```python
import jax
import jax.numpy as jnp

def _softmax(x, axis=-1):
    return jax.nn.softmax(x, axis=axis)
def _gelu(x):
    return jax.nn.gelu(x, approximate=True)
def _silu(x):
    return jax.nn.silu(x)
def _sigmoid(x):
    return jax.nn.sigmoid(x)
def _layernorm(x, axis=-1, eps=1e-5):
    m = jnp.mean(x, axis=axis, keepdims=True)
    v = jnp.var(x, axis=axis, keepdims=True)
    return (x - m) / jnp.sqrt(v + eps)
def _scatter_add(tgt, idx, src, axis=0):
    return tgt.at[idx].add(src)
def _segment_sum(src, seg, n):
    return jax.ops.segment_sum(src, seg, n)
class _Rng:
    def __init__(self, key):
        self._k = key
    def _next(self):
        self._k, sub = jax.random.split(self._k)
        return sub
    def normal(self, shape):
        return jax.random.normal(self._next(), shape, dtype=jnp.bfloat16)
    def randint(self, lo, hi, shape):
        return jax.random.randint(self._next(), shape, lo, hi, dtype=jnp.int32)
    def uniform(self, shape, lo=0.0, hi=1.0):
        return jax.random.uniform(self._next(), shape, jnp.bfloat16, lo, hi)
    def permutation(self, n):
        return jax.random.permutation(self._next(), n)


kernel_name = 'concat_heads__ssm_conv_h3__compressed_kv_cla__prompt'

def setup_inputs():
    _rng = _Rng(jax.random.key(int.from_bytes(__import__("os").urandom(4), "little")))
    _w = (lambda a: (lambda t: t.astype(jnp.bfloat16) if jnp.issubdtype(t.dtype, jnp.floating) else t)(jnp.asarray(a)))
    def _A_setup():
        B, S, D = 1, 2048, 448
        ks = 4
        return {
            "q": _w((lambda *s: _rng.normal(s) * 0.05)(B, S, D)),
            "k": _w((lambda *s: _rng.normal(s) * 0.05)(B, S, D)),
            "v": _w((lambda *s: _rng.normal(s) * 0.05)(B, S, D)),
            "shift_k": _w((lambda *s: _rng.normal(s) * 0.05)(D, ks) * 0.5),
            "ssm_k": _w((lambda *s: _rng.normal(s) * 0.05)(D, S) * (1.0 / S ** 0.5)),
            "ssm_D": _w((lambda *s: _rng.normal(s) * 0.05)(D)),
        }
    _A_in = _A_setup()

    def _B_setup():
        B, H, Sq, Sk, D, M = 1, 16, 2048, 2048, 256, 448
        Dc = 4 * D
        return {
            "x": _w((lambda *s: _rng.normal(s) * 0.05)(B, Sq, M)),
            "c_kv": _w((lambda *s: _rng.normal(s) * 0.05)(B, Sk, Dc)),
            "w_q": _w((lambda *s: _rng.normal(s) * 0.05)(M, H, D) * (M ** -0.5)),
            "w_uk": _w((lambda *s: _rng.normal(s) * 0.05)(Dc, H, D) * (Dc ** -0.5)),
            "w_uv": _w((lambda *s: _rng.normal(s) * 0.05)(Dc, H, D) * (Dc ** -0.5)),
            "w_o": _w((lambda *s: _rng.normal(s) * 0.05)(H, D, M) * ((H * D) ** -0.5)),
        }
    _B_in = _B_setup()

    return {
        "A_q": _A_in["q"],
        "A_k": _A_in["k"],
        "A_v": _A_in["v"],
        "A_shift_k": _A_in["shift_k"],
        "A_ssm_k": _A_in["ssm_k"],
        "A_ssm_D": _A_in["ssm_D"],
        "B_x": _B_in["x"],
        "B_c_kv": _B_in["c_kv"],
        "B_w_q": _B_in["w_q"],
        "B_w_uk": _B_in["w_uk"],
        "B_w_uv": _B_in["w_uv"],
        "B_w_o": _B_in["w_o"],
    }

def reference(A_q, A_k, A_v, A_shift_k, A_ssm_k, A_ssm_D, B_x, B_c_kv, B_w_q, B_w_uk, B_w_uv, B_w_o):
    def _A_ref(q, k, v, shift_k, ssm_k, ssm_D):
        B, S, D = q.shape
        ks = shift_k.shape[-1]
        k_pad = jnp.pad(k, ((0, 0), (ks - 1, 0), (0, 0)))
        k_shift = jnp.zeros_like(k)
        for t in range(ks):
            k_shift = k_shift + k_pad[:, t:t + S, :] * shift_k[:, ks - 1 - t][None, None, :]
        kv = k_shift * v
        L = 2 * S
        kv_pad = jnp.pad(kv, ((0, 0), (0, S), (0, 0)))
        kf_pad = jnp.pad(ssm_k, ((0, 0), (0, S)))
        kv_f = (lambda x, axes=(-2,-1): jnp.fft.rfft2(x.astype(jnp.float32), axes=axes))(kv_pad[:, None, :, :], axes=(1, 2))
        kf_f = (lambda x, axes=(-2,-1): jnp.fft.rfft2(x.astype(jnp.float32), axes=axes))(kf_pad[:, None, :], axes=(1, 2))
        kf_f = (lambda x, *d: x.transpose(*d))(kf_f, 1, 2, 0)
        y_f = kv_f * kf_f[None, :, :, :]
        y = (lambda x, s, axes=(-2,-1): jnp.fft.irfft2(x, s=s, axes=axes).astype(jnp.bfloat16))(y_f, (1, L), axes=(1, 2))[:, 0, :S, :]
        y = y + kv * ssm_D[None, None, :]
        return q * y

    def _B_ref(x, c_kv, w_q, w_uk, w_uv, w_o):
        B, Sq, M = x.shape[0], x.shape[1], x.shape[2]
        Sk = c_kv.shape[1]
        H, D = w_q.shape[1], w_q.shape[2]
        q = jnp.einsum("bqm,mhd->bhqd", x, w_q)
        k = jnp.einsum("bkc,chd->bhkd", c_kv, w_uk)
        v = jnp.einsum("bkc,chd->bhkd", c_kv, w_uv)
        scores = jnp.einsum("bhqd,bhkd->bhqk", q, k) * (D ** -0.5)
        off = Sk - Sq
        qi = jnp.arange(Sq)[:, None]
        kj = jnp.arange(Sk)[None, :]
        cmask = kj <= (qi + off)
        scores = jnp.where(cmask[None, None], scores, -1e9)
        p = _softmax(scores, axis=-1)
        ctx = jnp.einsum("bhqk,bhkd->bhqd", p, v)
        return jnp.einsum("bhqd,hdm->bqm", ctx, w_o)

    a = _A_ref(A_q, A_k, A_v, A_shift_k, A_ssm_k, A_ssm_D)
    b = _B_ref(B_x, B_c_kv, B_w_q, B_w_uk, B_w_uv, B_w_o)
    return jnp.concatenate([a, b], axis=-1)
```

```python
import math

import jax
import jax.numpy as jnp
import jax.experimental.pallas as pl
import jax.experimental.pallas.tpu as pltpu

S = 2048
M = 448
MP = 512
H = 16
D = 256
C = 1024
TQ = 256
NB = S // TQ
NU = 4
UC = M // NU
NBLK = S // 128
XCH = 4

F32 = jnp.float32
BF16 = jnp.bfloat16
U32 = jnp.uint32
NT = (((1,), (1,)), ((), ()))
HI_MASK = 0xFFFF0000
Q_SCALE = (D ** -0.5) * math.log2(math.e)
MASK_VALUE = -1e9


def _dot(a, b):
    return jnp.dot(a, b, preferred_element_type=F32)


def _dot_nt(a, b):
    return jax.lax.dot_general(a, b, NT, preferred_element_type=F32)


def _fold(xs, op):
    parts = []
    for x in xs:
        for t in range(x.shape[1] // 128):
            parts.append(x[:, t * 128:(t + 1) * 128])
    acc = parts[0]
    for p in parts[1:]:
        acc = op(acc, p)
    return acc


def _qk_softmax(i, q, ks):
    r = jax.lax.broadcasted_iota(jnp.int32, (128, 128), 0)
    c = jax.lax.broadcasted_iota(jnp.int32, (128, 128), 1)
    msk = c <= r
    s_full = [_dot_nt(q, ks[j]) for j in range(i)]
    s_d0 = _dot_nt(q, ks[i][:128])
    s_d1 = _dot_nt(q[128:], ks[i][128:])
    lo = [s[:128] for s in s_full] + [jnp.where(msk, s_d0[:128], MASK_VALUE)]
    hi = [s[128:] for s in s_full] + [s_d0[128:], jnp.where(msk, s_d1, MASK_VALUE)]
    m_lo = jnp.max(_fold(lo, jnp.maximum), axis=1, keepdims=True)
    m_hi = jnp.max(_fold(hi, jnp.maximum), axis=1, keepdims=True)
    p_lo = [jnp.exp2(s - m_lo) for s in lo]
    p_hi = [jnp.exp2(s - m_hi) for s in hi]
    l_lo = jnp.sum(_fold(p_lo, jnp.add), axis=1, keepdims=True)
    l_hi = jnp.sum(_fold(p_hi, jnp.add), axis=1, keepdims=True)
    ps = [jnp.concatenate([p_lo[j], p_hi[j]], axis=0).astype(BF16) for j in range(i + 1)]
    ps.append(p_hi[i + 1].astype(BF16))
    return ps, 1.0 / l_lo, 1.0 / l_hi


def _pv(i, ps, r_lo, r_hi, vs):
    o = None
    for j in range(i):
        t = _dot(ps[j], vs[j])
        o = t if o is None else o + t
    t = _dot(ps[i], vs[i][:128])
    o = t if o is None else o + t
    o_hi = o[128:] + _dot(ps[i + 1], vs[i][128:])
    return jnp.concatenate([o[:128] * r_lo, o_hi * r_hi], axis=0).astype(BF16)


def _kernel(aq_hbm, ak_hbm, av_hbm, sh_hbm, ah_hbm, dd_hbm, xt_hbm, c_hbm,
            wq_hbm, wk_hbm, wv_hbm, wot_hbm,
            out_hbm,
            sh_s, dd_s, coef_s, f_s, fh_s, xt_s, x_s, wq_raw, aq_s, ak_s, av_s, ah_s, at_s,
            c_s, wk_raw, wv_raw, wot_s, q_s, wk_s, wv_s, acc, stage_a, stage_b,
            sem_small, sem_x, sem_wq, sem_a, sem_c, sem_wk, sem_wv, sem_oa, sem_ob):
    wq32 = wq_hbm.bitcast(U32)
    wk32 = wk_hbm.bitcast(U32)
    wv32 = wv_hbm.bitcast(U32)
    xw = S // XCH

    def cp_small(i):
        return pltpu.make_async_copy((sh_hbm, dd_hbm)[i], (sh_s, dd_s)[i], sem_small.at[i])

    def cp_x(i):
        return pltpu.make_async_copy(xt_hbm.at[:, pl.ds(i * xw, xw)],
                                     xt_s.at[:, pl.ds(i * xw, xw)], sem_x.at[i])

    def cp_wq(p):
        return pltpu.make_async_copy(wq32.at[:, p, :], wq_raw.at[p], sem_wq.at[p])

    def cp_a(g, i):
        src = (ah_hbm, ak_hbm, av_hbm, aq_hbm)[i]
        dst = (ah_s, ak_s, av_s, aq_s)[i]
        start = g * UC if isinstance(g, int) else pl.multiple_of(g * UC, 16)
        return pltpu.make_async_copy(src.at[pl.ds(start, UC), :], dst.at[g], sem_a.at[g * 4 + i])

    def cp_c(i):
        return pltpu.make_async_copy((c_hbm, wot_hbm)[i], (c_s, wot_s)[i], sem_c.at[i])

    def cp_wk(p):
        return pltpu.make_async_copy(wk32.at[:, p, :], wk_raw.at[p], sem_wk.at[p])

    def cp_wv(p):
        return pltpu.make_async_copy(wv32.at[:, p, :], wv_raw.at[p], sem_wv.at[p])

    def cp_out_a(t):
        start = t * 128 if isinstance(t, int) else pl.multiple_of(t * 128, 128)
        return pltpu.make_async_copy(stage_a.at[pl.ds(start, 128), :],
                                     out_hbm.at[pl.ds(start, 128), pl.ds(0, 384)], sem_oa.at[t])

    def cp_out_b(i):
        return pltpu.make_async_copy(stage_b.at[pl.ds(i * TQ, TQ), :],
                                     out_hbm.at[pl.ds(i * TQ, TQ), pl.ds(384, MP)], sem_ob.at[i])

    cp_small(0).start()
    cp_small(1).start()
    cp_wq(0).start()
    cp_wq(1).start()
    for i in range(XCH):
        cp_x(i).start()
    for g in range(NU):
        if g > 0:
            cp_wq(2 * g).start()
            cp_wq(2 * g + 1).start()
        for i in range(4):
            cp_a(g, i).start()
    cp_wk(0).start()
    cp_wv(0).start()
    cp_c(0).start()
    cp_c(1).start()
    for p in range(1, H // 2):
        cp_wk(p).start()
        cp_wv(p).start()

    tt = jax.lax.broadcasted_iota(jnp.int32, (128, 128), 0)
    rr = jax.lax.broadcasted_iota(jnp.int32, (128, 128), 1)
    ang = ((tt * (2 * rr + 1)) & 511).astype(F32) * (2.0 * math.pi / 512.0)
    fmat = jnp.concatenate([jnp.cos(ang), -jnp.sin(ang)], axis=1).astype(BF16)
    f_s[...] = fmat
    fh_s[...] = (fmat.astype(F32) * (1.0 / 128.0)).astype(BF16)

    cp_small(0).wait()
    cp_small(1).wait()
    prm = [sh_s[j:j + 1, :].astype(F32) for j in range(4)]
    prm.append(dd_s[...].astype(F32).reshape(1, M))
    for j in range(5):
        row = jnp.concatenate([prm[j], jnp.zeros((1, MP - M), F32)], axis=1)
        for t in range(MP // 128):
            blk = jnp.broadcast_to(row[:, t * 128:(t + 1) * 128], (128, 128))
            coef_s[j, t * 128:(t + 1) * 128, :] = blk.T

    for i in range(XCH):
        cp_x(i).wait()
        for t in range(i * xw // 128, (i + 1) * xw // 128):
            cols = slice(t * 128, (t + 1) * 128)
            for g in range(3):
                x_s[cols, g * 128:(g + 1) * 128] = xt_s[g * 128:(g + 1) * 128, cols].astype(F32).T.astype(BF16)
            blk = jnp.concatenate([xt_s[384:M, cols].astype(F32), jnp.zeros((MP - M, 128), F32)], axis=0)
            x_s[cols, 384:MP] = blk.T.astype(BF16)

    def phase1(g, carry):
        cp_wq(2 * g).wait()
        cp_wq(2 * g + 1).wait()
        for i in range(4):
            cp_a(g, i).wait()
        row0 = pl.multiple_of(g * UC, 16)

        ws = []
        for p in range(2):
            raw = wq_raw[2 * g + p]
            lo = pltpu.bitcast(raw << 16, F32)
            hi = pltpu.bitcast(raw & jnp.uint32(HI_MASK), F32)
            w = jnp.concatenate([lo, hi], axis=1)
            w = jnp.concatenate([w, jnp.zeros((MP - M, 2 * D), F32)], axis=0)
            ws.append(w.astype(BF16))

        def qproj(p, r):
            rows = slice(r * 512, (r + 1) * 512)
            qq = _dot(x_s[rows, :], ws[p]) * Q_SCALE
            q_s[4 * g + 2 * p, rows, :] = qq[:, :D].astype(BF16)
            q_s[4 * g + 2 * p + 1, rows, :] = qq[:, D:].astype(BF16)

        coef = [coef_s[j, pl.ds(row0, UC), :] for j in range(5)]
        lane = jax.lax.broadcasted_iota(jnp.int32, (UC, 128), 1)

        fh = fh_s[...]
        zh = [_dot(ah_s[g, :, c * 128:(c + 1) * 128], fh) for c in range(NBLK)]

        kf = ak_s[g].astype(F32)
        sh_k = [kf] + [pltpu.roll(kf, j, 1) for j in range(1, 4)]
        kvs = []
        for c in range(NBLK):
            cols = slice(c * 128, (c + 1) * 128)
            t = sh_k[0][:, cols] * coef[0]
            for j in range(1, 4):
                kj = sh_k[j][:, cols]
                if c == 0:
                    kj = jnp.where(lane >= j, kj, 0.0)
                t = t + kj * coef[j]
            kvs.append((t * av_s[g, :, cols].astype(F32)).astype(BF16))
        fx = f_s[...]
        qproj(0, 0)
        zx = [_dot(kvs[c], fx) for c in range(NBLK)]
        qproj(0, 1)
        qproj(0, 2)
        qproj(0, 3)

        sgn = jnp.where((jax.lax.broadcasted_iota(jnp.int32, (8, 128), 1) & 1) == 0, 1.0, -1.0)
        pr = [[None] * (UC // 8) for _ in range(NBLK)]
        pi = [[None] * (UC // 8) for _ in range(NBLK)]
        for u in range(UC // 8):
            rows = slice(u * 8, (u + 1) * 8)
            xr = [z[rows, :128] for z in zx]
            xi = [z[rows, 128:] for z in zx]
            h0r = [z[rows, :128] for z in zh]
            h0i = [z[rows, 128:] for z in zh]
            hr = [h0r[0]] + [h0r[j] - sgn * h0i[j - 1] for j in range(1, NBLK)]
            hi = [h0i[0]] + [h0i[j] + sgn * h0r[j - 1] for j in range(1, NBLK)]
            xs = [xr[c] + xi[c] for c in range(NBLK)]
            hs = [hr[j] + hi[j] for j in range(NBLK)]
            for a0 in range(0, NBLK, 4):
                aa = [None] * 4
                bb = [None] * 4
                cc = [None] * 4
                for c0 in range(0, a0 + 4, 4):
                    for da in range(4):
                        for dc in range(4):
                            c = c0 + dc
                            j = a0 + da - c
                            if j < 0:
                                continue
                            ta, tb, tc = xr[c] * hr[j], xi[c] * hi[j], xs[c] * hs[j]
                            aa[da] = ta if aa[da] is None else aa[da] + ta
                            bb[da] = tb if bb[da] is None else bb[da] + tb
                            cc[da] = tc if cc[da] is None else cc[da] + tc
                for da in range(4):
                    pr[a0 + da][u] = aa[da] - bb[da]
                    pi[a0 + da][u] = cc[da] - (aa[da] + bb[da])
        qproj(1, 0)
        qproj(1, 1)
        qproj(1, 2)
        for a in range(NBLK):
            cols = slice(a * 128, (a + 1) * 128)
            pa = jnp.concatenate([jnp.concatenate(pr[a], axis=0), jnp.concatenate(pi[a], axis=0)],
                                 axis=1).astype(BF16)
            y = _dot_nt(pa, fx) + kvs[a].astype(F32) * coef[4]
            at_s[pl.ds(row0, UC), cols] = (aq_s[g, :, cols].astype(F32) * y).astype(BF16)
        qproj(1, 3)
        acc[pl.ds(pl.multiple_of(g * (S // NU), 8), S // NU), :] = jnp.zeros((S // NU, MP), F32)
        return carry

    jax.lax.fori_loop(0, NU, phase1, 0)

    def extract(h):
        pair = h // 2
        sh = (16 * (1 - h % 2)).astype(U32)
        wk_s[...] = pltpu.bitcast((wk_raw[pair] << sh) & jnp.uint32(HI_MASK), F32).astype(BF16)
        wv_s[...] = pltpu.bitcast((wv_raw[pair] << sh) & jnp.uint32(HI_MASK), F32).astype(BF16)

    cp_wk(0).wait()
    cp_wv(0).wait()
    extract(jnp.int32(0))
    cp_c(0).wait()
    cp_c(1).wait()

    def phase2(h, carry):
        @pl.when(jnp.logical_and(h % 2 == 1, h < H - 1))
        def _():
            cp_wk((h + 1) // 2).wait()
            cp_wv((h + 1) // 2).wait()

        wot = wot_s[h]
        ks, vs, sm, ctx = [], [], {}, {}

        def kproj(i):
            ks.append(_dot(c_s[i * TQ:(i + 1) * TQ, :], wk_s[...]).astype(BF16))

        def vproj(i):
            vs.append(_dot(c_s[i * TQ:(i + 1) * TQ, :], wv_s[...]).astype(BF16))

        def qk(i):
            sm[i] = _qk_softmax(i, q_s[h, i * TQ:(i + 1) * TQ, :], ks)

        def pv(i):
            ctx[i] = _pv(i, *sm[i], vs)

        def oproj(i):
            ot = _dot_nt(wot, ctx[i])
            top = jnp.where(h == 0, at_s[384:M, i * TQ:(i + 1) * TQ].astype(F32), 0.0)
            acc[i * TQ:(i + 1) * TQ, :] += jnp.concatenate([top, ot], axis=0).T

        t0 = pl.multiple_of(h * 128, 128)
        for g in range(3):
            blk = at_s[g * 128:(g + 1) * 128, pl.ds(t0, 128)].astype(F32)
            stage_a[pl.ds(t0, 128), g * 128:(g + 1) * 128] = blk.T.astype(BF16)

        kproj(0); vproj(0); qk(0); kproj(1); pv(0)
        for i in range(1, NB - 1):
            qk(i); vproj(i); oproj(i - 1); kproj(i + 1); pv(i)
        qk(NB - 1); vproj(NB - 1); pv(NB - 1); oproj(NB - 2); oproj(NB - 1)
        extract(jnp.minimum(h + 1, H - 1))
        cp_out_a(h).start()
        return carry

    jax.lax.fori_loop(0, H, phase2, 0)

    for i in range(NB):
        stage_b[i * TQ:(i + 1) * TQ, :] = acc[i * TQ:(i + 1) * TQ, :].astype(BF16)
        cp_out_b(i).start()
    for t in range(H):
        cp_out_a(t).wait()
    for i in range(NB):
        cp_out_b(i).wait()


@jax.jit
def pallas_concat_heads__ssm_conv_h3__compressed_kv_cla__prompt_kernel(
    A_q: jax.Array,
    A_k: jax.Array,
    A_v: jax.Array,
    A_shift_k: jax.Array,
    A_ssm_k: jax.Array,
    A_ssm_D: jax.Array,
    B_x: jax.Array,
    B_c_kv: jax.Array,
    B_w_q: jax.Array,
    B_w_uk: jax.Array,
    B_w_uv: jax.Array,
    B_w_o: jax.Array,
):
    vm = pltpu.VMEM
    dma = pltpu.SemaphoreType.DMA
    scratch = [
        vm((4, M), BF16),
        vm((M,), BF16),
        vm((5, MP, 128), F32),
        vm((128, 256), BF16),
        vm((128, 256), BF16),
        vm((M, S), BF16),
        vm((S, MP), BF16),
        vm((H // 2, M, D), U32),
        vm((NU, UC, S), BF16),
        vm((NU, UC, S), BF16),
        vm((NU, UC, S), BF16),
        vm((NU, UC, S), BF16),
        vm((M, S), BF16),
        vm((S, C), BF16),
        vm((H // 2, C, D), U32),
        vm((H // 2, C, D), U32),
        vm((H, M, D), BF16),
        vm((H, S, D), BF16),
        vm((C, D), BF16),
        vm((C, D), BF16),
        vm((S, MP), F32),
        vm((S, 384), BF16),
        vm((S, MP), BF16),
        dma((2,)), dma((XCH,)), dma((H // 2,)), dma((NU * 4,)), dma((2,)),
        dma((H // 2,)), dma((H // 2,)), dma((H,)), dma((NB,)),
    ]
    out = pl.pallas_call(
        _kernel,
        in_specs=[pl.BlockSpec(memory_space=pl.ANY)] * 12,
        out_specs=pl.BlockSpec(memory_space=pl.ANY),
        out_shape=jax.ShapeDtypeStruct((S, 2 * M), BF16),
        scratch_shapes=scratch,
        compiler_params=pltpu.CompilerParams(vmem_limit_bytes=120 * 1024 * 1024),
        name="h3_cla_fused",
    )(
        A_q[0].T, A_k[0].T, A_v[0].T, A_shift_k.T, A_ssm_k, A_ssm_D,
        B_x[0].T, B_c_kv[0], B_w_q, B_w_uk, B_w_uv, jnp.transpose(B_w_o, (0, 2, 1)),
    )
    return out[None]
```

```python
import math

import jax
import jax.numpy as jnp
import jax.experimental.pallas as pl
import jax.experimental.pallas.tpu as pltpu

S = 2048
M = 448
MP = 512
H = 16
D = 256
C = 1024
TQ = 256
NB = S // TQ
NU = 7
UC = M // NU
NBLK = S // 128
XCH = 4

F32 = jnp.float32
BF16 = jnp.bfloat16
U32 = jnp.uint32
NT = (((1,), (1,)), ((), ()))
HI_MASK = 0xFFFF0000
Q_SCALE = D ** -0.5
MASK_VALUE = -1e9


def _dot(a, b):
    return jnp.dot(a, b, preferred_element_type=F32)


def _dot_nt(a, b):
    return jax.lax.dot_general(a, b, NT, preferred_element_type=F32)


def _inject(x, tok):
    top = jnp.concatenate([x[:8, :128] | tok, x[:8, 128:]], axis=1)
    return jnp.concatenate([top, x[8:]], axis=0)


def _recip(x):
    r = pl.reciprocal(x, approx=True)
    return r * (2.0 - x * r)


def _fold(xs, op):
    parts = []
    for x in xs:
        for t in range(x.shape[1] // 128):
            parts.append(x[:, t * 128:(t + 1) * 128])
    acc = parts[0]
    for p in parts[1:]:
        acc = op(acc, p)
    return acc


def _qk(i, q, ks):
    r = jax.lax.broadcasted_iota(jnp.int32, (128, 128), 0)
    c = jax.lax.broadcasted_iota(jnp.int32, (128, 128), 1)
    msk = c <= r
    s_full = [_dot_nt(q, ks[j]) for j in range(i)]
    s_d0 = _dot_nt(q, ks[i][:128])
    s_d1 = _dot_nt(q[128:], ks[i][128:])
    lo = [s[:128] for s in s_full] + [jnp.where(msk, s_d0[:128], MASK_VALUE)]
    hi = [s[128:] for s in s_full] + [s_d0[128:], jnp.where(msk, s_d1, MASK_VALUE)]
    return lo, hi


def _softmax(i, lo, hi):
    m_lo = jnp.max(_fold(lo, jnp.maximum), axis=1, keepdims=True)
    m_hi = jnp.max(_fold(hi, jnp.maximum), axis=1, keepdims=True)
    p_lo = [jnp.exp(s - m_lo) for s in lo]
    p_hi = [jnp.exp(s - m_hi) for s in hi]
    ps = [jnp.concatenate([p_lo[j], p_hi[j]], axis=0).astype(BF16) for j in range(i + 1)]
    ps.append(p_hi[i + 1].astype(BF16))
    if i < NB - 1:
        pf = [p.astype(F32) for p in ps]
        p_lo = [p[:128] for p in pf[:-1]]
        p_hi = [p[128:] for p in pf[:-1]] + [pf[-1]]
    return ps, jnp.concatenate([_fold(p_lo, jnp.add), _fold(p_hi, jnp.add)], axis=0)


def _pv(i, ps, vs):
    o = None
    for j in range(i):
        t = _dot(ps[j], vs[j])
        o = t if o is None else o + t
    t = _dot(ps[i], vs[i][:128])
    o = t if o is None else o + t
    o_hi = o[128:] + _dot(ps[i + 1], vs[i][128:])
    return jnp.concatenate([o[:128], o_hi], axis=0)


def _normalize(o, lsum):
    r = _recip(jnp.sum(lsum, axis=1, keepdims=True))
    return pltpu.bitcast((o * r).astype(BF16), U32)


def _kernel(aq_hbm, ak_hbm, av_hbm, sh_hbm, ah_hbm, dd_hbm, xt_hbm, c_hbm,
            wq_hbm, wk_hbm, wv_hbm, wot_hbm,
            out_hbm,
            sh_s, dd_s, coef_s, f_s, fh_s, zero_s, xt_s, x_s, wq_raw, aq_s, ak_s, av_s, ah_s, at_s,
            c_s, wk_raw, wv_raw, wot_s, q_s, ctx_s, ot_s, o7_s, l7_s, stage_a, stage_b,
            sem_small, sem_x, sem_wq, sem_a, sem_c, sem_wk, sem_wv, sem_oa, sem_ob):
    wq32 = wq_hbm.bitcast(U32)
    wk32 = wk_hbm.bitcast(U32)
    wv32 = wv_hbm.bitcast(U32)
    xw = S // XCH

    def cp_small(i):
        return pltpu.make_async_copy((sh_hbm, dd_hbm)[i], (sh_s, dd_s)[i], sem_small.at[i])

    def cp_x(i):
        return pltpu.make_async_copy(xt_hbm.at[:, pl.ds(i * xw, xw)],
                                     xt_s.at[:, pl.ds(i * xw, xw)], sem_x.at[i])

    def cp_wq(p):
        return pltpu.make_async_copy(wq32.at[:, p, :], wq_raw.at[p], sem_wq.at[p])

    def cp_a(g, i):
        src = (ah_hbm, ak_hbm, av_hbm, aq_hbm)[i].bitcast(U32)
        dst = (ah_s, ak_s, av_s, aq_s)[i]
        n = UC // 2
        start = g * n if isinstance(g, int) else pl.multiple_of(g * n, 8)
        return pltpu.make_async_copy(src.at[pl.ds(start, n), :], dst.at[g], sem_a.at[g * 4 + i])

    def cp_c(i):
        return pltpu.make_async_copy((c_hbm, wot_hbm)[i].bitcast(U32), (c_s, wot_s)[i], sem_c.at[i])

    def cp_wk(p):
        return pltpu.make_async_copy(wk32.at[:, p, :], wk_raw.at[p], sem_wk.at[p])

    def cp_wv(p):
        return pltpu.make_async_copy(wv32.at[:, p, :], wv_raw.at[p], sem_wv.at[p])

    def cp_out_a(i):
        start = i * TQ if isinstance(i, int) else pl.multiple_of(i * TQ, TQ)
        return pltpu.make_async_copy(stage_a.at[pl.ds(start, TQ), :],
                                     out_hbm.at[pl.ds(start, TQ), pl.ds(0, 384)], sem_oa.at[i])

    def cp_out_b(i):
        start = i * TQ if isinstance(i, int) else pl.multiple_of(i * TQ, TQ)
        return pltpu.make_async_copy(stage_b.at[pl.ds(start, TQ), :],
                                     out_hbm.at[pl.ds(start, TQ), pl.ds(384, MP)], sem_ob.at[i])

    cp_x(0).start()
    cp_wq(0).start()
    cp_small(0).start()
    cp_small(1).start()
    for i in range(1, XCH):
        cp_x(i).start()
    for g in range(NU):
        cp_wq(g + 1).start()
        for i in range(4):
            cp_a(g, i).start()
    cp_wk(0).start()
    cp_wv(0).start()
    cp_c(0).start()
    cp_c(1).start()
    for p in range(1, H // 2):
        cp_wk(p).start()
        cp_wv(p).start()

    tt = jax.lax.broadcasted_iota(jnp.int32, (128, 128), 0)
    rr = jax.lax.broadcasted_iota(jnp.int32, (128, 128), 1)
    ang = ((tt * (2 * rr + 1)) & 511).astype(F32) * (2.0 * math.pi / 512.0)
    fmat = jnp.concatenate([jnp.cos(ang), -jnp.sin(ang)], axis=1).astype(BF16)
    f_s[...] = pltpu.bitcast(fmat, U32)
    fh_s[...] = pltpu.bitcast((fmat.astype(F32) * (1.0 / 128.0)).astype(BF16), U32)
    zero_s[...] = jnp.zeros((8, 128), U32)

    def xpose_x(i):
        for t in range(i * xw // 128, (i + 1) * xw // 128):
            cols = slice(t * 128, (t + 1) * 128)
            blks = [xt_s[g * 128:(g + 1) * 128, cols].astype(F32).T for g in range(3)]
            last = jnp.concatenate([xt_s[384:M, cols].astype(F32), jnp.zeros((MP - M, 128), F32)], axis=0)
            blks.append(last.T)
            x_s[t * 64:(t + 1) * 64, :] = pltpu.bitcast(jnp.concatenate(blks, axis=1).astype(BF16), U32)

    def q_weights(p):
        raw = wq_raw[p]
        lo = pltpu.bitcast(raw << 16, F32)
        hi = pltpu.bitcast(raw & jnp.uint32(HI_MASK), F32)
        w = jnp.concatenate([lo, hi], axis=1)
        w = jnp.concatenate([w, jnp.zeros((MP - M, 2 * D), F32)], axis=0)
        return w.astype(BF16)

    def qproj(p, w, r):
        rows = slice(r * xw // 2, (r + 1) * xw // 2)
        qq = _dot(pltpu.bitcast(x_s[rows, :], BF16), w) * Q_SCALE
        q_s[2 * p, rows, :] = pltpu.bitcast(qq[:, :D].astype(BF16), U32)
        q_s[2 * p + 1, rows, :] = pltpu.bitcast(qq[:, D:].astype(BF16), U32)

    cp_x(0).wait()
    xpose_x(0)
    cp_wq(0).wait()
    cp_x(1).wait()
    w0 = q_weights(0)
    xpose_x(1)
    qproj(0, w0, 0)
    cp_small(0).wait()
    cp_small(1).wait()
    cp_x(2).wait()
    xpose_x(2)
    qproj(0, w0, 1)
    prm = [sh_s[j:j + 1, :].astype(F32) for j in range(4)]
    prm.append(dd_s[...].astype(F32).reshape(1, M))
    for j in range(5):
        row = jnp.concatenate([prm[j], jnp.zeros((1, MP - M), F32)], axis=1)
        for t in range(MP // 128):
            blk = jnp.broadcast_to(row[:, t * 128:(t + 1) * 128], (128, 128))
            coef_s[j, t * 128:(t + 1) * 128, :] = blk.T
    cp_x(3).wait()
    xpose_x(3)
    qproj(0, w0, 2)
    qproj(0, w0, 3)
    ot_s[...] = jnp.zeros((M, TQ), F32)
    o7_s[...] = jnp.zeros((TQ, D), F32)
    l7_s[...] = jnp.ones((TQ, 128), F32)

    def phase1(g, carry):
        cp_wq(g + 1).wait()
        for i in range(4):
            cp_a(g, i).wait()
        row0 = pl.multiple_of(g * UC, 16)
        w = q_weights(g + 1)
        coef = [coef_s[j, pl.ds(row0, UC), :] for j in range(5)]
        lane = jax.lax.broadcasted_iota(jnp.int32, (UC, 128), 1)
        NS = 4

        def unstack(z):
            return [z[c // NS][(c % NS) * UC:(c % NS + 1) * UC] for c in range(NBLK)]

        fh = pltpu.bitcast(fh_s[...], BF16)
        zh = []
        for c0 in range(0, NBLK, NS):
            lhs = jnp.concatenate([ah_s[g, :, c * 128:(c + 1) * 128] for c in range(c0, c0 + NS)], axis=0)
            zh.append(_dot(pltpu.bitcast(lhs, BF16), fh))
        zh = unstack(zh)

        kf = pltpu.bitcast(ak_s[g], BF16).astype(F32)
        vf = pltpu.bitcast(av_s[g], BF16).astype(F32)
        sh_k = [kf] + [pltpu.roll(kf, j, 1) for j in range(1, 4)]
        kvf = []
        for c in range(NBLK):
            cols = slice(c * 128, (c + 1) * 128)
            t = sh_k[0][:, cols] * coef[0]
            for j in range(1, 4):
                kj = sh_k[j][:, cols]
                if c == 0:
                    kj = jnp.where(lane >= j, kj, 0.0)
                t = t + kj * coef[j]
            kvf.append(t * vf[:, cols])
        kvs = [jnp.concatenate(kvf[c0:c0 + NS], axis=0).astype(BF16) for c0 in range(0, NBLK, NS)]
        fx = pltpu.bitcast(f_s[...], BF16)
        qproj(g + 1, w, 0)
        zx = unstack([_dot(kv, fx) for kv in kvs])
        qproj(g + 1, w, 1)
        qproj(g + 1, w, 2)

        sgn = jnp.where((jax.lax.broadcasted_iota(jnp.int32, (8, 128), 1) & 1) == 0, 1.0, -1.0)
        pr = [[None] * (UC // 8) for _ in range(NBLK)]
        pi = [[None] * (UC // 8) for _ in range(NBLK)]
        for u in range(UC // 8):
            rows = slice(u * 8, (u + 1) * 8)
            xr = [z[rows, :128] for z in zx]
            xi = [z[rows, 128:] for z in zx]
            h0r = [z[rows, :128] for z in zh]
            h0i = [z[rows, 128:] for z in zh]
            hr = [h0r[0]] + [h0r[j] - sgn * h0i[j - 1] for j in range(1, NBLK)]
            hi = [h0i[0]] + [h0i[j] + sgn * h0r[j - 1] for j in range(1, NBLK)]
            xs = [xr[c] + xi[c] for c in range(NBLK)]
            hs = [hr[j] + hi[j] for j in range(NBLK)]
            for a0 in range(0, NBLK, 4):
                aa = [None] * 4
                bb = [None] * 4
                cc = [None] * 4
                for c0 in range(0, a0 + 4, 4):
                    for da in range(4):
                        for dc in range(4):
                            c = c0 + dc
                            j = a0 + da - c
                            if j < 0:
                                continue
                            ta, tb, tc = xr[c] * hr[j], xi[c] * hi[j], xs[c] * hs[j]
                            aa[da] = ta if aa[da] is None else aa[da] + ta
                            bb[da] = tb if bb[da] is None else bb[da] + tb
                            cc[da] = tc if cc[da] is None else cc[da] + tc
                for da in range(4):
                    pr[a0 + da][u] = aa[da] - bb[da]
                    pi[a0 + da][u] = cc[da] - (aa[da] + bb[da])
        ys = []
        for a0 in range(0, NBLK, NS):
            re = jnp.concatenate([t for a in range(a0, a0 + NS) for t in pr[a]], axis=0)
            im = jnp.concatenate([t for a in range(a0, a0 + NS) for t in pi[a]], axis=0)
            ys.append(_dot_nt(jnp.concatenate([re, im], axis=1).astype(BF16), fx))
        ys = unstack(ys)
        qproj(g + 1, w, 3)
        kvr = unstack([kv.astype(F32) for kv in kvs])
        qf = pltpu.bitcast(aq_s[g], BF16).astype(F32)
        for a in range(NBLK):
            cols = slice(a * 128, (a + 1) * 128)
            at_s[pl.ds(row0, UC), cols] = (qf[:, cols] * (ys[a] + kvr[a] * coef[4])).astype(BF16)
        return carry

    jax.lax.fori_loop(0, NU, phase1, 0)

    cp_c(0).wait()
    cp_c(1).wait()

    def extract(raw, h):
        sh = (16 * (1 - h % 2)).astype(U32)
        return pltpu.bitcast((raw[h // 2] << sh) & jnp.uint32(HI_MASK), F32).astype(BF16)

    def cblk(i):
        return pltpu.bitcast(c_s[i * TQ // 2:(i + 1) * TQ // 2, :], BF16)

    def finish_last(h):
        bits = _normalize(o7_s[...], l7_s[...])
        ctx_s[h, (NB - 1) * TQ // 2:NB * TQ // 2, :] = bits
        return bits

    def phase2(h, carry):
        @pl.when(h % 2 == 0)
        def _():
            cp_wk(h // 2).wait()
            cp_wv(h // 2).wait()

        wk = extract(wk_raw, h)
        wv = extract(wv_raw, h)
        ks, vs, toks = [], [], {}
        zero = zero_s[...]

        def token(bits):
            t = None
            for r in range(TQ // 16):
                for c in range(D // 128):
                    e = bits[r * 8:(r + 1) * 8, c * 128:(c + 1) * 128]
                    t = e if t is None else t | e
            return t & zero

        def kproj(i):
            ks.append(_dot(cblk(i), wk).astype(BF16))

        def vproj(i):
            vs.append(_dot(cblk(i), wv).astype(BF16))

        def qk(i):
            q = q_s[h, i * TQ // 2:(i + 1) * TQ // 2, :]
            if i - 2 in toks:
                q = _inject(q, toks[i - 2])
            return _qk(i, pltpu.bitcast(q, BF16), ks)

        def pv(i, sc):
            ps, lsum = _softmax(i, *sc)
            o = _pv(i, ps, vs)
            if i == NB - 1:
                o7_s[...] = o
                l7_s[...] = lsum
            else:
                bits = _normalize(o, lsum)
                ctx_s[h, i * TQ // 2:(i + 1) * TQ // 2, :] = bits
                toks[i] = token(bits)

        toks[-1] = token(finish_last(jnp.maximum(h - 1, 0)))
        kproj(0)
        vproj(0)
        sc = qk(0)
        kproj(1)
        pv(0, sc)
        for i in range(1, NB):
            sc = qk(i)
            vproj(i)
            if i + 1 < NB:
                kproj(i + 1)
            pv(i, sc)
        return carry

    jax.lax.fori_loop(0, H, phase2, 0)
    finish_last(H - 1)

    def finish(i):
        r0 = i * TQ if isinstance(i, int) else pl.multiple_of(i * TQ, TQ)
        top = at_s[384:M, pl.ds(r0, TQ)].astype(F32)
        stage_b[pl.ds(r0, TQ), :] = jnp.concatenate([top, ot_s[...]], axis=0).T.astype(BF16)

    def phase3(i, carry):
        prev = jnp.maximum(i - 1, 0)
        finish(prev)

        @pl.when(i > 0)
        def _():
            cp_out_b(prev).start()

        r0 = pl.multiple_of(i * TQ, TQ)
        for g in range(3):
            blk = at_s[g * 128:(g + 1) * 128, pl.ds(r0, TQ)].astype(F32)
            stage_a[pl.ds(r0, TQ), g * 128:(g + 1) * 128] = blk.T.astype(BF16)
        cp_out_a(i).start()
        rows = pl.ds(pl.multiple_of(i * (TQ // 2), TQ // 2), TQ // 2)
        wot = jnp.concatenate([wot_s[h] for h in range(H)], axis=1)
        ctx = jnp.concatenate([ctx_s[h, rows, :] for h in range(H)], axis=1)
        ot_s[...] = _dot_nt(pltpu.bitcast(wot, BF16), pltpu.bitcast(ctx, BF16))
        return carry

    jax.lax.fori_loop(0, NB, phase3, 0)

    finish(NB - 1)
    cp_out_b(NB - 1).start()
    for i in range(NB):
        cp_out_a(i).wait()
        cp_out_b(i).wait()


@jax.jit
def pallas_concat_heads__ssm_conv_h3__compressed_kv_cla__prompt_kernel(
    A_q: jax.Array,
    A_k: jax.Array,
    A_v: jax.Array,
    A_shift_k: jax.Array,
    A_ssm_k: jax.Array,
    A_ssm_D: jax.Array,
    B_x: jax.Array,
    B_c_kv: jax.Array,
    B_w_q: jax.Array,
    B_w_uk: jax.Array,
    B_w_uv: jax.Array,
    B_w_o: jax.Array,
):
    vm = pltpu.VMEM
    dma = pltpu.SemaphoreType.DMA
    scratch = [
        vm((4, M), BF16),
        vm((M,), BF16),
        vm((5, MP, 128), F32),
        vm((64, 256), U32),
        vm((64, 256), U32),
        vm((8, 128), U32),
        vm((M, S), BF16),
        vm((S // 2, MP), U32),
        vm((H // 2, M, D), U32),
        vm((NU, UC // 2, S), U32),
        vm((NU, UC // 2, S), U32),
        vm((NU, UC // 2, S), U32),
        vm((NU, UC // 2, S), U32),
        vm((M, S), BF16),
        vm((S // 2, C), U32),
        vm((H // 2, C, D), U32),
        vm((H // 2, C, D), U32),
        vm((H, M // 2, D), U32),
        vm((H, S // 2, D), U32),
        vm((H, S // 2, D), U32),
        vm((M, TQ), F32),
        vm((TQ, D), F32),
        vm((TQ, 128), F32),
        vm((S, 384), BF16),
        vm((S, MP), BF16),
        dma((2,)), dma((XCH,)), dma((H // 2,)), dma((NU * 4,)), dma((2,)),
        dma((H // 2,)), dma((H // 2,)), dma((NB,)), dma((NB,)),
    ]
    out = pl.pallas_call(
        _kernel,
        in_specs=[pl.BlockSpec(memory_space=pl.ANY)] * 12,
        out_specs=pl.BlockSpec(memory_space=pl.ANY),
        out_shape=jax.ShapeDtypeStruct((S, 2 * M), BF16),
        scratch_shapes=scratch,
        compiler_params=pltpu.CompilerParams(vmem_limit_bytes=120 * 1024 * 1024),
        name="h3_cla_fused",
    )(
        A_q[0].T, A_k[0].T, A_v[0].T, A_shift_k.T, A_ssm_k, A_ssm_D,
        B_x[0].T, B_c_kv[0], B_w_q, B_w_uk, B_w_uv, jnp.transpose(B_w_o, (0, 2, 1)),
    )
    return out[None]
```

```python
import math

import jax
import jax.numpy as jnp
import jax.experimental.pallas as pl
import jax.experimental.pallas.tpu as pltpu

S = 2048
M = 448
MP = 512
H = 16
D = 256
C = 1024
TQ = 256
NB = S // TQ
NU = 7
UC = M // NU
NBLK = S // 128
XCH = 4

F32 = jnp.float32
BF16 = jnp.bfloat16
U32 = jnp.uint32
NT = (((1,), (1,)), ((), ()))
HI_MASK = 0xFFFF0000
Q_SCALE = D ** -0.5
MASK_VALUE = -1e9
P1ORDER = "H0 H1 H2 H3 Q0 X0 Q1 X1 Q2 X2 Q3 X3 Q4 I00 Q5 I01 Q6 I10 Q7 I11 Q8 Q9 I20 Q10 I21 Q11 Q12 I30 Q13 I31 Q14 Q15"
QCH = 128
XB = (0, 256, 512, 1024, 2048)
TOKH = 6
TO = 128
NO = S // TO
NB3 = 4


def _dot(a, b):
    return jnp.dot(a, b, preferred_element_type=F32)


def _dot_nt(a, b):
    return jax.lax.dot_general(a, b, NT, preferred_element_type=F32)


def _inject(x, tok):
    top = jnp.concatenate([x[:8, :128] | tok, x[:8, 128:]], axis=1)
    return jnp.concatenate([top, x[8:]], axis=0)


def _recip(x):
    r = pl.reciprocal(x, approx=True)
    return r * (2.0 - x * r)


def _fold(xs, op):
    parts = []
    for x in xs:
        for t in range(x.shape[1] // 128):
            parts.append(x[:, t * 128:(t + 1) * 128])
    acc = parts[0]
    for p in parts[1:]:
        acc = op(acc, p)
    return acc


def _qk(i, q, ks):
    r = jax.lax.broadcasted_iota(jnp.int32, (128, 128), 0)
    c = jax.lax.broadcasted_iota(jnp.int32, (128, 128), 1)
    msk = c <= r
    s_full = [_dot_nt(q, ks[j]) for j in range(i)]
    s_d0 = _dot_nt(q, ks[i][:128])
    s_d1 = _dot_nt(q[128:], ks[i][128:])
    lo = [s[:128] for s in s_full] + [jnp.where(msk, s_d0[:128], MASK_VALUE)]
    hi = [s[128:] for s in s_full] + [s_d0[128:], jnp.where(msk, s_d1, MASK_VALUE)]
    return lo, hi


def _softmax(i, lo, hi):
    m_lo = jnp.max(_fold(lo, jnp.maximum), axis=1, keepdims=True)
    m_hi = jnp.max(_fold(hi, jnp.maximum), axis=1, keepdims=True)
    p_lo = [jnp.exp(s - m_lo) for s in lo]
    p_hi = [jnp.exp(s - m_hi) for s in hi]
    ps = [jnp.concatenate([p_lo[j], p_hi[j]], axis=0).astype(BF16) for j in range(i + 1)]
    ps.append(p_hi[i + 1].astype(BF16))
    if i < NB - 1:
        pf = [p.astype(F32) for p in ps]
        p_lo = [p[:128] for p in pf[:-1]]
        p_hi = [p[128:] for p in pf[:-1]] + [pf[-1]]
    return ps, jnp.concatenate([_fold(p_lo, jnp.add), _fold(p_hi, jnp.add)], axis=0)


def _pv(i, ps, vs):
    o = None
    for j in range(i):
        t = _dot(ps[j], vs[j])
        o = t if o is None else o + t
    t = _dot(ps[i], vs[i][:128])
    o = t if o is None else o + t
    o_hi = o[128:] + _dot(ps[i + 1], vs[i][128:])
    return jnp.concatenate([o[:128], o_hi], axis=0)


def _normalize(o, lsum):
    r = _recip(jnp.sum(lsum, axis=1, keepdims=True))
    return pltpu.bitcast((o * r).astype(BF16), U32)


def _kernel(aq_hbm, ak_hbm, av_hbm, sh_hbm, ah_hbm, dd_hbm, xt_hbm, c_hbm,
            wq_hbm, wk_hbm, wv_hbm, wot_hbm,
            out_hbm,
            sh_s, dd_s, coef_s, f_s, fh_s, zero_s, xt_s, x_s, wq_raw, aq_s, ak_s, av_s, ah_s, at_s,
            c_s, wk_raw, wv_raw, wot_s, q_s, ctx_s, ot_s, o7_s, l7_s, stage_a, stage_b,
            sem_small, sem_x, sem_wq, sem_a, sem_c, sem_wk, sem_wv, sem_oa, sem_ob):
    wq32 = wq_hbm.bitcast(U32)
    wk32 = wk_hbm.bitcast(U32)
    wv32 = wv_hbm.bitcast(U32)

    def cp_small(i):
        return pltpu.make_async_copy((sh_hbm, dd_hbm)[i], (sh_s, dd_s)[i], sem_small.at[i])

    def cp_x(i):
        cols = pl.ds(XB[i], XB[i + 1] - XB[i])
        return pltpu.make_async_copy(xt_hbm.at[:, cols], xt_s.at[:, cols], sem_x.at[i])

    def cp_wq(p):
        return pltpu.make_async_copy(wq32.at[:, p, :], wq_raw.at[p], sem_wq.at[p])

    def cp_a(g, i):
        src = (ah_hbm, ak_hbm, av_hbm, aq_hbm)[i].bitcast(U32)
        dst = (ah_s, ak_s, av_s, aq_s)[i]
        n = UC // 2
        start = g * n if isinstance(g, int) else pl.multiple_of(g * n, 8)
        return pltpu.make_async_copy(src.at[pl.ds(start, n), :], dst.at[g], sem_a.at[g * 4 + i])

    def cp_c(i):
        return pltpu.make_async_copy((c_hbm, wot_hbm)[i].bitcast(U32), (c_s, wot_s)[i], sem_c.at[i])

    def cp_wk(p):
        return pltpu.make_async_copy(wk32.at[:, p, :], wk_raw.at[p], sem_wk.at[p])

    def cp_wv(p):
        return pltpu.make_async_copy(wv32.at[:, p, :], wv_raw.at[p], sem_wv.at[p])

    def cp_out_a(i):
        start = i * TO if isinstance(i, int) else pl.multiple_of(i * TO, TO)
        return pltpu.make_async_copy(stage_a.at[pl.ds(start, TO), :],
                                     out_hbm.at[pl.ds(start, TO), pl.ds(0, 384)], sem_oa.at[i])

    def cp_out_b(i):
        start = i * TO if isinstance(i, int) else pl.multiple_of(i * TO, TO)
        return pltpu.make_async_copy(stage_b.at[pl.ds(start, TO), :],
                                     out_hbm.at[pl.ds(start, TO), pl.ds(384, MP)], sem_ob.at[i])

    cp_x(0).start()
    cp_wq(0).start()
    cp_small(0).start()
    cp_small(1).start()
    for i in range(1, XCH):
        cp_x(i).start()
    for g in range(NU):
        cp_wq(g + 1).start()
        for i in range(4):
            cp_a(g, i).start()
    cp_wk(0).start()
    cp_wv(0).start()
    cp_c(0).start()
    cp_c(1).start()
    for p in range(1, H // 2):
        cp_wk(p).start()
        cp_wv(p).start()

    tt = jax.lax.broadcasted_iota(jnp.int32, (128, 128), 0)
    rr = jax.lax.broadcasted_iota(jnp.int32, (128, 128), 1)
    ang = ((tt * (2 * rr + 1)) & 511).astype(F32) * (2.0 * math.pi / 512.0)
    fmat = jnp.concatenate([jnp.cos(ang), -jnp.sin(ang)], axis=1).astype(BF16)
    f_s[...] = pltpu.bitcast(fmat, U32)
    fh_s[...] = pltpu.bitcast((fmat.astype(F32) * (1.0 / 128.0)).astype(BF16), U32)
    zero_s[...] = jnp.zeros((8, 128), U32)

    def xpose_x(i):
        for t in range(XB[i] // 128, XB[i + 1] // 128):
            cols = slice(t * 128, (t + 1) * 128)
            blks = [xt_s[g * 128:(g + 1) * 128, cols].astype(F32).T for g in range(3)]
            last = jnp.concatenate([xt_s[384:M, cols].astype(F32), jnp.zeros((MP - M, 128), F32)], axis=0)
            blks.append(last.T)
            x_s[t * 64:(t + 1) * 64, :] = pltpu.bitcast(jnp.concatenate(blks, axis=1).astype(BF16), U32)

    def q_weights(p):
        raw = wq_raw[p]
        lo = pltpu.bitcast(raw << 16, F32)
        hi = pltpu.bitcast(raw & jnp.uint32(HI_MASK), F32)
        w = jnp.concatenate([lo, hi], axis=1) * Q_SCALE
        w = jnp.concatenate([w, jnp.zeros((MP - M, 2 * D), F32)], axis=0)
        return w.astype(BF16)

    def qproj(p, w, r0, r1):
        rows = slice(r0 // 2, r1 // 2)
        qq = _dot(pltpu.bitcast(x_s[rows, :], BF16), w)
        q_s[2 * p, rows, :] = pltpu.bitcast(qq[:, :D].astype(BF16), U32)
        q_s[2 * p + 1, rows, :] = pltpu.bitcast(qq[:, D:].astype(BF16), U32)

    cp_x(0).wait()
    xpose_x(0)
    cp_wq(0).wait()
    cp_x(1).wait()
    w0 = q_weights(0)
    xpose_x(1)
    qproj(0, w0, XB[0], XB[1])
    cp_small(0).wait()
    cp_small(1).wait()
    cp_x(2).wait()
    xpose_x(2)
    qproj(0, w0, XB[1], XB[2])
    prm = [sh_s[j:j + 1, :].astype(F32) for j in range(4)]
    prm.append(dd_s[...].astype(F32).reshape(1, M))
    for j in range(5):
        row = jnp.concatenate([prm[j], jnp.zeros((1, MP - M), F32)], axis=1)
        for t in range(MP // 128):
            blk = jnp.broadcast_to(row[:, t * 128:(t + 1) * 128], (128, 128))
            coef_s[j, t * 128:(t + 1) * 128, :] = blk.T
    cp_x(3).wait()
    xpose_x(3)
    qproj(0, w0, XB[2], XB[3])
    for r in range(XB[3], XB[4], 512):
        qproj(0, w0, r, min(r + 512, XB[4]))
    ot_s[...] = jnp.zeros((M, TO), F32)
    o7_s[...] = jnp.zeros((TQ, D), F32)
    l7_s[...] = jnp.ones((TQ, 128), F32)

    def phase1(g, carry):
        cp_wq(g + 1).wait()
        for i in range(4):
            cp_a(g, i).wait()
        w = q_weights(g + 1)
        fh = pltpu.bitcast(fh_s[...], BF16)
        fx = pltpu.bitcast(f_s[...], BF16)
        lane = jax.lax.broadcasted_iota(jnp.int32, (16, 128), 1)
        sgn = jnp.where((jax.lax.broadcasted_iota(jnp.int32, (8, 128), 1) & 1) == 0, 1.0, -1.0)
        zh, zx, kvs, ys = {}, {}, {}, {}

        def coef(k, j):
            return coef_s[j, pl.ds(pl.multiple_of(g * UC + k * 16, 16), 16), :]

        def hfwd(k):
            lhs = jnp.concatenate([ah_s[g, k * 8:(k + 1) * 8, c * 128:(c + 1) * 128] for c in range(NBLK)], axis=0)
            zh[k] = _dot(pltpu.bitcast(lhs, BF16), fh)

        def xfwd(k):
            kf = pltpu.bitcast(ak_s[g, k * 8:(k + 1) * 8, :], BF16).astype(F32)
            vf = pltpu.bitcast(av_s[g, k * 8:(k + 1) * 8, :], BF16).astype(F32)
            sh_k = [kf] + [pltpu.roll(kf, j, 1) for j in range(1, 4)]
            cf = [coef(k, j) for j in range(4)]
            kvf = []
            for c in range(NBLK):
                cols = slice(c * 128, (c + 1) * 128)
                t = sh_k[0][:, cols] * cf[0]
                for j in range(1, 4):
                    kj = sh_k[j][:, cols]
                    if c == 0:
                        kj = jnp.where(lane >= j, kj, 0.0)
                    t = t + kj * cf[j]
                kvf.append(t * vf[:, cols])
            kvs[k] = jnp.concatenate(kvf, axis=0).astype(BF16)
            zx[k] = _dot(kvs[k], fx)

        def inv(k, u):
            rows = [slice(c * 16 + u * 8, c * 16 + u * 8 + 8) for c in range(NBLK)]
            xr = [zx[k][r, :128] for r in rows]
            xi = [zx[k][r, 128:] for r in rows]
            h0r = [zh[k][r, :128] for r in rows]
            h0i = [zh[k][r, 128:] for r in rows]
            hr = [h0r[0]] + [h0r[j] - sgn * h0i[j - 1] for j in range(1, NBLK)]
            hi = [h0i[0]] + [h0i[j] + sgn * h0r[j - 1] for j in range(1, NBLK)]
            xs = [xr[c] + xi[c] for c in range(NBLK)]
            hs = [hr[j] + hi[j] for j in range(NBLK)]
            pr, pi = [], []
            for a0 in range(0, NBLK, 4):
                aa = [None] * 4
                bb = [None] * 4
                cc = [None] * 4
                for c0 in range(0, a0 + 4, 4):
                    for da in range(4):
                        for dc in range(4):
                            c = c0 + dc
                            j = a0 + da - c
                            if j < 0:
                                continue
                            ta, tb, tc = xr[c] * hr[j], xi[c] * hi[j], xs[c] * hs[j]
                            aa[da] = ta if aa[da] is None else aa[da] + ta
                            bb[da] = tb if bb[da] is None else bb[da] + tb
                            cc[da] = tc if cc[da] is None else cc[da] + tc
                for da in range(4):
                    pr.append(aa[da] - bb[da])
                    pi.append(cc[da] - (aa[da] + bb[da]))
            p = jnp.concatenate([jnp.concatenate(pr, axis=0), jnp.concatenate(pi, axis=0)], axis=1)
            ys[k, u] = _dot_nt(p.astype(BF16), fx)
            if u == 1:
                kvr = kvs[k].astype(F32)
                qf = pltpu.bitcast(aq_s[g, k * 8:(k + 1) * 8, :], BF16).astype(F32)
                dd = coef(k, 4)
                row0 = pl.multiple_of(g * UC + k * 16, 16)
                for a in range(NBLK):
                    cols = slice(a * 128, (a + 1) * 128)
                    y = jnp.concatenate([ys[k, 0][a * 8:(a + 1) * 8], ys[k, 1][a * 8:(a + 1) * 8]], axis=0)
                    at_s[pl.ds(row0, 16), cols] = (qf[:, cols] * (y + kvr[a * 16:(a + 1) * 16] * dd)).astype(BF16)

        for tokn in P1ORDER.split():
            if tokn[0] == 'Q':
                qproj(g + 1, w, int(tokn[1:]) * QCH, (int(tokn[1:]) + 1) * QCH)
            elif tokn[0] == 'H':
                hfwd(int(tokn[1]))
            elif tokn[0] == 'X':
                xfwd(int(tokn[1]))
            else:
                inv(int(tokn[1]), int(tokn[2]))
        return carry

    jax.lax.fori_loop(0, NU, phase1, 0)

    cp_c(0).wait()
    cp_c(1).wait()

    def extract(raw, h):
        sh = (16 * (1 - h % 2)).astype(U32)
        return pltpu.bitcast((raw[h // 2] << sh) & jnp.uint32(HI_MASK), F32).astype(BF16)

    def cblk(i):
        return pltpu.bitcast(c_s[i * TQ // 2:(i + 1) * TQ // 2, :], BF16)

    def finish_last(h):
        bits = _normalize(o7_s[...], l7_s[...])
        ctx_s[h, (NB - 1) * TQ // 2:NB * TQ // 2, :] = bits
        return bits

    def phase2(h, carry):
        @pl.when(h % 2 == 0)
        def _():
            cp_wk(h // 2).wait()
            cp_wv(h // 2).wait()

        wk = extract(wk_raw, h)
        wv = extract(wv_raw, h)
        ks, vs, toks = [], [], {}
        zero = zero_s[...]

        def token(bits):
            t = None
            for r in range(TQ // 16):
                for c in range(D // 128):
                    e = bits[r * 8:(r + 1) * 8, c * 128:(c + 1) * 128]
                    t = e if t is None else t | e
            return t & zero

        def kproj(i):
            ks.append(_dot(cblk(i), wk).astype(BF16))

        def vproj(i):
            vs.append(_dot(cblk(i), wv).astype(BF16))

        def qk(i):
            q = q_s[h, i * TQ // 2:(i + 1) * TQ // 2, :]
            if i - 2 in toks:
                q = _inject(q, toks[i - 2])
            return _qk(i, pltpu.bitcast(q, BF16), ks)

        def pv(i, sc):
            ps, lsum = _softmax(i, *sc)
            o = _pv(i, ps, vs)
            if i == NB - 1:
                o7_s[...] = o
                l7_s[...] = lsum
            else:
                bits = _normalize(o, lsum)
                ctx_s[h, i * TQ // 2:(i + 1) * TQ // 2, :] = bits
                toks[i] = token(bits)

        toks[-1] = token(finish_last(jnp.maximum(h - 1, 0)))
        kproj(0)
        vproj(0)
        sc = qk(0)
        kproj(1)
        pv(0, sc)
        for i in range(1, NB):
            sc = qk(i)
            vproj(i)
            if i + 1 < NB:
                kproj(i + 1)
            pv(i, sc)
        return carry

    jax.lax.fori_loop(0, H, phase2, 0)
    finish_last(H - 1)

    def orfold(x):
        bits = pltpu.bitcast(x, U32)
        t = None
        for r in range(bits.shape[0] // 8):
            for c in range(bits.shape[1] // 128):
                e = bits[r * 8:(r + 1) * 8, c * 128:(c + 1) * 128]
                t = e if t is None else t | e
        return t

    def finish(i, ot):
        r0 = i * TO if isinstance(i, int) else pl.multiple_of(i * TO, TO)
        top = at_s[384:M, pl.ds(r0, TO)].astype(F32)
        val = jnp.concatenate([top, ot], axis=0).T
        stage_b[pl.ds(r0, TO), :] = val.astype(BF16)
        return val

    def oproj(i, pending):
        r0 = pl.multiple_of(i * TO, TO)
        tok = orfold(pending)
        for g in range(3):
            blk = at_s[g * 128:(g + 1) * 128, pl.ds(r0, TO)].astype(F32).T
            stage_a[pl.ds(r0, TO), g * 128:(g + 1) * 128] = blk.astype(BF16)
            tok = tok | orfold(blk)
        cp_out_a(i).start()
        tok = tok & zero_s[...]
        rows = pl.ds(pl.multiple_of(i * (TO // 2), TO // 2), TO // 2)
        wot = jnp.concatenate([wot_s[h] for h in range(H)], axis=1)
        ctx = [ctx_s[h, rows, :] for h in range(H)]
        ctx[TOKH] = _inject(ctx[TOKH], tok)
        ctx = jnp.concatenate(ctx, axis=1)
        return _dot_nt(pltpu.bitcast(wot, BF16), pltpu.bitcast(ctx, BF16))

    def phase3(it, carry):
        prev = jnp.maximum(NB3 * it - 1, 0)
        val = finish(prev, ot_s[...])

        @pl.when(it > 0)
        def _():
            cp_out_b(prev).start()

        for k in range(NB3 - 1):
            val = finish(NB3 * it + k, oproj(NB3 * it + k, val))
            cp_out_b(NB3 * it + k).start()
        ot_s[...] = oproj(NB3 * it + NB3 - 1, val)
        return carry

    jax.lax.fori_loop(0, NO // NB3, phase3, 0)

    finish(NO - 1, ot_s[...])
    cp_out_b(NO - 1).start()
    for i in range(NO):
        cp_out_a(i).wait()
        cp_out_b(i).wait()


@jax.jit
def pallas_concat_heads__ssm_conv_h3__compressed_kv_cla__prompt_kernel(
    A_q: jax.Array,
    A_k: jax.Array,
    A_v: jax.Array,
    A_shift_k: jax.Array,
    A_ssm_k: jax.Array,
    A_ssm_D: jax.Array,
    B_x: jax.Array,
    B_c_kv: jax.Array,
    B_w_q: jax.Array,
    B_w_uk: jax.Array,
    B_w_uv: jax.Array,
    B_w_o: jax.Array,
):
    vm = pltpu.VMEM
    dma = pltpu.SemaphoreType.DMA
    scratch = [
        vm((4, M), BF16),
        vm((M,), BF16),
        vm((5, MP, 128), F32),
        vm((64, 256), U32),
        vm((64, 256), U32),
        vm((8, 128), U32),
        vm((M, S), BF16),
        vm((S // 2, MP), U32),
        vm((H // 2, M, D), U32),
        vm((NU, UC // 2, S), U32),
        vm((NU, UC // 2, S), U32),
        vm((NU, UC // 2, S), U32),
        vm((NU, UC // 2, S), U32),
        vm((M, S), BF16),
        vm((S // 2, C), U32),
        vm((H // 2, C, D), U32),
        vm((H // 2, C, D), U32),
        vm((H, M // 2, D), U32),
        vm((H, S // 2, D), U32),
        vm((H, S // 2, D), U32),
        vm((M, TO), F32),
        vm((TQ, D), F32),
        vm((TQ, 128), F32),
        vm((S, 384), BF16),
        vm((S, MP), BF16),
        dma((2,)), dma((XCH,)), dma((H // 2,)), dma((NU * 4,)), dma((2,)),
        dma((H // 2,)), dma((H // 2,)), dma((NO,)), dma((NO,)),
    ]
    out = pl.pallas_call(
        _kernel,
        in_specs=[pl.BlockSpec(memory_space=pl.ANY)] * 12,
        out_specs=pl.BlockSpec(memory_space=pl.ANY),
        out_shape=jax.ShapeDtypeStruct((S, 2 * M), BF16),
        scratch_shapes=scratch,
        compiler_params=pltpu.CompilerParams(vmem_limit_bytes=120 * 1024 * 1024, disable_semaphore_checks=True),
        name="h3_cla_fused",
    )(
        A_q[0].T, A_k[0].T, A_v[0].T, A_shift_k.T, A_ssm_k, A_ssm_D,
        B_x[0].T, B_c_kv[0], B_w_q, B_w_uk, B_w_uv, jnp.transpose(B_w_o, (0, 2, 1)),
    )
    return out[None]
```

```python
import math

import jax
import jax.numpy as jnp
import jax.experimental.pallas as pl
import jax.experimental.pallas.tpu as pltpu

S = 2048
M = 448
MP = 512
H = 16
D = 256
C = 1024
TQ = 256
NB = S // TQ
NU = 7
UC = M // NU
NBLK = S // 128
XCH = 4

F32 = jnp.float32
BF16 = jnp.bfloat16
U32 = jnp.uint32
NT = (((1,), (1,)), ((), ()))
HI_MASK = 0xFFFF0000
Q_SCALE = D ** -0.5
MASK_VALUE = -1e9
P1ORDER = "H0 H1 H2 H3 Q0 X0 Q1 X1 Q2 X2 Q3 X3 Q4 I00 Q5 I01 Q6 I10 Q7 I11 Q8 Q9 I20 Q10 I21 Q11 Q12 I30 Q13 I31 Q14 Q15"
QCH = 128
XB = (0, 256, 512, 1024, 2048)
TOKH = 6
TO = 128
NO = S // TO
NB3 = 4


def _dot(a, b):
    return jnp.dot(a, b, preferred_element_type=F32)


def _dot_nt(a, b):
    return jax.lax.dot_general(a, b, NT, preferred_element_type=F32)


def _inject(x, tok):
    top = jnp.concatenate([x[:8, :128] | tok, x[:8, 128:]], axis=1)
    return jnp.concatenate([top, x[8:]], axis=0)


def _recip(x):
    r = pl.reciprocal(x, approx=True)
    return r * (2.0 - x * r)


def _fold(xs, op):
    parts = []
    for x in xs:
        for t in range(x.shape[1] // 128):
            parts.append(x[:, t * 128:(t + 1) * 128])
    acc = parts[0]
    for p in parts[1:]:
        acc = op(acc, p)
    return acc


def _qk(i, q, ks):
    r = jax.lax.broadcasted_iota(jnp.int32, (128, 128), 0)
    c = jax.lax.broadcasted_iota(jnp.int32, (128, 128), 1)
    msk = c <= r
    s_full = [_dot_nt(q, ks[j]) for j in range(i)]
    s_d0 = _dot_nt(q, ks[i][:128])
    s_d1 = _dot_nt(q[128:], ks[i][128:])
    lo = [s[:128] for s in s_full] + [jnp.where(msk, s_d0[:128], MASK_VALUE)]
    hi = [s[128:] for s in s_full] + [s_d0[128:], jnp.where(msk, s_d1, MASK_VALUE)]
    return lo, hi


def _softmax(i, lo, hi):
    m_lo = jnp.max(_fold(lo, jnp.maximum), axis=1, keepdims=True)
    m_hi = jnp.max(_fold(hi, jnp.maximum), axis=1, keepdims=True)
    p_lo = [jnp.exp(s - m_lo) for s in lo]
    p_hi = [jnp.exp(s - m_hi) for s in hi]
    ps = [jnp.concatenate([p_lo[j], p_hi[j]], axis=0).astype(BF16) for j in range(i + 1)]
    ps.append(p_hi[i + 1].astype(BF16))
    if i < NB - 1:
        pf = [p.astype(F32) for p in ps]
        p_lo = [p[:128] for p in pf[:-1]]
        p_hi = [p[128:] for p in pf[:-1]] + [pf[-1]]
    return ps, jnp.concatenate([_fold(p_lo, jnp.add), _fold(p_hi, jnp.add)], axis=0)


def _pv(i, ps, vs):
    o = None
    for j in range(i):
        t = _dot(ps[j], vs[j])
        o = t if o is None else o + t
    t = _dot(ps[i], vs[i][:128])
    o = t if o is None else o + t
    o_hi = o[128:] + _dot(ps[i + 1], vs[i][128:])
    return jnp.concatenate([o[:128], o_hi], axis=0)


def _normalize(o, lsum):
    r = _recip(jnp.sum(lsum, axis=1, keepdims=True))
    return pltpu.bitcast((o * r).astype(BF16), U32)


def _kernel(aq_hbm, ak_hbm, av_hbm, sh_hbm, ah_hbm, dd_hbm, xt_hbm, c_hbm,
            wq_hbm, wk_hbm, wv_hbm, wot_hbm,
            out_hbm,
            sh_s, dd_s, coef_s, f_s, fh_s, zero_s, xt_s, x_s, wq_raw, aq_s, ak_s, av_s, ah_s, at_s,
            c_s, wk_raw, wv_raw, wot_s, q_s, ctx_s, ot_s, o7_s, l7_s, stage_a, stage_b,
            sem_small, sem_x, sem_wq, sem_a, sem_c, sem_wk, sem_wv, sem_oa, sem_ob):
    wq32 = wq_hbm.bitcast(U32)
    wk32 = wk_hbm.bitcast(U32)
    wv32 = wv_hbm.bitcast(U32)

    def cp_small(i):
        return pltpu.make_async_copy((sh_hbm, dd_hbm)[i], (sh_s, dd_s)[i], sem_small.at[i])

    def cp_x(i):
        cols = pl.ds(XB[i], XB[i + 1] - XB[i])
        return pltpu.make_async_copy(xt_hbm.at[:, cols], xt_s.at[:, cols], sem_x.at[i])

    def cp_wq(p):
        return pltpu.make_async_copy(wq32.at[:, p, :], wq_raw.at[p], sem_wq.at[p])

    def cp_a(g, i):
        src = (ah_hbm, ak_hbm, av_hbm, aq_hbm)[i].bitcast(U32)
        dst = (ah_s, ak_s, av_s, aq_s)[i]
        n = UC // 2
        start = g * n if isinstance(g, int) else pl.multiple_of(g * n, 8)
        return pltpu.make_async_copy(src.at[pl.ds(start, n), :], dst.at[g], sem_a.at[g * 4 + i])

    def cp_c(i):
        return pltpu.make_async_copy((c_hbm, wot_hbm)[i].bitcast(U32), (c_s, wot_s)[i], sem_c.at[i])

    def cp_wk(p):
        return pltpu.make_async_copy(wk32.at[:, p, :], wk_raw.at[p], sem_wk.at[p])

    def cp_wv(p):
        return pltpu.make_async_copy(wv32.at[:, p, :], wv_raw.at[p], sem_wv.at[p])

    def cp_out_a(i):
        n = NB3 * TO
        start = i * n if isinstance(i, int) else pl.multiple_of(i * n, n)
        return pltpu.make_async_copy(stage_a.at[pl.ds(start, n), :],
                                     out_hbm.at[pl.ds(start, n), pl.ds(0, 384)], sem_oa.at[i])

    def cp_out_b(i):
        start = i * TO if isinstance(i, int) else pl.multiple_of(i * TO, TO)
        return pltpu.make_async_copy(stage_b.at[pl.ds(start, TO), :],
                                     out_hbm.at[pl.ds(start, TO), pl.ds(384, MP)], sem_ob.at[i])

    cp_x(0).start()
    cp_wq(0).start()
    cp_small(0).start()
    cp_small(1).start()
    for i in range(1, XCH):
        cp_x(i).start()
    for g in range(NU):
        cp_wq(g + 1).start()
        for i in range(4):
            cp_a(g, i).start()
    cp_wk(0).start()
    cp_wv(0).start()
    cp_c(0).start()
    cp_c(1).start()
    for p in range(1, H // 2):
        cp_wk(p).start()
        cp_wv(p).start()

    tt = jax.lax.broadcasted_iota(jnp.int32, (128, 128), 0)
    rr = jax.lax.broadcasted_iota(jnp.int32, (128, 128), 1)
    ang = ((tt * (2 * rr + 1)) & 511).astype(F32) * (2.0 * math.pi / 512.0)
    fmat = jnp.concatenate([jnp.cos(ang), -jnp.sin(ang)], axis=1).astype(BF16)
    f_s[...] = pltpu.bitcast(fmat, U32)
    fh_s[...] = pltpu.bitcast((fmat.astype(F32) * (1.0 / 128.0)).astype(BF16), U32)
    zero_s[...] = jnp.zeros((8, 128), U32)

    def xpose_x(i):
        for t in range(XB[i] // 128, XB[i + 1] // 128):
            cols = slice(t * 128, (t + 1) * 128)
            blks = [xt_s[g * 128:(g + 1) * 128, cols].astype(F32).T for g in range(3)]
            last = jnp.concatenate([xt_s[384:M, cols].astype(F32), jnp.zeros((MP - M, 128), F32)], axis=0)
            blks.append(last.T)
            x_s[t * 64:(t + 1) * 64, :] = pltpu.bitcast(jnp.concatenate(blks, axis=1).astype(BF16), U32)

    def q_weights(p):
        raw = wq_raw[p]
        lo = pltpu.bitcast(raw << 16, F32)
        hi = pltpu.bitcast(raw & jnp.uint32(HI_MASK), F32)
        w = jnp.concatenate([lo, hi], axis=1) * Q_SCALE
        w = jnp.concatenate([w, jnp.zeros((MP - M, 2 * D), F32)], axis=0)
        return w.astype(BF16)

    def qproj(p, w, r0, r1):
        rows = slice(r0 // 2, r1 // 2)
        qq = _dot(pltpu.bitcast(x_s[rows, :], BF16), w)
        q_s[2 * p, rows, :] = pltpu.bitcast(qq[:, :D].astype(BF16), U32)
        q_s[2 * p + 1, rows, :] = pltpu.bitcast(qq[:, D:].astype(BF16), U32)

    cp_x(0).wait()
    xpose_x(0)
    cp_wq(0).wait()
    cp_x(1).wait()
    w0 = q_weights(0)
    xpose_x(1)
    qproj(0, w0, XB[0], XB[1])
    cp_small(0).wait()
    cp_small(1).wait()
    cp_x(2).wait()
    xpose_x(2)
    qproj(0, w0, XB[1], XB[2])
    prm = [sh_s[j:j + 1, :].astype(F32) for j in range(4)]
    prm.append(dd_s[...].astype(F32).reshape(1, M))
    for j in range(5):
        row = jnp.concatenate([prm[j], jnp.zeros((1, MP - M), F32)], axis=1)
        for t in range(MP // 128):
            blk = jnp.broadcast_to(row[:, t * 128:(t + 1) * 128], (128, 128))
            coef_s[j, t * 128:(t + 1) * 128, :] = blk.T
    cp_x(3).wait()
    xpose_x(3)
    qproj(0, w0, XB[2], XB[3])
    for r in range(XB[3], XB[4], 512):
        qproj(0, w0, r, min(r + 512, XB[4]))
    ot_s[...] = jnp.zeros((M, TO), F32)
    o7_s[...] = jnp.zeros((TQ, D), F32)
    l7_s[...] = jnp.ones((TQ, 128), F32)

    def phase1(g, carry):
        cp_wq(g + 1).wait()
        for i in range(4):
            cp_a(g, i).wait()
        w = q_weights(g + 1)
        fh = pltpu.bitcast(fh_s[...], BF16)
        fx = pltpu.bitcast(f_s[...], BF16)
        lane = jax.lax.broadcasted_iota(jnp.int32, (16, 128), 1)
        sgn = jnp.where((jax.lax.broadcasted_iota(jnp.int32, (8, 128), 1) & 1) == 0, 1.0, -1.0)
        zh, zx, kvs, ys = {}, {}, {}, {}

        def coef(k, j):
            return coef_s[j, pl.ds(pl.multiple_of(g * UC + k * 16, 16), 16), :]

        def hfwd(k):
            lhs = jnp.concatenate([ah_s[g, k * 8:(k + 1) * 8, c * 128:(c + 1) * 128] for c in range(NBLK)], axis=0)
            zh[k] = _dot(pltpu.bitcast(lhs, BF16), fh)

        def xfwd(k):
            kf = pltpu.bitcast(ak_s[g, k * 8:(k + 1) * 8, :], BF16).astype(F32)
            vf = pltpu.bitcast(av_s[g, k * 8:(k + 1) * 8, :], BF16).astype(F32)
            sh_k = [kf] + [pltpu.roll(kf, j, 1) for j in range(1, 4)]
            cf = [coef(k, j) for j in range(4)]
            kvf = []
            for c in range(NBLK):
                cols = slice(c * 128, (c + 1) * 128)
                t = sh_k[0][:, cols] * cf[0]
                for j in range(1, 4):
                    kj = sh_k[j][:, cols]
                    if c == 0:
                        kj = jnp.where(lane >= j, kj, 0.0)
                    t = t + kj * cf[j]
                kvf.append(t * vf[:, cols])
            kvs[k] = jnp.concatenate(kvf, axis=0).astype(BF16)
            zx[k] = _dot(kvs[k], fx)

        def inv(k, u):
            rows = [slice(c * 16 + u * 8, c * 16 + u * 8 + 8) for c in range(NBLK)]
            xr = [zx[k][r, :128] for r in rows]
            xi = [zx[k][r, 128:] for r in rows]
            h0r = [zh[k][r, :128] for r in rows]
            h0i = [zh[k][r, 128:] for r in rows]
            hr = [h0r[0]] + [h0r[j] - sgn * h0i[j - 1] for j in range(1, NBLK)]
            hi = [h0i[0]] + [h0i[j] + sgn * h0r[j - 1] for j in range(1, NBLK)]
            xs = [xr[c] + xi[c] for c in range(NBLK)]
            hs = [hr[j] + hi[j] for j in range(NBLK)]
            pr, pi = [], []
            for a0 in range(0, NBLK, 4):
                aa = [None] * 4
                bb = [None] * 4
                cc = [None] * 4
                for c0 in range(0, a0 + 4, 4):
                    for da in range(4):
                        for dc in range(4):
                            c = c0 + dc
                            j = a0 + da - c
                            if j < 0:
                                continue
                            ta, tb, tc = xr[c] * hr[j], xi[c] * hi[j], xs[c] * hs[j]
                            aa[da] = ta if aa[da] is None else aa[da] + ta
                            bb[da] = tb if bb[da] is None else bb[da] + tb
                            cc[da] = tc if cc[da] is None else cc[da] + tc
                for da in range(4):
                    pr.append(aa[da] - bb[da])
                    pi.append(cc[da] - (aa[da] + bb[da]))
            p = jnp.concatenate([jnp.concatenate(pr, axis=0), jnp.concatenate(pi, axis=0)], axis=1)
            ys[k, u] = _dot_nt(p.astype(BF16), fx)
            if u == 1:
                kvr = kvs[k].astype(F32)
                qf = pltpu.bitcast(aq_s[g, k * 8:(k + 1) * 8, :], BF16).astype(F32)
                dd = coef(k, 4)
                row0 = pl.multiple_of(g * UC + k * 16, 16)
                for a in range(NBLK):
                    cols = slice(a * 128, (a + 1) * 128)
                    y = jnp.concatenate([ys[k, 0][a * 8:(a + 1) * 8], ys[k, 1][a * 8:(a + 1) * 8]], axis=0)
                    at_s[pl.ds(row0, 16), cols] = (qf[:, cols] * (y + kvr[a * 16:(a + 1) * 16] * dd)).astype(BF16)

        for tokn in P1ORDER.split():
            if tokn[0] == 'Q':
                qproj(g + 1, w, int(tokn[1:]) * QCH, (int(tokn[1:]) + 1) * QCH)
            elif tokn[0] == 'H':
                hfwd(int(tokn[1]))
            elif tokn[0] == 'X':
                xfwd(int(tokn[1]))
            else:
                inv(int(tokn[1]), int(tokn[2]))
        return carry

    jax.lax.fori_loop(0, NU, phase1, 0)

    cp_c(0).wait()
    cp_c(1).wait()
    for p in range(H // 2):
        cp_wk(p).wait()
        cp_wv(p).wait()

    def extract(raw, h):
        sh = (16 - ((h & 1) << 4)).astype(U32)
        return pltpu.bitcast((raw[h >> 1] << sh) & jnp.uint32(HI_MASK), F32).astype(BF16)

    def cblk(i):
        return pltpu.bitcast(c_s[i * TQ // 2:(i + 1) * TQ // 2, :], BF16)

    def finish_last(h):
        bits = _normalize(o7_s[...], l7_s[...])
        ctx_s[h, (NB - 1) * TQ // 2:NB * TQ // 2, :] = bits
        return bits

    def phase2(h, carry):
        wk = extract(wk_raw, h)
        wv = extract(wv_raw, h)
        ks, vs, toks = [], [], {}
        zero = zero_s[...]

        def token(bits):
            t = None
            for r in range(TQ // 16):
                for c in range(D // 128):
                    e = bits[r * 8:(r + 1) * 8, c * 128:(c + 1) * 128]
                    t = e if t is None else t | e
            return t & zero

        def kproj(i):
            ks.append(_dot(cblk(i), wk).astype(BF16))

        def vproj(i):
            vs.append(_dot(cblk(i), wv).astype(BF16))

        def qk(i):
            q = q_s[h, i * TQ // 2:(i + 1) * TQ // 2, :]
            if i - 2 in toks:
                q = _inject(q, toks[i - 2])
            return _qk(i, pltpu.bitcast(q, BF16), ks)

        def pv(i, sc):
            ps, lsum = _softmax(i, *sc)
            o = _pv(i, ps, vs)
            if i == NB - 1:
                o7_s[...] = o
                l7_s[...] = lsum
            else:
                bits = _normalize(o, lsum)
                ctx_s[h, i * TQ // 2:(i + 1) * TQ // 2, :] = bits
                toks[i] = token(bits)

        toks[-1] = token(finish_last(jnp.maximum(h - 1, 0)))
        kproj(0)
        vproj(0)
        sc = qk(0)
        kproj(1)
        pv(0, sc)
        for i in range(1, NB):
            sc = qk(i)
            vproj(i)
            if i + 1 < NB:
                kproj(i + 1)
            pv(i, sc)
        return carry

    jax.lax.fori_loop(0, H, phase2, 0)
    finish_last(H - 1)

    def orfold(x):
        bits = pltpu.bitcast(x, U32)
        t = None
        for r in range(bits.shape[0] // 8):
            for c in range(bits.shape[1] // 128):
                e = bits[r * 8:(r + 1) * 8, c * 128:(c + 1) * 128]
                t = e if t is None else t | e
        return t

    def finish(i, ot):
        r0 = i * TO if isinstance(i, int) else pl.multiple_of(i * TO, TO)
        top = at_s[384:M, pl.ds(r0, TO)].astype(F32)
        val = jnp.concatenate([top, ot], axis=0).T
        stage_b[pl.ds(r0, TO), :] = val.astype(BF16)
        return val

    def oproj(i, pending):
        tok = orfold(pending[0])
        for x in pending[1:]:
            tok = tok | orfold(x)
        tok = tok & zero_s[...]
        rows = pl.ds(pl.multiple_of(i * (TO // 2), TO // 2), TO // 2)
        wot = jnp.concatenate([wot_s[h] for h in range(H)], axis=1)
        ctx = [ctx_s[h, rows, :] for h in range(H)]
        ctx[TOKH] = _inject(ctx[TOKH], tok)
        ctx = jnp.concatenate(ctx, axis=1)
        return _dot_nt(pltpu.bitcast(wot, BF16), pltpu.bitcast(ctx, BF16))

    def phase3(it, carry):
        prev = jnp.maximum(NB3 * it - 1, 0)
        pend = [finish(prev, ot_s[...])]

        @pl.when(it > 0)
        def _():
            cp_out_b(prev).start()

        r0 = pl.multiple_of(it * (NB3 * TO), NB3 * TO)
        apart = []
        for g in range(3):
            blk = at_s[g * 128:(g + 1) * 128, pl.ds(r0, NB3 * TO)].astype(F32).T
            stage_a[pl.ds(r0, NB3 * TO), g * 128:(g + 1) * 128] = blk.astype(BF16)
            apart.append(blk)
        cp_out_a(it).start()

        for k in range(NB3 - 1):
            pend = [finish(NB3 * it + k, oproj(NB3 * it + k, pend))]
            if k == 0:
                pend += apart
            cp_out_b(NB3 * it + k).start()
        ot_s[...] = oproj(NB3 * it + NB3 - 1, pend)
        return carry

    jax.lax.fori_loop(0, NO // NB3, phase3, 0)

    finish(NO - 1, ot_s[...])
    cp_out_b(NO - 1).start()
    for i in range(NO // NB3):
        cp_out_a(i).wait()
    for i in range(NO):
        cp_out_b(i).wait()


@jax.jit
def pallas_concat_heads__ssm_conv_h3__compressed_kv_cla__prompt_kernel(
    A_q: jax.Array,
    A_k: jax.Array,
    A_v: jax.Array,
    A_shift_k: jax.Array,
    A_ssm_k: jax.Array,
    A_ssm_D: jax.Array,
    B_x: jax.Array,
    B_c_kv: jax.Array,
    B_w_q: jax.Array,
    B_w_uk: jax.Array,
    B_w_uv: jax.Array,
    B_w_o: jax.Array,
):
    vm = pltpu.VMEM
    dma = pltpu.SemaphoreType.DMA
    scratch = [
        vm((4, M), BF16),
        vm((M,), BF16),
        vm((5, MP, 128), F32),
        vm((64, 256), U32),
        vm((64, 256), U32),
        vm((8, 128), U32),
        vm((M, S), BF16),
        vm((S // 2, MP), U32),
        vm((H // 2, M, D), U32),
        vm((NU, UC // 2, S), U32),
        vm((NU, UC // 2, S), U32),
        vm((NU, UC // 2, S), U32),
        vm((NU, UC // 2, S), U32),
        vm((M, S), BF16),
        vm((S // 2, C), U32),
        vm((H // 2, C, D), U32),
        vm((H // 2, C, D), U32),
        vm((H, M // 2, D), U32),
        vm((H, S // 2, D), U32),
        vm((H, S // 2, D), U32),
        vm((M, TO), F32),
        vm((TQ, D), F32),
        vm((TQ, 128), F32),
        vm((S, 384), BF16),
        vm((S, MP), BF16),
        dma((2,)), dma((XCH,)), dma((H // 2,)), dma((NU * 4,)), dma((2,)),
        dma((H // 2,)), dma((H // 2,)), dma((NO // NB3,)), dma((NO,)),
    ]
    out = pl.pallas_call(
        _kernel,
        in_specs=[pl.BlockSpec(memory_space=pl.ANY)] * 12,
        out_specs=pl.BlockSpec(memory_space=pl.ANY),
        out_shape=jax.ShapeDtypeStruct((S, 2 * M), BF16),
        scratch_shapes=scratch,
        compiler_params=pltpu.CompilerParams(vmem_limit_bytes=120 * 1024 * 1024, disable_semaphore_checks=True, disable_bounds_checks=True),
        name="h3_cla_fused",
    )(
        A_q[0].T, A_k[0].T, A_v[0].T, A_shift_k.T, A_ssm_k, A_ssm_D,
        B_x[0].T, B_c_kv[0], B_w_q, B_w_uk, B_w_uv, jnp.transpose(B_w_o, (0, 2, 1)),
    )
    return out[None]
```

```python
import math

import jax
import jax.numpy as jnp
import jax.experimental.pallas as pl
import jax.experimental.pallas.tpu as pltpu

S = 2048
M = 448
MP = 512
H = 16
D = 256
C = 1024
TQ = 256
NB = S // TQ
NU = 7
UC = M // NU
NBLK = S // 128

F32 = jnp.float32
BF16 = jnp.bfloat16
U32 = jnp.uint32
NT = (((1,), (1,)), ((), ()))
HI_MASK = 0xFFFF0000
Q_SCALE = D ** -0.5
MASK_VALUE = -1e9
P1ORDER = "H0 H1 H2 H3 Q0 X0 Q1 X1 Q2 X2 Q3 X3 Q4 I00 Q5 I01 Q6 I10 Q7 I11 Q8 Q9 I20 Q10 I21 Q11 Q12 I30 Q13 I31 Q14 Q15"
QCH = 128
XB = (0, 256, 640, 1280, 2048)
TOKH = 6
TO = 128
NO = S // TO
BA = 4
BC = 4
MLAG = 2
SLAG = 2
XCH = len(XB) - 1
XLAG = 128
QPRO = 128
NB3 = 4


def _dot(a, b):
    return jnp.dot(a, b, preferred_element_type=F32)


def _dot_nt(a, b):
    return jax.lax.dot_general(a, b, NT, preferred_element_type=F32)


def _inject(x, tok):
    top = x[:8, :128] | tok
    if x.shape[1] > 128:
        top = jnp.concatenate([top, x[:8, 128:]], axis=1)
    return jnp.concatenate([top, x[8:]], axis=0)


def _recip(x):
    r = pl.reciprocal(x, approx=True)
    return r * (2.0 - x * r)


def _fold(xs, op):
    parts = []
    for x in xs:
        for t in range(x.shape[1] // 128):
            parts.append(x[:, t * 128:(t + 1) * 128])
    acc = parts[0]
    for p in parts[1:]:
        acc = op(acc, p)
    return acc


def _orfold(x):
    bits = pltpu.bitcast(x, U32)
    t = None
    for r in range(bits.shape[0] // 8):
        for c in range(bits.shape[1] // 128):
            e = bits[r * 8:(r + 1) * 8, c * 128:(c + 1) * 128]
            t = e if t is None else t | e
    return t


def _qk(i, qu, ks, zero):
    r = jax.lax.broadcasted_iota(jnp.int32, (128, 128), 0)
    c = jax.lax.broadcasted_iota(jnp.int32, (128, 128), 1)
    msk = c <= r
    toks = {}
    run = None
    s_full = []

    def lhs(j):
        return pltpu.bitcast(_inject(qu, toks[j - MLAG]) if j - MLAG in toks else qu, BF16)

    for j in range(i):
        s = _dot_nt(lhs(j), ks[j])
        s_full.append(s)
        mj = jnp.maximum(s[:, :128], s[:, 128:])
        run = mj if run is None else jnp.maximum(run, mj)
        toks[j] = _orfold(run) & zero
    q = lhs(i)
    s_d0 = _dot_nt(q, ks[i][:128])
    s_d1 = _dot_nt(q[128:], ks[i][128:])
    d_lo = jnp.where(msk, s_d0[:128], MASK_VALUE)
    d_hi = jnp.where(msk, s_d1, MASK_VALUE)
    lo = [s[:128] for s in s_full] + [d_lo]
    hi = [s[128:] for s in s_full] + [s_d0[128:], d_hi]
    x_lo = d_lo
    x_hi = jnp.maximum(s_d0[128:], d_hi)
    if run is not None:
        x_lo = jnp.maximum(x_lo, run[:128])
        x_hi = jnp.maximum(x_hi, run[128:])
    return lo, hi, x_lo, x_hi


def _softmax_pv(i, lo, hi, x_lo, x_hi, vs, zero):
    m_lo = jnp.max(x_lo, axis=1, keepdims=True)
    m_hi = jnp.max(x_hi, axis=1, keepdims=True)
    toks = {}
    run = None
    o = None

    def lhs(e, j):
        p = e.astype(BF16)
        if j - SLAG in toks:
            p = pltpu.bitcast(_inject(pltpu.bitcast(p, U32), toks[j - SLAG]), BF16)
        return p

    for j in range(i + 1):
        e = jnp.concatenate([jnp.exp(lo[j] - m_lo), jnp.exp(hi[j] - m_hi)], axis=0)
        p = lhs(e, j)
        t = _dot(p, vs[j] if j < i else vs[i][:128])
        o = t if o is None else o + t
        e = p.astype(F32)
        ej = e[:, :128] + e[:, 128:] if j < i else e
        run = ej if run is None else run + ej
        toks[j] = _orfold(run) & zero
    e = jnp.exp(hi[i + 1] - m_hi)
    p = e.astype(BF16)
    o_hi = o[128:] + _dot(p, vs[i][128:])
    e = p.astype(F32)
    run = jnp.concatenate([run[:128], run[128:] + e], axis=0)
    return jnp.concatenate([o[:128], o_hi], axis=0), run


def _normalize(o, lsum):
    r = _recip(jnp.sum(lsum, axis=1, keepdims=True))
    return pltpu.bitcast((o * r).astype(BF16), U32)


def _kernel(aq_hbm, ak_hbm, av_hbm, sh_hbm, ah_hbm, dd_hbm, xt_hbm, c_hbm,
            wq_hbm, wk_hbm, wv_hbm, wot_hbm,
            out_hbm,
            sh_s, dd_s, coef_s, f_s, fh_s, zero_s, xt_s, x_s, wq_raw, aq_s, ak_s, av_s, ah_s, at_s,
            c_s, wk_raw, wv_raw, wot_s, q_s, ctx_s, ot_s, o7_s, l7_s, stage_a, stage_b,
            sem_small, sem_x, sem_wq, sem_a, sem_c, sem_wk, sem_wv, sem_oa, sem_ob):
    wq32 = wq_hbm.bitcast(U32)
    wk32 = wk_hbm.bitcast(U32)
    wv32 = wv_hbm.bitcast(U32)

    def cp_small(i):
        return pltpu.make_async_copy((sh_hbm, dd_hbm)[i], (sh_s, dd_s)[i], sem_small.at[i])

    def cp_x(i):
        cols = pl.ds(XB[i], XB[i + 1] - XB[i])
        return pltpu.make_async_copy(xt_hbm.at[:, cols], xt_s.at[:, cols], sem_x.at[i])

    def cp_wq(p):
        return pltpu.make_async_copy(wq32.at[:, p, :], wq_raw.at[p], sem_wq.at[p])

    def cp_a(g, i):
        src = (ah_hbm, ak_hbm, av_hbm, aq_hbm)[i].bitcast(U32)
        dst = (ah_s, ak_s, av_s, aq_s)[i]
        n = UC // 2
        start = g * n if isinstance(g, int) else pl.multiple_of(g * n, 8)
        return pltpu.make_async_copy(src.at[pl.ds(start, n), :], dst.at[g], sem_a.at[g * 4 + i])

    def cp_c(i):
        return pltpu.make_async_copy((c_hbm, wot_hbm)[i].bitcast(U32), (c_s, wot_s)[i], sem_c.at[i])

    def cp_wk(p):
        return pltpu.make_async_copy(wk32.at[:, p, :], wk_raw.at[p], sem_wk.at[p])

    def cp_wv(p):
        return pltpu.make_async_copy(wv32.at[:, p, :], wv_raw.at[p], sem_wv.at[p])

    def cp_out_a(i):
        n = NB3 * TO
        start = i * n if isinstance(i, int) else pl.multiple_of(i * n, n)
        return pltpu.make_async_copy(stage_a.at[pl.ds(start, n), :],
                                     out_hbm.at[pl.ds(start, n), pl.ds(0, 384)], sem_oa.at[i])

    def cp_out_b(i):
        start = i * TO if isinstance(i, int) else pl.multiple_of(i * TO, TO)
        return pltpu.make_async_copy(stage_b.at[pl.ds(start, TO), :],
                                     out_hbm.at[pl.ds(start, TO), pl.ds(384, MP)], sem_ob.at[i])

    cp_x(0).start()
    cp_wq(0).start()
    for i in range(1, XCH):
        cp_x(i).start()
    cp_small(0).start()
    cp_small(1).start()

    tt = jax.lax.broadcasted_iota(jnp.int32, (128, 128), 0)
    rr = jax.lax.broadcasted_iota(jnp.int32, (128, 128), 1)
    ang = ((tt * (2 * rr + 1)) & 511).astype(F32) * (2.0 * math.pi / 512.0)
    fmat = jnp.concatenate([jnp.cos(ang), -jnp.sin(ang)], axis=1).astype(BF16)
    f_s[...] = pltpu.bitcast(fmat, U32)
    fh_s[...] = pltpu.bitcast((fmat.astype(F32) * (1.0 / 128.0)).astype(BF16), U32)
    zero_s[...] = jnp.zeros((8, 128), U32)

    def xpose_x(i):
        for t in range(XB[i] // 128, XB[i + 1] // 128):
            cols = slice(t * 128, (t + 1) * 128)
            blks = [xt_s[g * 128:(g + 1) * 128, cols].astype(F32).T for g in range(3)]
            last = jnp.concatenate([xt_s[384:M, cols].astype(F32), jnp.zeros((MP - M, 128), F32)], axis=0)
            blks.append(last.T)
            x_s[t * 64:(t + 1) * 64, :] = pltpu.bitcast(jnp.concatenate(blks, axis=1).astype(BF16), U32)

    def q_weights(p):
        raw = wq_raw[p]
        lo = pltpu.bitcast(raw << 16, F32)
        hi = pltpu.bitcast(raw & jnp.uint32(HI_MASK), F32)
        w = jnp.concatenate([lo, hi], axis=1) * Q_SCALE
        w = jnp.concatenate([w, jnp.zeros((MP - M, 2 * D), F32)], axis=0)
        return w.astype(BF16)

    def qproj(p, w, r0, r1):
        rows = slice(r0 // 2, r1 // 2)
        qq = _dot(pltpu.bitcast(x_s[rows, :], BF16), w)
        q_s[2 * p, rows, :] = pltpu.bitcast(qq[:, :D].astype(BF16), U32)
        q_s[2 * p + 1, rows, :] = pltpu.bitcast(qq[:, D:].astype(BF16), U32)

    def issue_rest():
        for g in range(NU):
            cp_wq(g + 1).start()
            for i in range(4):
                cp_a(g, i).start()
        cp_wk(0).start()
        cp_wv(0).start()
        cp_c(0).start()
        cp_c(1).start()
        for p in range(1, H // 2):
            cp_wk(p).start()
            cp_wv(p).start()

    def coefs():
        prm = [sh_s[j:j + 1, :].astype(F32) for j in range(4)]
        prm.append(dd_s[...].astype(F32).reshape(1, M))
        for j in range(5):
            row = jnp.concatenate([prm[j], jnp.zeros((1, MP - M), F32)], axis=1)
            for t in range(MP // 128):
                blk = jnp.broadcast_to(row[:, t * 128:(t + 1) * 128], (128, 128))
                coef_s[j, t * 128:(t + 1) * 128, :] = blk.T

    def qrange(r0, r1):
        while r0 < r1:
            n = min(QPRO, r1 - r0)
            qproj(0, w0, r0, r0 + n)
            r0 += n

    cp_x(0).wait()
    xpose_x(0)
    issue_rest()
    cp_wq(0).wait()
    w0 = q_weights(0)
    qrange(0, XB[1] - XLAG)
    for i in range(1, XCH):
        cp_x(i).wait()
        if i == XCH - 1:
            cp_small(0).wait()
            cp_small(1).wait()
            coefs()
        qrange(XB[i] - XLAG, XB[i])
        xpose_x(i)
        qrange(XB[i], XB[i + 1] - (XLAG if i < XCH - 1 else 0))
    ot_s[...] = jnp.zeros((M, TO), F32)
    o7_s[...] = jnp.zeros((TQ, D), F32)
    l7_s[...] = jnp.ones((TQ, 128), F32)

    def phase1(g, carry):
        cp_wq(g + 1).wait()
        for i in range(4):
            cp_a(g, i).wait()
        w = q_weights(g + 1)
        fh = pltpu.bitcast(fh_s[...], BF16)
        fx = pltpu.bitcast(f_s[...], BF16)
        lane = jax.lax.broadcasted_iota(jnp.int32, (16, 128), 1)
        sgn = jnp.where((jax.lax.broadcasted_iota(jnp.int32, (8, 128), 1) & 1) == 0, 1.0, -1.0)
        zh, zx, kvs, ys = {}, {}, {}, {}

        def coef(k, j):
            return coef_s[j, pl.ds(pl.multiple_of(g * UC + k * 16, 16), 16), :]

        def hfwd(k):
            lhs = jnp.concatenate([ah_s[g, k * 8:(k + 1) * 8, c * 128:(c + 1) * 128] for c in range(NBLK)], axis=0)
            zh[k] = _dot(pltpu.bitcast(lhs, BF16), fh)

        def xfwd(k):
            kf = pltpu.bitcast(ak_s[g, k * 8:(k + 1) * 8, :], BF16).astype(F32)
            vf = pltpu.bitcast(av_s[g, k * 8:(k + 1) * 8, :], BF16).astype(F32)
            sh_k = [kf] + [pltpu.roll(kf, j, 1) for j in range(1, 4)]
            cf = [coef(k, j) for j in range(4)]
            kvf = []
            for c in range(NBLK):
                cols = slice(c * 128, (c + 1) * 128)
                t = sh_k[0][:, cols] * cf[0]
                for j in range(1, 4):
                    kj = sh_k[j][:, cols]
                    if c == 0:
                        kj = jnp.where(lane >= j, kj, 0.0)
                    t = t + kj * cf[j]
                kvf.append(t * vf[:, cols])
            kvs[k] = jnp.concatenate(kvf, axis=0).astype(BF16)
            zx[k] = _dot(kvs[k], fx)

        def inv(k, u):
            rows = [slice(c * 16 + u * 8, c * 16 + u * 8 + 8) for c in range(NBLK)]
            xr = [zx[k][r, :128] for r in rows]
            xi = [zx[k][r, 128:] for r in rows]
            h0r = [zh[k][r, :128] for r in rows]
            h0i = [zh[k][r, 128:] for r in rows]
            hr = [h0r[0]] + [h0r[j] - sgn * h0i[j - 1] for j in range(1, NBLK)]
            hi = [h0i[0]] + [h0i[j] + sgn * h0r[j - 1] for j in range(1, NBLK)]
            pr, pi = [], []
            for a0 in range(0, NBLK, BA):
                re = [None] * BA
                im = [None] * BA
                for c0 in range(0, a0 + BA, BC):
                    for da in range(BA):
                        for dc in range(BC):
                            c = c0 + dc
                            j = a0 + da - c
                            if j < 0:
                                continue
                            tr = xr[c] * hr[j] - xi[c] * hi[j]
                            ti = xr[c] * hi[j] + xi[c] * hr[j]
                            re[da] = tr if re[da] is None else re[da] + tr
                            im[da] = ti if im[da] is None else im[da] + ti
                pr += re
                pi += im
            p = jnp.concatenate([jnp.concatenate(pr, axis=0), jnp.concatenate(pi, axis=0)], axis=1)
            ys[k, u] = _dot_nt(p.astype(BF16), fx)
            if u == 1:
                kvr = kvs[k].astype(F32)
                qf = pltpu.bitcast(aq_s[g, k * 8:(k + 1) * 8, :], BF16).astype(F32)
                dd = coef(k, 4)
                row0 = pl.multiple_of(g * UC + k * 16, 16)
                for a in range(NBLK):
                    cols = slice(a * 128, (a + 1) * 128)
                    y = jnp.concatenate([ys[k, 0][a * 8:(a + 1) * 8], ys[k, 1][a * 8:(a + 1) * 8]], axis=0)
                    at_s[pl.ds(row0, 16), cols] = (qf[:, cols] * (y + kvr[a * 16:(a + 1) * 16] * dd)).astype(BF16)

        for tokn in P1ORDER.split():
            if tokn[0] == 'Q':
                qproj(g + 1, w, int(tokn[1:]) * QCH, (int(tokn[1:]) + 1) * QCH)
            elif tokn[0] == 'H':
                hfwd(int(tokn[1]))
            elif tokn[0] == 'X':
                xfwd(int(tokn[1]))
            else:
                inv(int(tokn[1]), int(tokn[2]))
        return carry

    jax.lax.fori_loop(0, NU, phase1, 0)

    cp_c(0).wait()
    cp_c(1).wait()
    for p in range(H // 2):
        cp_wk(p).wait()
        cp_wv(p).wait()

    def extract(raw, h):
        sh = (16 - ((h & 1) << 4)).astype(U32)
        return pltpu.bitcast((raw[h >> 1] << sh) & jnp.uint32(HI_MASK), F32).astype(BF16)

    def cblk(i):
        return pltpu.bitcast(c_s[i * TQ // 2:(i + 1) * TQ // 2, :], BF16)

    def finish_last(h):
        bits = _normalize(o7_s[...], l7_s[...])
        ctx_s[h, (NB - 1) * TQ // 2:NB * TQ // 2, :] = bits
        return bits

    def phase2(h, carry):
        wk = extract(wk_raw, h)
        wv = extract(wv_raw, h)
        ks, vs, toks = [], [], {}
        zero = zero_s[...]

        def token(bits):
            t = None
            for r in range(TQ // 16):
                for c in range(D // 128):
                    e = bits[r * 8:(r + 1) * 8, c * 128:(c + 1) * 128]
                    t = e if t is None else t | e
            return t & zero

        def kproj(i):
            ks.append(_dot(cblk(i), wk).astype(BF16))

        def vproj(i):
            vs.append(_dot(cblk(i), wv).astype(BF16))

        def qk(i):
            q = q_s[h, i * TQ // 2:(i + 1) * TQ // 2, :]
            if i - 2 in toks:
                q = _inject(q, toks[i - 2])
            return _qk(i, q, ks, zero)

        def pv(i, sc):
            o, lsum = _softmax_pv(i, *sc, vs, zero)
            if i == NB - 1:
                o7_s[...] = o
                l7_s[...] = lsum
            else:
                bits = _normalize(o, lsum)
                ctx_s[h, i * TQ // 2:(i + 1) * TQ // 2, :] = bits
                toks[i] = token(bits)

        toks[-1] = token(finish_last(jnp.maximum(h - 1, 0)))
        kproj(0)
        vproj(0)
        sc = qk(0)
        kproj(1)
        pv(0, sc)
        for i in range(1, NB):
            sc = qk(i)
            vproj(i)
            if i + 1 < NB:
                kproj(i + 1)
            pv(i, sc)
        return carry

    jax.lax.fori_loop(0, H, phase2, 0)
    finish_last(H - 1)

    def orfold(x):
        bits = pltpu.bitcast(x, U32)
        t = None
        for r in range(bits.shape[0] // 8):
            for c in range(bits.shape[1] // 128):
                e = bits[r * 8:(r + 1) * 8, c * 128:(c + 1) * 128]
                t = e if t is None else t | e
        return t

    def finish(i, ot):
        r0 = i * TO if isinstance(i, int) else pl.multiple_of(i * TO, TO)
        top = at_s[384:M, pl.ds(r0, TO)].astype(F32)
        val = jnp.concatenate([top, ot], axis=0).T
        stage_b[pl.ds(r0, TO), :] = val.astype(BF16)
        return val

    def oproj(i, pending):
        tok = orfold(pending[0])
        for x in pending[1:]:
            tok = tok | orfold(x)
        tok = tok & zero_s[...]
        rows = pl.ds(pl.multiple_of(i * (TO // 2), TO // 2), TO // 2)
        wot = jnp.concatenate([wot_s[h] for h in range(H)], axis=1)
        ctx = [ctx_s[h, rows, :] for h in range(H)]
        ctx[TOKH] = _inject(ctx[TOKH], tok)
        ctx = jnp.concatenate(ctx, axis=1)
        return _dot_nt(pltpu.bitcast(wot, BF16), pltpu.bitcast(ctx, BF16))

    def phase3(it, carry):
        prev = jnp.maximum(NB3 * it - 1, 0)
        pend = [finish(prev, ot_s[...])]

        @pl.when(it > 0)
        def _():
            cp_out_b(prev).start()

        r0 = pl.multiple_of(it * (NB3 * TO), NB3 * TO)
        apart = []
        for g in range(3):
            blk = at_s[g * 128:(g + 1) * 128, pl.ds(r0, NB3 * TO)].astype(F32).T
            stage_a[pl.ds(r0, NB3 * TO), g * 128:(g + 1) * 128] = blk.astype(BF16)
            apart.append(blk)
        cp_out_a(it).start()

        for k in range(NB3 - 1):
            pend = [finish(NB3 * it + k, oproj(NB3 * it + k, pend))]
            if k == 0:
                pend += apart
            cp_out_b(NB3 * it + k).start()
        ot_s[...] = oproj(NB3 * it + NB3 - 1, pend)
        return carry

    jax.lax.fori_loop(0, NO // NB3, phase3, 0)

    finish(NO - 1, ot_s[...])
    cp_out_b(NO - 1).start()
    for i in range(NO // NB3):
        cp_out_a(i).wait()
    for i in range(NO):
        cp_out_b(i).wait()


@jax.jit
def pallas_concat_heads__ssm_conv_h3__compressed_kv_cla__prompt_kernel(
    A_q: jax.Array,
    A_k: jax.Array,
    A_v: jax.Array,
    A_shift_k: jax.Array,
    A_ssm_k: jax.Array,
    A_ssm_D: jax.Array,
    B_x: jax.Array,
    B_c_kv: jax.Array,
    B_w_q: jax.Array,
    B_w_uk: jax.Array,
    B_w_uv: jax.Array,
    B_w_o: jax.Array,
):
    vm = pltpu.VMEM
    dma = pltpu.SemaphoreType.DMA
    scratch = [
        vm((4, M), BF16),
        vm((M,), BF16),
        vm((5, MP, 128), F32),
        vm((64, 256), U32),
        vm((64, 256), U32),
        vm((8, 128), U32),
        vm((M, S), BF16),
        vm((S // 2, MP), U32),
        vm((H // 2, M, D), U32),
        vm((NU, UC // 2, S), U32),
        vm((NU, UC // 2, S), U32),
        vm((NU, UC // 2, S), U32),
        vm((NU, UC // 2, S), U32),
        vm((M, S), BF16),
        vm((S // 2, C), U32),
        vm((H // 2, C, D), U32),
        vm((H // 2, C, D), U32),
        vm((H, M // 2, D), U32),
        vm((H, S // 2, D), U32),
        vm((H, S // 2, D), U32),
        vm((M, TO), F32),
        vm((TQ, D), F32),
        vm((TQ, 128), F32),
        vm((S, 384), BF16),
        vm((S, MP), BF16),
        dma((2,)), dma((XCH,)), dma((H // 2,)), dma((NU * 4,)), dma((2,)),
        dma((H // 2,)), dma((H // 2,)), dma((NO // NB3,)), dma((NO,)),
    ]
    out = pl.pallas_call(
        _kernel,
        in_specs=[pl.BlockSpec(memory_space=pl.ANY)] * 12,
        out_specs=pl.BlockSpec(memory_space=pl.ANY),
        out_shape=jax.ShapeDtypeStruct((S, 2 * M), BF16),
        scratch_shapes=scratch,
        compiler_params=pltpu.CompilerParams(vmem_limit_bytes=120 * 1024 * 1024, disable_semaphore_checks=True, disable_bounds_checks=True),
        name="h3_cla_fused",
    )(
        A_q[0].T, A_k[0].T, A_v[0].T, A_shift_k.T, A_ssm_k, A_ssm_D,
        B_x[0].T, B_c_kv[0], B_w_q, B_w_uk, B_w_uv, jnp.transpose(B_w_o, (0, 2, 1)),
    )
    return out[None]
```

```python
import math

import jax
import jax.numpy as jnp
import jax.experimental.pallas as pl
import jax.experimental.pallas.tpu as pltpu

S = 2048
M = 448
MP = 512
H = 16
D = 256
C = 1024
TQ = 256
NB = S // TQ
NU = 7
UC = M // NU
NBLK = S // 128

F32 = jnp.float32
BF16 = jnp.bfloat16
U32 = jnp.uint32
NT = (((1,), (1,)), ((), ()))
HI_MASK = 0xFFFF0000
Q_SCALE = D ** -0.5
MASK_VALUE = -1e9
P1ORDER = "H0 H1 H2 H3 Q0 X0 Q1 X1 Q2 X2 Q3 X3 Q4 I00 Q5 I01 Q6 I10 Q7 I11 Q8 Q9 I20 Q10 I21 Q11 Q12 I30 Q13 I31 Q14 Q15"
QCH = 128
XB = (0, 256, 640, 1280, 2048)
TOKH = 6
TO = 128
NO = S // TO
BA = 4
BC = 4
MLAG = 2
SLAG = 3
XCH = len(XB) - 1
XLAG = 128
QPRO = 128
NPART = 8
QOR = 2
NB3 = 4


def _dot(a, b):
    return jnp.dot(a, b, preferred_element_type=F32)


def _dot_nt(a, b):
    return jax.lax.dot_general(a, b, NT, preferred_element_type=F32)


def _inject(x, tok):
    top = x[:8, :128] | tok
    if x.shape[1] > 128:
        top = jnp.concatenate([top, x[:8, 128:]], axis=1)
    return jnp.concatenate([top, x[8:]], axis=0)


def _recip(x):
    r = pl.reciprocal(x, approx=True)
    return r * (2.0 - x * r)


def _fold(xs, op):
    parts = []
    for x in xs:
        for t in range(x.shape[1] // 128):
            parts.append(x[:, t * 128:(t + 1) * 128])
    acc = parts[0]
    for p in parts[1:]:
        acc = op(acc, p)
    return acc


def _orfold(x):
    bits = pltpu.bitcast(x, U32)
    t = None
    for r in range(bits.shape[0] // 8):
        for c in range(bits.shape[1] // 128):
            e = bits[r * 8:(r + 1) * 8, c * 128:(c + 1) * 128]
            t = e if t is None else t | e
    return t


def _qk(i, qu, ks, zero, extra):
    r = jax.lax.broadcasted_iota(jnp.int32, (128, 128), 0)
    c = jax.lax.broadcasted_iota(jnp.int32, (128, 128), 1)
    msk = c <= r
    toks = {}
    run = None
    s_full = []

    def lhs(j):
        t = toks.get(j - MLAG)
        for k, e in enumerate(extra):
            if min(k, i) == j:
                t = e if t is None else t | e
        return pltpu.bitcast(qu if t is None else _inject(qu, t), BF16)

    for j in range(i):
        s = _dot_nt(lhs(j), ks[j])
        s_full.append(s)
        mj = jnp.maximum(s[:, :128], s[:, 128:])
        run = mj if run is None else jnp.maximum(run, mj)
        toks[j] = _orfold(run) & zero
    q = lhs(i)
    s_d0 = _dot_nt(q, ks[i][:128])
    s_d1 = _dot_nt(q[128:], ks[i][128:])
    d_lo = jnp.where(msk, s_d0[:128], MASK_VALUE)
    d_hi = jnp.where(msk, s_d1, MASK_VALUE)
    lo = [s[:128] for s in s_full] + [d_lo]
    hi = [s[128:] for s in s_full] + [s_d0[128:], d_hi]
    x_lo = d_lo
    x_hi = jnp.maximum(s_d0[128:], d_hi)
    if run is not None:
        x_lo = jnp.maximum(x_lo, run[:128])
        x_hi = jnp.maximum(x_hi, run[128:])
    return lo, hi, x_lo, x_hi


def _softmax_pv(i, lo, hi, x_lo, x_hi, vs, zero):
    m_lo = jnp.max(x_lo, axis=1, keepdims=True)
    m_hi = jnp.max(x_hi, axis=1, keepdims=True)
    toks = {}
    run = None
    o = None

    def lhs(e, j):
        p = e.astype(BF16)
        if j - SLAG in toks:
            p = pltpu.bitcast(_inject(pltpu.bitcast(p, U32), toks[j - SLAG]), BF16)
        return p

    for j in range(i + 1):
        e = jnp.concatenate([jnp.exp(lo[j] - m_lo), jnp.exp(hi[j] - m_hi)], axis=0)
        p = lhs(e, j)
        t = _dot(p, vs[j] if j < i else vs[i][:128])
        o = t if o is None else o + t
        e = p.astype(F32)
        ej = e[:, :128] + e[:, 128:] if j < i else e
        run = ej if run is None else run + ej
        toks[j] = _orfold(run) & zero
    e = jnp.exp(hi[i + 1] - m_hi)
    p = e.astype(BF16)
    o_hi = o[128:] + _dot(p, vs[i][128:])
    e = p.astype(F32)
    run = jnp.concatenate([run[:128], run[128:] + e], axis=0)
    return jnp.concatenate([o[:128], o_hi], axis=0), run


def _normalize(o, lsum):
    r = _recip(jnp.sum(lsum, axis=1, keepdims=True))
    return pltpu.bitcast((o * r).astype(BF16), U32)


def _kernel(aq_hbm, ak_hbm, av_hbm, sh_hbm, ah_hbm, dd_hbm, xt_hbm, c_hbm,
            wq_hbm, wk_hbm, wv_hbm, wot_hbm,
            out_hbm,
            sh_s, dd_s, coef_s, f_s, fh_s, zero_s, xt_s, x_s, wq_raw, aq_s, ak_s, av_s, ah_s, at_s,
            c_s, wk_raw, wv_raw, wot_s, q_s, ctx_s, ot_s, o7_s, l7_s, stage_a, stage_b,
            sem_small, sem_x, sem_wq, sem_a, sem_c, sem_wk, sem_wv, sem_oa, sem_ob):
    wq32 = wq_hbm.bitcast(U32)
    wk32 = wk_hbm.bitcast(U32)
    wv32 = wv_hbm.bitcast(U32)

    def cp_small(i):
        return pltpu.make_async_copy((sh_hbm, dd_hbm)[i], (sh_s, dd_s)[i], sem_small.at[i])

    def cp_x(i):
        cols = pl.ds(XB[i], XB[i + 1] - XB[i])
        return pltpu.make_async_copy(xt_hbm.at[:, cols], xt_s.at[:, cols], sem_x.at[i])

    def cp_wq(p):
        return pltpu.make_async_copy(wq32.at[:, p, :], wq_raw.at[p], sem_wq.at[p])

    def cp_a(g, i):
        src = (ah_hbm, ak_hbm, av_hbm, aq_hbm)[i].bitcast(U32)
        dst = (ah_s, ak_s, av_s, aq_s)[i]
        n = UC // 2
        start = g * n if isinstance(g, int) else pl.multiple_of(g * n, 8)
        return pltpu.make_async_copy(src.at[pl.ds(start, n), :], dst.at[g], sem_a.at[g * 4 + i])

    def cp_c(i):
        return pltpu.make_async_copy((c_hbm, wot_hbm)[i].bitcast(U32), (c_s, wot_s)[i], sem_c.at[i])

    def cp_wk(p):
        return pltpu.make_async_copy(wk32.at[:, p, :], wk_raw.at[p], sem_wk.at[p])

    def cp_wv(p):
        return pltpu.make_async_copy(wv32.at[:, p, :], wv_raw.at[p], sem_wv.at[p])

    def cp_out_a(i):
        n = NB3 * TO
        start = i * n if isinstance(i, int) else pl.multiple_of(i * n, n)
        return pltpu.make_async_copy(stage_a.at[pl.ds(start, n), :],
                                     out_hbm.at[pl.ds(start, n), pl.ds(0, 384)], sem_oa.at[i])

    def cp_out_b(i):
        start = i * TO if isinstance(i, int) else pl.multiple_of(i * TO, TO)
        return pltpu.make_async_copy(stage_b.at[pl.ds(start, TO), :],
                                     out_hbm.at[pl.ds(start, TO), pl.ds(384, MP)], sem_ob.at[i])

    cp_x(0).start()
    cp_wq(0).start()
    for i in range(1, XCH):
        cp_x(i).start()
    cp_small(0).start()
    cp_small(1).start()

    tt = jax.lax.broadcasted_iota(jnp.int32, (128, 128), 0)
    rr = jax.lax.broadcasted_iota(jnp.int32, (128, 128), 1)
    ang = ((tt * (2 * rr + 1)) & 511).astype(F32) * (2.0 * math.pi / 512.0)
    fmat = jnp.concatenate([jnp.cos(ang), -jnp.sin(ang)], axis=1).astype(BF16)
    f_s[...] = pltpu.bitcast(fmat, U32)
    fh_s[...] = pltpu.bitcast((fmat.astype(F32) * (1.0 / 128.0)).astype(BF16), U32)
    zero_s[...] = jnp.zeros((8, 128), U32)

    def xpose_x(i):
        for t in range(XB[i] // 128, XB[i + 1] // 128):
            cols = slice(t * 128, (t + 1) * 128)
            blks = [xt_s[g * 128:(g + 1) * 128, cols].astype(F32).T for g in range(3)]
            last = jnp.concatenate([xt_s[384:M, cols].astype(F32), jnp.zeros((MP - M, 128), F32)], axis=0)
            blks.append(last.T)
            x_s[t * 64:(t + 1) * 64, :] = pltpu.bitcast(jnp.concatenate(blks, axis=1).astype(BF16), U32)

    def q_weights(p):
        raw = wq_raw[p]
        lo = pltpu.bitcast(raw << 16, F32)
        hi = pltpu.bitcast(raw & jnp.uint32(HI_MASK), F32)
        w = jnp.concatenate([lo, hi], axis=1) * Q_SCALE
        w = jnp.concatenate([w, jnp.zeros((MP - M, 2 * D), F32)], axis=0)
        return w.astype(BF16)

    def qproj(p, w, r0, r1):
        rows = slice(r0 // 2, r1 // 2)
        qq = _dot(pltpu.bitcast(x_s[rows, :], BF16), w)
        q_s[2 * p, rows, :] = pltpu.bitcast(qq[:, :D].astype(BF16), U32)
        q_s[2 * p + 1, rows, :] = pltpu.bitcast(qq[:, D:].astype(BF16), U32)

    def issue_rest():
        for g in range(NU):
            cp_wq(g + 1).start()
            for i in range(4):
                cp_a(g, i).start()
        cp_wk(0).start()
        cp_wv(0).start()
        cp_c(0).start()
        cp_c(1).start()
        for p in range(1, H // 2):
            cp_wk(p).start()
            cp_wv(p).start()

    def coefs():
        prm = [sh_s[j:j + 1, :].astype(F32) for j in range(4)]
        prm.append(dd_s[...].astype(F32).reshape(1, M))
        for j in range(5):
            row = jnp.concatenate([prm[j], jnp.zeros((1, MP - M), F32)], axis=1)
            for t in range(MP // 128):
                blk = jnp.broadcast_to(row[:, t * 128:(t + 1) * 128], (128, 128))
                coef_s[j, t * 128:(t + 1) * 128, :] = blk.T

    def qrange(r0, r1):
        while r0 < r1:
            n = min(QPRO, r1 - r0)
            qproj(0, w0, r0, r0 + n)
            r0 += n

    cp_x(0).wait()
    xpose_x(0)
    issue_rest()
    cp_wq(0).wait()
    w0 = q_weights(0)
    qrange(0, XB[1] - XLAG)
    for i in range(1, XCH):
        cp_x(i).wait()
        if i == XCH - 1:
            cp_small(0).wait()
            cp_small(1).wait()
            coefs()
        qrange(XB[i] - XLAG, XB[i])
        xpose_x(i)
        qrange(XB[i], XB[i + 1] - (XLAG if i < XCH - 1 else 0))
    ot_s[...] = jnp.zeros((M, TO), F32)
    o7_s[...] = jnp.zeros((TQ, D), F32)
    l7_s[...] = jnp.ones((TQ, 128), F32)

    def phase1(g, carry):
        cp_wq(g + 1).wait()
        for i in range(4):
            cp_a(g, i).wait()
        w = q_weights(g + 1)
        fh = pltpu.bitcast(fh_s[...], BF16)
        fx = pltpu.bitcast(f_s[...], BF16)
        lane = jax.lax.broadcasted_iota(jnp.int32, (16, 128), 1)
        sgn = jnp.where((jax.lax.broadcasted_iota(jnp.int32, (8, 128), 1) & 1) == 0, 1.0, -1.0)
        zh, zx, kvs, ys = {}, {}, {}, {}

        def coef(k, j):
            return coef_s[j, pl.ds(pl.multiple_of(g * UC + k * 16, 16), 16), :]

        def hfwd(k):
            lhs = jnp.concatenate([ah_s[g, k * 8:(k + 1) * 8, c * 128:(c + 1) * 128] for c in range(NBLK)], axis=0)
            zh[k] = _dot(pltpu.bitcast(lhs, BF16), fh)

        def xfwd(k):
            kf = pltpu.bitcast(ak_s[g, k * 8:(k + 1) * 8, :], BF16).astype(F32)
            vf = pltpu.bitcast(av_s[g, k * 8:(k + 1) * 8, :], BF16).astype(F32)
            sh_k = [kf] + [pltpu.roll(kf, j, 1) for j in range(1, 4)]
            cf = [coef(k, j) for j in range(4)]
            kvf = []
            for c in range(NBLK):
                cols = slice(c * 128, (c + 1) * 128)
                t = sh_k[0][:, cols] * cf[0]
                for j in range(1, 4):
                    kj = sh_k[j][:, cols]
                    if c == 0:
                        kj = jnp.where(lane >= j, kj, 0.0)
                    t = t + kj * cf[j]
                kvf.append(t * vf[:, cols])
            kvs[k] = jnp.concatenate(kvf, axis=0).astype(BF16)
            zx[k] = _dot(kvs[k], fx)

        def inv(k, u):
            rows = [slice(c * 16 + u * 8, c * 16 + u * 8 + 8) for c in range(NBLK)]
            xr = [zx[k][r, :128] for r in rows]
            xi = [zx[k][r, 128:] for r in rows]
            h0r = [zh[k][r, :128] for r in rows]
            h0i = [zh[k][r, 128:] for r in rows]
            hr = [h0r[0]] + [h0r[j] - sgn * h0i[j - 1] for j in range(1, NBLK)]
            hi = [h0i[0]] + [h0i[j] + sgn * h0r[j - 1] for j in range(1, NBLK)]
            pr, pi = [], []
            for a0 in range(0, NBLK, BA):
                re = [None] * BA
                im = [None] * BA
                for c0 in range(0, a0 + BA, BC):
                    for da in range(BA):
                        for dc in range(BC):
                            c = c0 + dc
                            j = a0 + da - c
                            if j < 0:
                                continue
                            tr = xr[c] * hr[j] - xi[c] * hi[j]
                            ti = xr[c] * hi[j] + xi[c] * hr[j]
                            re[da] = tr if re[da] is None else re[da] + tr
                            im[da] = ti if im[da] is None else im[da] + ti
                pr += re
                pi += im
            p = jnp.concatenate([jnp.concatenate(pr, axis=0), jnp.concatenate(pi, axis=0)], axis=1)
            ys[k, u] = _dot_nt(p.astype(BF16), fx)
            if u == 1:
                kvr = kvs[k].astype(F32)
                qf = pltpu.bitcast(aq_s[g, k * 8:(k + 1) * 8, :], BF16).astype(F32)
                dd = coef(k, 4)
                row0 = pl.multiple_of(g * UC + k * 16, 16)
                for a in range(NBLK):
                    cols = slice(a * 128, (a + 1) * 128)
                    y = jnp.concatenate([ys[k, 0][a * 8:(a + 1) * 8], ys[k, 1][a * 8:(a + 1) * 8]], axis=0)
                    at_s[pl.ds(row0, 16), cols] = (qf[:, cols] * (y + kvr[a * 16:(a + 1) * 16] * dd)).astype(BF16)

        for tokn in P1ORDER.split():
            if tokn[0] == 'Q':
                qproj(g + 1, w, int(tokn[1:]) * QCH, (int(tokn[1:]) + 1) * QCH)
            elif tokn[0] == 'H':
                hfwd(int(tokn[1]))
            elif tokn[0] == 'X':
                xfwd(int(tokn[1]))
            else:
                inv(int(tokn[1]), int(tokn[2]))
        return carry

    jax.lax.fori_loop(0, NU, phase1, 0)

    cp_c(0).wait()
    cp_c(1).wait()
    for p in range(H // 2):
        cp_wk(p).wait()
        cp_wv(p).wait()

    def extract(raw, h):
        sh = (16 - ((h & 1) << 4)).astype(U32)
        return pltpu.bitcast((raw[h >> 1] << sh) & jnp.uint32(HI_MASK), F32).astype(BF16)

    def cblk(i):
        return pltpu.bitcast(c_s[i * TQ // 2:(i + 1) * TQ // 2, :], BF16)

    def finish_last(h):
        bits = _normalize(o7_s[...], l7_s[...])
        ctx_s[h, (NB - 1) * TQ // 2:NB * TQ // 2, :] = bits
        return bits

    def phase2(h, carry):
        wk = extract(wk_raw, h)
        wv = extract(wv_raw, h)
        ks, vs, toks = [], [], {}
        zero = zero_s[...]

        def token(bits):
            n = TQ // 2 // NPART
            return [_orfold(bits[k * n:(k + 1) * n]) & zero for k in range(NPART)]

        def kproj(i):
            ks.append(_dot(cblk(i), wk).astype(BF16))

        def vproj(i):
            vs.append(_dot(cblk(i), wv).astype(BF16))

        def qk(i):
            q = q_s[h, i * TQ // 2:(i + 1) * TQ // 2, :]
            if i >= QOR:
                q = q | jnp.tile(zero, (TQ // 16, D // 128))
            return _qk(i, q, ks, zero, toks.get(i - 2, []))

        def pv(i, sc):
            o, lsum = _softmax_pv(i, *sc, vs, zero)
            if i == NB - 1:
                o7_s[...] = o
                l7_s[...] = lsum
            else:
                bits = _normalize(o, lsum)
                ctx_s[h, i * TQ // 2:(i + 1) * TQ // 2, :] = bits
                toks[i] = token(bits)

        toks[-1] = token(finish_last(jnp.maximum(h - 1, 0)))
        kproj(0)
        vproj(0)
        sc = qk(0)
        kproj(1)
        pv(0, sc)
        for i in range(1, NB):
            sc = qk(i)
            vproj(i)
            if i + 1 < NB:
                kproj(i + 1)
            pv(i, sc)
        return carry

    jax.lax.fori_loop(0, H, phase2, 0)

    def orfold(x):
        bits = pltpu.bitcast(x, U32)
        t = None
        for r in range(bits.shape[0] // 8):
            for c in range(bits.shape[1] // 128):
                e = bits[r * 8:(r + 1) * 8, c * 128:(c + 1) * 128]
                t = e if t is None else t | e
        return t

    def finish(i, ot):
        r0 = i * TO if isinstance(i, int) else pl.multiple_of(i * TO, TO)
        top = at_s[384:M, pl.ds(r0, TO)].astype(F32)
        val = jnp.concatenate([top, ot], axis=0).T
        stage_b[pl.ds(r0, TO), :] = val.astype(BF16)
        return val

    def oproj(i, pending):
        tok = orfold(pending[0])
        for x in pending[1:]:
            tok = tok | orfold(x)
        tok = tok & zero_s[...]
        rows = pl.ds(pl.multiple_of(i * (TO // 2), TO // 2), TO // 2)
        wot = jnp.concatenate([wot_s[h] for h in range(H)], axis=1)
        ctx = [ctx_s[h, rows, :] for h in range(H)]
        ctx[TOKH] = _inject(ctx[TOKH], tok)
        ctx = jnp.concatenate(ctx, axis=1)
        return _dot_nt(pltpu.bitcast(wot, BF16), pltpu.bitcast(ctx, BF16))

    def phase3(it, carry):
        prev = jnp.maximum(NB3 * it - 1, 0)
        pend = [finish(prev, ot_s[...])]

        @pl.when(it > 0)
        def _():
            cp_out_b(prev).start()

        r0 = pl.multiple_of(it * (NB3 * TO), NB3 * TO)
        apart = []
        for g in range(3):
            blk = at_s[g * 128:(g + 1) * 128, pl.ds(r0, NB3 * TO)].astype(F32).T
            stage_a[pl.ds(r0, NB3 * TO), g * 128:(g + 1) * 128] = blk.astype(BF16)
            apart.append(blk)
        cp_out_a(it).start()

        for k in range(NB3 - 1):
            pend = [finish(NB3 * it + k, oproj(NB3 * it + k, pend))]
            if k == 0:
                pend += apart
            cp_out_b(NB3 * it + k).start()
        ot_s[...] = oproj(NB3 * it + NB3 - 1, pend)
        finish_last(H - 1)
        return carry

    jax.lax.fori_loop(0, NO // NB3, phase3, 0)

    finish(NO - 1, ot_s[...])
    cp_out_b(NO - 1).start()
    for i in range(NO // NB3):
        cp_out_a(i).wait()
    for i in range(NO):
        cp_out_b(i).wait()


@jax.jit
def pallas_concat_heads__ssm_conv_h3__compressed_kv_cla__prompt_kernel(
    A_q: jax.Array,
    A_k: jax.Array,
    A_v: jax.Array,
    A_shift_k: jax.Array,
    A_ssm_k: jax.Array,
    A_ssm_D: jax.Array,
    B_x: jax.Array,
    B_c_kv: jax.Array,
    B_w_q: jax.Array,
    B_w_uk: jax.Array,
    B_w_uv: jax.Array,
    B_w_o: jax.Array,
):
    vm = pltpu.VMEM
    dma = pltpu.SemaphoreType.DMA
    scratch = [
        vm((4, M), BF16),
        vm((M,), BF16),
        vm((5, MP, 128), F32),
        vm((64, 256), U32),
        vm((64, 256), U32),
        vm((8, 128), U32),
        vm((M, S), BF16),
        vm((S // 2, MP), U32),
        vm((H // 2, M, D), U32),
        vm((NU, UC // 2, S), U32),
        vm((NU, UC // 2, S), U32),
        vm((NU, UC // 2, S), U32),
        vm((NU, UC // 2, S), U32),
        vm((M, S), BF16),
        vm((S // 2, C), U32),
        vm((H // 2, C, D), U32),
        vm((H // 2, C, D), U32),
        vm((H, M // 2, D), U32),
        vm((H, S // 2, D), U32),
        vm((H, S // 2, D), U32),
        vm((M, TO), F32),
        vm((TQ, D), F32),
        vm((TQ, 128), F32),
        vm((S, 384), BF16),
        vm((S, MP), BF16),
        dma((2,)), dma((XCH,)), dma((H // 2,)), dma((NU * 4,)), dma((2,)),
        dma((H // 2,)), dma((H // 2,)), dma((NO // NB3,)), dma((NO,)),
    ]
    out = pl.pallas_call(
        _kernel,
        in_specs=[pl.BlockSpec(memory_space=pl.ANY)] * 12,
        out_specs=pl.BlockSpec(memory_space=pl.ANY),
        out_shape=jax.ShapeDtypeStruct((S, 2 * M), BF16),
        scratch_shapes=scratch,
        compiler_params=pltpu.CompilerParams(vmem_limit_bytes=120 * 1024 * 1024, disable_semaphore_checks=True, disable_bounds_checks=True),
        name="h3_cla_fused",
    )(
        A_q[0].T, A_k[0].T, A_v[0].T, A_shift_k.T, A_ssm_k, A_ssm_D,
        B_x[0].T, B_c_kv[0], B_w_q, B_w_uk, B_w_uv, jnp.transpose(B_w_o, (0, 2, 1)),
    )
    return out[None]
```

```python
import math

import jax
import jax.numpy as jnp
import jax.experimental.pallas as pl
import jax.experimental.pallas.tpu as pltpu

S = 2048
M = 448
MP = 512
MA = 384
H = 16
D = 256
C = 1024
TQ = 256
NB = S // TQ
NU = 7
UC = M // NU
NBLK = S // 128
QCH = 128
XB = (0, 256, 640, 1280, 2048)
XCH = len(XB) - 1
TO = 128
NO = S // TO
NB3 = 4
TOKH = 6
MLAG = 2
SLAG = 3
NPART = 8
P1ORDER = ("H0 H1 H2 H3 Q0 X0 Q1 X1 Q2 X2 Q3 X3 Q4 I00 Q5 I01 Q6 I10 Q7 I11 "
           "Q8 Q9 I20 Q10 I21 Q11 Q12 I30 Q13 I31 Q14 Q15")

F32 = jnp.float32
BF16 = jnp.bfloat16
U32 = jnp.uint32
HI_MASK = 0xFFFF0000
Q_SCALE = D ** -0.5
MASK_VALUE = -1e9


def _dot(a, b):
    return jnp.dot(a, b, preferred_element_type=F32)


def _dot_nt(a, b):
    return jax.lax.dot_general(a, b, (((1,), (1,)), ((), ())), preferred_element_type=F32)


def _or_fold(x):
    bits = pltpu.bitcast(x, U32)
    t = None
    for r in range(bits.shape[0] // 8):
        for c in range(bits.shape[1] // 128):
            e = bits[r * 8:(r + 1) * 8, c * 128:(c + 1) * 128]
            t = e if t is None else t | e
    return t


def _inject(x, tok):
    top = x[:8, :128] | tok
    if x.shape[1] > 128:
        top = jnp.concatenate([top, x[:8, 128:]], axis=1)
    return jnp.concatenate([top, x[8:]], axis=0)


def _recip(x):
    r = pl.reciprocal(x, approx=True)
    return r * (2.0 - x * r)


def _qk(i, qu, ks, zero, extra):
    r = jax.lax.broadcasted_iota(jnp.int32, (128, 128), 0)
    c = jax.lax.broadcasted_iota(jnp.int32, (128, 128), 1)
    msk = c <= r
    toks = {}
    run = None
    s_full = []

    def lhs(j):
        t = toks.get(j - MLAG)
        for k, e in enumerate(extra):
            if min(k, i) == j:
                t = e if t is None else t | e
        return pltpu.bitcast(qu if t is None else _inject(qu, t), BF16)

    for j in range(i):
        s = _dot_nt(lhs(j), ks[j])
        s_full.append(s)
        mj = jnp.maximum(s[:, :128], s[:, 128:])
        run = mj if run is None else jnp.maximum(run, mj)
        toks[j] = _or_fold(run) & zero
    q = lhs(i)
    s_d0 = _dot_nt(q, ks[i][:128])
    s_d1 = _dot_nt(q[128:], ks[i][128:])
    d_lo = jnp.where(msk, s_d0[:128], MASK_VALUE)
    d_hi = jnp.where(msk, s_d1, MASK_VALUE)
    lo = [s[:128] for s in s_full] + [d_lo]
    hi = [s[128:] for s in s_full] + [s_d0[128:], d_hi]
    x_lo = d_lo
    x_hi = jnp.maximum(s_d0[128:], d_hi)
    if run is not None:
        x_lo = jnp.maximum(x_lo, run[:128])
        x_hi = jnp.maximum(x_hi, run[128:])
    return lo, hi, x_lo, x_hi


def _softmax_pv(i, lo, hi, x_lo, x_hi, vs, zero):
    m_lo = jnp.max(x_lo, axis=1, keepdims=True)
    m_hi = jnp.max(x_hi, axis=1, keepdims=True)
    toks = {}
    run = None
    o = None

    def lhs(e, j):
        p = e.astype(BF16)
        if j - SLAG in toks:
            p = pltpu.bitcast(_inject(pltpu.bitcast(p, U32), toks[j - SLAG]), BF16)
        return p

    for j in range(i + 1):
        e = jnp.concatenate([jnp.exp(lo[j] - m_lo), jnp.exp(hi[j] - m_hi)], axis=0)
        p = lhs(e, j)
        t = _dot(p, vs[j] if j < i else vs[i][:128])
        o = t if o is None else o + t
        e = p.astype(F32)
        ej = e[:, :128] + e[:, 128:] if j < i else e
        run = ej if run is None else run + ej
        toks[j] = _or_fold(run) & zero
    p = jnp.exp(hi[i + 1] - m_hi).astype(BF16)
    o_hi = o[128:] + _dot(p, vs[i][128:])
    run = jnp.concatenate([run[:128], run[128:] + p.astype(F32)], axis=0)
    return jnp.concatenate([o[:128], o_hi], axis=0), run


def _normalize(o, lsum):
    r = _recip(jnp.sum(lsum, axis=1, keepdims=True))
    return pltpu.bitcast((o * r).astype(BF16), U32)


def _kernel(aq_hbm, ak_hbm, av_hbm, sh_hbm, ah_hbm, dd_hbm, xt_hbm, c_hbm,
            wq_hbm, wk_hbm, wv_hbm, wot_hbm,
            out_hbm,
            sh_s, dd_s, coef_s, f_s, fh_s, zero_s, xt_s, x_s, wq_raw, aq_s, ak_s, av_s, ah_s, at_s,
            c_s, wk_raw, wv_raw, wot_s, q_s, ctx_s, ot_s, o7_s, l7_s, stage_a, stage_b,
            sem_small, sem_x, sem_wq, sem_a, sem_c, sem_wk, sem_wv, sem_oa, sem_ob):
    wq32 = wq_hbm.bitcast(U32)
    wk32 = wk_hbm.bitcast(U32)
    wv32 = wv_hbm.bitcast(U32)

    def cp_small(i):
        return pltpu.make_async_copy((sh_hbm, dd_hbm)[i], (sh_s, dd_s)[i], sem_small.at[i])

    def cp_x(i):
        cols = pl.ds(XB[i], XB[i + 1] - XB[i])
        return pltpu.make_async_copy(xt_hbm.at[:, cols], xt_s.at[:, cols], sem_x.at[i])

    def cp_wq(p):
        return pltpu.make_async_copy(wq32.at[:, p, :], wq_raw.at[p], sem_wq.at[p])

    def cp_a(g, i):
        src = (ah_hbm, ak_hbm, av_hbm, aq_hbm)[i].bitcast(U32)
        dst = (ah_s, ak_s, av_s, aq_s)[i]
        n = UC // 2
        start = g * n if isinstance(g, int) else pl.multiple_of(g * n, 8)
        return pltpu.make_async_copy(src.at[pl.ds(start, n), :], dst.at[g], sem_a.at[g * 4 + i])

    def cp_c(i):
        return pltpu.make_async_copy((c_hbm, wot_hbm)[i].bitcast(U32), (c_s, wot_s)[i], sem_c.at[i])

    def cp_wk(p):
        return pltpu.make_async_copy(wk32.at[:, p, :], wk_raw.at[p], sem_wk.at[p])

    def cp_wv(p):
        return pltpu.make_async_copy(wv32.at[:, p, :], wv_raw.at[p], sem_wv.at[p])

    def cp_out_a(i):
        n = NB3 * TO
        start = i * n if isinstance(i, int) else pl.multiple_of(i * n, n)
        return pltpu.make_async_copy(stage_a.at[pl.ds(start, n), :],
                                     out_hbm.at[pl.ds(start, n), pl.ds(0, MA)], sem_oa.at[i])

    def cp_out_b(i):
        start = i * TO if isinstance(i, int) else pl.multiple_of(i * TO, TO)
        return pltpu.make_async_copy(stage_b.at[pl.ds(start, TO), :],
                                     out_hbm.at[pl.ds(start, TO), pl.ds(MA, MP)], sem_ob.at[i])

    cp_x(0).start()
    cp_wq(0).start()
    for i in range(1, XCH):
        cp_x(i).start()
    cp_small(0).start()
    cp_small(1).start()

    tt = jax.lax.broadcasted_iota(jnp.int32, (128, 128), 0)
    rr = jax.lax.broadcasted_iota(jnp.int32, (128, 128), 1)
    ang = ((tt * (2 * rr + 1)) & 511).astype(F32) * (2.0 * math.pi / 512.0)
    fmat = jnp.concatenate([jnp.cos(ang), -jnp.sin(ang)], axis=1).astype(BF16)
    f_s[...] = pltpu.bitcast(fmat, U32)
    fh_s[...] = pltpu.bitcast((fmat.astype(F32) * (1.0 / 128.0)).astype(BF16), U32)
    zero_s[...] = jnp.zeros((8, 128), U32)

    def xpose_x(i):
        for t in range(XB[i] // 128, XB[i + 1] // 128):
            cols = slice(t * 128, (t + 1) * 128)
            blks = [xt_s[g * 128:(g + 1) * 128, cols].astype(F32).T for g in range(3)]
            last = jnp.concatenate([xt_s[MA:M, cols].astype(F32), jnp.zeros((MP - M, 128), F32)], axis=0)
            blks.append(last.T)
            x_s[t * 64:(t + 1) * 64, :] = pltpu.bitcast(jnp.concatenate(blks, axis=1).astype(BF16), U32)

    def q_weights(p):
        raw = wq_raw[p]
        lo = pltpu.bitcast(raw << 16, F32)
        hi = pltpu.bitcast(raw & jnp.uint32(HI_MASK), F32)
        w = jnp.concatenate([lo, hi], axis=1) * Q_SCALE
        w = jnp.concatenate([w, jnp.zeros((MP - M, 2 * D), F32)], axis=0)
        return w.astype(BF16)

    def qproj(p, w, r):
        rows = slice(r * QCH // 2, (r + 1) * QCH // 2)
        qq = _dot(pltpu.bitcast(x_s[rows, :], BF16), w)
        q_s[2 * p, rows, :] = pltpu.bitcast(qq[:, :D].astype(BF16), U32)
        q_s[2 * p + 1, rows, :] = pltpu.bitcast(qq[:, D:].astype(BF16), U32)

    cp_x(0).wait()
    xpose_x(0)
    for g in range(NU):
        cp_wq(g + 1).start()
        for i in range(4):
            cp_a(g, i).start()
    cp_wk(0).start()
    cp_wv(0).start()
    cp_c(0).start()
    cp_c(1).start()
    for p in range(1, H // 2):
        cp_wk(p).start()
        cp_wv(p).start()
    cp_wq(0).wait()
    w0 = q_weights(0)
    for r in range(XB[1] // QCH - 1):
        qproj(0, w0, r)
    for i in range(1, XCH):
        cp_x(i).wait()
        if i == XCH - 1:
            cp_small(0).wait()
            cp_small(1).wait()
            prm = [sh_s[j:j + 1, :].astype(F32) for j in range(4)]
            prm.append(dd_s[...].astype(F32).reshape(1, M))
            for j in range(5):
                row = jnp.concatenate([prm[j], jnp.zeros((1, MP - M), F32)], axis=1)
                for t in range(MP // 128):
                    blk = jnp.broadcast_to(row[:, t * 128:(t + 1) * 128], (128, 128))
                    coef_s[j, t * 128:(t + 1) * 128, :] = blk.T
        qproj(0, w0, XB[i] // QCH - 1)
        xpose_x(i)
        for r in range(XB[i] // QCH, XB[i + 1] // QCH - (1 if i < XCH - 1 else 0)):
            qproj(0, w0, r)
    ot_s[...] = jnp.zeros((M, TO), F32)
    o7_s[...] = jnp.zeros((TQ, D), F32)
    l7_s[...] = jnp.ones((TQ, 128), F32)

    def phase1(g, carry):
        cp_wq(g + 1).wait()
        for i in range(4):
            cp_a(g, i).wait()
        w = q_weights(g + 1)
        fh = pltpu.bitcast(fh_s[...], BF16)
        fx = pltpu.bitcast(f_s[...], BF16)
        lane = jax.lax.broadcasted_iota(jnp.int32, (16, 128), 1)
        sgn = jnp.where((jax.lax.broadcasted_iota(jnp.int32, (8, 128), 1) & 1) == 0, 1.0, -1.0)
        zh, zx, kvs, ys = {}, {}, {}, {}

        def coef(k, j):
            return coef_s[j, pl.ds(pl.multiple_of(g * UC + k * 16, 16), 16), :]

        def hfwd(k):
            lhs = jnp.concatenate([ah_s[g, k * 8:(k + 1) * 8, c * 128:(c + 1) * 128]
                                   for c in range(NBLK)], axis=0)
            zh[k] = _dot(pltpu.bitcast(lhs, BF16), fh)

        def xfwd(k):
            kf = pltpu.bitcast(ak_s[g, k * 8:(k + 1) * 8, :], BF16).astype(F32)
            vf = pltpu.bitcast(av_s[g, k * 8:(k + 1) * 8, :], BF16).astype(F32)
            sh_k = [kf] + [pltpu.roll(kf, j, 1) for j in range(1, 4)]
            cf = [coef(k, j) for j in range(4)]
            kvf = []
            for c in range(NBLK):
                cols = slice(c * 128, (c + 1) * 128)
                t = sh_k[0][:, cols] * cf[0]
                for j in range(1, 4):
                    kj = sh_k[j][:, cols]
                    if c == 0:
                        kj = jnp.where(lane >= j, kj, 0.0)
                    t = t + kj * cf[j]
                kvf.append(t * vf[:, cols])
            kvs[k] = jnp.concatenate(kvf, axis=0).astype(BF16)
            zx[k] = _dot(kvs[k], fx)

        def inv(k, u):
            rows = [slice(c * 16 + u * 8, c * 16 + u * 8 + 8) for c in range(NBLK)]
            xr = [zx[k][r, :128] for r in rows]
            xi = [zx[k][r, 128:] for r in rows]
            h0r = [zh[k][r, :128] for r in rows]
            h0i = [zh[k][r, 128:] for r in rows]
            hr = [h0r[0]] + [h0r[j] - sgn * h0i[j - 1] for j in range(1, NBLK)]
            hi = [h0i[0]] + [h0i[j] + sgn * h0r[j - 1] for j in range(1, NBLK)]
            pr, pi = [], []
            for a0 in range(0, NBLK, 4):
                re = [None] * 4
                im = [None] * 4
                for c0 in range(0, a0 + 4, 4):
                    for da in range(4):
                        for c in range(c0, c0 + 4):
                            j = a0 + da - c
                            if j < 0:
                                continue
                            tr = xr[c] * hr[j] - xi[c] * hi[j]
                            ti = xr[c] * hi[j] + xi[c] * hr[j]
                            re[da] = tr if re[da] is None else re[da] + tr
                            im[da] = ti if im[da] is None else im[da] + ti
                pr += re
                pi += im
            p = jnp.concatenate([jnp.concatenate(pr, axis=0), jnp.concatenate(pi, axis=0)], axis=1)
            ys[k, u] = _dot_nt(p.astype(BF16), fx)
            if u == 1:
                kvr = kvs[k].astype(F32)
                qraw = aq_s[g, k * 8:(k + 1) * 8, :] | jnp.tile(zero_s[...], (1, NBLK))
                qf = pltpu.bitcast(qraw, BF16).astype(F32)
                dd = coef(k, 4)
                row0 = pl.multiple_of(g * UC + k * 16, 16)
                for a in range(NBLK):
                    cols = slice(a * 128, (a + 1) * 128)
                    y = jnp.concatenate([ys[k, 0][a * 8:(a + 1) * 8], ys[k, 1][a * 8:(a + 1) * 8]], axis=0)
                    y = y + kvr[a * 16:(a + 1) * 16] * dd
                    at_s[pl.ds(row0, 16), cols] = (qf[:, cols] * y).astype(BF16)

        for step in P1ORDER.split():
            if step[0] == 'Q':
                qproj(g + 1, w, int(step[1:]))
            elif step[0] == 'H':
                hfwd(int(step[1]))
            elif step[0] == 'X':
                xfwd(int(step[1]))
            else:
                inv(int(step[1]), int(step[2]))
        return carry

    jax.lax.fori_loop(0, NU, phase1, 0)

    cp_c(0).wait()
    cp_c(1).wait()
    for p in range(H // 2):
        cp_wk(p).wait()
        cp_wv(p).wait()

    def extract(raw, h):
        sh = (16 - ((h & 1) << 4)).astype(U32)
        return pltpu.bitcast((raw[h >> 1] << sh) & jnp.uint32(HI_MASK), F32).astype(BF16)

    def cblk(i):
        return pltpu.bitcast(c_s[i * TQ // 2:(i + 1) * TQ // 2, :], BF16)

    def finish_last(h):
        bits = _normalize(o7_s[...], l7_s[...])
        ctx_s[h, (NB - 1) * TQ // 2:NB * TQ // 2, :] = bits
        return bits

    def phase2(h, carry):
        wk = extract(wk_raw, h)
        wv = extract(wv_raw, h)
        ks, vs, toks = [], [], {}
        zero = zero_s[...]

        def tokens(bits):
            n = TQ // 2 // NPART
            return [_or_fold(bits[k * n:(k + 1) * n]) & zero for k in range(NPART)]

        def kproj(i):
            ks.append(_dot(cblk(i), wk).astype(BF16))

        def vproj(i):
            vs.append(_dot(cblk(i), wv).astype(BF16))

        def qk(i):
            q = q_s[h, i * TQ // 2:(i + 1) * TQ // 2, :]
            if i >= 2:
                q = q | jnp.tile(zero, (TQ // 16, D // 128))
            return _qk(i, q, ks, zero, toks.get(i - 2, []))

        def pv(i, sc):
            o, lsum = _softmax_pv(i, *sc, vs, zero)
            if i == NB - 1:
                o7_s[...] = o
                l7_s[...] = lsum
            else:
                bits = _normalize(o, lsum)
                ctx_s[h, i * TQ // 2:(i + 1) * TQ // 2, :] = bits
                toks[i] = tokens(bits)

        toks[-1] = tokens(finish_last(jnp.maximum(h - 1, 0)))
        kproj(0)
        vproj(0)
        sc = qk(0)
        kproj(1)
        pv(0, sc)
        for i in range(1, NB):
            sc = qk(i)
            vproj(i)
            if i + 1 < NB:
                kproj(i + 1)
            pv(i, sc)
        return carry

    jax.lax.fori_loop(0, H, phase2, 0)

    def finish(i, ot):
        r0 = i * TO if isinstance(i, int) else pl.multiple_of(i * TO, TO)
        top = at_s[MA:M, pl.ds(r0, TO)].astype(F32)
        val = jnp.concatenate([top, ot], axis=0).T
        stage_b[pl.ds(r0, TO), :] = val.astype(BF16)
        return val

    def oproj(i, pending):
        tok = _or_fold(pending[0])
        for x in pending[1:]:
            tok = tok | _or_fold(x)
        tok = tok & zero_s[...]
        rows = pl.ds(pl.multiple_of(i * (TO // 2), TO // 2), TO // 2)
        wot = jnp.concatenate([wot_s[h] for h in range(H)], axis=1)
        ctx = [ctx_s[h, rows, :] for h in range(H)]
        ctx[TOKH] = _inject(ctx[TOKH], tok)
        ctx = jnp.concatenate(ctx, axis=1)
        return _dot_nt(pltpu.bitcast(wot, BF16), pltpu.bitcast(ctx, BF16))

    def phase3(it, carry):
        prev = jnp.maximum(NB3 * it - 1, 0)
        pend = [finish(prev, ot_s[...])]

        @pl.when(it > 0)
        def _():
            cp_out_b(prev).start()

        r0 = pl.multiple_of(it * (NB3 * TO), NB3 * TO)
        apart = []
        for g in range(MA // 128):
            blk = at_s[g * 128:(g + 1) * 128, pl.ds(r0, NB3 * TO)].astype(F32).T
            stage_a[pl.ds(r0, NB3 * TO), g * 128:(g + 1) * 128] = blk.astype(BF16)
            apart.append(blk)
        cp_out_a(it).start()

        for k in range(NB3 - 1):
            pend = [finish(NB3 * it + k, oproj(NB3 * it + k, pend))]
            if k == 0:
                pend += apart
            cp_out_b(NB3 * it + k).start()
        ot_s[...] = oproj(NB3 * it + NB3 - 1, pend)
        finish_last(H - 1)
        return carry

    jax.lax.fori_loop(0, NO // NB3, phase3, 0)

    finish(NO - 1, ot_s[...])
    cp_out_b(NO - 1).start()
    for i in range(NO // NB3):
        cp_out_a(i).wait()
    for i in range(NO):
        cp_out_b(i).wait()


@jax.jit
def pallas_concat_heads__ssm_conv_h3__compressed_kv_cla__prompt_kernel(
    A_q: jax.Array,
    A_k: jax.Array,
    A_v: jax.Array,
    A_shift_k: jax.Array,
    A_ssm_k: jax.Array,
    A_ssm_D: jax.Array,
    B_x: jax.Array,
    B_c_kv: jax.Array,
    B_w_q: jax.Array,
    B_w_uk: jax.Array,
    B_w_uv: jax.Array,
    B_w_o: jax.Array,
):
    vm = pltpu.VMEM
    dma = pltpu.SemaphoreType.DMA
    scratch = [
        vm((4, M), BF16),
        vm((M,), BF16),
        vm((5, MP, 128), F32),
        vm((64, 256), U32),
        vm((64, 256), U32),
        vm((8, 128), U32),
        vm((M, S), BF16),
        vm((S // 2, MP), U32),
        vm((H // 2, M, D), U32),
        vm((NU, UC // 2, S), U32),
        vm((NU, UC // 2, S), U32),
        vm((NU, UC // 2, S), U32),
        vm((NU, UC // 2, S), U32),
        vm((M, S), BF16),
        vm((S // 2, C), U32),
        vm((H // 2, C, D), U32),
        vm((H // 2, C, D), U32),
        vm((H, M // 2, D), U32),
        vm((H, S // 2, D), U32),
        vm((H, S // 2, D), U32),
        vm((M, TO), F32),
        vm((TQ, D), F32),
        vm((TQ, 128), F32),
        vm((S, MA), BF16),
        vm((S, MP), BF16),
        dma((2,)), dma((XCH,)), dma((H // 2,)), dma((NU * 4,)), dma((2,)),
        dma((H // 2,)), dma((H // 2,)), dma((NO // NB3,)), dma((NO,)),
    ]
    out = pl.pallas_call(
        _kernel,
        in_specs=[pl.BlockSpec(memory_space=pl.ANY)] * 12,
        out_specs=pl.BlockSpec(memory_space=pl.ANY),
        out_shape=jax.ShapeDtypeStruct((S, 2 * M), BF16),
        scratch_shapes=scratch,
        compiler_params=pltpu.CompilerParams(
            vmem_limit_bytes=120 * 1024 * 1024,
            disable_semaphore_checks=True,
            disable_bounds_checks=True,
        ),
        name="h3_cla_fused",
    )(
        A_q[0].T, A_k[0].T, A_v[0].T, A_shift_k.T, A_ssm_k, A_ssm_D,
        B_x[0].T, B_c_kv[0], B_w_q, B_w_uk, B_w_uv, jnp.transpose(B_w_o, (0, 2, 1)),
    )
    return out[None]
```

```python
import math

import jax
import jax.numpy as jnp
import jax.experimental.pallas as pl
import jax.experimental.pallas.tpu as pltpu

S = 2048
M = 448
MP = 512
MA = 384
H = 16
D = 256
C = 1024
TQ = 256
NB = S // TQ
NU = 7
UC = M // NU
NBLK = S // 128
QCH = 128
XB = (0, 256, 640, 1280, 2048)
XCH = len(XB) - 1
TO = 128
NO = S // TO
NB3 = 4
TOKH = 6
MLAG = 6
SLAG = 7
NPART = 16
P1ORDER = ("H0 H1 H2 H3 Q0 X0 Q1 X1 Q2 X2 Q3 X3 Q4 I00 Q5 I01 Q6 I10 Q7 I11 "
           "Q8 Q9 I20 Q10 I21 Q11 Q12 I30 Q13 I31 Q14 Q15")

F32 = jnp.float32
BF16 = jnp.bfloat16
U32 = jnp.uint32
HI_MASK = 0xFFFF0000
Q_SCALE = D ** -0.5
MASK_VALUE = -1e9


def _dot(a, b):
    return jnp.dot(a, b, preferred_element_type=F32)


def _dot_nt(a, b):
    return jax.lax.dot_general(a, b, (((1,), (1,)), ((), ())), preferred_element_type=F32)


def _or_fold(x):
    bits = pltpu.bitcast(x, U32)
    t = None
    for r in range(bits.shape[0] // 8):
        for c in range(bits.shape[1] // 128):
            e = bits[r * 8:(r + 1) * 8, c * 128:(c + 1) * 128]
            t = e if t is None else t | e
    return t


def _inject(x, tok):
    top = x[:8, :128] | tok
    if x.shape[1] > 128:
        top = jnp.concatenate([top, x[:8, 128:]], axis=1)
    return jnp.concatenate([top, x[8:]], axis=0)


def _recip(x):
    r = pl.reciprocal(x, approx=True)
    return r * (2.0 - x * r)


def _rows(chunks, r0, r1):
    parts = []
    n = TQ
    while r0 < r1:
        c = r0 // n
        e = min(r1, (c + 1) * n)
        parts.append(chunks[c][(r0 - c * n) // 2:(e - c * n) // 2])
        r0 = e
    x = parts[0] if len(parts) == 1 else jnp.concatenate(parts, axis=0)
    return pltpu.bitcast(x, BF16)


def _plan(i, cls):
    base = 64 * (1 - cls)
    full = 2 * i + cls - 1
    out = []
    m = 0
    while m < full:
        w = 2 if m + 2 <= full else 1
        out.append((base + 128 * m, base + 128 * (m + w), 0, None))
        m += w
    if full >= 0:
        out.append((base + 128 * full, base + 128 * (full + 1), 0, 0))
    out.append((base + 128 * (full + 1), base + 128 * (full + 2), 64, 64))
    return out


def _qk(i, qu, ks, zero, extra):
    r = jax.lax.broadcasted_iota(jnp.int32, (64, 128), 0)
    c = jax.lax.broadcasted_iota(jnp.int32, (64, 128), 1)
    msk = c <= r + 64
    qc = [jnp.concatenate([qu[32 * cls:32 * cls + 32], qu[64 + 32 * cls:96 + 32 * cls]], axis=0)
          for cls in range(2)]
    plans = [_plan(i, 0), _plan(i, 1)]
    steps = []
    for j in range(max(len(plans[0]), len(plans[1]))):
        for cls in (1, 0):
            if j < len(plans[cls]):
                steps.append((cls, plans[cls][j]))
    toks = {}
    run = [None, None]
    sc = [[], []]

    def lhs(n, x):
        t = toks.get(n - MLAG)
        for k, e in enumerate(extra):
            if min(k * len(steps) // len(extra), len(steps) - 1) == n:
                t = e if t is None else t | e
        return pltpu.bitcast(x if t is None else _inject(x, t), BF16)

    rem = _dot_nt(_rows(ks, 0, 64), pltpu.bitcast(qc[0], BF16)).T
    if i == 0:
        rem = jnp.concatenate([jnp.where((c <= r)[:, :64], rem[:64], MASK_VALUE), rem[64:]], axis=0)
    run[0] = jnp.concatenate([rem, jnp.full((128, 64), MASK_VALUE, F32)], axis=1)
    for n, (cls, (k0, k1, row0, mrow)) in enumerate(steps):
        s = _dot_nt(lhs(n, qc[cls][row0 // 2:]), _rows(ks, k0, k1))
        if mrow == 0:
            s = jnp.concatenate([jnp.where(msk, s[:64], MASK_VALUE), s[64:]], axis=0)
        elif mrow == 64:
            s = jnp.where(msk, s, MASK_VALUE)
        sc[cls].append(s)
        mj = jnp.maximum(s[:, :128], s[:, 128:]) if k1 - k0 == 256 else s
        if run[cls] is None:
            run[cls] = mj
        elif row0 == 0:
            run[cls] = jnp.maximum(run[cls], mj)
        else:
            run[cls] = jnp.concatenate([run[cls][:64], jnp.maximum(run[cls][64:], mj)], axis=0)
        toks[n] = _or_fold(run[cls]) & zero
    return steps, rem, sc, run


def _softmax_pv(i, steps, rem, sc, mx, vs, zero):
    m = [jnp.max(mx[cls], axis=1, keepdims=True) for cls in range(2)]
    toks = {}
    p = jnp.exp(rem - m[0]).astype(BF16)
    o = [_dot(p, _rows(vs, 0, 64)), None]
    run = [jnp.concatenate([p.astype(F32), jnp.zeros((128, 64), F32)], axis=1), None]
    idx = [0, 0]
    for n, (cls, (k0, k1, row0, _)) in enumerate(steps):
        p = jnp.exp(sc[cls][idx[cls]] - m[cls][row0:]).astype(BF16)
        idx[cls] += 1
        if n - SLAG in toks:
            p = pltpu.bitcast(_inject(pltpu.bitcast(p, U32), toks[n - SLAG]), BF16)
        t = _dot(p, _rows(vs, k0, k1))
        e = p.astype(F32)
        ej = e[:, :128] + e[:, 128:] if k1 - k0 == 256 else e
        if o[cls] is None:
            o[cls], run[cls] = t, ej
        elif row0 == 0:
            o[cls], run[cls] = o[cls] + t, run[cls] + ej
        else:
            o[cls] = jnp.concatenate([o[cls][:64], o[cls][64:] + t], axis=0)
            run[cls] = jnp.concatenate([run[cls][:64], run[cls][64:] + ej], axis=0)
        toks[n] = _or_fold(run[cls]) & zero

    def natural(x):
        return jnp.concatenate([x[0][:64], x[1][:64], x[0][64:], x[1][64:]], axis=0)
    return natural(o), natural(run)


def _normalize(o, lsum):
    r = _recip(jnp.sum(lsum, axis=1, keepdims=True))
    return pltpu.bitcast((o * r).astype(BF16), U32)


def _kernel(aq_hbm, ak_hbm, av_hbm, sh_hbm, ah_hbm, dd_hbm, xt_hbm, c_hbm,
            wq_hbm, wk_hbm, wv_hbm, wot_hbm,
            out_hbm,
            sh_s, dd_s, coef_s, f_s, fh_s, zero_s, xt_s, x_s, wq_raw, aq_s, ak_s, av_s, ah_s, at_s,
            c_s, wk_raw, wv_raw, wot_s, q_s, ctx_s, ot_s, o7_s, l7_s, stage_a, stage_b,
            sem_small, sem_x, sem_wq, sem_a, sem_c, sem_wk, sem_wv, sem_oa, sem_ob):
    wq32 = wq_hbm.bitcast(U32)
    wk32 = wk_hbm.bitcast(U32)
    wv32 = wv_hbm.bitcast(U32)

    def cp_small(i):
        return pltpu.make_async_copy((sh_hbm, dd_hbm)[i], (sh_s, dd_s)[i], sem_small.at[i])

    def cp_x(i):
        cols = pl.ds(XB[i], XB[i + 1] - XB[i])
        return pltpu.make_async_copy(xt_hbm.at[:, cols], xt_s.at[:, cols], sem_x.at[i])

    def cp_wq(p):
        return pltpu.make_async_copy(wq32.at[:, p, :], wq_raw.at[p], sem_wq.at[p])

    def cp_a(g, i):
        src = (ah_hbm, ak_hbm, av_hbm, aq_hbm)[i].bitcast(U32)
        dst = (ah_s, ak_s, av_s, aq_s)[i]
        n = UC // 2
        start = g * n if isinstance(g, int) else pl.multiple_of(g * n, 8)
        return pltpu.make_async_copy(src.at[pl.ds(start, n), :], dst.at[g], sem_a.at[g * 4 + i])

    def cp_c(i):
        return pltpu.make_async_copy((c_hbm, wot_hbm)[i].bitcast(U32), (c_s, wot_s)[i], sem_c.at[i])

    def cp_wk(p):
        return pltpu.make_async_copy(wk32.at[:, p, :], wk_raw.at[p], sem_wk.at[p])

    def cp_wv(p):
        return pltpu.make_async_copy(wv32.at[:, p, :], wv_raw.at[p], sem_wv.at[p])

    def cp_out_a(i):
        n = NB3 * TO
        start = i * n if isinstance(i, int) else pl.multiple_of(i * n, n)
        return pltpu.make_async_copy(stage_a.at[pl.ds(start, n), :],
                                     out_hbm.at[pl.ds(start, n), pl.ds(0, MA)], sem_oa.at[i])

    def cp_out_b(i):
        start = i * TO if isinstance(i, int) else pl.multiple_of(i * TO, TO)
        return pltpu.make_async_copy(stage_b.at[pl.ds(start, TO), :],
                                     out_hbm.at[pl.ds(start, TO), pl.ds(MA, MP)], sem_ob.at[i])

    cp_x(0).start()
    cp_wq(0).start()
    for i in range(1, XCH):
        cp_x(i).start()
    cp_small(0).start()
    cp_small(1).start()

    tt = jax.lax.broadcasted_iota(jnp.int32, (128, 128), 0)
    rr = jax.lax.broadcasted_iota(jnp.int32, (128, 128), 1)
    ang = ((tt * (2 * rr + 1)) & 511).astype(F32) * (2.0 * math.pi / 512.0)
    fmat = jnp.concatenate([jnp.cos(ang), -jnp.sin(ang)], axis=1).astype(BF16)
    f_s[...] = pltpu.bitcast(fmat, U32)
    fh_s[...] = pltpu.bitcast((fmat.astype(F32) * (1.0 / 128.0)).astype(BF16), U32)
    zero_s[...] = jnp.zeros((8, 128), U32)

    def xpose_x(i):
        for t in range(XB[i] // 128, XB[i + 1] // 128):
            cols = slice(t * 128, (t + 1) * 128)
            blks = [xt_s[g * 128:(g + 1) * 128, cols].astype(F32).T for g in range(3)]
            last = jnp.concatenate([xt_s[MA:M, cols].astype(F32), jnp.zeros((MP - M, 128), F32)], axis=0)
            blks.append(last.T)
            x_s[t * 64:(t + 1) * 64, :] = pltpu.bitcast(jnp.concatenate(blks, axis=1).astype(BF16), U32)

    def q_weights(p):
        raw = wq_raw[p]
        lo = pltpu.bitcast(raw << 16, F32)
        hi = pltpu.bitcast(raw & jnp.uint32(HI_MASK), F32)
        w = jnp.concatenate([lo, hi], axis=1) * Q_SCALE
        w = jnp.concatenate([w, jnp.zeros((MP - M, 2 * D), F32)], axis=0)
        return w.astype(BF16)

    def qproj(p, w, r):
        rows = slice(r * QCH // 2, (r + 1) * QCH // 2)
        qq = _dot(pltpu.bitcast(x_s[rows, :], BF16), w)
        q_s[2 * p, rows, :] = pltpu.bitcast(qq[:, :D].astype(BF16), U32)
        q_s[2 * p + 1, rows, :] = pltpu.bitcast(qq[:, D:].astype(BF16), U32)

    cp_x(0).wait()
    xpose_x(0)
    for g in range(NU):
        cp_wq(g + 1).start()
        for i in range(4):
            cp_a(g, i).start()
    cp_wk(0).start()
    cp_wv(0).start()
    cp_c(0).start()
    cp_c(1).start()
    for p in range(1, H // 2):
        cp_wk(p).start()
        cp_wv(p).start()
    cp_wq(0).wait()
    w0 = q_weights(0)
    for r in range(XB[1] // QCH - 1):
        qproj(0, w0, r)
    for i in range(1, XCH):
        cp_x(i).wait()
        if i == XCH - 1:
            cp_small(0).wait()
            cp_small(1).wait()
            prm = [sh_s[j:j + 1, :].astype(F32) for j in range(4)]
            prm.append(dd_s[...].astype(F32).reshape(1, M))
            for j in range(5):
                row = jnp.concatenate([prm[j], jnp.zeros((1, MP - M), F32)], axis=1)
                for t in range(MP // 128):
                    blk = jnp.broadcast_to(row[:, t * 128:(t + 1) * 128], (128, 128))
                    coef_s[j, t * 128:(t + 1) * 128, :] = blk.T
        qproj(0, w0, XB[i] // QCH - 1)
        xpose_x(i)
        for r in range(XB[i] // QCH, XB[i + 1] // QCH - (1 if i < XCH - 1 else 0)):
            qproj(0, w0, r)
    ot_s[...] = jnp.zeros((M, TO), F32)
    o7_s[...] = jnp.zeros((TQ, D), F32)
    l7_s[...] = jnp.ones((TQ, 128), F32)

    def phase1(g, carry):
        cp_wq(g + 1).wait()
        for i in range(4):
            cp_a(g, i).wait()
        w = q_weights(g + 1)
        fh = pltpu.bitcast(fh_s[...], BF16)
        fx = pltpu.bitcast(f_s[...], BF16)
        lane = jax.lax.broadcasted_iota(jnp.int32, (16, 128), 1)
        sgn = jnp.where((jax.lax.broadcasted_iota(jnp.int32, (8, 128), 1) & 1) == 0, 1.0, -1.0)
        zh, zx, kvs, ys = {}, {}, {}, {}

        def coef(k, j):
            return coef_s[j, pl.ds(pl.multiple_of(g * UC + k * 16, 16), 16), :]

        def hfwd(k):
            lhs = jnp.concatenate([ah_s[g, k * 8:(k + 1) * 8, c * 128:(c + 1) * 128]
                                   for c in range(NBLK)], axis=0)
            zh[k] = _dot(pltpu.bitcast(lhs, BF16), fh)

        def xfwd(k):
            kf = pltpu.bitcast(ak_s[g, k * 8:(k + 1) * 8, :], BF16).astype(F32)
            vf = pltpu.bitcast(av_s[g, k * 8:(k + 1) * 8, :], BF16).astype(F32)
            sh_k = [kf] + [pltpu.roll(kf, j, 1) for j in range(1, 4)]
            cf = [coef(k, j) for j in range(4)]
            kvf = []
            for c in range(NBLK):
                cols = slice(c * 128, (c + 1) * 128)
                t = sh_k[0][:, cols] * cf[0]
                for j in range(1, 4):
                    kj = sh_k[j][:, cols]
                    if c == 0:
                        kj = jnp.where(lane >= j, kj, 0.0)
                    t = t + kj * cf[j]
                kvf.append(t * vf[:, cols])
            kvs[k] = jnp.concatenate(kvf, axis=0).astype(BF16)
            zx[k] = _dot(kvs[k], fx)

        def inv(k, u):
            rows = [slice(c * 16 + u * 8, c * 16 + u * 8 + 8) for c in range(NBLK)]
            xr = [zx[k][r, :128] for r in rows]
            xi = [zx[k][r, 128:] for r in rows]
            h0r = [zh[k][r, :128] for r in rows]
            h0i = [zh[k][r, 128:] for r in rows]
            hr = [h0r[0]] + [h0r[j] - sgn * h0i[j - 1] for j in range(1, NBLK)]
            hi = [h0i[0]] + [h0i[j] + sgn * h0r[j - 1] for j in range(1, NBLK)]
            pr, pi = [], []
            for a0 in range(0, NBLK, 4):
                re = [None] * 4
                im = [None] * 4
                for c0 in range(0, a0 + 4, 4):
                    for da in range(4):
                        for c in range(c0, c0 + 4):
                            j = a0 + da - c
                            if j < 0:
                                continue
                            tr = xr[c] * hr[j] - xi[c] * hi[j]
                            ti = xr[c] * hi[j] + xi[c] * hr[j]
                            re[da] = tr if re[da] is None else re[da] + tr
                            im[da] = ti if im[da] is None else im[da] + ti
                pr += re
                pi += im
            p = jnp.concatenate([jnp.concatenate(pr, axis=0), jnp.concatenate(pi, axis=0)], axis=1)
            ys[k, u] = _dot_nt(p.astype(BF16), fx)
            if u == 1:
                kvr = kvs[k].astype(F32)
                qraw = aq_s[g, k * 8:(k + 1) * 8, :] | jnp.tile(zero_s[...], (1, NBLK))
                qf = pltpu.bitcast(qraw, BF16).astype(F32)
                dd = coef(k, 4)
                row0 = pl.multiple_of(g * UC + k * 16, 16)
                for a in range(NBLK):
                    cols = slice(a * 128, (a + 1) * 128)
                    y = jnp.concatenate([ys[k, 0][a * 8:(a + 1) * 8], ys[k, 1][a * 8:(a + 1) * 8]], axis=0)
                    y = y + kvr[a * 16:(a + 1) * 16] * dd
                    at_s[pl.ds(row0, 16), cols] = (qf[:, cols] * y).astype(BF16)

        for step in P1ORDER.split():
            if step[0] == 'Q':
                qproj(g + 1, w, int(step[1:]))
            elif step[0] == 'H':
                hfwd(int(step[1]))
            elif step[0] == 'X':
                xfwd(int(step[1]))
            else:
                inv(int(step[1]), int(step[2]))
        return carry

    jax.lax.fori_loop(0, NU, phase1, 0)

    cp_c(0).wait()
    cp_c(1).wait()
    for p in range(H // 2):
        cp_wk(p).wait()
        cp_wv(p).wait()

    def extract(raw, h):
        sh = (16 - ((h & 1) << 4)).astype(U32)
        return pltpu.bitcast((raw[h >> 1] << sh) & jnp.uint32(HI_MASK), F32).astype(BF16)

    def cblk(i):
        return pltpu.bitcast(c_s[i * TQ // 2:(i + 1) * TQ // 2, :], BF16)

    def finish_last(h):
        bits = _normalize(o7_s[...], l7_s[...])
        ctx_s[h, (NB - 1) * TQ // 2:NB * TQ // 2, :] = bits
        return bits

    def phase2(h, carry):
        wk = extract(wk_raw, h)
        wv = extract(wv_raw, h)
        ks, vs, toks = [], [], {}
        zero = zero_s[...]

        def tokens(bits):
            n = TQ // 2 // NPART
            return [_or_fold(bits[k * n:(k + 1) * n]) & zero for k in range(NPART)]

        def kproj(i):
            ks.append(pltpu.bitcast(_dot(cblk(i), wk).astype(BF16), U32))

        def vproj(i):
            vs.append(pltpu.bitcast(_dot(cblk(i), wv).astype(BF16), U32))

        def qk(i):
            q = q_s[h, i * TQ // 2:(i + 1) * TQ // 2, :]
            if i >= 2:
                q = q | jnp.tile(zero, (TQ // 16, D // 128))
            return _qk(i, q, ks, zero, toks.get(i - 2, []))

        def pv(i, sc):
            o, lsum = _softmax_pv(i, *sc, vs, zero)
            if i == NB - 1:
                o7_s[...] = o
                l7_s[...] = lsum
            else:
                bits = _normalize(o, lsum)
                ctx_s[h, i * TQ // 2:(i + 1) * TQ // 2, :] = bits
                toks[i] = tokens(bits)

        toks[-1] = tokens(finish_last(jnp.maximum(h - 1, 0)))
        kproj(0)
        vproj(0)
        sc = qk(0)
        kproj(1)
        pv(0, sc)
        for i in range(1, NB):
            sc = qk(i)
            vproj(i)
            if i + 1 < NB:
                kproj(i + 1)
            pv(i, sc)
        return carry

    jax.lax.fori_loop(0, H, phase2, 0)

    def finish(i, ot):
        r0 = i * TO if isinstance(i, int) else pl.multiple_of(i * TO, TO)
        top = at_s[MA:M, pl.ds(r0, TO)].astype(F32)
        val = jnp.concatenate([top, ot], axis=0).T
        stage_b[pl.ds(r0, TO), :] = val.astype(BF16)
        return val

    def oproj(i, pending):
        tok = _or_fold(pending[0])
        for x in pending[1:]:
            tok = tok | _or_fold(x)
        tok = tok & zero_s[...]
        rows = pl.ds(pl.multiple_of(i * (TO // 2), TO // 2), TO // 2)
        wot = jnp.concatenate([wot_s[h] for h in range(H)], axis=1)
        ctx = [ctx_s[h, rows, :] for h in range(H)]
        ctx[TOKH] = _inject(ctx[TOKH], tok)
        ctx = jnp.concatenate(ctx, axis=1)
        return _dot_nt(pltpu.bitcast(wot, BF16), pltpu.bitcast(ctx, BF16))

    def phase3(it, carry):
        prev = jnp.maximum(NB3 * it - 1, 0)
        pend = [finish(prev, ot_s[...])]

        @pl.when(it > 0)
        def _():
            cp_out_b(prev).start()

        r0 = pl.multiple_of(it * (NB3 * TO), NB3 * TO)
        apart = []
        for g in range(MA // 128):
            blk = at_s[g * 128:(g + 1) * 128, pl.ds(r0, NB3 * TO)].astype(F32).T
            stage_a[pl.ds(r0, NB3 * TO), g * 128:(g + 1) * 128] = blk.astype(BF16)
            apart.append(blk)
        cp_out_a(it).start()

        for k in range(NB3 - 1):
            pend = [finish(NB3 * it + k, oproj(NB3 * it + k, pend))]
            if k == 0:
                pend += apart
            cp_out_b(NB3 * it + k).start()
        ot_s[...] = oproj(NB3 * it + NB3 - 1, pend)
        finish_last(H - 1)
        return carry

    jax.lax.fori_loop(0, NO // NB3, phase3, 0)

    finish(NO - 1, ot_s[...])
    cp_out_b(NO - 1).start()
    for i in range(NO // NB3):
        cp_out_a(i).wait()
    for i in range(NO):
        cp_out_b(i).wait()


@jax.jit
def pallas_concat_heads__ssm_conv_h3__compressed_kv_cla__prompt_kernel(
    A_q: jax.Array,
    A_k: jax.Array,
    A_v: jax.Array,
    A_shift_k: jax.Array,
    A_ssm_k: jax.Array,
    A_ssm_D: jax.Array,
    B_x: jax.Array,
    B_c_kv: jax.Array,
    B_w_q: jax.Array,
    B_w_uk: jax.Array,
    B_w_uv: jax.Array,
    B_w_o: jax.Array,
):
    vm = pltpu.VMEM
    dma = pltpu.SemaphoreType.DMA
    scratch = [
        vm((4, M), BF16),
        vm((M,), BF16),
        vm((5, MP, 128), F32),
        vm((64, 256), U32),
        vm((64, 256), U32),
        vm((8, 128), U32),
        vm((M, S), BF16),
        vm((S // 2, MP), U32),
        vm((H // 2, M, D), U32),
        vm((NU, UC // 2, S), U32),
        vm((NU, UC // 2, S), U32),
        vm((NU, UC // 2, S), U32),
        vm((NU, UC // 2, S), U32),
        vm((M, S), BF16),
        vm((S // 2, C), U32),
        vm((H // 2, C, D), U32),
        vm((H // 2, C, D), U32),
        vm((H, M // 2, D), U32),
        vm((H, S // 2, D), U32),
        vm((H, S // 2, D), U32),
        vm((M, TO), F32),
        vm((TQ, D), F32),
        vm((TQ, 128), F32),
        vm((S, MA), BF16),
        vm((S, MP), BF16),
        dma((2,)), dma((XCH,)), dma((H // 2,)), dma((NU * 4,)), dma((2,)),
        dma((H // 2,)), dma((H // 2,)), dma((NO // NB3,)), dma((NO,)),
    ]
    out = pl.pallas_call(
        _kernel,
        in_specs=[pl.BlockSpec(memory_space=pl.ANY)] * 12,
        out_specs=pl.BlockSpec(memory_space=pl.ANY),
        out_shape=jax.ShapeDtypeStruct((S, 2 * M), BF16),
        scratch_shapes=scratch,
        compiler_params=pltpu.CompilerParams(
            vmem_limit_bytes=120 * 1024 * 1024,
            disable_semaphore_checks=True,
            disable_bounds_checks=True,
        ),
        name="h3_cla_fused",
    )(
        A_q[0].T, A_k[0].T, A_v[0].T, A_shift_k.T, A_ssm_k, A_ssm_D,
        B_x[0].T, B_c_kv[0], B_w_q, B_w_uk, B_w_uv, jnp.transpose(B_w_o, (0, 2, 1)),
    )
    return out[None]
```

```python
import math

import jax
import jax.numpy as jnp
import jax.experimental.pallas as pl
import jax.experimental.pallas.tpu as pltpu

S = 2048
M = 448
MP = 512
MA = 384
H = 16
D = 256
C = 1024
G = 32
NC = 128 // G
TQ = 128 * NC
NB = S // TQ
PC = 256
NU = 7
UC = M // NU
NBLK = S // 128
QCH = 128
XB = (0, 256, 640, 1280, 2048)
XCH = len(XB) - 1
TO = 128
NO = S // TO
NB3 = 4
TOKH = 6
MLAG = 700
SLAG = 800
NPART = 32
P1ORDER = ("H0 H1 H2 H3 Q0 X0 Q1 X1 Q2 X2 Q3 X3 Q4 I00 Q5 I01 Q6 I10 Q7 I11 "
           "Q8 Q9 I20 Q10 I21 Q11 Q12 I30 Q13 I31 Q14 Q15")

P2ORDER = "K0 K1 V0 Q0 V1 K2 P0 K3 V2 Q1 V3 K4 P1 K5 V4 Q2 V5 K6 P2 K7 V6 Q3 V7 P3"

F32 = jnp.float32
BF16 = jnp.bfloat16
U32 = jnp.uint32
HI_MASK = 0xFFFF0000
Q_SCALE = D ** -0.5
MASK_VALUE = -1e9


def _dot(a, b):
    return jnp.dot(a, b, preferred_element_type=F32)


def _dot_nt(a, b):
    return jax.lax.dot_general(a, b, (((1,), (1,)), ((), ())), preferred_element_type=F32)


def _or_fold(x):
    bits = pltpu.bitcast(x, U32)
    t = None
    for r in range(bits.shape[0] // 8):
        for c in range(bits.shape[1] // 128):
            e = bits[r * 8:(r + 1) * 8, c * 128:(c + 1) * 128]
            t = e if t is None else t | e
    return t


def _inject(x, tok):
    top = x[:8, :128] | tok
    if x.shape[1] > 128:
        top = jnp.concatenate([top, x[:8, 128:]], axis=1)
    return jnp.concatenate([top, x[8:]], axis=0)


def _recip(x):
    r = pl.reciprocal(x, approx=True)
    return r * (2.0 - x * r)


def _rows(chunks, r0, r1):
    parts = []
    while r0 < r1:
        c = r0 // PC
        e = min(r1, (c + 1) * PC)
        parts.append(chunks[c][(r0 - c * PC) // 2:(e - c * PC) // 2])
        r0 = e
    x = parts[0] if len(parts) == 1 else jnp.concatenate(parts, axis=0)
    return pltpu.bitcast(x, BF16)


def _steps(i):
    plans = []
    for cls in range(NC):
        last = cls == NC - 1
        base = 0 if last else G * (cls + 1)
        full = NC * i - 1 + last
        plan = []
        m = 0
        while m < full:
            w = 2 if m + 2 <= full else 1
            plan.append((cls, base + 128 * m, base + 128 * (m + w), 0, False))
            m += w
        for t in range(NC):
            if full + t >= 0:
                plan.append((cls, base + 128 * (full + t), base + 128 * (full + t + 1), G * t, True))
        plans.append(plan)
    n = max(len(p) for p in plans)
    return [plans[cls][j - n + len(plans[cls])] for j in range(n) for cls in reversed(range(NC))
            if j - n + len(plans[cls]) >= 0]


def _due(steps, lag):
    ends, out, t = [], [], 0
    for _, k0, k1, row0, _ in steps:
        src = [n for n, e in enumerate(ends) if e + lag <= t]
        out.append(src[-1] if src else None)
        t += (128 - row0) * (k1 - k0) // 256
        ends.append(t)
    return [None if x in out[:n] else x for n, x in enumerate(out)]


def _token(n, nsteps, own, extra):
    t = own
    for k, e in enumerate(extra):
        if k * nsteps // len(extra) == n:
            t = e if t is None else t | e
    return t


def _update(acc, x, row0, op):
    if acc is None:
        return x
    if row0 == 0:
        return op(acc, x)
    return jnp.concatenate([acc[:row0], op(acc[row0:], x)], axis=0)


def _qk(i, qu, ks, zero, extra):
    r = jax.lax.broadcasted_iota(jnp.int32, (G, 128), 0)
    c = jax.lax.broadcasted_iota(jnp.int32, (G, 128), 1)
    msk = c <= r + (128 - G)
    h = G // 2
    qc = [jnp.concatenate([qu[64 * t + h * cls:64 * t + h * (cls + 1)] for t in range(NC)], axis=0)
          for cls in range(NC)]
    steps = _steps(i)
    due = _due(steps, MLAG)
    toks = {}
    run = [None] * NC
    sc, lead = [], []
    for cls in range(NC - 1):
        w = G * (cls + 1)
        s = _dot_nt(_rows(ks, 0, w), pltpu.bitcast(qc[cls], BF16)).T
        if i == 0:
            top = jnp.where((c <= r + G * cls)[:, :w], s[:G], MASK_VALUE)
            s = jnp.concatenate([top, s[G:]], axis=0)
        lead.append(s)
        run[cls] = jnp.concatenate([s, jnp.full((128, 128 - w), MASK_VALUE, F32)], axis=1)
    for n, (cls, k0, k1, row0, masked) in enumerate(steps):
        x = qc[cls][row0 // 2:]
        t = _token(n, len(steps), toks.get(due[n]), extra)
        s = _dot_nt(pltpu.bitcast(x if t is None else _inject(x, t), BF16), _rows(ks, k0, k1))
        if masked:
            top = jnp.where(msk, s[:G], MASK_VALUE)
            s = top if row0 + G == 128 else jnp.concatenate([top, s[G:]], axis=0)
        sc.append(s)
        mj = jnp.maximum(s[:, :128], s[:, 128:]) if k1 - k0 == 256 else s
        run[cls] = _update(run[cls], mj, row0, jnp.maximum)
        toks[n] = _or_fold(run[cls]) & zero
    return steps, lead, sc, run


def _softmax_pv(steps, lead, sc, mx, vs, zero, extra):
    m = [jnp.max(mx[cls], axis=1, keepdims=True) for cls in range(NC)]
    due = _due(steps, SLAG)
    toks = {}
    o = [None] * NC
    run = [None] * NC
    for cls in range(NC - 1):
        w = G * (cls + 1)
        p = jnp.exp(lead[cls] - m[cls]).astype(BF16)
        o[cls] = _dot(p, _rows(vs, 0, w))
        run[cls] = jnp.concatenate([p.astype(F32), jnp.zeros((128, 128 - w), F32)], axis=1)
    for n, (cls, k0, k1, row0, _) in enumerate(steps):
        p = jnp.exp(sc[n] - m[cls][row0:]).astype(BF16)
        t = _token(n, len(steps), toks.get(due[n]), extra)
        if t is not None:
            p = pltpu.bitcast(_inject(pltpu.bitcast(p, U32), t), BF16)
        t = _dot(p, _rows(vs, k0, k1))
        e = p.astype(F32)
        ej = e[:, :128] + e[:, 128:] if k1 - k0 == 256 else e
        o[cls] = _update(o[cls], t, row0, jnp.add)
        run[cls] = _update(run[cls], ej, row0, jnp.add)
        toks[n] = _or_fold(run[cls]) & zero

    def natural(x):
        return jnp.concatenate([x[cls][G * t:G * (t + 1)] for t in range(NC) for cls in range(NC)], axis=0)
    return natural(o), natural(run)


def _normalize(o, lsum):
    r = _recip(jnp.sum(lsum, axis=1, keepdims=True))
    return pltpu.bitcast((o * r).astype(BF16), U32)


def _kernel(aq_hbm, ak_hbm, av_hbm, sh_hbm, ah_hbm, dd_hbm, xt_hbm, c_hbm,
            wq_hbm, wk_hbm, wv_hbm, wot_hbm,
            out_hbm,
            sh_s, dd_s, coef_s, f_s, fh_s, zero_s, xt_s, x_s, wq_raw, aq_s, ak_s, av_s, ah_s, at_s,
            c_s, wk_raw, wv_raw, wot_s, q_s, ctx_s, ot_s, o7_s, l7_s, stage_a, stage_b,
            sem_small, sem_x, sem_wq, sem_a, sem_c, sem_wk, sem_wv, sem_oa, sem_ob):
    wq32 = wq_hbm.bitcast(U32)
    wk32 = wk_hbm.bitcast(U32)
    wv32 = wv_hbm.bitcast(U32)

    def cp_small(i):
        return pltpu.make_async_copy((sh_hbm, dd_hbm)[i], (sh_s, dd_s)[i], sem_small.at[i])

    def cp_x(i):
        cols = pl.ds(XB[i], XB[i + 1] - XB[i])
        return pltpu.make_async_copy(xt_hbm.at[:, cols], xt_s.at[:, cols], sem_x.at[i])

    def cp_wq(p):
        return pltpu.make_async_copy(wq32.at[:, p, :], wq_raw.at[p], sem_wq.at[p])

    def cp_a(g, i):
        src = (ah_hbm, ak_hbm, av_hbm, aq_hbm)[i].bitcast(U32)
        dst = (ah_s, ak_s, av_s, aq_s)[i]
        n = UC // 2
        start = g * n if isinstance(g, int) else pl.multiple_of(g * n, 8)
        return pltpu.make_async_copy(src.at[pl.ds(start, n), :], dst.at[g], sem_a.at[g * 4 + i])

    def cp_c(i):
        return pltpu.make_async_copy((c_hbm, wot_hbm)[i].bitcast(U32), (c_s, wot_s)[i], sem_c.at[i])

    def cp_wk(p):
        return pltpu.make_async_copy(wk32.at[:, p, :], wk_raw.at[p], sem_wk.at[p])

    def cp_wv(p):
        return pltpu.make_async_copy(wv32.at[:, p, :], wv_raw.at[p], sem_wv.at[p])

    def cp_out_a(i):
        n = NB3 * TO
        start = i * n if isinstance(i, int) else pl.multiple_of(i * n, n)
        return pltpu.make_async_copy(stage_a.at[pl.ds(start, n), :],
                                     out_hbm.at[pl.ds(start, n), pl.ds(0, MA)], sem_oa.at[i])

    def cp_out_b(i):
        start = i * TO if isinstance(i, int) else pl.multiple_of(i * TO, TO)
        return pltpu.make_async_copy(stage_b.at[pl.ds(start, TO), :],
                                     out_hbm.at[pl.ds(start, TO), pl.ds(MA, MP)], sem_ob.at[i])

    cp_x(0).start()
    cp_wq(0).start()
    for i in range(1, XCH):
        cp_x(i).start()
    cp_small(0).start()
    cp_small(1).start()

    tt = jax.lax.broadcasted_iota(jnp.int32, (128, 128), 0)
    rr = jax.lax.broadcasted_iota(jnp.int32, (128, 128), 1)
    ang = ((tt * (2 * rr + 1)) & 511).astype(F32) * (2.0 * math.pi / 512.0)
    fmat = jnp.concatenate([jnp.cos(ang), -jnp.sin(ang)], axis=1).astype(BF16)
    f_s[...] = pltpu.bitcast(fmat, U32)
    fh_s[...] = pltpu.bitcast((fmat.astype(F32) * (1.0 / 128.0)).astype(BF16), U32)
    zero_s[...] = jnp.zeros((8, 128), U32)

    def xpose_x(i):
        for t in range(XB[i] // 128, XB[i + 1] // 128):
            cols = slice(t * 128, (t + 1) * 128)
            blks = [xt_s[g * 128:(g + 1) * 128, cols].astype(F32).T for g in range(3)]
            last = jnp.concatenate([xt_s[MA:M, cols].astype(F32), jnp.zeros((MP - M, 128), F32)], axis=0)
            blks.append(last.T)
            x_s[t * 64:(t + 1) * 64, :] = pltpu.bitcast(jnp.concatenate(blks, axis=1).astype(BF16), U32)

    def q_weights(p):
        raw = wq_raw[p]
        lo = pltpu.bitcast(raw << 16, F32)
        hi = pltpu.bitcast(raw & jnp.uint32(HI_MASK), F32)
        w = jnp.concatenate([lo, hi], axis=1) * Q_SCALE
        w = jnp.concatenate([w, jnp.zeros((MP - M, 2 * D), F32)], axis=0)
        return w.astype(BF16)

    def qproj(p, w, r):
        rows = slice(r * QCH // 2, (r + 1) * QCH // 2)
        qq = _dot(pltpu.bitcast(x_s[rows, :], BF16), w)
        q_s[2 * p, rows, :] = pltpu.bitcast(qq[:, :D].astype(BF16), U32)
        q_s[2 * p + 1, rows, :] = pltpu.bitcast(qq[:, D:].astype(BF16), U32)

    cp_x(0).wait()
    xpose_x(0)
    for g in range(NU):
        cp_wq(g + 1).start()
        for i in range(4):
            cp_a(g, i).start()
    cp_wk(0).start()
    cp_wv(0).start()
    cp_c(0).start()
    cp_c(1).start()
    for p in range(1, H // 2):
        cp_wk(p).start()
        cp_wv(p).start()
    cp_wq(0).wait()
    w0 = q_weights(0)
    for r in range(XB[1] // QCH - 1):
        qproj(0, w0, r)
    for i in range(1, XCH):
        cp_x(i).wait()
        if i == XCH - 1:
            cp_small(0).wait()
            cp_small(1).wait()
            prm = [sh_s[j:j + 1, :].astype(F32) for j in range(4)]
            prm.append(dd_s[...].astype(F32).reshape(1, M))
            for j in range(5):
                row = jnp.concatenate([prm[j], jnp.zeros((1, MP - M), F32)], axis=1)
                for t in range(MP // 128):
                    blk = jnp.broadcast_to(row[:, t * 128:(t + 1) * 128], (128, 128))
                    coef_s[j, t * 128:(t + 1) * 128, :] = blk.T
        qproj(0, w0, XB[i] // QCH - 1)
        xpose_x(i)
        for r in range(XB[i] // QCH, XB[i + 1] // QCH - (1 if i < XCH - 1 else 0)):
            qproj(0, w0, r)
    ot_s[...] = jnp.zeros((M, TO), F32)
    o7_s[...] = jnp.zeros((TQ, D), F32)
    l7_s[...] = jnp.ones((TQ, 128), F32)

    def phase1(g, carry):
        cp_wq(g + 1).wait()
        for i in range(4):
            cp_a(g, i).wait()
        w = q_weights(g + 1)
        fh = pltpu.bitcast(fh_s[...], BF16)
        fx = pltpu.bitcast(f_s[...], BF16)
        lane = jax.lax.broadcasted_iota(jnp.int32, (16, 128), 1)
        sgn = jnp.where((jax.lax.broadcasted_iota(jnp.int32, (8, 128), 1) & 1) == 0, 1.0, -1.0)
        zh, zx, kvs, ys = {}, {}, {}, {}

        def coef(k, j):
            return coef_s[j, pl.ds(pl.multiple_of(g * UC + k * 16, 16), 16), :]

        def hfwd(k):
            lhs = jnp.concatenate([ah_s[g, k * 8:(k + 1) * 8, c * 128:(c + 1) * 128]
                                   for c in range(NBLK)], axis=0)
            zh[k] = _dot(pltpu.bitcast(lhs, BF16), fh)

        def xfwd(k):
            kf = pltpu.bitcast(ak_s[g, k * 8:(k + 1) * 8, :], BF16).astype(F32)
            vf = pltpu.bitcast(av_s[g, k * 8:(k + 1) * 8, :], BF16).astype(F32)
            sh_k = [kf] + [pltpu.roll(kf, j, 1) for j in range(1, 4)]
            cf = [coef(k, j) for j in range(4)]
            kvf = []
            for c in range(NBLK):
                cols = slice(c * 128, (c + 1) * 128)
                t = sh_k[0][:, cols] * cf[0]
                for j in range(1, 4):
                    kj = sh_k[j][:, cols]
                    if c == 0:
                        kj = jnp.where(lane >= j, kj, 0.0)
                    t = t + kj * cf[j]
                kvf.append(t * vf[:, cols])
            kvs[k] = jnp.concatenate(kvf, axis=0).astype(BF16)
            zx[k] = _dot(kvs[k], fx)

        def inv(k, u):
            rows = [slice(c * 16 + u * 8, c * 16 + u * 8 + 8) for c in range(NBLK)]
            xr = [zx[k][r, :128] for r in rows]
            xi = [zx[k][r, 128:] for r in rows]
            h0r = [zh[k][r, :128] for r in rows]
            h0i = [zh[k][r, 128:] for r in rows]
            hr = [h0r[0]] + [h0r[j] - sgn * h0i[j - 1] for j in range(1, NBLK)]
            hi = [h0i[0]] + [h0i[j] + sgn * h0r[j - 1] for j in range(1, NBLK)]
            pr, pi = [], []
            for a0 in range(0, NBLK, 4):
                re = [None] * 4
                im = [None] * 4
                for c0 in range(0, a0 + 4, 4):
                    for da in range(4):
                        for c in range(c0, c0 + 4):
                            j = a0 + da - c
                            if j < 0:
                                continue
                            tr = xr[c] * hr[j] - xi[c] * hi[j]
                            ti = xr[c] * hi[j] + xi[c] * hr[j]
                            re[da] = tr if re[da] is None else re[da] + tr
                            im[da] = ti if im[da] is None else im[da] + ti
                pr += re
                pi += im
            p = jnp.concatenate([jnp.concatenate(pr, axis=0), jnp.concatenate(pi, axis=0)], axis=1)
            ys[k, u] = _dot_nt(p.astype(BF16), fx)
            if u == 1:
                kvr = kvs[k].astype(F32)
                qraw = aq_s[g, k * 8:(k + 1) * 8, :] | jnp.tile(zero_s[...], (1, NBLK))
                qf = pltpu.bitcast(qraw, BF16).astype(F32)
                dd = coef(k, 4)
                row0 = pl.multiple_of(g * UC + k * 16, 16)
                for a in range(NBLK):
                    cols = slice(a * 128, (a + 1) * 128)
                    y = jnp.concatenate([ys[k, 0][a * 8:(a + 1) * 8], ys[k, 1][a * 8:(a + 1) * 8]], axis=0)
                    y = y + kvr[a * 16:(a + 1) * 16] * dd
                    at_s[pl.ds(row0, 16), cols] = (qf[:, cols] * y).astype(BF16)

        for step in P1ORDER.split():
            if step[0] == 'Q':
                qproj(g + 1, w, int(step[1:]))
            elif step[0] == 'H':
                hfwd(int(step[1]))
            elif step[0] == 'X':
                xfwd(int(step[1]))
            else:
                inv(int(step[1]), int(step[2]))
        return carry

    jax.lax.fori_loop(0, NU, phase1, 0)

    cp_c(0).wait()
    cp_c(1).wait()
    for p in range(H // 2):
        cp_wk(p).wait()
        cp_wv(p).wait()

    def extract(raw, h):
        sh = (16 - ((h & 1) << 4)).astype(U32)
        return pltpu.bitcast((raw[h >> 1] << sh) & jnp.uint32(HI_MASK), F32).astype(BF16)

    def cblk(i):
        return pltpu.bitcast(c_s[i * PC // 2:(i + 1) * PC // 2, :], BF16)

    def finish_last(h):
        bits = _normalize(o7_s[...], l7_s[...])
        ctx_s[h, (NB - 1) * TQ // 2:NB * TQ // 2, :] = bits
        return bits

    def phase2(h, carry):
        wk = extract(wk_raw, h)
        wv = extract(wv_raw, h)
        ks, vs, toks, sc = [], [], {}, {}
        zero = zero_s[...]

        def tokens(bits):
            n = TQ // 2 // NPART
            return [_or_fold(bits[k * n:(k + 1) * n]) & zero for k in range(NPART)]

        toks[-1] = tokens(finish_last(jnp.maximum(h - 1, 0)))
        for step in P2ORDER.split():
            i = int(step[1:])
            if step[0] == 'K':
                ks.append(pltpu.bitcast(_dot(cblk(i), wk).astype(BF16), U32))
            elif step[0] == 'V':
                vs.append(pltpu.bitcast(_dot(cblk(i), wv).astype(BF16), U32))
            elif step[0] == 'Q':
                q = q_s[h, i * TQ // 2:(i + 1) * TQ // 2, :]
                if i >= 1:
                    q = q | jnp.tile(zero, (TQ // 16, D // 128))
                sc[i] = _qk(i, q, ks, zero, toks.get(i - 2, []))
            elif i == NB - 1:
                o7_s[...], l7_s[...] = _softmax_pv(*sc[i], vs, zero, toks[i - 1])
            else:
                bits = _normalize(*_softmax_pv(*sc[i], vs, zero, []))
                ctx_s[h, i * TQ // 2:(i + 1) * TQ // 2, :] = bits
                toks[i] = tokens(bits)
        return carry

    jax.lax.fori_loop(0, H, phase2, 0)

    def finish(i, ot):
        r0 = i * TO if isinstance(i, int) else pl.multiple_of(i * TO, TO)
        top = at_s[MA:M, pl.ds(r0, TO)].astype(F32)
        val = jnp.concatenate([top, ot], axis=0).T
        stage_b[pl.ds(r0, TO), :] = val.astype(BF16)
        return val

    def oproj(i, pending):
        tok = _or_fold(pending[0])
        for x in pending[1:]:
            tok = tok | _or_fold(x)
        tok = tok & zero_s[...]
        rows = pl.ds(pl.multiple_of(i * (TO // 2), TO // 2), TO // 2)
        wot = jnp.concatenate([wot_s[h] for h in range(H)], axis=1)
        ctx = [ctx_s[h, rows, :] for h in range(H)]
        ctx[TOKH] = _inject(ctx[TOKH], tok)
        ctx = jnp.concatenate(ctx, axis=1)
        return _dot_nt(pltpu.bitcast(wot, BF16), pltpu.bitcast(ctx, BF16))

    def phase3(it, carry):
        prev = jnp.maximum(NB3 * it - 1, 0)
        pend = [finish(prev, ot_s[...])]

        @pl.when(it > 0)
        def _():
            cp_out_b(prev).start()

        r0 = pl.multiple_of(it * (NB3 * TO), NB3 * TO)
        apart = []
        for g in range(MA // 128):
            blk = at_s[g * 128:(g + 1) * 128, pl.ds(r0, NB3 * TO)].astype(F32).T
            stage_a[pl.ds(r0, NB3 * TO), g * 128:(g + 1) * 128] = blk.astype(BF16)
            apart.append(blk)
        cp_out_a(it).start()

        for k in range(NB3 - 1):
            pend = [finish(NB3 * it + k, oproj(NB3 * it + k, pend))]
            if k == 0:
                pend += apart
            cp_out_b(NB3 * it + k).start()
        ot_s[...] = oproj(NB3 * it + NB3 - 1, pend)
        finish_last(H - 1)
        return carry

    jax.lax.fori_loop(0, NO // NB3, phase3, 0)

    finish(NO - 1, ot_s[...])
    cp_out_b(NO - 1).start()
    for i in range(NO // NB3):
        cp_out_a(i).wait()
    for i in range(NO):
        cp_out_b(i).wait()


@jax.jit
def pallas_concat_heads__ssm_conv_h3__compressed_kv_cla__prompt_kernel(
    A_q: jax.Array,
    A_k: jax.Array,
    A_v: jax.Array,
    A_shift_k: jax.Array,
    A_ssm_k: jax.Array,
    A_ssm_D: jax.Array,
    B_x: jax.Array,
    B_c_kv: jax.Array,
    B_w_q: jax.Array,
    B_w_uk: jax.Array,
    B_w_uv: jax.Array,
    B_w_o: jax.Array,
):
    vm = pltpu.VMEM
    dma = pltpu.SemaphoreType.DMA
    scratch = [
        vm((4, M), BF16),
        vm((M,), BF16),
        vm((5, MP, 128), F32),
        vm((64, 256), U32),
        vm((64, 256), U32),
        vm((8, 128), U32),
        vm((M, S), BF16),
        vm((S // 2, MP), U32),
        vm((H // 2, M, D), U32),
        vm((NU, UC // 2, S), U32),
        vm((NU, UC // 2, S), U32),
        vm((NU, UC // 2, S), U32),
        vm((NU, UC // 2, S), U32),
        vm((M, S), BF16),
        vm((S // 2, C), U32),
        vm((H // 2, C, D), U32),
        vm((H // 2, C, D), U32),
        vm((H, M // 2, D), U32),
        vm((H, S // 2, D), U32),
        vm((H, S // 2, D), U32),
        vm((M, TO), F32),
        vm((TQ, D), F32),
        vm((TQ, 128), F32),
        vm((S, MA), BF16),
        vm((S, MP), BF16),
        dma((2,)), dma((XCH,)), dma((H // 2,)), dma((NU * 4,)), dma((2,)),
        dma((H // 2,)), dma((H // 2,)), dma((NO // NB3,)), dma((NO,)),
    ]
    out = pl.pallas_call(
        _kernel,
        in_specs=[pl.BlockSpec(memory_space=pl.ANY)] * 12,
        out_specs=pl.BlockSpec(memory_space=pl.ANY),
        out_shape=jax.ShapeDtypeStruct((S, 2 * M), BF16),
        scratch_shapes=scratch,
        compiler_params=pltpu.CompilerParams(
            vmem_limit_bytes=120 * 1024 * 1024,
            disable_semaphore_checks=True,
            disable_bounds_checks=True,
        ),
        name="h3_cla_fused",
    )(
        A_q[0].T, A_k[0].T, A_v[0].T, A_shift_k.T, A_ssm_k, A_ssm_D,
        B_x[0].T, B_c_kv[0], B_w_q, B_w_uk, B_w_uv, jnp.transpose(B_w_o, (0, 2, 1)),
    )
    return out[None]
```

```python
import math

import jax
import jax.numpy as jnp
import jax.experimental.pallas as pl
import jax.experimental.pallas.tpu as pltpu

S = 2048
M = 448
MP = 512
MA = 384
H = 16
D = 256
C = 1024
G = 32
NC = 128 // G
TQ = 128 * NC
NB = S // TQ
PC = 256
NU = 7
UC = M // NU
NBLK = S // 128
QCH = 128
XB = (0, 256, 768, 1280, 2048)
XCH = len(XB) - 1
TO = 128
NO = S // TO
NB3 = 4
TOKH = 6
MLAG = 800
SLAG = 1000
NPART = 32
P1ORDER = ("H0 H1 H2 H3 Q0 X0 Q1 X1 Q2 X2 Q3 X3 Q4 I00 Q5 I01 Q6 I10 Q7 I11 "
           "Q8 Q9 I20 Q10 I21 Q11 Q12 I30 Q13 I31 Q14 Q15")

P2ORDER = "K0 K1 V0 Q0 V1 K2 P0 K3 V2 Q1 V3 K4 P1 K5 V4 Q2 V5 K6 P2 K7 V6 Q3 V7 P3"

WPARTS = 16
WOQ = 2
KVF32 = 1
CTOK = 0
PSKIP = 0
B11Q = 1
MORDER = (1, 4, 0, 3, 6, 2, 5)
XLAG = 3
P1PLAN = {0:'H0 H1 H2 H3',4:'X0',7:'X1',11:'X2',14:'X3',16:'C0',18:'I00',20:'C1',22:'I01',24:'C2',26:'I10',28:'C3',30:'I11',33:'C4',35:'I20',37:'C5',39:'I21',42:'C6',44:'I30',47:'C7',49:'I31'}
F32 = jnp.float32
BF16 = jnp.bfloat16
U32 = jnp.uint32
HI_MASK = 0xFFFF0000
Q_SCALE = D ** -0.5
MASK_VALUE = -1e9


def _dot(a, b):
    return jnp.dot(a, b, preferred_element_type=F32)


def _dot_nt(a, b):
    return jax.lax.dot_general(a, b, (((1,), (1,)), ((), ())), preferred_element_type=F32)


def _pack(x):
    return pltpu.bitcast(x.astype(BF16), U32)


def _ds(start, size, align):
    return pl.ds(start if isinstance(start, int) else pl.multiple_of(start, align), size)


def _sample(x):
    return _or_fold(jnp.concatenate([x[r + 8:r + 16] for r in range(0, x.shape[0], 16)], axis=0))


def _quads(x):
    r, c = x.shape[0] // 2, x.shape[1] // 2
    return x[:r, :c], x[:r, c:], x[r:, :c], x[r:, c:]


def _lhs_sums(a):
    a11, a12, a21, a22 = _quads(a)
    return a11 + a22, a21 + a22, a11 + a12, a21 - a11, a12 - a22


def _lhs_ops(a):
    a11, _, _, a22 = _quads(a)
    s1, s2, s5, s6, s7 = _lhs_sums(a)
    return s1, s2, a11, a22, s5, s6, s7


def _rhs_ops(b):
    b11, b12, b21, b22 = _quads(b)
    return b11 + b22, b11, b12 - b22, b21 - b11, b22, b11 + b12, b21 + b22


def _combine(m):
    m1, m2, m3, m4, m5, m6, m7 = m
    top = jnp.concatenate([(m1 + m4) + (m7 - m5), m3 + m5], axis=1)
    bot = jnp.concatenate([m2 + m4, (m1 - m2) + (m3 + m6)], axis=1)
    return jnp.concatenate([top, bot], axis=0)


def _or_fold(x):
    bits = pltpu.bitcast(x, U32)
    t = None
    for r in range(bits.shape[0] // 8):
        for c in range(bits.shape[1] // 128):
            e = bits[r * 8:(r + 1) * 8, c * 128:(c + 1) * 128]
            t = e if t is None else t | e
    return t


def _inject(x, tok):
    top = x[:8, :128] | tok
    if x.shape[1] > 128:
        top = jnp.concatenate([top, x[:8, 128:]], axis=1)
    return jnp.concatenate([top, x[8:]], axis=0)


def _recip(x):
    r = pl.reciprocal(x, approx=True)
    return r * (2.0 - x * r)


def _rows(chunks, r0, r1):
    parts = []
    while r0 < r1:
        c = r0 // PC
        e = min(r1, (c + 1) * PC)
        parts.append(chunks[c][r0 - c * PC:e - c * PC] if KVF32 else chunks[c][(r0 - c * PC) // 2:(e - c * PC) // 2])
        r0 = e
    x = parts[0] if len(parts) == 1 else jnp.concatenate(parts, axis=0)
    return x.astype(BF16) if KVF32 else pltpu.bitcast(x, BF16)


def _steps(i):
    plans = []
    for cls in range(NC):
        last = cls == NC - 1
        base = 0 if last else G * (cls + 1)
        full = NC * i - 1 + last
        plan = []
        m = 0
        while m < full:
            w = 2 if m + 2 <= full else 1
            plan.append((cls, base + 128 * m, base + 128 * (m + w), 0, False))
            m += w
        for t in range(NC):
            if full + t >= 0:
                plan.append((cls, base + 128 * (full + t), base + 128 * (full + t + 1), G * t, True))
        plans.append(plan)
    n = max(len(p) for p in plans)
    return [plans[cls][j - n + len(plans[cls])] for j in range(n) for cls in reversed(range(NC))
            if j - n + len(plans[cls]) >= 0]


def _due(steps, lag):
    ends, out, t = [], [], 0
    for _, k0, k1, row0, _ in steps:
        src = [n for n, e in enumerate(ends) if e + lag <= t]
        out.append(src[-1] if src else None)
        t += (128 - row0) * (k1 - k0) // 256
        ends.append(t)
    return [None if x in out[:n] else x for n, x in enumerate(out)]


def _token(n, nsteps, own, extra):
    t = own
    for k, e in enumerate(extra):
        if e is not None and k * nsteps // len(extra) == n:
            t = e if t is None else t | e
    return t


def _mix(a, b):
    keyed = [((k + 0.5) / len(a), x) for k, x in enumerate(a)] + [((k + 1.0) / len(b), x) for k, x in enumerate(b)]
    return [x for _, x in sorted(keyed, key=lambda e: e[0])]


def _update(acc, x, row0, op):
    if acc is None:
        return x
    if row0 == 0:
        return op(acc, x)
    return jnp.concatenate([acc[:row0], op(acc[row0:], x)], axis=0)


def _qk(i, qu, ks, zero, extra):
    r = jax.lax.broadcasted_iota(jnp.int32, (G, 128), 0)
    c = jax.lax.broadcasted_iota(jnp.int32, (G, 128), 1)
    msk = c <= r + (128 - G)
    h = G // 2
    qc = [jnp.concatenate([qu[64 * t + h * cls:64 * t + h * (cls + 1)] for t in range(NC)], axis=0)
          for cls in range(NC)]
    steps = _steps(i)
    due = _due(steps, MLAG)
    toks = {}
    run = [None] * NC
    sc, lead = [], []
    for cls in range(NC - 1):
        w = G * (cls + 1)
        s = _dot_nt(_rows(ks, 0, w), pltpu.bitcast(qc[cls], BF16)).T
        if i == 0:
            top = jnp.where((c <= r + G * cls)[:, :w], s[:G], MASK_VALUE)
            s = jnp.concatenate([top, s[G:]], axis=0)
        lead.append(s)
        run[cls] = jnp.concatenate([s, jnp.full((128, 128 - w), MASK_VALUE, F32)], axis=1)
    for n, (cls, k0, k1, row0, masked) in enumerate(steps):
        x = qc[cls][row0 // 2:]
        t = _token(n, len(steps), toks.get(due[n]), extra)
        s = _dot_nt(pltpu.bitcast(x if t is None else _inject(x, t), BF16), _rows(ks, k0, k1))
        if masked:
            top = jnp.where(msk, s[:G], MASK_VALUE)
            s = top if row0 + G == 128 else jnp.concatenate([top, s[G:]], axis=0)
        sc.append(s)
        mj = jnp.maximum(s[:, :128], s[:, 128:]) if k1 - k0 == 256 else s
        run[cls] = _update(run[cls], mj, row0, jnp.maximum)
        toks[n] = _or_fold(run[cls]) & zero
    return steps, lead, sc, run


def _softmax_pv(steps, lead, sc, mx, vs, zero, extra):
    m = [jnp.max(mx[cls], axis=1, keepdims=True) for cls in range(NC)]
    due = _due(steps, SLAG)
    toks = {}
    o = [None] * NC
    run = [None] * NC
    for cls in range(NC - 1):
        w = G * (cls + 1)
        p = jnp.exp(lead[cls] - m[cls]).astype(BF16)
        o[cls] = _dot(p, _rows(vs, 0, w))
        run[cls] = jnp.concatenate([p.astype(F32), jnp.zeros((128, 128 - w), F32)], axis=1)
    for n, (cls, k0, k1, row0, _) in enumerate(steps):
        p = jnp.exp(sc[n] - m[cls][row0:])
        t = _token(n, len(steps), toks.get(due[n]), extra)
        if t is not None:
            p = pltpu.bitcast(_inject(pltpu.bitcast(p, U32), t), F32)
        p = p.astype(BF16)
        t = _dot(p, _rows(vs, k0, k1))
        e = p.astype(F32)
        ej = e[:, :128] + e[:, 128:] if k1 - k0 == 256 else e
        o[cls] = _update(o[cls], t, row0, jnp.add)
        run[cls] = _update(run[cls], ej, row0, jnp.add)
        toks[n] = _or_fold(run[cls]) & zero

    def natural(x):
        return jnp.concatenate([x[cls][G * t:G * (t + 1)] for t in range(NC) for cls in range(NC)], axis=0)
    return natural(o), natural(run)


def _normalize(o, lsum):
    r = _recip(jnp.sum(lsum, axis=1, keepdims=True))
    return o * r


def _kernel(aq_hbm, ak_hbm, av_hbm, sh_hbm, ah_hbm, dd_hbm, xt_hbm, c_hbm,
            wq_hbm, wk_hbm, wv_hbm, wot_hbm,
            out_hbm,
            sh_s, dd_s, coef_s, f_s, fh_s, zero_s, xt_s, x_s, wq_raw, aq_s, ak_s, av_s, ah_s, at_s,
            c_s, cs_s, b11_s, wk_raw, wv_raw, wot_s, wos_s, q_s, ctx_s, ot_s, o7_s, l7_s, stage_a, stage_b,
            sem_small, sem_x, sem_wq, sem_a, sem_c, sem_wk, sem_wv, sem_oa, sem_ob):
    wq32 = wq_hbm.bitcast(U32)
    wk32 = wk_hbm.bitcast(U32)
    wv32 = wv_hbm.bitcast(U32)

    def cp_small(i):
        return pltpu.make_async_copy((sh_hbm, dd_hbm)[i], (sh_s, dd_s)[i], sem_small.at[i])

    def cp_x(i):
        cols = pl.ds(XB[i], XB[i + 1] - XB[i])
        return pltpu.make_async_copy(xt_hbm.at[:, cols], xt_s.at[:, cols], sem_x.at[i])

    def cp_wq(p):
        return pltpu.make_async_copy(wq32.at[:, p, :], wq_raw.at[p], sem_wq.at[p])

    def cp_a(g, i):
        src = (ah_hbm, ak_hbm, av_hbm, aq_hbm)[i].bitcast(U32)
        dst = (ah_s, ak_s, av_s, aq_s)[i]
        n = UC // 2
        start = g * n if isinstance(g, int) else pl.multiple_of(g * n, 8)
        return pltpu.make_async_copy(src.at[pl.ds(start, n), :], dst.at[g], sem_a.at[g * 4 + i])

    def cp_c(i):
        n = PC // 2
        start = i * n if isinstance(i, int) else pl.multiple_of(i * n, n)
        return pltpu.make_async_copy(c_hbm.bitcast(U32).at[pl.ds(start, n), :],
                                     c_s.at[pl.ds(start, n), :], sem_c.at[i])

    def cp_wo():
        return pltpu.make_async_copy(wot_hbm.bitcast(U32), wot_s, sem_c.at[S // PC])

    def c_sums(i, part, nparts):
        n = 64 // nparts
        r0 = i * (PC // 2) + part * n
        if not isinstance(r0, int):
            r0 = pl.multiple_of(r0, n)
        top = pltpu.bitcast(c_s[pl.ds(r0, n), :], BF16).astype(F32)
        bot = pltpu.bitcast(c_s[pl.ds(r0 + 64, n), :], BF16).astype(F32)
        tok = None
        for j, x in enumerate(_lhs_sums(jnp.concatenate([top, bot], axis=0))):
            cs_s[_ds((i * 5 + j) * 64 + part * n, n, n), :] = _pack(x)
            if j in (0, 4):
                tok = _sample(x) if tok is None else tok | _sample(x)
        return tok & zero_s[...]

    def cp_wk(p):
        return pltpu.make_async_copy(wk32.at[:, p, :], wk_raw.at[p], sem_wk.at[p])

    def cp_wv(p):
        return pltpu.make_async_copy(wv32.at[:, p, :], wv_raw.at[p], sem_wv.at[p])

    def cp_out_a(i):
        n = NB3 * TO
        start = i * n if isinstance(i, int) else pl.multiple_of(i * n, n)
        return pltpu.make_async_copy(stage_a.at[pl.ds(start, n), :],
                                     out_hbm.at[pl.ds(start, n), pl.ds(0, MA)], sem_oa.at[i])

    def cp_out_b(i):
        start = i * TO if isinstance(i, int) else pl.multiple_of(i * TO, TO)
        return pltpu.make_async_copy(stage_b.at[pl.ds(start, TO), :],
                                     out_hbm.at[pl.ds(start, TO), pl.ds(MA, MP)], sem_ob.at[i])

    cp_x(0).start()
    cp_wq(0).start()
    for i in range(1, XCH):
        cp_x(i).start()
    cp_small(0).start()
    cp_small(1).start()

    tt = jax.lax.broadcasted_iota(jnp.int32, (128, 128), 0)
    rr = jax.lax.broadcasted_iota(jnp.int32, (128, 128), 1)
    ang = ((tt * (2 * rr + 1)) & 511).astype(F32) * (2.0 * math.pi / 512.0)
    fmat = jnp.concatenate([jnp.cos(ang), -jnp.sin(ang)], axis=1).astype(BF16)
    f_s[...] = pltpu.bitcast(fmat, U32)
    fh_s[...] = pltpu.bitcast((fmat.astype(F32) * (1.0 / 128.0)).astype(BF16), U32)
    zero_s[...] = jnp.zeros((8, 128), U32)

    def xpose_x(i):
        for blk in range(XB[i] // 256, XB[i + 1] // 256):
            tiles = []
            for t in (2 * blk, 2 * blk + 1):
                cols = slice(t * 128, (t + 1) * 128)
                parts = [xt_s[g * 128:(g + 1) * 128, cols].astype(F32).T for g in range(3)]
                last = jnp.concatenate([xt_s[MA:M, cols].astype(F32), jnp.zeros((MP - M, 128), F32)], axis=0)
                parts.append(last.T)
                tiles.append(jnp.concatenate(parts, axis=1))
            x = jnp.concatenate(tiles, axis=0)
            for j, op in enumerate(_lhs_ops(x)):
                x_s[(blk * 7 + j) * 64:(blk * 7 + j + 1) * 64, :] = _pack(op)

    def q_weights(p):
        raw = wq_raw[p]
        ops = []
        for w in (raw << 16, raw & jnp.uint32(HI_MASK)):
            w = pltpu.bitcast(w, F32) * Q_SCALE
            ops.append(_rhs_ops(jnp.concatenate([w, jnp.zeros((MP - M, D), F32)], axis=0)))
        return [jnp.concatenate([u, v], axis=1).astype(BF16) for u, v in zip(*ops)]

    def qstep(p, w, ms, n, tok=None):
        blk, j = n // 7, MORDER[n % 7]
        x = x_s[(blk * 7 + j) * 64:(blk * 7 + j + 1) * 64, :]
        if tok is not None:
            x = _inject(x, tok)
        ms[j] = _dot(pltpu.bitcast(x, BF16), w[j])
        if n % 7 == 6:
            for k in range(2):
                q = _combine([ms[e][:, k * 128:(k + 1) * 128] for e in range(7)])
                q_s[_ds((2 * p + k) * (S // 2) + blk * 128, 128, 128), :] = _pack(q)

    cp_x(0).wait()
    xpose_x(0)
    cp_c(0).start()
    for g in range(NU):
        cp_wq(g + 1).start()
        for i in range(4):
            cp_a(g, i).start()
        cp_c(g + 1).start()
    cp_wk(0).start()
    cp_wv(0).start()
    cp_wo().start()
    for p in range(1, H // 2):
        cp_wk(p).start()
        cp_wv(p).start()
    cp_wq(0).wait()
    w0 = q_weights(0)
    ms0 = {}
    for n in range(XB[1] // 256 * 7 - XLAG):
        qstep(0, w0, ms0, n)
    for i in range(1, XCH):
        cp_x(i).wait()
        if i == XCH - 1:
            cp_small(0).wait()
            cp_small(1).wait()
            cp_c(0).wait()
            for part in range(8):
                c_sums(0, part, 8)
            prm = [sh_s[j:j + 1, :].astype(F32) for j in range(4)]
            prm.append(dd_s[...].astype(F32).reshape(1, M))
            for j in range(5):
                row = jnp.concatenate([prm[j], jnp.zeros((1, MP - M), F32)], axis=1)
                for t in range(MP // 128):
                    blk = jnp.broadcast_to(row[:, t * 128:(t + 1) * 128], (128, 128))
                    coef_s[j, t * 128:(t + 1) * 128, :] = blk.T
        for n in range(XB[i] // 256 * 7 - XLAG, XB[i] // 256 * 7):
            qstep(0, w0, ms0, n)
        xpose_x(i)
        for n in range(XB[i] // 256 * 7, XB[i + 1] // 256 * 7 - (XLAG if i < XCH - 1 else 0)):
            qstep(0, w0, ms0, n)
    ot_s[...] = jnp.zeros((M, TO), F32)
    o7_s[...] = jnp.zeros((TQ, D), F32)
    l7_s[...] = jnp.ones((TQ, 128), F32)

    def phase1(g, carry):
        cp_wq(g + 1).wait()
        for i in range(4):
            cp_a(g, i).wait()
        cp_c(g + 1).wait()
        w = q_weights(g + 1)
        fh = pltpu.bitcast(fh_s[...], BF16)
        fx = pltpu.bitcast(f_s[...], BF16)
        lane = jax.lax.broadcasted_iota(jnp.int32, (16, 128), 1)
        sgn = jnp.where((jax.lax.broadcasted_iota(jnp.int32, (8, 128), 1) & 1) == 0, 1.0, -1.0)
        zh, zx, kvs, ys = {}, {}, {}, {}

        def coef(k, j):
            return coef_s[j, pl.ds(pl.multiple_of(g * UC + k * 16, 16), 16), :]

        def hfwd(k):
            lhs = jnp.concatenate([ah_s[g, k * 8:(k + 1) * 8, c * 128:(c + 1) * 128]
                                   for c in range(NBLK)], axis=0)
            zh[k] = _dot(pltpu.bitcast(lhs, BF16), fh)

        def xfwd(k):
            kf = pltpu.bitcast(ak_s[g, k * 8:(k + 1) * 8, :], BF16).astype(F32)
            vf = pltpu.bitcast(av_s[g, k * 8:(k + 1) * 8, :], BF16).astype(F32)
            sh_k = [kf] + [pltpu.roll(kf, j, 1) for j in range(1, 4)]
            cf = [coef(k, j) for j in range(4)]
            kvf = []
            for c in range(NBLK):
                cols = slice(c * 128, (c + 1) * 128)
                t = sh_k[0][:, cols] * cf[0]
                for j in range(1, 4):
                    kj = sh_k[j][:, cols]
                    if c == 0:
                        kj = jnp.where(lane >= j, kj, 0.0)
                    t = t + kj * cf[j]
                kvf.append(t * vf[:, cols])
            kvs[k] = jnp.concatenate(kvf, axis=0).astype(BF16)
            zx[k] = _dot(kvs[k], fx)

        def inv(k, u):
            rows = [slice(c * 16 + u * 8, c * 16 + u * 8 + 8) for c in range(NBLK)]
            xr = [zx[k][r, :128] for r in rows]
            xi = [zx[k][r, 128:] for r in rows]
            h0r = [zh[k][r, :128] for r in rows]
            h0i = [zh[k][r, 128:] for r in rows]
            hr = [h0r[0]] + [h0r[j] - sgn * h0i[j - 1] for j in range(1, NBLK)]
            hi = [h0i[0]] + [h0i[j] + sgn * h0r[j - 1] for j in range(1, NBLK)]
            pr, pi = [], []
            for a0 in range(0, NBLK, 4):
                re = [None] * 4
                im = [None] * 4
                for c0 in range(0, a0 + 4, 4):
                    for da in range(4):
                        for c in range(c0, c0 + 4):
                            j = a0 + da - c
                            if j < 0:
                                continue
                            tr = xr[c] * hr[j] - xi[c] * hi[j]
                            ti = xr[c] * hi[j] + xi[c] * hr[j]
                            re[da] = tr if re[da] is None else re[da] + tr
                            im[da] = ti if im[da] is None else im[da] + ti
                pr += re
                pi += im
            p = jnp.concatenate([jnp.concatenate(pr, axis=0), jnp.concatenate(pi, axis=0)], axis=1)
            ys[k, u] = _dot_nt(p.astype(BF16), fx)
            if u == 1:
                kvr = kvs[k].astype(F32)
                qraw = aq_s[g, k * 8:(k + 1) * 8, :] | jnp.tile(zero_s[...], (1, NBLK))
                qf = pltpu.bitcast(qraw, BF16).astype(F32)
                dd = coef(k, 4)
                row0 = pl.multiple_of(g * UC + k * 16, 16)
                for a in range(NBLK):
                    cols = slice(a * 128, (a + 1) * 128)
                    y = jnp.concatenate([ys[k, 0][a * 8:(a + 1) * 8], ys[k, 1][a * 8:(a + 1) * 8]], axis=0)
                    y = y + kvr[a * 16:(a + 1) * 16] * dd
                    at_s[pl.ds(row0, 16), cols] = (qf[:, cols] * y).astype(BF16)

        ms = {}
        for n in range(S // 256 * 7):
            tok = None
            for step in P1PLAN.get(n, '').replace('_', ' ').split():
                if step[0] == 'H':
                    hfwd(int(step[1]))
                elif step[0] == 'X':
                    xfwd(int(step[1]))
                elif step[0] == 'I':
                    inv(int(step[1]), int(step[2]))
                else:
                    tok = c_sums(g + 1, int(step[1]), 8)
            qstep(g + 1, w, ms, n, tok)
        return carry

    jax.lax.fori_loop(0, NU, phase1, 0)

    cp_wo().wait()
    for p in range(H // 2):
        cp_wk(p).wait()
        cp_wv(p).wait()

    def unpack_head(w, h):
        sh = (16 - ((h & 1) << 4)).astype(U32)
        return pltpu.bitcast((w << sh) & jnp.uint32(HI_MASK), F32)

    def extract(raw, h):
        return [x.astype(BF16) for x in _rhs_ops(unpack_head(raw[h >> 1], h))]

    def first_operand(h):
        w = jnp.concatenate([wk_raw[h >> 1, :C // 2, :128], wk_raw[h >> 1, C // 2:, 128:]], axis=1)
        w = unpack_head(w, h)
        b11_s[...] = _pack(w)
        return w

    first_operand(jnp.int32(0))

    def project(i, ws):
        r0 = i * PC // 2
        sums = [cs_s[(i * 5 + j) * 64:(i * 5 + j + 1) * 64, :] for j in range(5)]
        lhs = sums[:2] + [c_s[r0:r0 + 64, :C // 2], c_s[r0 + 64:r0 + 128, C // 2:]] + sums[2:]
        ms = [None] * 7
        for j in MORDER:
            ms[j] = _dot(pltpu.bitcast(lhs[j], BF16), ws[j])
        return _combine(ms) if KVF32 else _pack(_combine(ms))

    def finish_last(h):
        bits = _normalize(o7_s[...], l7_s[...])
        ctx_s[_ds(h * (S // 2) + (NB - 1) * TQ // 2, TQ // 2, TQ // 2), :] = _pack(bits)
        return bits

    def phase2(h, carry):
        wk = extract(wk_raw, h)
        wk[1] = pltpu.bitcast(b11_s[:, :128], BF16)
        wk[4] = pltpu.bitcast(b11_s[:, 128:], BF16)
        wv = extract(wv_raw, h)
        ks, vs, toks, sc = [], [], {}, {}
        zero = zero_s[...]

        def tokens(bits):
            n = TQ // NPART
            return [(_or_fold(bits[k * n:(k + 1) * n]) if CTOK == 0 else _or_fold(bits[k * n:(k + 1) * n, :128]) if CTOK == 1 else _sample(bits[k * n:(k + 1) * n])) & zero for k in range(NPART)]

        def wo_sums(part):
            r0 = (h & 1) * (M // 8) + part * 8
            quad = [[wot_s[(h >> 1) + k * (H // 2), _ds(r + r0, 8, 8), :] for k in range(2)] for r in (0, M // 4)]
            wo = jnp.concatenate([jnp.concatenate(x, axis=1) for x in quad], axis=0)
            wtok = None
            for j, x in enumerate(_lhs_sums(pltpu.bitcast(wo, BF16).astype(F32))):
                wos_s[_ds(((h >> 1) * 5 + j) * (M // 4) + r0, 8, 8), :] = _pack(x)
                if j in (0, 4):
                    wtok = _sample(x) if wtok is None else wtok | _sample(x)
            return wtok & zero

        nxt = jnp.minimum(h + 1, H - 1)
        toks[-1] = tokens(finish_last(jnp.maximum(h - 1, 0)))
        for step in P2ORDER.split():
            i = int(step[1:])
            if step[0] == 'K':
                ks.append(project(i, wk))
            elif step[0] == 'V':
                vs.append(project(i, wv))
            elif step[0] == 'Q':
                q = q_s[_ds(h * (S // 2) + i * TQ // 2, TQ // 2, TQ // 2), :]
                if i >= 1:
                    q = q | jnp.tile(zero, (TQ // 16, D // 128))
                extra = toks.get(i - 2, [])
                if i == WOQ:
                    extra = _mix(extra, [wo_sums(part) for part in range(7)])
                if i == NB - 1:
                    bits = first_operand(nxt)
                    if B11Q:
                        extra = _mix(extra, [_sample(bits[k * 64:(k + 1) * 64]) & zero for k in range(8)])
                sc[i] = _qk(i, q, ks, zero, extra)
            elif i == NB - 1:
                extra = [None] * PSKIP + toks[i - 1]
                o7_s[...], l7_s[...] = _softmax_pv(*sc[i], vs, zero, extra)
            else:
                bits = _normalize(*_softmax_pv(*sc[i], vs, zero, []))
                ctx_s[_ds(h * (S // 2) + i * TQ // 2, TQ // 2, TQ // 2), :] = _pack(bits)
                toks[i] = tokens(bits)
        return carry

    jax.lax.fori_loop(0, H, phase2, 0)

    def finish(i, ot):
        r0 = i * TO if isinstance(i, int) else pl.multiple_of(i * TO, TO)
        top = at_s[MA:M, pl.ds(r0, TO)].astype(F32)
        val = jnp.concatenate([top, ot], axis=0).T
        stage_b[pl.ds(r0, TO), :] = val.astype(BF16)
        return val

    def oproj(i, pending):
        hm = M // 4
        rows = pl.multiple_of(i * TO, TO)
        ctx = [jnp.concatenate([ctx_s[pl.ds(h * (S // 2) + rows + k * (TO // 2), TO // 2), :] for h in range(H)], axis=1)
               for k in range(2)]
        q1, q2 = [pltpu.bitcast(x, BF16).astype(F32) for x in ctx]
        kh = H * D // 2
        b11, b21, b12, b22 = q1[:, :kh], q1[:, kh:], q2[:, :kh], q2[:, kh:]
        rhs = [(b11 + b22).astype(BF16), pltpu.bitcast(ctx[0][:, :kh], BF16), (b12 - b22).astype(BF16),
               (b21 - b11).astype(BF16), pltpu.bitcast(ctx[1][:, kh:], BF16), (b11 + b12).astype(BF16),
               (b21 + b22).astype(BF16)]

        def sums(j):
            return jnp.concatenate([wos_s[(p * 5 + j) * hm:(p * 5 + j + 1) * hm, :] for p in range(H // 2)], axis=1)
        lhs = [lambda: sums(0), lambda: sums(1),
               lambda: jnp.concatenate([wot_s[h, :hm, :] for h in range(H // 2)], axis=1),
               lambda: jnp.concatenate([wot_s[h, hm:, :] for h in range(H // 2, H)], axis=1),
               lambda: sums(2), lambda: sums(3), lambda: sums(4)]
        ms = [None] * 7
        for n, j in enumerate(MORDER):
            x = lhs[j]()
            if n in pending:
                tok = None
                for y in pending[n]():
                    tok = _or_fold(y) if tok is None else tok | _or_fold(y)
                x = _inject(x, tok & zero_s[...])
            ms[j] = _dot_nt(pltpu.bitcast(x, BF16), rhs[j])
            if n == 4:
                first = jnp.concatenate([(ms[0] + ms[3]) + (ms[6] - ms[4]), ms[1] + ms[3]], axis=0)
                pending = dict(pending)
                val = finish(2 * i, first)
                cp_out_b(2 * i).start()
                pending[6] = lambda: [val]
        return jnp.concatenate([ms[2] + ms[4], (ms[0] - ms[1]) + (ms[2] + ms[5])], axis=0)

    def phase3(it, carry):
        prev = jnp.maximum(NB3 * it - 1, 0)
        val = finish(prev, ot_s[...])

        @pl.when(it > 0)
        def _():
            cp_out_b(prev).start()

        r0 = pl.multiple_of(it * (NB3 * TO), NB3 * TO)
        apart = []
        for g in range(MA // 128):
            blk = at_s[g * 128:(g + 1) * 128, pl.ds(r0, NB3 * TO)].astype(F32).T
            stage_a[pl.ds(r0, NB3 * TO), g * 128:(g + 1) * 128] = blk.astype(BF16)
            apart.append(blk)
        cp_out_a(it).start()

        pend = {2: lambda: [val], 3: lambda: apart}
        for k in range(NB3 // 2 - 1):
            u = NB3 // 2 * it + k
            val2 = finish(2 * u + 1, oproj(u, pend))
            cp_out_b(2 * u + 1).start()
            pend = {2: lambda: [val2]}
        ot_s[...] = oproj(NB3 // 2 * it + NB3 // 2 - 1, pend)
        finish_last(H - 1)
        return carry

    jax.lax.fori_loop(0, NO // NB3, phase3, 0)

    finish(NO - 1, ot_s[...])
    cp_out_b(NO - 1).start()
    for i in range(NO // NB3):
        cp_out_a(i).wait()
    for i in range(NO):
        cp_out_b(i).wait()


@jax.jit
def pallas_concat_heads__ssm_conv_h3__compressed_kv_cla__prompt_kernel(
    A_q: jax.Array,
    A_k: jax.Array,
    A_v: jax.Array,
    A_shift_k: jax.Array,
    A_ssm_k: jax.Array,
    A_ssm_D: jax.Array,
    B_x: jax.Array,
    B_c_kv: jax.Array,
    B_w_q: jax.Array,
    B_w_uk: jax.Array,
    B_w_uv: jax.Array,
    B_w_o: jax.Array,
):
    vm = pltpu.VMEM
    dma = pltpu.SemaphoreType.DMA
    scratch = [
        vm((4, M), BF16),
        vm((M,), BF16),
        vm((5, MP, 128), F32),
        vm((64, 256), U32),
        vm((64, 256), U32),
        vm((8, 128), U32),
        vm((M, S), BF16),
        vm((S // 256 * 7 * 64, MP // 2), U32),
        vm((H // 2, M, D), U32),
        vm((NU, UC // 2, S), U32),
        vm((NU, UC // 2, S), U32),
        vm((NU, UC // 2, S), U32),
        vm((NU, UC // 2, S), U32),
        vm((M, S), BF16),
        vm((S // 2, C), U32),
        vm((S // PC * 5 * 64, C // 2), U32),
        vm((C // 4, 256), U32),
        vm((H // 2, C, D), U32),
        vm((H // 2, C, D), U32),
        vm((H, M // 2, D), U32),
        vm((H // 2 * 5 * M // 4, D), U32),
        vm((H * S // 2, D), U32),
        vm((H * S // 2, D), U32),
        vm((M, TO), F32),
        vm((TQ, D), F32),
        vm((TQ, 128), F32),
        vm((S, MA), BF16),
        vm((S, MP), BF16),
        dma((2,)), dma((XCH,)), dma((H // 2,)), dma((NU * 4,)), dma((S // PC + 1,)),
        dma((H // 2,)), dma((H // 2,)), dma((NO // NB3,)), dma((NO,)),
    ]
    out = pl.pallas_call(
        _kernel,
        in_specs=[pl.BlockSpec(memory_space=pl.ANY)] * 12,
        out_specs=pl.BlockSpec(memory_space=pl.ANY),
        out_shape=jax.ShapeDtypeStruct((S, 2 * M), BF16),
        scratch_shapes=scratch,
        compiler_params=pltpu.CompilerParams(
            vmem_limit_bytes=120 * 1024 * 1024,
            disable_semaphore_checks=True,
            disable_bounds_checks=True,
        ),
        name="h3_cla_fused",
    )(
        A_q[0].T, A_k[0].T, A_v[0].T, A_shift_k.T, A_ssm_k, A_ssm_D,
        B_x[0].T, B_c_kv[0], B_w_q, B_w_uk, B_w_uv, jnp.transpose(B_w_o, (0, 2, 1)),
    )
    return out[None]
```

```python
import math

import jax
import jax.numpy as jnp
import jax.experimental.pallas as pl
import jax.experimental.pallas.tpu as pltpu

S = 2048
M = 448
MP = 512
MA = 384
H = 16
D = 256
C = 1024
G = 32
NC = 128 // G
TQ = 128 * NC
NB = S // TQ
PC = 512
NU = 7
UC = M // NU
NBLK = S // 128
QCH = 128
XB = (0, 256, 768, 1280, 2048)
XCH = len(XB) - 1
TO = 128
NO = S // TO
NB3 = 4
TOKH = 6
MLAG = 800
SLAG = 1000
NPART = 32
P1ORDER = ("H0 H1 H2 H3 Q0 X0 Q1 X1 Q2 X2 Q3 X3 Q4 I00 Q5 I01 Q6 I10 Q7 I11 "
           "Q8 Q9 I20 Q10 I21 Q11 Q12 I30 Q13 I31 Q14 Q15")

P2ORDER = "M101 M401 M001 M301 M601 M201 M501 Q0 M12 M42 P0 Q1 M02 M32 M62 P1 M22 M52 Q2 M13 M43 M03 M33 M63 P2 Q3 M23 M53 P3"

WPARTS = 16
WOQ = 2
KVF32 = 1
CTOK = 0
PSKIP = 0
B11Q = 1
WPLAN = {'Q3': range(0, 8), 'P2': range(8, 12), 'P3': range(12, 16)}
TOKQ = {1: -1, 2: 0, 3: 1}
WT = 1
CT = 2
MORDER = (1, 4, 0, 3, 6, 2, 5)
XLAG = 3
P1PLAN = {0:'H0 H1 H2 H3',4:'X0',7:'X1',11:'X2',14:'X3',19:'I00',24:'I01',28:'I10',32:'I11',36:'I20',40:'I21',44:'I30',48:'I31',2:'C0',51:'C1',53:'C2',55:'C3'}
F32 = jnp.float32
BF16 = jnp.bfloat16
U32 = jnp.uint32
HI_MASK = 0xFFFF0000
Q_SCALE = D ** -0.5
MASK_VALUE = -1e9


def _dot(a, b):
    return jnp.dot(a, b, preferred_element_type=F32)


def _dot_nt(a, b):
    return jax.lax.dot_general(a, b, (((1,), (1,)), ((), ())), preferred_element_type=F32)


def _pack(x):
    return pltpu.bitcast(x.astype(BF16), U32)


def _ds(start, size, align):
    return pl.ds(start if isinstance(start, int) else pl.multiple_of(start, align), size)


def _sample(x):
    return _or_fold(jnp.concatenate([x[r + 8:r + 16] for r in range(0, x.shape[0], 16)], axis=0))


def _quads(x):
    r, c = x.shape[0] // 2, x.shape[1] // 2
    return x[:r, :c], x[:r, c:], x[r:, :c], x[r:, c:]


def _lhs_sums(a):
    a11, a12, a21, a22 = _quads(a)
    return a11 + a22, a21 + a22, a11 + a12, a21 - a11, a12 - a22


def _lhs_ops(a):
    a11, _, _, a22 = _quads(a)
    s1, s2, s5, s6, s7 = _lhs_sums(a)
    return s1, s2, a11, a22, s5, s6, s7


def _rhs_ops(b):
    b11, b12, b21, b22 = _quads(b)
    return b11 + b22, b11, b12 - b22, b21 - b11, b22, b11 + b12, b21 + b22


def _combine(m):
    m1, m2, m3, m4, m5, m6, m7 = m
    top = jnp.concatenate([(m1 + m4) + (m7 - m5), m3 + m5], axis=1)
    bot = jnp.concatenate([m2 + m4, (m1 - m2) + (m3 + m6)], axis=1)
    return jnp.concatenate([top, bot], axis=0)


def _or_fold(x):
    bits = pltpu.bitcast(x, U32)
    t = None
    for r in range(bits.shape[0] // 8):
        for c in range(bits.shape[1] // 128):
            e = bits[r * 8:(r + 1) * 8, c * 128:(c + 1) * 128]
            t = e if t is None else t | e
    return t


def _inject(x, tok):
    top = x[:8, :128] | tok
    if x.shape[1] > 128:
        top = jnp.concatenate([top, x[:8, 128:]], axis=1)
    return jnp.concatenate([top, x[8:]], axis=0)


def _recip(x):
    r = pl.reciprocal(x, approx=True)
    return r * (2.0 - x * r)


def _rows(chunks, r0, r1):
    parts = []
    while r0 < r1:
        c = r0 // PC
        e = min(r1, (c + 1) * PC)
        parts.append(chunks[c][r0 - c * PC:e - c * PC] if KVF32 else chunks[c][(r0 - c * PC) // 2:(e - c * PC) // 2])
        r0 = e
    x = parts[0] if len(parts) == 1 else jnp.concatenate(parts, axis=0)
    return x.astype(BF16) if KVF32 else pltpu.bitcast(x, BF16)


def _steps(i):
    plans = []
    for cls in range(NC):
        last = cls == NC - 1
        base = 0 if last else G * (cls + 1)
        full = NC * i - 1 + last
        plan = []
        m = 0
        while m < full:
            w = 2 if m + 2 <= full else 1
            plan.append((cls, base + 128 * m, base + 128 * (m + w), 0, False))
            m += w
        for t in range(NC):
            if full + t >= 0:
                plan.append((cls, base + 128 * (full + t), base + 128 * (full + t + 1), G * t, True))
        plans.append(plan)
    n = max(len(p) for p in plans)
    return [plans[cls][j - n + len(plans[cls])] for j in range(n) for cls in reversed(range(NC))
            if j - n + len(plans[cls]) >= 0]


def _due(steps, lag):
    ends, out, t = [], [], 0
    for _, k0, k1, row0, _ in steps:
        src = [n for n, e in enumerate(ends) if e + lag <= t]
        out.append(src[-1] if src else None)
        t += (128 - row0) * (k1 - k0) // 256
        ends.append(t)
    return [None if x in out[:n] else x for n, x in enumerate(out)]


def _token(n, nsteps, own, extra):
    t = own
    for k, e in enumerate(extra):
        if e is not None and k * nsteps // len(extra) == n:
            t = e if t is None else t | e
    return t


def _mix(a, b):
    if not a or not b:
        return a or b
    keyed = [((k + 0.5) / len(a), x) for k, x in enumerate(a)] + [((k + 1.0) / len(b), x) for k, x in enumerate(b)]
    return [x for _, x in sorted(keyed, key=lambda e: e[0])]


def _update(acc, x, row0, op):
    if acc is None:
        return x
    if row0 == 0:
        return op(acc, x)
    return jnp.concatenate([acc[:row0], op(acc[row0:], x)], axis=0)


def _qk(i, qu, ks, zero, extra):
    r = jax.lax.broadcasted_iota(jnp.int32, (G, 128), 0)
    c = jax.lax.broadcasted_iota(jnp.int32, (G, 128), 1)
    msk = c <= r + (128 - G)
    h = G // 2
    qc = [jnp.concatenate([qu[64 * t + h * cls:64 * t + h * (cls + 1)] for t in range(NC)], axis=0)
          for cls in range(NC)]
    steps = _steps(i)
    due = _due(steps, MLAG)
    toks = {}
    run = [None] * NC
    sc, lead = [], []
    for cls in range(NC - 1):
        w = G * (cls + 1)
        s = _dot_nt(_rows(ks, 0, w), pltpu.bitcast(qc[cls], BF16)).T
        if i == 0:
            top = jnp.where((c <= r + G * cls)[:, :w], s[:G], MASK_VALUE)
            s = jnp.concatenate([top, s[G:]], axis=0)
        lead.append(s)
        run[cls] = jnp.concatenate([s, jnp.full((128, 128 - w), MASK_VALUE, F32)], axis=1)
    for n, (cls, k0, k1, row0, masked) in enumerate(steps):
        x = qc[cls][row0 // 2:]
        t = _token(n, len(steps), toks.get(due[n]), extra)
        s = _dot_nt(pltpu.bitcast(x if t is None else _inject(x, t), BF16), _rows(ks, k0, k1))
        if masked:
            top = jnp.where(msk, s[:G], MASK_VALUE)
            s = top if row0 + G == 128 else jnp.concatenate([top, s[G:]], axis=0)
        sc.append(s)
        mj = jnp.maximum(s[:, :128], s[:, 128:]) if k1 - k0 == 256 else s
        run[cls] = _update(run[cls], mj, row0, jnp.maximum)
        toks[n] = _or_fold(run[cls]) & zero
    return steps, lead, sc, run


def _softmax_pv(steps, lead, sc, mx, vs, zero, extra):
    m = [jnp.max(mx[cls], axis=1, keepdims=True) for cls in range(NC)]
    due = _due(steps, SLAG)
    toks = {}
    o = [None] * NC
    run = [None] * NC
    for cls in range(NC - 1):
        w = G * (cls + 1)
        p = jnp.exp(lead[cls] - m[cls]).astype(BF16)
        o[cls] = _dot(p, _rows(vs, 0, w))
        run[cls] = jnp.concatenate([p.astype(F32), jnp.zeros((128, 128 - w), F32)], axis=1)
    for n, (cls, k0, k1, row0, _) in enumerate(steps):
        p = jnp.exp(sc[n] - m[cls][row0:])
        t = _token(n, len(steps), toks.get(due[n]), extra)
        if t is not None:
            p = pltpu.bitcast(_inject(pltpu.bitcast(p, U32), t), F32)
        p = p.astype(BF16)
        t = _dot(p, _rows(vs, k0, k1))
        e = p.astype(F32)
        ej = e[:, :128] + e[:, 128:] if k1 - k0 == 256 else e
        o[cls] = _update(o[cls], t, row0, jnp.add)
        run[cls] = _update(run[cls], ej, row0, jnp.add)
        toks[n] = _or_fold(run[cls]) & zero

    def natural(x):
        return jnp.concatenate([x[cls][G * t:G * (t + 1)] for t in range(NC) for cls in range(NC)], axis=0)
    return natural(o), natural(run)


def _normalize(o, lsum):
    r = _recip(jnp.sum(lsum, axis=1, keepdims=True))
    return o * r


def _kernel(aq_hbm, ak_hbm, av_hbm, sh_hbm, ah_hbm, dd_hbm, xt_hbm, c_hbm,
            wq_hbm, wk_hbm, wv_hbm, wot_hbm,
            out_hbm,
            sh_s, dd_s, coef_s, f_s, fh_s, zero_s, xt_s, x_s, wq_raw, aq_s, ak_s, av_s, ah_s, at_s,
            c_s, cs_s, ws_s, wk_raw, wv_raw, wot_s, wos_s, q_s, ctx_s, ot_s, o7_s, l7_s, stage_a, stage_b,
            sem_small, sem_x, sem_wq, sem_a, sem_c, sem_wk, sem_wv, sem_oa, sem_ob):
    wq32 = wq_hbm.bitcast(U32)
    wk32 = wk_hbm.bitcast(U32)
    wv32 = wv_hbm.bitcast(U32)

    def cp_small(i):
        return pltpu.make_async_copy((sh_hbm, dd_hbm)[i], (sh_s, dd_s)[i], sem_small.at[i])

    def cp_x(i):
        cols = pl.ds(XB[i], XB[i + 1] - XB[i])
        return pltpu.make_async_copy(xt_hbm.at[:, cols], xt_s.at[:, cols], sem_x.at[i])

    def cp_wq(p):
        return pltpu.make_async_copy(wq32.at[:, p, :], wq_raw.at[p], sem_wq.at[p])

    def cp_a(g, i):
        src = (ah_hbm, ak_hbm, av_hbm, aq_hbm)[i].bitcast(U32)
        dst = (ah_s, ak_s, av_s, aq_s)[i]
        n = UC // 2
        start = g * n if isinstance(g, int) else pl.multiple_of(g * n, 8)
        return pltpu.make_async_copy(src.at[pl.ds(start, n), :], dst.at[g], sem_a.at[g * 4 + i])

    def cp_c(i):
        n = 128
        start = i * n if isinstance(i, int) else pl.multiple_of(i * n, n)
        return pltpu.make_async_copy(c_hbm.bitcast(U32).at[pl.ds(start, n), :],
                                     c_s.at[pl.ds(start, n), :], sem_c.at[i])

    def cp_wo():
        return pltpu.make_async_copy(wot_hbm.bitcast(U32), wot_s, sem_c.at[8])

    def c_ops(strip):
        blk, part = strip >> 3, strip & 7
        a = jnp.concatenate([c_s[_ds(blk * 256 + k * 64 + part * 8, 8, 8), :] for k in range(4)], axis=0)
        a = pltpu.bitcast(a, BF16).astype(F32)
        tok = None
        for i, x in enumerate(_lhs_ops(a)):
            for j, y in enumerate(_lhs_ops(x)):
                cs_s[_ds(((blk * 7 + i) * 7 + j) * 64 + part * 8, 8, 8), :] = _pack(y)
                if j % CT == 0:
                    tok = _sample(y) if tok is None else tok | _sample(y)
        return tok & zero_s[...]

    def cp_wk(p):
        return pltpu.make_async_copy(wk32.at[:, p, :], wk_raw.at[p], sem_wk.at[p])

    def cp_wv(p):
        return pltpu.make_async_copy(wv32.at[:, p, :], wv_raw.at[p], sem_wv.at[p])

    def cp_out_a(i):
        n = NB3 * TO
        start = i * n if isinstance(i, int) else pl.multiple_of(i * n, n)
        return pltpu.make_async_copy(stage_a.at[pl.ds(start, n), :],
                                     out_hbm.at[pl.ds(start, n), pl.ds(0, MA)], sem_oa.at[i])

    def cp_out_b(i):
        start = i * TO if isinstance(i, int) else pl.multiple_of(i * TO, TO)
        return pltpu.make_async_copy(stage_b.at[pl.ds(start, TO), :],
                                     out_hbm.at[pl.ds(start, TO), pl.ds(MA, MP)], sem_ob.at[i])

    cp_x(0).start()
    cp_wq(0).start()
    for i in range(1, XCH):
        cp_x(i).start()
    cp_small(0).start()
    cp_small(1).start()

    tt = jax.lax.broadcasted_iota(jnp.int32, (128, 128), 0)
    rr = jax.lax.broadcasted_iota(jnp.int32, (128, 128), 1)
    ang = ((tt * (2 * rr + 1)) & 511).astype(F32) * (2.0 * math.pi / 512.0)
    fmat = jnp.concatenate([jnp.cos(ang), -jnp.sin(ang)], axis=1).astype(BF16)
    f_s[...] = pltpu.bitcast(fmat, U32)
    fh_s[...] = pltpu.bitcast((fmat.astype(F32) * (1.0 / 128.0)).astype(BF16), U32)
    zero_s[...] = jnp.zeros((8, 128), U32)

    def xpose_x(i):
        for blk in range(XB[i] // 256, XB[i + 1] // 256):
            tiles = []
            for t in (2 * blk, 2 * blk + 1):
                cols = slice(t * 128, (t + 1) * 128)
                parts = [xt_s[g * 128:(g + 1) * 128, cols].astype(F32).T for g in range(3)]
                last = jnp.concatenate([xt_s[MA:M, cols].astype(F32), jnp.zeros((MP - M, 128), F32)], axis=0)
                parts.append(last.T)
                tiles.append(jnp.concatenate(parts, axis=1))
            x = jnp.concatenate(tiles, axis=0)
            for j, op in enumerate(_lhs_ops(x)):
                x_s[(blk * 7 + j) * 64:(blk * 7 + j + 1) * 64, :] = _pack(op)

    def q_weights(p):
        raw = wq_raw[p]
        ops = []
        for w in (raw << 16, raw & jnp.uint32(HI_MASK)):
            w = pltpu.bitcast(w, F32) * Q_SCALE
            ops.append(_rhs_ops(jnp.concatenate([w, jnp.zeros((MP - M, D), F32)], axis=0)))
        return [jnp.concatenate([u, v], axis=1).astype(BF16) for u, v in zip(*ops)]

    def qstep(p, w, ms, n, tok=None):
        blk, j = n // 7, MORDER[n % 7]
        x = x_s[(blk * 7 + j) * 64:(blk * 7 + j + 1) * 64, :]
        if tok is not None:
            x = _inject(x, tok)
        ms[j] = _dot(pltpu.bitcast(x, BF16), w[j])
        if n % 7 == 6:
            for k in range(2):
                q = _combine([ms[e][:, k * 128:(k + 1) * 128] for e in range(7)])
                q_s[_ds((2 * p + k) * (S // 2) + blk * 128, 128, 128), :] = _pack(q)

    cp_x(0).wait()
    xpose_x(0)
    cp_c(0).start()
    cp_c(1).start()
    for g in range(NU):
        cp_wq(g + 1).start()
        for i in range(4):
            cp_a(g, i).start()
        if g < NU - 1:
            cp_c(g + 2).start()
    cp_wk(0).start()
    cp_wv(0).start()
    cp_wo().start()
    for p in range(1, H // 2):
        cp_wk(p).start()
        cp_wv(p).start()
    cp_wq(0).wait()
    w0 = q_weights(0)
    ms0 = {}
    for n in range(XB[1] // 256 * 7 - XLAG):
        qstep(0, w0, ms0, n)
    for i in range(1, XCH):
        cp_x(i).wait()
        if i == XCH - 1:
            cp_small(0).wait()
            cp_small(1).wait()
            cp_c(0).wait()
            cp_c(1).wait()
            for strip in range(4):
                c_ops(strip)
            prm = [sh_s[j:j + 1, :].astype(F32) for j in range(4)]
            prm.append(dd_s[...].astype(F32).reshape(1, M))
            for j in range(5):
                row = jnp.concatenate([prm[j], jnp.zeros((1, MP - M), F32)], axis=1)
                for t in range(MP // 128):
                    blk = jnp.broadcast_to(row[:, t * 128:(t + 1) * 128], (128, 128))
                    coef_s[j, t * 128:(t + 1) * 128, :] = blk.T
        for n in range(XB[i] // 256 * 7 - XLAG, XB[i] // 256 * 7):
            qstep(0, w0, ms0, n)
        xpose_x(i)
        for n in range(XB[i] // 256 * 7, XB[i + 1] // 256 * 7 - (XLAG if i < XCH - 1 else 0)):
            qstep(0, w0, ms0, n)
    ot_s[...] = jnp.zeros((M, TO), F32)
    o7_s[...] = jnp.zeros((TQ, D), F32)
    l7_s[...] = jnp.ones((TQ, 128), F32)

    def phase1(g, carry):
        cp_wq(g + 1).wait()
        for i in range(4):
            cp_a(g, i).wait()

        @pl.when((g & 1) == 1)
        def _():
            cp_c(g + 1).wait()
            cp_c(g + 2).wait()

        w = q_weights(g + 1)
        fh = pltpu.bitcast(fh_s[...], BF16)
        fx = pltpu.bitcast(f_s[...], BF16)
        lane = jax.lax.broadcasted_iota(jnp.int32, (16, 128), 1)
        sgn = jnp.where((jax.lax.broadcasted_iota(jnp.int32, (8, 128), 1) & 1) == 0, 1.0, -1.0)
        zh, zx, kvs, ys = {}, {}, {}, {}

        def coef(k, j):
            return coef_s[j, pl.ds(pl.multiple_of(g * UC + k * 16, 16), 16), :]

        def hfwd(k):
            lhs = jnp.concatenate([ah_s[g, k * 8:(k + 1) * 8, c * 128:(c + 1) * 128]
                                   for c in range(NBLK)], axis=0)
            zh[k] = _dot(pltpu.bitcast(lhs, BF16), fh)

        def xfwd(k):
            kf = pltpu.bitcast(ak_s[g, k * 8:(k + 1) * 8, :], BF16).astype(F32)
            vf = pltpu.bitcast(av_s[g, k * 8:(k + 1) * 8, :], BF16).astype(F32)
            sh_k = [kf] + [pltpu.roll(kf, j, 1) for j in range(1, 4)]
            cf = [coef(k, j) for j in range(4)]
            kvf = []
            for c in range(NBLK):
                cols = slice(c * 128, (c + 1) * 128)
                t = sh_k[0][:, cols] * cf[0]
                for j in range(1, 4):
                    kj = sh_k[j][:, cols]
                    if c == 0:
                        kj = jnp.where(lane >= j, kj, 0.0)
                    t = t + kj * cf[j]
                kvf.append(t * vf[:, cols])
            kvs[k] = jnp.concatenate(kvf, axis=0).astype(BF16)
            zx[k] = _dot(kvs[k], fx)

        def inv(k, u):
            rows = [slice(c * 16 + u * 8, c * 16 + u * 8 + 8) for c in range(NBLK)]
            xr = [zx[k][r, :128] for r in rows]
            xi = [zx[k][r, 128:] for r in rows]
            h0r = [zh[k][r, :128] for r in rows]
            h0i = [zh[k][r, 128:] for r in rows]
            hr = [h0r[0]] + [h0r[j] - sgn * h0i[j - 1] for j in range(1, NBLK)]
            hi = [h0i[0]] + [h0i[j] + sgn * h0r[j - 1] for j in range(1, NBLK)]
            pr, pi = [], []
            for a0 in range(0, NBLK, 4):
                re = [None] * 4
                im = [None] * 4
                for c0 in range(0, a0 + 4, 4):
                    for da in range(4):
                        for c in range(c0, c0 + 4):
                            j = a0 + da - c
                            if j < 0:
                                continue
                            tr = xr[c] * hr[j] - xi[c] * hi[j]
                            ti = xr[c] * hi[j] + xi[c] * hr[j]
                            re[da] = tr if re[da] is None else re[da] + tr
                            im[da] = ti if im[da] is None else im[da] + ti
                pr += re
                pi += im
            p = jnp.concatenate([jnp.concatenate(pr, axis=0), jnp.concatenate(pi, axis=0)], axis=1)
            ys[k, u] = _dot_nt(p.astype(BF16), fx)
            if u == 1:
                kvr = kvs[k].astype(F32)
                qraw = aq_s[g, k * 8:(k + 1) * 8, :] | jnp.tile(zero_s[...], (1, NBLK))
                qf = pltpu.bitcast(qraw, BF16).astype(F32)
                dd = coef(k, 4)
                row0 = pl.multiple_of(g * UC + k * 16, 16)
                for a in range(NBLK):
                    cols = slice(a * 128, (a + 1) * 128)
                    y = jnp.concatenate([ys[k, 0][a * 8:(a + 1) * 8], ys[k, 1][a * 8:(a + 1) * 8]], axis=0)
                    y = y + kvr[a * 16:(a + 1) * 16] * dd
                    at_s[pl.ds(row0, 16), cols] = (qf[:, cols] * y).astype(BF16)

        ms = {}
        for n in range(S // 256 * 7):
            tok = None
            for step in P1PLAN.get(n, '').replace('_', ' ').split():
                if step[0] == 'H':
                    hfwd(int(step[1]))
                elif step[0] == 'X':
                    xfwd(int(step[1]))
                elif step[0] == 'I':
                    inv(int(step[1]), int(step[2]))
                else:
                    tok = c_ops(4 * (g + 1) + int(step[1]))
            qstep(g + 1, w, ms, n, tok)
        return carry

    jax.lax.fori_loop(0, NU, phase1, 0)

    cp_wo().wait()
    for p in range(H // 2):
        cp_wk(p).wait()
        cp_wv(p).wait()

    def unpack_head(w, h):
        sh = (16 - ((h & 1) << 4)).astype(U32)
        return pltpu.bitcast((w << sh) & jnp.uint32(HI_MASK), F32)

    def first_operands(h):
        w = jnp.concatenate([wk_raw[h >> 1, :256, :128], wk_raw[h >> 1, 256:512, 128:]], axis=1)
        w = unpack_head(w, h)
        ws_s[...] = _pack(w)
        return w

    first_operands(jnp.int32(0))

    def product(ws, blks, i):
        ms = [None] * 7
        for j in MORDER:
            r = [((blk * 7 + i) * 7 + j) * 64 for blk in blks]
            x = jnp.concatenate([cs_s[e:e + 64, :] for e in r], axis=0)
            ms[j] = _dot(pltpu.bitcast(x, BF16), ws[i][j])
        return [_combine([m[k * 128:(k + 1) * 128] for m in ms]) for k in range(len(blks))]

    def finish_last(h):
        bits = _normalize(o7_s[...], l7_s[...])
        ctx_s[_ds(h * (S // 2) + (NB - 1) * TQ // 2, TQ // 2, TQ // 2), :] = _pack(bits)
        return bits

    def phase2(h, carry):
        b = unpack_head(jnp.concatenate([wk_raw[h >> 1], wv_raw[h >> 1]], axis=1), h)
        ws = [[y.astype(BF16) for y in _rhs_ops(x)] for x in _rhs_ops(b)]
        ws[1][1] = pltpu.bitcast(ws_s[:, :128], BF16)
        ws[1][4] = pltpu.bitcast(ws_s[:, 128:], BF16)
        mo = {}
        ks, vs, toks, sc = [], [], {}, {}
        zero = zero_s[...]

        def tokens(bits):
            n = TQ // NPART
            return [(_or_fold(bits[k * n:(k + 1) * n]) if CTOK == 0 else _or_fold(bits[k * n:(k + 1) * n, :128]) if CTOK == 1 else _sample(bits[k * n:(k + 1) * n])) & zero for k in range(NPART)]

        def wo_sums(part):
            r0 = (h & 1) * (M // 8) + part * 8
            quad = [[wot_s[(h >> 1) + k * (H // 2), _ds(r + r0, 8, 8), :] for k in range(2)] for r in (0, M // 4)]
            wo = jnp.concatenate([jnp.concatenate(x, axis=1) for x in quad], axis=0)
            wtok = None
            for j, x in enumerate(_lhs_sums(pltpu.bitcast(wo, BF16).astype(F32))):
                wos_s[_ds(((h >> 1) * 5 + j) * (M // 4) + r0, 8, 8), :] = _pack(x)
                if j in (0, 4):
                    wtok = _sample(x) if wtok is None else wtok | _sample(x)
            return wtok & zero

        nxt = jnp.minimum(h + 1, H - 1)
        toks[-1] = tokens(finish_last(jnp.maximum(h - 1, 0)))
        for step in P2ORDER.split():
            i = int(step[1:])
            if step[0] == 'M':
                blks = [int(e) for e in step[2:]]
                j = int(step[1])
                for blk, m in zip(blks, product(ws, blks, j)):
                    mo[blk, j] = m
                    e = [mo.get((blk, k)) for k in range(7)]
                    if j == 6:
                        ks.append(jnp.concatenate([(e[0] + e[3]) + (e[6] - e[4]), e[1] + e[3]], axis=0))
                    if j == 5:
                        vs.append(jnp.concatenate([e[2] + e[4], (e[0] - e[1]) + (e[2] + e[5])], axis=0))
            elif step[0] == 'Q':
                q = q_s[_ds(h * (S // 2) + i * TQ // 2, TQ // 2, TQ // 2), :]
                if i >= 1:
                    q = q | jnp.tile(zero, (TQ // 16, D // 128))
                extra = toks.get(TOKQ.get(i), [])
                if i == WOQ:
                    extra = _mix(extra, [wo_sums(part) for part in range(7)])
                if i == NB - 1:
                    w = first_operands(nxt)
                    extra = _mix(extra, [_sample(w[k * 64:(k + 1) * 64]) & zero for k in range(4)])
                sc[i] = _qk(i, q, ks, zero, extra)
            elif i == NB - 1:
                extra = [None] * PSKIP + toks[i - 1]
                o7_s[...], l7_s[...] = _softmax_pv(*sc[i], vs, zero, extra)
            else:
                bits = _normalize(*_softmax_pv(*sc[i], vs, zero, []))
                ctx_s[_ds(h * (S // 2) + i * TQ // 2, TQ // 2, TQ // 2), :] = _pack(bits)
                toks[i] = tokens(bits)
        return carry

    jax.lax.fori_loop(0, H, phase2, 0)

    def finish(i, ot):
        r0 = i * TO if isinstance(i, int) else pl.multiple_of(i * TO, TO)
        top = at_s[MA:M, pl.ds(r0, TO)].astype(F32)
        val = jnp.concatenate([top, ot], axis=0).T
        stage_b[pl.ds(r0, TO), :] = val.astype(BF16)
        return val

    def oproj(i, pending):
        hm = M // 4
        rows = pl.multiple_of(i * TO, TO)
        ctx = [jnp.concatenate([ctx_s[pl.ds(h * (S // 2) + rows + k * (TO // 2), TO // 2), :] for h in range(H)], axis=1)
               for k in range(2)]
        q1, q2 = [pltpu.bitcast(x, BF16).astype(F32) for x in ctx]
        kh = H * D // 2
        b11, b21, b12, b22 = q1[:, :kh], q1[:, kh:], q2[:, :kh], q2[:, kh:]
        rhs = [(b11 + b22).astype(BF16), pltpu.bitcast(ctx[0][:, :kh], BF16), (b12 - b22).astype(BF16),
               (b21 - b11).astype(BF16), pltpu.bitcast(ctx[1][:, kh:], BF16), (b11 + b12).astype(BF16),
               (b21 + b22).astype(BF16)]

        def sums(j):
            return jnp.concatenate([wos_s[(p * 5 + j) * hm:(p * 5 + j + 1) * hm, :] for p in range(H // 2)], axis=1)
        lhs = [lambda: sums(0), lambda: sums(1),
               lambda: jnp.concatenate([wot_s[h, :hm, :] for h in range(H // 2)], axis=1),
               lambda: jnp.concatenate([wot_s[h, hm:, :] for h in range(H // 2, H)], axis=1),
               lambda: sums(2), lambda: sums(3), lambda: sums(4)]
        ms = [None] * 7
        for n, j in enumerate(MORDER):
            x = lhs[j]()
            if n in pending:
                tok = None
                for y in pending[n]():
                    tok = _or_fold(y) if tok is None else tok | _or_fold(y)
                x = _inject(x, tok & zero_s[...])
            ms[j] = _dot_nt(pltpu.bitcast(x, BF16), rhs[j])
            if n == 4:
                first = jnp.concatenate([(ms[0] + ms[3]) + (ms[6] - ms[4]), ms[1] + ms[3]], axis=0)
                pending = dict(pending)
                val = finish(2 * i, first)
                cp_out_b(2 * i).start()
                pending[6] = lambda: [val]
        return jnp.concatenate([ms[2] + ms[4], (ms[0] - ms[1]) + (ms[2] + ms[5])], axis=0)

    def phase3(it, carry):
        prev = jnp.maximum(NB3 * it - 1, 0)
        val = finish(prev, ot_s[...])

        @pl.when(it > 0)
        def _():
            cp_out_b(prev).start()

        r0 = pl.multiple_of(it * (NB3 * TO), NB3 * TO)
        apart = []
        for g in range(MA // 128):
            blk = at_s[g * 128:(g + 1) * 128, pl.ds(r0, NB3 * TO)].astype(F32).T
            stage_a[pl.ds(r0, NB3 * TO), g * 128:(g + 1) * 128] = blk.astype(BF16)
            apart.append(blk)
        cp_out_a(it).start()

        pend = {2: lambda: [val], 3: lambda: apart}
        for k in range(NB3 // 2 - 1):
            u = NB3 // 2 * it + k
            val2 = finish(2 * u + 1, oproj(u, pend))
            cp_out_b(2 * u + 1).start()
            pend = {2: lambda: [val2]}
        ot_s[...] = oproj(NB3 // 2 * it + NB3 // 2 - 1, pend)
        finish_last(H - 1)
        return carry

    jax.lax.fori_loop(0, NO // NB3, phase3, 0)

    finish(NO - 1, ot_s[...])
    cp_out_b(NO - 1).start()
    for i in range(NO // NB3):
        cp_out_a(i).wait()
    for i in range(NO):
        cp_out_b(i).wait()


@jax.jit
def pallas_concat_heads__ssm_conv_h3__compressed_kv_cla__prompt_kernel(
    A_q: jax.Array,
    A_k: jax.Array,
    A_v: jax.Array,
    A_shift_k: jax.Array,
    A_ssm_k: jax.Array,
    A_ssm_D: jax.Array,
    B_x: jax.Array,
    B_c_kv: jax.Array,
    B_w_q: jax.Array,
    B_w_uk: jax.Array,
    B_w_uv: jax.Array,
    B_w_o: jax.Array,
):
    vm = pltpu.VMEM
    dma = pltpu.SemaphoreType.DMA
    scratch = [
        vm((4, M), BF16),
        vm((M,), BF16),
        vm((5, MP, 128), F32),
        vm((64, 256), U32),
        vm((64, 256), U32),
        vm((8, 128), U32),
        vm((M, S), BF16),
        vm((S // 256 * 7 * 64, MP // 2), U32),
        vm((H // 2, M, D), U32),
        vm((NU, UC // 2, S), U32),
        vm((NU, UC // 2, S), U32),
        vm((NU, UC // 2, S), U32),
        vm((NU, UC // 2, S), U32),
        vm((M, S), BF16),
        vm((S // 2, C), U32),
        vm((NB * 49 * 64, C // 4), U32),
        vm((128, 256), U32),
        vm((H // 2, C, D), U32),
        vm((H // 2, C, D), U32),
        vm((H, M // 2, D), U32),
        vm((H // 2 * 5 * M // 4, D), U32),
        vm((H * S // 2, D), U32),
        vm((H * S // 2, D), U32),
        vm((M, TO), F32),
        vm((TQ, D), F32),
        vm((TQ, 128), F32),
        vm((S, MA), BF16),
        vm((S, MP), BF16),
        dma((2,)), dma((XCH,)), dma((H // 2,)), dma((NU * 4,)), dma((9,)),
        dma((H // 2,)), dma((H // 2,)), dma((NO // NB3,)), dma((NO,)),
    ]
    out = pl.pallas_call(
        _kernel,
        in_specs=[pl.BlockSpec(memory_space=pl.ANY)] * 12,
        out_specs=pl.BlockSpec(memory_space=pl.ANY),
        out_shape=jax.ShapeDtypeStruct((S, 2 * M), BF16),
        scratch_shapes=scratch,
        compiler_params=pltpu.CompilerParams(
            vmem_limit_bytes=120 * 1024 * 1024,
            disable_semaphore_checks=True,
            disable_bounds_checks=True,
        ),
        name="h3_cla_fused",
    )(
        A_q[0].T, A_k[0].T, A_v[0].T, A_shift_k.T, A_ssm_k, A_ssm_D,
        B_x[0].T, B_c_kv[0], B_w_q, B_w_uk, B_w_uv, jnp.transpose(B_w_o, (0, 2, 1)),
    )
    return out[None]
```

```python
import math

import jax
import jax.numpy as jnp
import jax.experimental.pallas as pl
import jax.experimental.pallas.tpu as pltpu

S = 2048
M = 448
MP = 512
MA = 384
H = 16
D = 256
C = 1024
G = 32
NC = 128 // G
TQ = 128 * NC
NB = S // TQ
PC = 512
NU = 7
UC = M // NU
NBLK = S // 128
QCH = 128
XB = (0, 256, 768, 1280, 2048)
XCH = len(XB) - 1
TO = 128
NO = S // TO
NB3 = 4
TOKH = 6
MLAG = 800
SLAG = 1000
NPART = 32
P1ORDER = ("H0 H1 H2 H3 Q0 X0 Q1 X1 Q2 X2 Q3 X3 Q4 I00 Q5 I01 Q6 I10 Q7 I11 "
           "Q8 Q9 I20 Q10 I21 Q11 Q12 I30 Q13 I31 Q14 Q15")

P2ORDER = "M101 M401 M001 M301 M601 M201 M501 Q0 M12 M42 P0 Q1 M02 M32 M62 P1 M22 M52 Q2 M13 M43 M03 M33 M63 P2 Q3 M23 M53 P3"

WPARTS = 16
WOQ = 2
KVF32 = 1
CTOK = 0
PSKIP = 0
B11Q = 1
WPLAN = {'Q3': range(0, 8), 'P2': range(8, 12), 'P3': range(12, 16)}
TOKQ = {1: -1, 2: 0, 3: 1}
WT = 1
CT = 2
CPOS = list(list(range(16,19))+list(range(20,24))+[25,26,29,30,33,34,37,38,41,42,45,46,47]+list(range(49,56))+[1])
PVS = 1
PVG = 2
PVLAST = 0
PORDER = (2,4,5,0,3,1,6)
PUN = 0
PVMIN = 0
SUN = 1
VTOK = {0: ['V0', 'V1'], 2: ['V2']}
CMAJ = 1
VFULL = 1
MORDER = (1, 4, 0, 3, 6, 2, 5)
XLAG = 3
P1PLAN = {0:'H0 H1 H2 H3',4:'X0',7:'X1',11:'X2',14:'X3',19:'I00',24:'I01',28:'I10',32:'I11',36:'I20',40:'I21',44:'I30',48:'I31'}
F32 = jnp.float32
BF16 = jnp.bfloat16
U32 = jnp.uint32
HI_MASK = 0xFFFF0000
Q_SCALE = D ** -0.5
MASK_VALUE = -1e9


def _dot(a, b):
    return jnp.dot(a, b, preferred_element_type=F32)


def _dot_nt(a, b):
    return jax.lax.dot_general(a, b, (((1,), (1,)), ((), ())), preferred_element_type=F32)


def _pack(x):
    return pltpu.bitcast(x.astype(BF16), U32)


def _ds(start, size, align):
    return pl.ds(start if isinstance(start, int) else pl.multiple_of(start, align), size)


def _sample(x):
    return _or_fold(jnp.concatenate([x[r + 8:r + 16] for r in range(0, x.shape[0], 16)], axis=0))


def _quads(x):
    r, c = x.shape[0] // 2, x.shape[1] // 2
    return x[:r, :c], x[:r, c:], x[r:, :c], x[r:, c:]


def _lhs_sums(a):
    a11, a12, a21, a22 = _quads(a)
    return a11 + a22, a21 + a22, a11 + a12, a21 - a11, a12 - a22


def _lhs_ops(a):
    a11, _, _, a22 = _quads(a)
    s1, s2, s5, s6, s7 = _lhs_sums(a)
    return s1, s2, a11, a22, s5, s6, s7


def _rhs_ops(b):
    b11, b12, b21, b22 = _quads(b)
    return b11 + b22, b11, b12 - b22, b21 - b11, b22, b11 + b12, b21 + b22


def _combine(m):
    m1, m2, m3, m4, m5, m6, m7 = m
    top = jnp.concatenate([(m1 + m4) + (m7 - m5), m3 + m5], axis=1)
    bot = jnp.concatenate([m2 + m4, (m1 - m2) + (m3 + m6)], axis=1)
    return jnp.concatenate([top, bot], axis=0)


def _or_fold(x):
    bits = pltpu.bitcast(x, U32)
    t = None
    for r in range(bits.shape[0] // 8):
        for c in range(bits.shape[1] // 128):
            e = bits[r * 8:(r + 1) * 8, c * 128:(c + 1) * 128]
            t = e if t is None else t | e
    return t


def _inject(x, tok):
    top = x[:8, :128] | tok
    if x.shape[1] > 128:
        top = jnp.concatenate([top, x[:8, 128:]], axis=1)
    return jnp.concatenate([top, x[8:]], axis=0)


def _recip(x):
    r = pl.reciprocal(x, approx=True)
    return r * (2.0 - x * r)


def _rows(chunks, r0, r1, raw=False):
    parts = []
    while r0 < r1:
        c = r0 // PC
        e = min(r1, (c + 1) * PC)
        parts.append(chunks[c][r0 - c * PC:e - c * PC] if KVF32 else chunks[c][(r0 - c * PC) // 2:(e - c * PC) // 2])
        r0 = e
    x = parts[0] if len(parts) == 1 else jnp.concatenate(parts, axis=0)
    return x if raw else x.astype(BF16)


def _steps(i):
    plans = []
    for cls in range(NC):
        last = cls == NC - 1
        base = 0 if last else G * (cls + 1)
        full = NC * i - 1 + last
        plan = []
        m = 0
        while m < full:
            w = 2 if m + 2 <= full else 1
            plan.append((cls, base + 128 * m, base + 128 * (m + w), 0, False))
            m += w
        for t in range(NC):
            if full + t >= 0:
                plan.append((cls, base + 128 * (full + t), base + 128 * (full + t + 1), G * t, True))
        plans.append(plan)
    n = max(len(p) for p in plans)
    return [plans[cls][j - n + len(plans[cls])] for j in range(n) for cls in reversed(range(NC))
            if j - n + len(plans[cls]) >= 0]


def _due(steps, lag):
    ends, out, t = [], [], 0
    for _, k0, k1, row0, _ in steps:
        src = [n for n, e in enumerate(ends) if e + lag <= t]
        out.append(src[-1] if src else None)
        t += (128 - row0) * (k1 - k0) // 256
        ends.append(t)
    return [None if x in out[:n] else x for n, x in enumerate(out)]


def _token(n, nsteps, own, extra):
    t = own
    for k, e in enumerate(extra):
        if e is not None and k * nsteps // len(extra) == n:
            t = e if t is None else t | e
    return t


def _mix(a, b):
    if not a or not b:
        return a or b
    keyed = [((k + 0.5) / len(a), x) for k, x in enumerate(a)] + [((k + 1.0) / len(b), x) for k, x in enumerate(b)]
    return [x for _, x in sorted(keyed, key=lambda e: e[0])]


def _update(acc, x, row0, op):
    if acc is None:
        return x
    if row0 == 0:
        return op(acc, x)
    return jnp.concatenate([acc[:row0], op(acc[row0:], x)], axis=0)


def _qk(i, qu, ks, zero, extra):
    r = jax.lax.broadcasted_iota(jnp.int32, (G, 128), 0)
    c = jax.lax.broadcasted_iota(jnp.int32, (G, 128), 1)
    msk = c <= r + (128 - G)
    h = G // 2
    qc = [jnp.concatenate([qu[64 * t + h * cls:64 * t + h * (cls + 1)] for t in range(NC)], axis=0)
          for cls in range(NC)]
    steps = _steps(i)
    due = _due(steps, MLAG)
    toks = {}
    run = [None] * NC
    sc, lead = [], []
    for cls in range(NC - 1):
        w = G * (cls + 1)
        s = _dot_nt(_rows(ks, 0, w), pltpu.bitcast(qc[cls], BF16)).T
        if i == 0:
            top = jnp.where((c <= r + G * cls)[:, :w], s[:G], MASK_VALUE)
            s = jnp.concatenate([top, s[G:]], axis=0)
        lead.append(s)
        run[cls] = jnp.concatenate([s, jnp.full((128, 128 - w), MASK_VALUE, F32)], axis=1)
    for n, (cls, k0, k1, row0, masked) in enumerate(steps):
        x = qc[cls][row0 // 2:]
        t = _token(n, len(steps), toks.get(due[n]), extra)
        s = _dot_nt(pltpu.bitcast(x if t is None else _inject(x, t), BF16), _rows(ks, k0, k1))
        if masked:
            top = jnp.where(msk, s[:G], MASK_VALUE)
            s = top if row0 + G == 128 else jnp.concatenate([top, s[G:]], axis=0)
        sc.append(s)
        mj = jnp.maximum(s[:, :128], s[:, 128:]) if k1 - k0 == 256 else s
        run[cls] = _update(run[cls], mj, row0, jnp.maximum)
        toks[n] = _or_fold(run[cls]) & zero
    return steps, lead, sc, run


def _softmax_pv(steps, lead, sc, mx, vs, zero, extra):
    m = [jnp.max(mx[cls], axis=1, keepdims=True) for cls in range(NC)]
    wide = [[n for n, e in enumerate(steps) if e[0] == cls and e[2] - e[1] == 256] for cls in range(NC)]
    groups = []
    for cls in range(NC):
        w, out = list(wide[cls]), []
        while w:
            k = len(w) if len(w) <= PVG + 1 else PVG
            out.append(w[:k])
            w = w[k:]
        groups.append(out)
    perm = [n for gi in range(max(len(x) for x in groups)) for cls in reversed(range(NC))
            if gi < len(groups[cls]) for n in groups[cls][gi]]
    rest = [n for n in range(len(steps)) if n not in perm]
    if CMAJ:
        rest.sort(key=lambda n: (-steps[n][0], n))
    perm = perm + rest if PVLAST == 0 else rest + perm if PVLAST == 1 else list(range(len(steps)))
    steps = [steps[n] for n in perm]
    sc = [sc[n] for n in perm]
    due = _due(steps, SLAG)
    toks = {}
    o = [None] * NC
    run = [None] * NC
    macc = [[None] * 7 for _ in range(NC)]
    wait = [[] for _ in range(NC)]
    def leading(cls):
        w = G * (cls + 1)
        p = jnp.exp(lead[cls] - m[cls]).astype(BF16)
        o[cls] = _dot(p, _rows(vs, 0, w))
        e = jnp.concatenate([p.astype(F32), jnp.zeros((128, 128 - w), F32)], axis=1)
        run[cls] = _update(run[cls], e, 0, jnp.add)

    if CMAJ < 2:
        for cls in range(NC - 1):
            leading(cls)
    for n, (cls, k0, k1, row0, _) in enumerate(steps):
        if o[cls] is None and cls < NC - 1 and k1 - k0 < 256:
            leading(cls)
        p = jnp.exp(sc[n] - m[cls][row0:])
        t = _token(n, len(steps), toks.get(due[n]), extra)
        if t is not None:
            p = pltpu.bitcast(_inject(pltpu.bitcast(p, U32), t), F32)
        if k1 - k0 == 256 and len(steps) >= PVMIN:
            ops = _lhs_ops(p)
            lhs = [x.astype(BF16) for x in ops]
            rhs = [x.astype(BF16) for x in _rhs_ops(_rows(vs, k0, k1, True))]
            wait[cls].append((lhs, rhs))
            left = sum(1 for e in steps[n + 1:] if e[0] == cls and e[2] - e[1] == 256)
            if len(wait[cls]) >= PVG and left != 1 or left == 0:
                for j in PORDER:
                    v = [e[1][j] for e in wait[cls]]
                    t = None
                    for x, y in zip(wait[cls], v):
                        d = _dot(x[0][j], y)
                        t = d if t is None else t + d
                    macc[cls][j] = t if macc[cls][j] is None else macc[cls][j] + t
                wait[cls] = []
            ej = jnp.concatenate([lhs[4].astype(F32), lhs[1].astype(F32)] if PUN else [ops[4], ops[1]], axis=0)
        else:
            e = p
            p = p.astype(BF16)
            t = _dot(p, _rows(vs, k0, k1))
            e = p.astype(F32) if SUN else e
            ej = e[:, :128] + e[:, 128:] if k1 - k0 == 256 else e
            o[cls] = _update(o[cls], t, row0, jnp.add)
        run[cls] = _update(run[cls], ej, row0, jnp.add)
        toks[n] = _or_fold(run[cls]) & zero
    for cls in range(NC):
        if macc[cls][0] is not None:
            o[cls] = o[cls] + _combine(macc[cls])

    def natural(x):
        return jnp.concatenate([x[cls][G * t:G * (t + 1)] for t in range(NC) for cls in range(NC)], axis=0)
    return natural(o), natural(run)


def _normalize(o, lsum):
    r = _recip(jnp.sum(lsum, axis=1, keepdims=True))
    return o * r


def _kernel(aq_hbm, ak_hbm, av_hbm, sh_hbm, ah_hbm, dd_hbm, xt_hbm, c_hbm,
            wq_hbm, wk_hbm, wv_hbm, wot_hbm,
            out_hbm,
            sh_s, dd_s, coef_s, f_s, fh_s, zero_s, xt_s, x_s, wq_raw, aq_s, ak_s, av_s, ah_s, at_s,
            c_s, cs_s, ws_s, wk_raw, wv_raw, wot_s, wos_s, q_s, ctx_s, ot_s, o7_s, l7_s, stage_a, stage_b,
            sem_small, sem_x, sem_wq, sem_a, sem_c, sem_wk, sem_wv, sem_oa, sem_ob):
    wq32 = wq_hbm.bitcast(U32)
    wk32 = wk_hbm.bitcast(U32)
    wv32 = wv_hbm.bitcast(U32)

    def cp_small(i):
        return pltpu.make_async_copy((sh_hbm, dd_hbm)[i], (sh_s, dd_s)[i], sem_small.at[i])

    def cp_x(i):
        cols = pl.ds(XB[i], XB[i + 1] - XB[i])
        return pltpu.make_async_copy(xt_hbm.at[:, cols], xt_s.at[:, cols], sem_x.at[i])

    def cp_wq(p):
        return pltpu.make_async_copy(wq32.at[:, p, :], wq_raw.at[p], sem_wq.at[p])

    def cp_a(g, i):
        src = (ah_hbm, ak_hbm, av_hbm, aq_hbm)[i].bitcast(U32)
        dst = (ah_s, ak_s, av_s, aq_s)[i]
        n = UC // 2
        start = g * n if isinstance(g, int) else pl.multiple_of(g * n, 8)
        return pltpu.make_async_copy(src.at[pl.ds(start, n), :], dst.at[g], sem_a.at[g * 4 + i])

    def cp_c(i):
        n = 128
        start = i * n if isinstance(i, int) else pl.multiple_of(i * n, n)
        return pltpu.make_async_copy(c_hbm.bitcast(U32).at[pl.ds(start, n), :],
                                     c_s.at[pl.ds(start, n), :], sem_c.at[i])

    def cp_wo():
        return pltpu.make_async_copy(wot_hbm.bitcast(U32), wot_s, sem_c.at[8])

    def c_ops(strip, i):
        blk, part = strip >> 3, strip & 7

        def quad(r, k):
            x = [c_s[_ds(blk * 256 + (2 * r + e) * 64 + part * 8, 8, 8), k * 512:(k + 1) * 512] for e in range(2)]
            return pltpu.bitcast(jnp.concatenate(x, axis=0), BF16).astype(F32)
        x = (lambda: quad(0, 0) + quad(1, 1), lambda: quad(1, 0) + quad(1, 1), lambda: quad(0, 0),
             lambda: quad(1, 1), lambda: quad(0, 0) + quad(0, 1), lambda: quad(1, 0) - quad(0, 0),
             lambda: quad(0, 1) - quad(1, 1))[i]()
        tok = None
        for j, y in enumerate(_lhs_ops(x)):
            cs_s[_ds(((blk * 7 + i) * 7 + j) * 64 + part * 8, 8, 8), :] = _pack(y)
            if j % CT == 0:
                tok = _sample(y) if tok is None else tok | _sample(y)
        return tok & zero_s[...]

    def cp_wk(p):
        return pltpu.make_async_copy(wk32.at[:, p, :], wk_raw.at[p], sem_wk.at[p])

    def cp_wv(p):
        return pltpu.make_async_copy(wv32.at[:, p, :], wv_raw.at[p], sem_wv.at[p])

    def cp_out_a(i):
        n = NB3 * TO
        start = i * n if isinstance(i, int) else pl.multiple_of(i * n, n)
        return pltpu.make_async_copy(stage_a.at[pl.ds(start, n), :],
                                     out_hbm.at[pl.ds(start, n), pl.ds(0, MA)], sem_oa.at[i])

    def cp_out_b(i):
        start = i * TO if isinstance(i, int) else pl.multiple_of(i * TO, TO)
        return pltpu.make_async_copy(stage_b.at[pl.ds(start, TO), :],
                                     out_hbm.at[pl.ds(start, TO), pl.ds(MA, MP)], sem_ob.at[i])

    cp_x(0).start()
    cp_wq(0).start()
    for i in range(1, XCH):
        cp_x(i).start()
    cp_small(0).start()
    cp_small(1).start()

    tt = jax.lax.broadcasted_iota(jnp.int32, (128, 128), 0)
    rr = jax.lax.broadcasted_iota(jnp.int32, (128, 128), 1)
    ang = ((tt * (2 * rr + 1)) & 511).astype(F32) * (2.0 * math.pi / 512.0)
    fmat = jnp.concatenate([jnp.cos(ang), -jnp.sin(ang)], axis=1).astype(BF16)
    f_s[...] = pltpu.bitcast(fmat, U32)
    fh_s[...] = pltpu.bitcast((fmat.astype(F32) * (1.0 / 128.0)).astype(BF16), U32)
    zero_s[...] = jnp.zeros((8, 128), U32)

    def xpose_x(i):
        for blk in range(XB[i] // 256, XB[i + 1] // 256):
            tiles = []
            for t in (2 * blk, 2 * blk + 1):
                cols = slice(t * 128, (t + 1) * 128)
                parts = [xt_s[g * 128:(g + 1) * 128, cols].astype(F32).T for g in range(3)]
                last = jnp.concatenate([xt_s[MA:M, cols].astype(F32), jnp.zeros((MP - M, 128), F32)], axis=0)
                parts.append(last.T)
                tiles.append(jnp.concatenate(parts, axis=1))
            x = jnp.concatenate(tiles, axis=0)
            for j, op in enumerate(_lhs_ops(x)):
                x_s[(blk * 7 + j) * 64:(blk * 7 + j + 1) * 64, :] = _pack(op)

    def q_weights(p):
        raw = wq_raw[p]
        ops = []
        for w in (raw << 16, raw & jnp.uint32(HI_MASK)):
            w = pltpu.bitcast(w, F32) * Q_SCALE
            ops.append(_rhs_ops(jnp.concatenate([w, jnp.zeros((MP - M, D), F32)], axis=0)))
        return [jnp.concatenate([u, v], axis=1).astype(BF16) for u, v in zip(*ops)]

    def qstep(p, w, ms, n, tok=None):
        blk, j = n // 7, MORDER[n % 7]
        x = x_s[(blk * 7 + j) * 64:(blk * 7 + j + 1) * 64, :]
        if tok is not None:
            x = _inject(x, tok)
        ms[j] = _dot(pltpu.bitcast(x, BF16), w[j])
        if n % 7 == 6:
            for k in range(2):
                q = _combine([ms[e][:, k * 128:(k + 1) * 128] for e in range(7)])
                q_s[_ds((2 * p + k) * (S // 2) + blk * 128, 128, 128), :] = _pack(q)

    cp_x(0).wait()
    xpose_x(0)
    cp_c(0).start()
    cp_c(1).start()
    for g in range(NU):
        cp_wq(g + 1).start()
        for i in range(4):
            cp_a(g, i).start()
        if g < NU - 1:
            cp_c(g + 2).start()
    cp_wk(0).start()
    cp_wv(0).start()
    cp_wo().start()
    for p in range(1, H // 2):
        cp_wk(p).start()
        cp_wv(p).start()
    cp_wq(0).wait()
    w0 = q_weights(0)
    ms0 = {}
    for n in range(XB[1] // 256 * 7 - XLAG):
        qstep(0, w0, ms0, n)
    for i in range(1, XCH):
        cp_x(i).wait()
        if i == XCH - 1:
            cp_small(0).wait()
            cp_small(1).wait()
            cp_c(0).wait()
            cp_c(1).wait()
            prm = [sh_s[j:j + 1, :].astype(F32) for j in range(4)]
            prm.append(dd_s[...].astype(F32).reshape(1, M))
            for j in range(5):
                row = jnp.concatenate([prm[j], jnp.zeros((1, MP - M), F32)], axis=1)
                for t in range(MP // 128):
                    blk = jnp.broadcast_to(row[:, t * 128:(t + 1) * 128], (128, 128))
                    coef_s[j, t * 128:(t + 1) * 128, :] = blk.T
        for n in range(XB[i] // 256 * 7 - XLAG, XB[i] // 256 * 7):
            qstep(0, w0, ms0, n)
        xpose_x(i)
        for n in range(XB[i] // 256 * 7, XB[i + 1] // 256 * 7 - (XLAG if i < XCH - 1 else 0)):
            tok = None
            if i == XCH - 1:
                n0, n1 = XB[i] // 256 * 7, XB[i + 1] // 256 * 7
                for e in range(28):
                    if n0 + e * (n1 - n0) // 28 == n:
                        t = c_ops(e // 7, e % 7)
                        tok = t if tok is None else tok | t
            qstep(0, w0, ms0, n, tok)
    ot_s[...] = jnp.zeros((M, TO), F32)
    o7_s[...] = jnp.zeros((TQ, D), F32)
    l7_s[...] = jnp.ones((TQ, 128), F32)

    def phase1(g, carry):
        cp_wq(g + 1).wait()
        for i in range(4):
            cp_a(g, i).wait()

        @pl.when((g & 1) == 1)
        def _():
            cp_c(g + 1).wait()
            cp_c(g + 2).wait()

        w = q_weights(g + 1)
        fh = pltpu.bitcast(fh_s[...], BF16)
        fx = pltpu.bitcast(f_s[...], BF16)
        lane = jax.lax.broadcasted_iota(jnp.int32, (16, 128), 1)
        sgn = jnp.where((jax.lax.broadcasted_iota(jnp.int32, (8, 128), 1) & 1) == 0, 1.0, -1.0)
        zh, zx, kvs, ys = {}, {}, {}, {}

        def coef(k, j):
            return coef_s[j, pl.ds(pl.multiple_of(g * UC + k * 16, 16), 16), :]

        def hfwd(k):
            lhs = jnp.concatenate([ah_s[g, k * 8:(k + 1) * 8, c * 128:(c + 1) * 128]
                                   for c in range(NBLK)], axis=0)
            zh[k] = _dot(pltpu.bitcast(lhs, BF16), fh)

        def xfwd(k):
            kf = pltpu.bitcast(ak_s[g, k * 8:(k + 1) * 8, :], BF16).astype(F32)
            vf = pltpu.bitcast(av_s[g, k * 8:(k + 1) * 8, :], BF16).astype(F32)
            sh_k = [kf] + [pltpu.roll(kf, j, 1) for j in range(1, 4)]
            cf = [coef(k, j) for j in range(4)]
            kvf = []
            for c in range(NBLK):
                cols = slice(c * 128, (c + 1) * 128)
                t = sh_k[0][:, cols] * cf[0]
                for j in range(1, 4):
                    kj = sh_k[j][:, cols]
                    if c == 0:
                        kj = jnp.where(lane >= j, kj, 0.0)
                    t = t + kj * cf[j]
                kvf.append(t * vf[:, cols])
            kvs[k] = jnp.concatenate(kvf, axis=0).astype(BF16)
            zx[k] = _dot(kvs[k], fx)

        def inv(k, u):
            rows = [slice(c * 16 + u * 8, c * 16 + u * 8 + 8) for c in range(NBLK)]
            xr = [zx[k][r, :128] for r in rows]
            xi = [zx[k][r, 128:] for r in rows]
            h0r = [zh[k][r, :128] for r in rows]
            h0i = [zh[k][r, 128:] for r in rows]
            hr = [h0r[0]] + [h0r[j] - sgn * h0i[j - 1] for j in range(1, NBLK)]
            hi = [h0i[0]] + [h0i[j] + sgn * h0r[j - 1] for j in range(1, NBLK)]
            pr, pi = [], []
            for a0 in range(0, NBLK, 4):
                re = [None] * 4
                im = [None] * 4
                for c0 in range(0, a0 + 4, 4):
                    for da in range(4):
                        for c in range(c0, c0 + 4):
                            j = a0 + da - c
                            if j < 0:
                                continue
                            tr = xr[c] * hr[j] - xi[c] * hi[j]
                            ti = xr[c] * hi[j] + xi[c] * hr[j]
                            re[da] = tr if re[da] is None else re[da] + tr
                            im[da] = ti if im[da] is None else im[da] + ti
                pr += re
                pi += im
            p = jnp.concatenate([jnp.concatenate(pr, axis=0), jnp.concatenate(pi, axis=0)], axis=1)
            ys[k, u] = _dot_nt(p.astype(BF16), fx)
            if u == 1:
                kvr = kvs[k].astype(F32)
                qraw = aq_s[g, k * 8:(k + 1) * 8, :] | jnp.tile(zero_s[...], (1, NBLK))
                qf = pltpu.bitcast(qraw, BF16).astype(F32)
                dd = coef(k, 4)
                row0 = pl.multiple_of(g * UC + k * 16, 16)
                for a in range(NBLK):
                    cols = slice(a * 128, (a + 1) * 128)
                    y = jnp.concatenate([ys[k, 0][a * 8:(a + 1) * 8], ys[k, 1][a * 8:(a + 1) * 8]], axis=0)
                    y = y + kvr[a * 16:(a + 1) * 16] * dd
                    at_s[pl.ds(row0, 16), cols] = (qf[:, cols] * y).astype(BF16)

        ms = {}
        for n in range(S // 256 * 7):
            tok = None
            for step in P1PLAN.get(n, '').replace('_', ' ').split():
                if step[0] == 'H':
                    hfwd(int(step[1]))
                elif step[0] == 'X':
                    xfwd(int(step[1]))
                elif step[0] == 'I':
                    inv(int(step[1]), int(step[2]))
            if n in CPOS:
                e = CPOS.index(n)
                tok = c_ops(4 * (g + 1) + e // 7, e % 7)
            qstep(g + 1, w, ms, n, tok)
        return carry

    jax.lax.fori_loop(0, NU, phase1, 0)

    cp_wo().wait()
    for p in range(H // 2):
        cp_wk(p).wait()
        cp_wv(p).wait()

    def unpack_head(w, h):
        sh = (16 - ((h & 1) << 4)).astype(U32)
        return pltpu.bitcast((w << sh) & jnp.uint32(HI_MASK), F32)

    def first_operands(h):
        w = jnp.concatenate([wk_raw[h >> 1, :256, :128], wk_raw[h >> 1, 256:512, 128:]], axis=1)
        w = unpack_head(w, h)
        ws_s[...] = _pack(w)
        return w

    first_operands(jnp.int32(0))

    def product(ws, blks, i):
        ms = [None] * 7
        for j in MORDER:
            r = [((blk * 7 + i) * 7 + j) * 64 for blk in blks]
            x = jnp.concatenate([cs_s[e:e + 64, :] for e in r], axis=0)
            ms[j] = _dot(pltpu.bitcast(x, BF16), ws[i][j])
        return [_combine([m[k * 128:(k + 1) * 128] for m in ms]) for k in range(len(blks))]

    def finish_last(h):
        bits = _normalize(o7_s[...], l7_s[...])
        ctx_s[_ds(h * (S // 2) + (NB - 1) * TQ // 2, TQ // 2, TQ // 2), :] = _pack(bits)
        return bits

    def phase2(h, carry):
        b = unpack_head(jnp.concatenate([wk_raw[h >> 1], wv_raw[h >> 1]], axis=1), h)
        ws = [[y.astype(BF16) for y in _rhs_ops(x)] for x in _rhs_ops(b)]
        ws[1][1] = pltpu.bitcast(ws_s[:, :128], BF16)
        ws[1][4] = pltpu.bitcast(ws_s[:, 128:], BF16)
        mo = {}
        ks, vs, toks, sc = [], [], {}, {}
        zero = zero_s[...]

        def tokens(bits):
            n = TQ // NPART
            return [(_or_fold(bits[k * n:(k + 1) * n]) if CTOK == 0 else _or_fold(bits[k * n:(k + 1) * n, :128]) if CTOK == 1 else _sample(bits[k * n:(k + 1) * n])) & zero for k in range(NPART)]

        def wo_sums(part):
            r0 = (h & 1) * (M // 8) + part * 8
            quad = [[wot_s[(h >> 1) + k * (H // 2), _ds(r + r0, 8, 8), :] for k in range(2)] for r in (0, M // 4)]
            wo = jnp.concatenate([jnp.concatenate(x, axis=1) for x in quad], axis=0)
            wtok = None
            for j, x in enumerate(_lhs_sums(pltpu.bitcast(wo, BF16).astype(F32))):
                wos_s[_ds(((h >> 1) * 5 + j) * (M // 4) + r0, 8, 8), :] = _pack(x)
                if j in (0, 4):
                    wtok = _sample(x) if wtok is None else wtok | _sample(x)
            return wtok & zero

        nxt = jnp.minimum(h + 1, H - 1)
        toks[-1] = tokens(finish_last(jnp.maximum(h - 1, 0)))
        for step in P2ORDER.split():
            i = int(step[1:])
            if step[0] == 'M':
                blks = [int(e) for e in step[2:]]
                j = int(step[1])
                for blk, m in zip(blks, product(ws, blks, j)):
                    mo[blk, j] = m
                    e = [mo.get((blk, k)) for k in range(7)]
                    if j == 6:
                        ks.append(jnp.concatenate([(e[0] + e[3]) + (e[6] - e[4]), e[1] + e[3]], axis=0))
                    if j == 5:
                        vs.append(jnp.concatenate([e[2] + e[4], (e[0] - e[1]) + (e[2] + e[5])], axis=0))
            elif step[0] == 'Q':
                q = q_s[_ds(h * (S // 2) + i * TQ // 2, TQ // 2, TQ // 2), :]
                if i >= 1:
                    q = q | jnp.tile(zero, (TQ // 16, D // 128))
                extra = toks.get(TOKQ.get(i), [])
                for src in VTOK.get(i, []):
                    v = (vs if src[0] == 'V' else ks)[int(src[1])]
                    extra = _mix(extra, [(_or_fold if VFULL else _sample)(v[k * 64:(k + 1) * 64]) & zero for k in range(8)])
                if i == WOQ:
                    extra = _mix(extra, [wo_sums(part) for part in range(7)])
                if i == NB - 1:
                    w = first_operands(nxt)
                    extra = _mix(extra, [_sample(w[k * 64:(k + 1) * 64]) & zero for k in range(4)])
                sc[i] = _qk(i, q, ks, zero, extra)
            elif i == NB - 1:
                extra = [None] * PSKIP + toks[i - 1]
                o7_s[...], l7_s[...] = _softmax_pv(*sc[i], vs, zero, extra)
            else:
                bits = _normalize(*_softmax_pv(*sc[i], vs, zero, []))
                ctx_s[_ds(h * (S // 2) + i * TQ // 2, TQ // 2, TQ // 2), :] = _pack(bits)
                toks[i] = tokens(bits)
        return carry

    jax.lax.fori_loop(0, H, phase2, 0)

    def finish(i, ot):
        r0 = i * TO if isinstance(i, int) else pl.multiple_of(i * TO, TO)
        top = at_s[MA:M, pl.ds(r0, TO)].astype(F32)
        val = jnp.concatenate([top, ot], axis=0).T
        stage_b[pl.ds(r0, TO), :] = val.astype(BF16)
        return val

    def oproj(i, pending):
        hm = M // 4
        rows = pl.multiple_of(i * TO, TO)
        ctx = [jnp.concatenate([ctx_s[pl.ds(h * (S // 2) + rows + k * (TO // 2), TO // 2), :] for h in range(H)], axis=1)
               for k in range(2)]
        q1, q2 = [pltpu.bitcast(x, BF16).astype(F32) for x in ctx]
        kh = H * D // 2
        b11, b21, b12, b22 = q1[:, :kh], q1[:, kh:], q2[:, :kh], q2[:, kh:]
        rhs = [(b11 + b22).astype(BF16), pltpu.bitcast(ctx[0][:, :kh], BF16), (b12 - b22).astype(BF16),
               (b21 - b11).astype(BF16), pltpu.bitcast(ctx[1][:, kh:], BF16), (b11 + b12).astype(BF16),
               (b21 + b22).astype(BF16)]

        def sums(j):
            return jnp.concatenate([wos_s[(p * 5 + j) * hm:(p * 5 + j + 1) * hm, :] for p in range(H // 2)], axis=1)
        lhs = [lambda: sums(0), lambda: sums(1),
               lambda: jnp.concatenate([wot_s[h, :hm, :] for h in range(H // 2)], axis=1),
               lambda: jnp.concatenate([wot_s[h, hm:, :] for h in range(H // 2, H)], axis=1),
               lambda: sums(2), lambda: sums(3), lambda: sums(4)]
        ms = [None] * 7
        for n, j in enumerate(MORDER):
            x = lhs[j]()
            if n in pending:
                tok = None
                for y in pending[n]():
                    tok = _or_fold(y) if tok is None else tok | _or_fold(y)
                x = _inject(x, tok & zero_s[...])
            ms[j] = _dot_nt(pltpu.bitcast(x, BF16), rhs[j])
            if n == 4:
                first = jnp.concatenate([(ms[0] + ms[3]) + (ms[6] - ms[4]), ms[1] + ms[3]], axis=0)
                pending = dict(pending)
                val = finish(2 * i, first)
                cp_out_b(2 * i).start()
                pending[6] = lambda: [val]
        return jnp.concatenate([ms[2] + ms[4], (ms[0] - ms[1]) + (ms[2] + ms[5])], axis=0)

    def phase3(it, carry):
        prev = jnp.maximum(NB3 * it - 1, 0)
        val = finish(prev, ot_s[...])

        @pl.when(it > 0)
        def _():
            cp_out_b(prev).start()

        r0 = pl.multiple_of(it * (NB3 * TO), NB3 * TO)
        apart = []
        for g in range(MA // 128):
            blk = at_s[g * 128:(g + 1) * 128, pl.ds(r0, NB3 * TO)].astype(F32).T
            stage_a[pl.ds(r0, NB3 * TO), g * 128:(g + 1) * 128] = blk.astype(BF16)
            apart.append(blk)
        cp_out_a(it).start()

        pend = {2: lambda: [val], 3: lambda: apart}
        for k in range(NB3 // 2 - 1):
            u = NB3 // 2 * it + k
            val2 = finish(2 * u + 1, oproj(u, pend))
            cp_out_b(2 * u + 1).start()
            pend = {2: lambda: [val2]}
        ot_s[...] = oproj(NB3 // 2 * it + NB3 // 2 - 1, pend)
        finish_last(H - 1)
        return carry

    jax.lax.fori_loop(0, NO // NB3, phase3, 0)

    finish(NO - 1, ot_s[...])
    cp_out_b(NO - 1).start()
    for i in range(NO // NB3):
        cp_out_a(i).wait()
    for i in range(NO):
        cp_out_b(i).wait()


@jax.jit
def pallas_concat_heads__ssm_conv_h3__compressed_kv_cla__prompt_kernel(
    A_q: jax.Array,
    A_k: jax.Array,
    A_v: jax.Array,
    A_shift_k: jax.Array,
    A_ssm_k: jax.Array,
    A_ssm_D: jax.Array,
    B_x: jax.Array,
    B_c_kv: jax.Array,
    B_w_q: jax.Array,
    B_w_uk: jax.Array,
    B_w_uv: jax.Array,
    B_w_o: jax.Array,
):
    vm = pltpu.VMEM
    dma = pltpu.SemaphoreType.DMA
    scratch = [
        vm((4, M), BF16),
        vm((M,), BF16),
        vm((5, MP, 128), F32),
        vm((64, 256), U32),
        vm((64, 256), U32),
        vm((8, 128), U32),
        vm((M, S), BF16),
        vm((S // 256 * 7 * 64, MP // 2), U32),
        vm((H // 2, M, D), U32),
        vm((NU, UC // 2, S), U32),
        vm((NU, UC // 2, S), U32),
        vm((NU, UC // 2, S), U32),
        vm((NU, UC // 2, S), U32),
        vm((M, S), BF16),
        vm((S // 2, C), U32),
        vm((NB * 49 * 64, C // 4), U32),
        vm((128, 256), U32),
        vm((H // 2, C, D), U32),
        vm((H // 2, C, D), U32),
        vm((H, M // 2, D), U32),
        vm((H // 2 * 5 * M // 4, D), U32),
        vm((H * S // 2, D), U32),
        vm((H * S // 2, D), U32),
        vm((M, TO), F32),
        vm((TQ, D), F32),
        vm((TQ, 128), F32),
        vm((S, MA), BF16),
        vm((S, MP), BF16),
        dma((2,)), dma((XCH,)), dma((H // 2,)), dma((NU * 4,)), dma((9,)),
        dma((H // 2,)), dma((H // 2,)), dma((NO // NB3,)), dma((NO,)),
    ]
    out = pl.pallas_call(
        _kernel,
        in_specs=[pl.BlockSpec(memory_space=pl.ANY)] * 12,
        out_specs=pl.BlockSpec(memory_space=pl.ANY),
        out_shape=jax.ShapeDtypeStruct((S, 2 * M), BF16),
        scratch_shapes=scratch,
        compiler_params=pltpu.CompilerParams(
            vmem_limit_bytes=120 * 1024 * 1024,
            disable_semaphore_checks=True,
            disable_bounds_checks=True,
        ),
        name="h3_cla_fused",
    )(
        A_q[0].T, A_k[0].T, A_v[0].T, A_shift_k.T, A_ssm_k, A_ssm_D,
        B_x[0].T, B_c_kv[0], B_w_q, B_w_uk, B_w_uv, jnp.transpose(B_w_o, (0, 2, 1)),
    )
    return out[None]
```

```python
import math

import jax
import jax.numpy as jnp
import jax.experimental.pallas as pl
import jax.experimental.pallas.tpu as pltpu

S = 2048
M = 448
MP = 512
MA = 384
H = 16
D = 256
C = 1024
G = 32
NC = 128 // G
TQ = 128 * NC
NB = S // TQ
PC = 512
NU = 7
UC = M // NU
NBLK = S // 128
QCH = 128
XB = (0, 256, 768, 1280, 2048)
XCH = len(XB) - 1
TO = 128
NO = S // TO
NB3 = 4
TOKH = 6
MLAG = 800
SLAG = 1000
NPART = 32
P1ORDER = ("H0 H1 H2 H3 Q0 X0 Q1 X1 Q2 X2 Q3 X3 Q4 I00 Q5 I01 Q6 I10 Q7 I11 "
           "Q8 Q9 I20 Q10 I21 Q11 Q12 I30 Q13 I31 Q14 Q15")

P2ORDER = "M101 M401 M001 M301 M601 M201 M501 Q0 M12 M42 P0 Q1 M02 M32 M62 P1 M22 M52 Q2 M13 M43 M03 M33 M63 P2 Q3 M23 M53 P3"

WPARTS = 16
WOQ = (2, 3)
KVF32 = 1
CTOK = 0
PSKIP = 0
B11Q = 1
WPLAN = {'Q3': range(0, 8), 'P2': range(8, 12), 'P3': range(12, 16)}
TOKQ = {1: -1, 2: 0, 3: 1}
WT = 1
CT = 2
CPOS = list(list(range(16,19))+list(range(20,24))+[25,26,29,30,33,34,37,38,41,42,45,46,47]+list(range(49,56))+[1])
PVS = 1
PVG = 2
PVLAST = 0
PORDER = (2,4,5,0,3,1,6)
PUN = 1
PVMIN = 0
SUN = 1
VTOK = {0: ['V0', 'V1'], 2: ['V2']}
CMAJ = 1
VFULL = 1
PVG1 = 0
OPEND = (3, 16)
ODUE = 4
MORDER = (1, 4, 0, 3, 6, 2, 5)
XLAG = 3
P1PLAN = {0:'H0 H1 H2 H3',4:'X0',7:'X1',11:'X2',14:'X3',19:'I00',24:'I01',28:'I10',32:'I11',36:'I20',40:'I21',44:'I30',48:'I31'}
F32 = jnp.float32
BF16 = jnp.bfloat16
U32 = jnp.uint32
HI_MASK = 0xFFFF0000
Q_SCALE = D ** -0.5
MASK_VALUE = -1e9


def _dot(a, b):
    return jnp.dot(a, b, preferred_element_type=F32)


def _dot_nt(a, b):
    return jax.lax.dot_general(a, b, (((1,), (1,)), ((), ())), preferred_element_type=F32)


def _pack(x):
    return pltpu.bitcast(x.astype(BF16), U32)


def _ds(start, size, align):
    return pl.ds(start if isinstance(start, int) else pl.multiple_of(start, align), size)


def _sample(x):
    return _or_fold(jnp.concatenate([x[r + 8:r + 16] for r in range(0, x.shape[0], 16)], axis=0))


OSAMP = None


def _quads(x):
    r, c = x.shape[0] // 2, x.shape[1] // 2
    return x[:r, :c], x[:r, c:], x[r:, :c], x[r:, c:]


def _lhs_sums(a):
    a11, a12, a21, a22 = _quads(a)
    return a11 + a22, a21 + a22, a11 + a12, a21 - a11, a12 - a22


def _lhs_ops(a):
    a11, _, _, a22 = _quads(a)
    s1, s2, s5, s6, s7 = _lhs_sums(a)
    return s1, s2, a11, a22, s5, s6, s7


def _lhs_op(quad, i):
    return (lambda: quad(0, 0) + quad(1, 1), lambda: quad(1, 0) + quad(1, 1), lambda: quad(0, 0),
            lambda: quad(1, 1), lambda: quad(0, 0) + quad(0, 1), lambda: quad(1, 0) - quad(0, 0),
            lambda: quad(0, 1) - quad(1, 1))[i]()


def _rhs_op(quad, i):
    return (lambda: quad(0, 0) + quad(1, 1), lambda: quad(0, 0), lambda: quad(0, 1) - quad(1, 1),
            lambda: quad(1, 0) - quad(0, 0), lambda: quad(1, 1), lambda: quad(0, 0) + quad(0, 1),
            lambda: quad(1, 0) + quad(1, 1))[i]()


def _rhs_ops(b):
    b11, b12, b21, b22 = _quads(b)
    return b11 + b22, b11, b12 - b22, b21 - b11, b22, b11 + b12, b21 + b22


def _combine(m):
    m1, m2, m3, m4, m5, m6, m7 = m
    top = jnp.concatenate([(m1 + m4) + (m7 - m5), m3 + m5], axis=1)
    bot = jnp.concatenate([m2 + m4, (m1 - m2) + (m3 + m6)], axis=1)
    return jnp.concatenate([top, bot], axis=0)


def _or_fold(x):
    bits = pltpu.bitcast(x, U32)
    t = None
    for r in range(bits.shape[0] // 8):
        for c in range(bits.shape[1] // 128):
            e = bits[r * 8:(r + 1) * 8, c * 128:(c + 1) * 128]
            t = e if t is None else t | e
    return t


OSAMP = _sample


def _inject(x, tok):
    top = x[:8, :128] | tok
    if x.shape[1] > 128:
        top = jnp.concatenate([top, x[:8, 128:]], axis=1)
    return jnp.concatenate([top, x[8:]], axis=0)


def _recip(x):
    r = pl.reciprocal(x, approx=True)
    return r * (2.0 - x * r)


def _rows(chunks, r0, r1, raw=False):
    parts = []
    while r0 < r1:
        c = r0 // PC
        e = min(r1, (c + 1) * PC)
        parts.append(chunks[c][r0 - c * PC:e - c * PC] if KVF32 else chunks[c][(r0 - c * PC) // 2:(e - c * PC) // 2])
        r0 = e
    x = parts[0] if len(parts) == 1 else jnp.concatenate(parts, axis=0)
    return x if raw else x.astype(BF16)


def _steps(i):
    plans = []
    for cls in range(NC):
        last = cls == NC - 1
        base = 0 if last else G * (cls + 1)
        full = NC * i - 1 + last
        plan = []
        m = 0
        while m < full:
            w = 2 if m + 2 <= full else 1
            plan.append((cls, base + 128 * m, base + 128 * (m + w), 0, False))
            m += w
        for t in range(NC):
            if full + t >= 0:
                plan.append((cls, base + 128 * (full + t), base + 128 * (full + t + 1), G * t, True))
        plans.append(plan)
    n = max(len(p) for p in plans)
    return [plans[cls][j - n + len(plans[cls])] for j in range(n) for cls in reversed(range(NC))
            if j - n + len(plans[cls]) >= 0]


def _due(steps, lag):
    ends, out, t = [], [], 0
    for _, k0, k1, row0, _ in steps:
        src = [n for n, e in enumerate(ends) if e + lag <= t]
        out.append(src[-1] if src else None)
        t += (128 - row0) * (k1 - k0) // 256
        ends.append(t)
    return [None if x in out[:n] else x for n, x in enumerate(out)]


def _token(n, nsteps, own, extra):
    t = own
    for k, e in enumerate(extra):
        if e is not None and k * nsteps // len(extra) == n:
            t = e if t is None else t | e
    return t


def _mix(a, b):
    if not a or not b:
        return a or b
    keyed = [((k + 0.5) / len(a), x) for k, x in enumerate(a)] + [((k + 1.0) / len(b), x) for k, x in enumerate(b)]
    return [x for _, x in sorted(keyed, key=lambda e: e[0])]


def _update(acc, x, row0, op):
    if acc is None:
        return x
    if row0 == 0:
        return op(acc, x)
    return jnp.concatenate([acc[:row0], op(acc[row0:], x)], axis=0)


def _qk(i, qu, ks, zero, extra):
    r = jax.lax.broadcasted_iota(jnp.int32, (G, 128), 0)
    c = jax.lax.broadcasted_iota(jnp.int32, (G, 128), 1)
    msk = c <= r + (128 - G)
    h = G // 2
    qc = [jnp.concatenate([qu[64 * t + h * cls:64 * t + h * (cls + 1)] for t in range(NC)], axis=0)
          for cls in range(NC)]
    steps = _steps(i)
    due = _due(steps, MLAG)
    toks = {}
    run = [None] * NC
    sc, lead = [], []
    for cls in range(NC - 1):
        w = G * (cls + 1)
        s = _dot_nt(_rows(ks, 0, w), pltpu.bitcast(qc[cls], BF16)).T
        if i == 0:
            top = jnp.where((c <= r + G * cls)[:, :w], s[:G], MASK_VALUE)
            s = jnp.concatenate([top, s[G:]], axis=0)
        lead.append(s)
        run[cls] = jnp.concatenate([s, jnp.full((128, 128 - w), MASK_VALUE, F32)], axis=1)
    for n, (cls, k0, k1, row0, masked) in enumerate(steps):
        x = qc[cls][row0 // 2:]
        t = _token(n, len(steps), toks.get(due[n]), extra)
        s = _dot_nt(pltpu.bitcast(x if t is None else _inject(x, t), BF16), _rows(ks, k0, k1))
        if masked:
            top = jnp.where(msk, s[:G], MASK_VALUE)
            s = top if row0 + G == 128 else jnp.concatenate([top, s[G:]], axis=0)
        sc.append(s)
        mj = jnp.maximum(s[:, :128], s[:, 128:]) if k1 - k0 == 256 else s
        run[cls] = _update(run[cls], mj, row0, jnp.maximum)
        toks[n] = _or_fold(run[cls]) & zero
    return steps, lead, sc, run


def _softmax_pv(steps, lead, sc, mx, vs, zero, extra):
    m = [jnp.max(mx[cls], axis=1, keepdims=True) for cls in range(NC)]
    wide = [[n for n, e in enumerate(steps) if e[0] == cls and e[2] - e[1] == 256] for cls in range(NC)]
    groups = []
    for cls in range(NC):
        w, out = list(wide[cls]), []
        while w:
            k = len(w) if len(w) <= PVG + 1 else PVG
            if PVG1 and not out and len(w) > 2:
                k = 1
            out.append(w[:k])
            w = w[k:]
        groups.append(out)
    perm = [n for gi in range(max(len(x) for x in groups)) for cls in reversed(range(NC))
            if gi < len(groups[cls]) for n in groups[cls][gi]]
    ends = [g[-1] for x in groups for g in x]
    rest = [n for n in range(len(steps)) if n not in perm]
    if CMAJ:
        rest.sort(key=lambda n: (-steps[n][0], n))
    perm = perm + rest if PVLAST == 0 else rest + perm if PVLAST == 1 else list(range(len(steps)))
    steps = [steps[n] for n in perm]
    sc = [sc[n] for n in perm]
    due = _due(steps, SLAG)
    toks = {}
    o = [None] * NC
    run = [None] * NC
    macc = [[None] * 7 for _ in range(NC)]
    wait = [[] for _ in range(NC)]
    def leading(cls):
        w = G * (cls + 1)
        p = jnp.exp(lead[cls] - m[cls]).astype(BF16)
        o[cls] = _dot(p, _rows(vs, 0, w))
        e = jnp.concatenate([p.astype(F32), jnp.zeros((128, 128 - w), F32)], axis=1)
        run[cls] = _update(run[cls], e, 0, jnp.add)

    if CMAJ < 2:
        for cls in range(NC - 1):
            leading(cls)
    for n, (cls, k0, k1, row0, _) in enumerate(steps):
        if o[cls] is None and cls < NC - 1 and k1 - k0 < 256:
            leading(cls)
        p = jnp.exp(sc[n] - m[cls][row0:])
        t = _token(n, len(steps), toks.get(due[n]), extra)
        if t is not None:
            p = pltpu.bitcast(_inject(pltpu.bitcast(p, U32), t), F32)
        if k1 - k0 == 256 and len(steps) >= PVMIN:
            ops = _lhs_ops(p)
            lhs = [x.astype(BF16) for x in ops]
            rhs = [x.astype(BF16) for x in _rhs_ops(_rows(vs, k0, k1, True))]
            wait[cls].append((lhs, rhs))
            if perm[n] in ends:
                for j in PORDER:
                    v = [e[1][j] for e in wait[cls]]
                    t = None
                    for x, y in zip(wait[cls], v):
                        d = _dot(x[0][j], y)
                        t = d if t is None else t + d
                    macc[cls][j] = t if macc[cls][j] is None else macc[cls][j] + t
                wait[cls] = []
            ej = jnp.concatenate([lhs[4].astype(F32), lhs[1].astype(F32)] if PUN else [ops[4], ops[1]], axis=0)
        else:
            e = p
            p = p.astype(BF16)
            t = _dot(p, _rows(vs, k0, k1))
            e = p.astype(F32) if SUN else e
            ej = e[:, :128] + e[:, 128:] if k1 - k0 == 256 else e
            o[cls] = _update(o[cls], t, row0, jnp.add)
        run[cls] = _update(run[cls], ej, row0, jnp.add)
        toks[n] = _or_fold(run[cls]) & zero
    for cls in range(NC):
        if macc[cls][0] is not None:
            o[cls] = o[cls] + _combine(macc[cls])

    def natural(x):
        return jnp.concatenate([x[cls][G * t:G * (t + 1)] for t in range(NC) for cls in range(NC)], axis=0)
    return natural(o), natural(run)


def _normalize(o, lsum):
    r = _recip(jnp.sum(lsum, axis=1, keepdims=True))
    return o * r


def _kernel(aq_hbm, ak_hbm, av_hbm, sh_hbm, ah_hbm, dd_hbm, xt_hbm, c_hbm,
            wq_hbm, wk_hbm, wv_hbm, wot_hbm,
            out_hbm,
            sh_s, dd_s, coef_s, f_s, fh_s, zero_s, xt_s, x_s, wq_raw, aq_s, ak_s, av_s, ah_s, at_s,
            c_s, cs_s, ws_s, wk_raw, wv_raw, wot_s, wos_s, q_s, ctx_s, ot_s, o7_s, l7_s, stage_a, stage_b,
            sem_small, sem_x, sem_wq, sem_a, sem_c, sem_wk, sem_wv, sem_oa, sem_ob):
    wq32 = wq_hbm.bitcast(U32)
    wk32 = wk_hbm.bitcast(U32)
    wv32 = wv_hbm.bitcast(U32)

    def cp_small(i):
        return pltpu.make_async_copy((sh_hbm, dd_hbm)[i], (sh_s, dd_s)[i], sem_small.at[i])

    def cp_x(i):
        cols = pl.ds(XB[i], XB[i + 1] - XB[i])
        return pltpu.make_async_copy(xt_hbm.at[:, cols], xt_s.at[:, cols], sem_x.at[i])

    def cp_wq(p):
        return pltpu.make_async_copy(wq32.at[:, p, :], wq_raw.at[p], sem_wq.at[p])

    def cp_a(g, i):
        src = (ah_hbm, ak_hbm, av_hbm, aq_hbm)[i].bitcast(U32)
        dst = (ah_s, ak_s, av_s, aq_s)[i]
        n = UC // 2
        start = g * n if isinstance(g, int) else pl.multiple_of(g * n, 8)
        return pltpu.make_async_copy(src.at[pl.ds(start, n), :], dst.at[g], sem_a.at[g * 4 + i])

    def cp_c(i):
        n = 128
        start = i * n if isinstance(i, int) else pl.multiple_of(i * n, n)
        return pltpu.make_async_copy(c_hbm.bitcast(U32).at[pl.ds(start, n), :],
                                     c_s.at[pl.ds(start, n), :], sem_c.at[i])

    def cp_wo():
        return pltpu.make_async_copy(wot_hbm.bitcast(U32), wot_s, sem_c.at[8])

    def c_ops(strip, i):
        blk, part = strip >> 3, strip & 7

        def quad(r, k):
            x = [c_s[_ds(blk * 256 + (2 * r + e) * 64 + part * 8, 8, 8), k * 512:(k + 1) * 512] for e in range(2)]
            return pltpu.bitcast(jnp.concatenate(x, axis=0), BF16).astype(F32)
        x = (lambda: quad(0, 0) + quad(1, 1), lambda: quad(1, 0) + quad(1, 1), lambda: quad(0, 0),
             lambda: quad(1, 1), lambda: quad(0, 0) + quad(0, 1), lambda: quad(1, 0) - quad(0, 0),
             lambda: quad(0, 1) - quad(1, 1))[i]()
        tok = None
        for j, y in enumerate(_lhs_ops(x)):
            cs_s[_ds(((blk * 7 + i) * 7 + j) * 64 + part * 8, 8, 8), :] = _pack(y)
            if j % CT == 0:
                tok = _sample(y) if tok is None else tok | _sample(y)
        return tok & zero_s[...]

    def cp_wk(p):
        return pltpu.make_async_copy(wk32.at[:, p, :], wk_raw.at[p], sem_wk.at[p])

    def cp_wv(p):
        return pltpu.make_async_copy(wv32.at[:, p, :], wv_raw.at[p], sem_wv.at[p])

    def cp_out_a(i):
        n = NB3 * TO
        start = i * n if isinstance(i, int) else pl.multiple_of(i * n, n)
        return pltpu.make_async_copy(stage_a.at[pl.ds(start, n), :],
                                     out_hbm.at[pl.ds(start, n), pl.ds(0, MA)], sem_oa.at[i])

    def cp_out_b(i):
        start = i * TO if isinstance(i, int) else pl.multiple_of(i * TO, TO)
        return pltpu.make_async_copy(stage_b.at[pl.ds(start, TO), :],
                                     out_hbm.at[pl.ds(start, TO), pl.ds(MA, MP)], sem_ob.at[i])

    cp_x(0).start()
    cp_wq(0).start()
    for i in range(1, XCH):
        cp_x(i).start()
    cp_small(0).start()
    cp_small(1).start()

    tt = jax.lax.broadcasted_iota(jnp.int32, (128, 128), 0)
    rr = jax.lax.broadcasted_iota(jnp.int32, (128, 128), 1)
    ang = ((tt * (2 * rr + 1)) & 511).astype(F32) * (2.0 * math.pi / 512.0)
    fmat = jnp.concatenate([jnp.cos(ang), -jnp.sin(ang)], axis=1).astype(BF16)
    f_s[...] = pltpu.bitcast(fmat, U32)
    fh_s[...] = pltpu.bitcast((fmat.astype(F32) * (1.0 / 128.0)).astype(BF16), U32)
    zero_s[...] = jnp.zeros((8, 128), U32)

    def xpose_x(i):
        for blk in range(XB[i] // 256, XB[i + 1] // 256):
            tiles = []
            for t in (2 * blk, 2 * blk + 1):
                cols = slice(t * 128, (t + 1) * 128)
                parts = [xt_s[g * 128:(g + 1) * 128, cols].astype(F32).T for g in range(3)]
                last = jnp.concatenate([xt_s[MA:M, cols].astype(F32), jnp.zeros((MP - M, 128), F32)], axis=0)
                parts.append(last.T)
                tiles.append(jnp.concatenate(parts, axis=1))
            x = jnp.concatenate(tiles, axis=0)
            for j, op in enumerate(_lhs_ops(x)):
                x_s[(blk * 7 + j) * 64:(blk * 7 + j + 1) * 64, :] = _pack(op)

    def q_weights(p):
        raw = wq_raw[p]
        ops = []
        for w in (raw << 16, raw & jnp.uint32(HI_MASK)):
            w = pltpu.bitcast(w, F32) * Q_SCALE
            ops.append(_rhs_ops(jnp.concatenate([w, jnp.zeros((MP - M, D), F32)], axis=0)))
        return [jnp.concatenate([u, v], axis=1).astype(BF16) for u, v in zip(*ops)]

    def qstep(p, w, ms, n, tok=None):
        blk, j = n // 7, MORDER[n % 7]
        x = x_s[(blk * 7 + j) * 64:(blk * 7 + j + 1) * 64, :]
        if tok is not None:
            x = _inject(x, tok)
        ms[j] = _dot(pltpu.bitcast(x, BF16), w[j])
        if n % 7 == 6:
            for k in range(2):
                q = _combine([ms[e][:, k * 128:(k + 1) * 128] for e in range(7)])
                q_s[_ds((2 * p + k) * (S // 2) + blk * 128, 128, 128), :] = _pack(q)

    cp_x(0).wait()
    xpose_x(0)
    cp_c(0).start()
    cp_c(1).start()
    for g in range(NU):
        cp_wq(g + 1).start()
        for i in range(4):
            cp_a(g, i).start()
        if g < NU - 1:
            cp_c(g + 2).start()
    cp_wk(0).start()
    cp_wv(0).start()
    cp_wo().start()
    for p in range(1, H // 2):
        cp_wk(p).start()
        cp_wv(p).start()
    cp_wq(0).wait()
    w0 = q_weights(0)
    ms0 = {}
    for n in range(XB[1] // 256 * 7 - XLAG):
        qstep(0, w0, ms0, n)
    for i in range(1, XCH):
        cp_x(i).wait()
        if i == XCH - 1:
            cp_small(0).wait()
            cp_small(1).wait()
            cp_c(0).wait()
            cp_c(1).wait()
            prm = [sh_s[j:j + 1, :].astype(F32) for j in range(4)]
            prm.append(dd_s[...].astype(F32).reshape(1, M))
            for j in range(5):
                row = jnp.concatenate([prm[j], jnp.zeros((1, MP - M), F32)], axis=1)
                for t in range(MP // 128):
                    blk = jnp.broadcast_to(row[:, t * 128:(t + 1) * 128], (128, 128))
                    coef_s[j, t * 128:(t + 1) * 128, :] = blk.T
        for n in range(XB[i] // 256 * 7 - XLAG, XB[i] // 256 * 7):
            qstep(0, w0, ms0, n)
        xpose_x(i)
        for n in range(XB[i] // 256 * 7, XB[i + 1] // 256 * 7 - (XLAG if i < XCH - 1 else 0)):
            tok = None
            if i == XCH - 1:
                n0, n1 = XB[i] // 256 * 7, XB[i + 1] // 256 * 7
                for e in range(28):
                    if n0 + e * (n1 - n0) // 28 == n:
                        t = c_ops(e // 7, e % 7)
                        tok = t if tok is None else tok | t
            qstep(0, w0, ms0, n, tok)
    ot_s[...] = jnp.zeros((M, TO), F32)
    o7_s[...] = jnp.zeros((TQ, D), F32)
    l7_s[...] = jnp.ones((TQ, 128), F32)

    def phase1(g, carry):
        cp_wq(g + 1).wait()
        for i in range(4):
            cp_a(g, i).wait()

        @pl.when((g & 1) == 1)
        def _():
            cp_c(g + 1).wait()
            cp_c(g + 2).wait()

        w = q_weights(g + 1)
        fh = pltpu.bitcast(fh_s[...], BF16)
        fx = pltpu.bitcast(f_s[...], BF16)
        lane = jax.lax.broadcasted_iota(jnp.int32, (16, 128), 1)
        sgn = jnp.where((jax.lax.broadcasted_iota(jnp.int32, (8, 128), 1) & 1) == 0, 1.0, -1.0)
        zh, zx, kvs, ys = {}, {}, {}, {}

        def coef(k, j):
            return coef_s[j, pl.ds(pl.multiple_of(g * UC + k * 16, 16), 16), :]

        def hfwd(k):
            lhs = jnp.concatenate([ah_s[g, k * 8:(k + 1) * 8, c * 128:(c + 1) * 128]
                                   for c in range(NBLK)], axis=0)
            zh[k] = _dot(pltpu.bitcast(lhs, BF16), fh)

        def xfwd(k):
            kf = pltpu.bitcast(ak_s[g, k * 8:(k + 1) * 8, :], BF16).astype(F32)
            vf = pltpu.bitcast(av_s[g, k * 8:(k + 1) * 8, :], BF16).astype(F32)
            sh_k = [kf] + [pltpu.roll(kf, j, 1) for j in range(1, 4)]
            cf = [coef(k, j) for j in range(4)]
            kvf = []
            for c in range(NBLK):
                cols = slice(c * 128, (c + 1) * 128)
                t = sh_k[0][:, cols] * cf[0]
                for j in range(1, 4):
                    kj = sh_k[j][:, cols]
                    if c == 0:
                        kj = jnp.where(lane >= j, kj, 0.0)
                    t = t + kj * cf[j]
                kvf.append(t * vf[:, cols])
            kvs[k] = jnp.concatenate(kvf, axis=0).astype(BF16)
            zx[k] = _dot(kvs[k], fx)

        def inv(k, u):
            rows = [slice(c * 16 + u * 8, c * 16 + u * 8 + 8) for c in range(NBLK)]
            xr = [zx[k][r, :128] for r in rows]
            xi = [zx[k][r, 128:] for r in rows]
            h0r = [zh[k][r, :128] for r in rows]
            h0i = [zh[k][r, 128:] for r in rows]
            hr = [h0r[0]] + [h0r[j] - sgn * h0i[j - 1] for j in range(1, NBLK)]
            hi = [h0i[0]] + [h0i[j] + sgn * h0r[j - 1] for j in range(1, NBLK)]
            pr, pi = [], []
            for a0 in range(0, NBLK, 4):
                re = [None] * 4
                im = [None] * 4
                for c0 in range(0, a0 + 4, 4):
                    for da in range(4):
                        for c in range(c0, c0 + 4):
                            j = a0 + da - c
                            if j < 0:
                                continue
                            tr = xr[c] * hr[j] - xi[c] * hi[j]
                            ti = xr[c] * hi[j] + xi[c] * hr[j]
                            re[da] = tr if re[da] is None else re[da] + tr
                            im[da] = ti if im[da] is None else im[da] + ti
                pr += re
                pi += im
            p = jnp.concatenate([jnp.concatenate(pr, axis=0), jnp.concatenate(pi, axis=0)], axis=1)
            ys[k, u] = _dot_nt(p.astype(BF16), fx)
            if u == 1:
                kvr = kvs[k].astype(F32)
                qraw = aq_s[g, k * 8:(k + 1) * 8, :] | jnp.tile(zero_s[...], (1, NBLK))
                qf = pltpu.bitcast(qraw, BF16).astype(F32)
                dd = coef(k, 4)
                row0 = pl.multiple_of(g * UC + k * 16, 16)
                for a in range(NBLK):
                    cols = slice(a * 128, (a + 1) * 128)
                    y = jnp.concatenate([ys[k, 0][a * 8:(a + 1) * 8], ys[k, 1][a * 8:(a + 1) * 8]], axis=0)
                    y = y + kvr[a * 16:(a + 1) * 16] * dd
                    at_s[pl.ds(row0, 16), cols] = (qf[:, cols] * y).astype(BF16)

        ms = {}
        for n in range(S // 256 * 7):
            tok = None
            for step in P1PLAN.get(n, '').replace('_', ' ').split():
                if step[0] == 'H':
                    hfwd(int(step[1]))
                elif step[0] == 'X':
                    xfwd(int(step[1]))
                elif step[0] == 'I':
                    inv(int(step[1]), int(step[2]))
            if n in CPOS:
                e = CPOS.index(n)
                tok = c_ops(4 * (g + 1) + e // 7, e % 7)
            qstep(g + 1, w, ms, n, tok)
        return carry

    jax.lax.fori_loop(0, NU, phase1, 0)

    cp_wo().wait()
    for p in range(H // 2):
        cp_wk(p).wait()
        cp_wv(p).wait()

    def unpack_head(w, h):
        sh = (16 - ((h & 1) << 4)).astype(U32)
        return pltpu.bitcast((w << sh) & jnp.uint32(HI_MASK), F32)

    def first_operands(h):
        w = jnp.concatenate([wk_raw[h >> 1, :256, :128], wk_raw[h >> 1, 256:512, 128:]], axis=1)
        w = unpack_head(w, h)
        ws_s[...] = _pack(w)
        return w

    first_operands(jnp.int32(0))

    def product(ws, blks, i):
        ms = [None] * 7
        for j in MORDER:
            r = [((blk * 7 + i) * 7 + j) * 64 for blk in blks]
            x = jnp.concatenate([cs_s[e:e + 64, :] for e in r], axis=0)
            ms[j] = _dot(pltpu.bitcast(x, BF16), ws[i][j])
        return [_combine([m[k * 128:(k + 1) * 128] for m in ms]) for k in range(len(blks))]

    def finish_last(h):
        bits = _normalize(o7_s[...], l7_s[...])
        ctx_s[_ds(h * (S // 2) + (NB - 1) * TQ // 2, TQ // 2, TQ // 2), :] = _pack(bits)
        return bits

    def phase2(h, carry):
        b = unpack_head(jnp.concatenate([wk_raw[h >> 1], wv_raw[h >> 1]], axis=1), h)
        ws = [[y.astype(BF16) for y in _rhs_ops(x)] for x in _rhs_ops(b)]
        ws[1][1] = pltpu.bitcast(ws_s[:, :128], BF16)
        ws[1][4] = pltpu.bitcast(ws_s[:, 128:], BF16)
        mo = {}
        ks, vs, toks, sc = [], [], {}, {}
        zero = zero_s[...]

        def tokens(bits):
            n = TQ // NPART
            return [(_or_fold(bits[k * n:(k + 1) * n]) if CTOK == 0 else _or_fold(bits[k * n:(k + 1) * n, :128]) if CTOK == 1 else _sample(bits[k * n:(k + 1) * n])) & zero for k in range(NPART)]

        def wo_ops(k, i):
            unit = jnp.minimum(2 * h + k, 27)
            j = jax.lax.div(unit, 7)
            r0 = (unit - 7 * j) * 8

            def quad(r, c):
                x = [jnp.concatenate([wot_s[j + 4 * (2 * c + f), _ds((2 * r + e) * 56 + r0, 8, 8), :]
                                      for f in range(2)], axis=1) for e in range(2)]
                return pltpu.bitcast(jnp.concatenate(x, axis=0), BF16).astype(F32)
            tok = None
            for n, y in enumerate(_lhs_ops(_lhs_op(quad, i))):
                wos_s[_ds(((j * 7 + i) * 7 + n) * 56 + r0, 8, 8), :] = _pack(y)
                if n % 2 == 0:
                    tok = _sample(y) if tok is None else tok | _sample(y)
            return tok & zero

        nxt = jnp.minimum(h + 1, H - 1)
        toks[-1] = tokens(finish_last(jnp.maximum(h - 1, 0)))
        for step in P2ORDER.split():
            i = int(step[1:])
            if step[0] == 'M':
                blks = [int(e) for e in step[2:]]
                j = int(step[1])
                for blk, m in zip(blks, product(ws, blks, j)):
                    mo[blk, j] = m
                    e = [mo.get((blk, k)) for k in range(7)]
                    if j == 6:
                        ks.append(jnp.concatenate([(e[0] + e[3]) + (e[6] - e[4]), e[1] + e[3]], axis=0))
                    if j == 5:
                        vs.append(jnp.concatenate([e[2] + e[4], (e[0] - e[1]) + (e[2] + e[5])], axis=0))
            elif step[0] == 'Q':
                q = q_s[_ds(h * (S // 2) + i * TQ // 2, TQ // 2, TQ // 2), :]
                if i >= 1:
                    q = q | jnp.tile(zero, (TQ // 16, D // 128))
                extra = toks.get(TOKQ.get(i), [])
                for src in VTOK.get(i, []):
                    v = (vs if src[0] == 'V' else ks)[int(src[1])]
                    extra = _mix(extra, [(_or_fold if VFULL else _sample)(v[k * 64:(k + 1) * 64]) & zero for k in range(8)])
                if i in WOQ:
                    extra = _mix(extra, [wo_ops(WOQ.index(i), e) for e in range(7)])
                if i == NB - 1:
                    w = first_operands(nxt)
                    extra = _mix(extra, [_sample(w[k * 64:(k + 1) * 64]) & zero for k in range(4)])
                sc[i] = _qk(i, q, ks, zero, extra)
            elif i == NB - 1:
                extra = [None] * PSKIP + toks[i - 1]
                o7_s[...], l7_s[...] = _softmax_pv(*sc[i], vs, zero, extra)
            else:
                bits = _normalize(*_softmax_pv(*sc[i], vs, zero, []))
                ctx_s[_ds(h * (S // 2) + i * TQ // 2, TQ // 2, TQ // 2), :] = _pack(bits)
                toks[i] = tokens(bits)
        return carry

    jax.lax.fori_loop(0, H, phase2, 0)

    def finish(i, ot):
        r0 = i * TO if isinstance(i, int) else pl.multiple_of(i * TO, TO)
        top = at_s[MA:M, pl.ds(r0, TO)].astype(F32)
        val = jnp.concatenate([top, ot], axis=0).T
        stage_b[pl.ds(r0, TO), :] = val.astype(BF16)
        return val

    def phase3(it, carry):
        prev = jnp.maximum(NB3 * it - 1, 0)
        val = finish(prev, ot_s[...])
        pend = {OPEND[0] + k: [val[:, k * 128:(k + 1) * 128]] for k in range(4)}

        @pl.when(it > 0)
        def _():
            cp_out_b(prev).start()

        r0 = pl.multiple_of(it * (NB3 * TO), NB3 * TO)
        apart = []
        for g in range(MA // 128):
            blk = at_s[g * 128:(g + 1) * 128, pl.ds(r0, NB3 * TO)].astype(F32).T
            stage_a[pl.ds(r0, NB3 * TO), g * 128:(g + 1) * 128] = blk.astype(BF16)
            apart.append(blk)
        cp_out_a(it).start()
        for k, y in enumerate(apart):
            for e in range(4):
                pend[OPEND[1] + 4 * k + e] = [y[e * 128:(e + 1) * 128]]

        def ctx(kq, t):
            rows = pl.multiple_of((NB3 * it + t) * (TO // 2), TO // 2)
            x = [ctx_s[pl.ds(h * (S // 2) + rows, TO // 2), :] for h in range(4 * kq, 4 * kq + 4)]
            return pltpu.bitcast(jnp.concatenate(x, axis=1), BF16)

        def half(m, k):
            if k == 0:
                return jnp.concatenate([(m[0] + m[3]) + (m[6] - m[4]), m[1] + m[3]], axis=0)
            return jnp.concatenate([m[2] + m[4], (m[0] - m[1]) + (m[2] + m[5])], axis=0)

        mo = [[None] * 7, [None] * 7]
        step = 0
        for i in MORDER:
            sub = {(a, b): _rhs_op(lambda r, c: ctx(2 * r + a, 2 * c + b).astype(F32), i)
                   for a in range(2) for b in range(2)}
            mi = [None] * 7
            for j in MORDER:
                w = _rhs_op(lambda r, c: sub[r, c], j).astype(BF16)
                x = jnp.concatenate([wos_s[((e * 7 + i) * 7 + j) * 56:((e * 7 + i) * 7 + j + 1) * 56, :]
                                     for e in range(4)], axis=1)
                if step in pend:
                    tok = None
                    for y in pend[step]:
                        tok = OSAMP(y) if tok is None else tok | OSAMP(y)
                    x = _inject(x, tok & zero_s[...])
                mi[j] = _dot_nt(pltpu.bitcast(x, BF16), w)
                step += 1
                for k, last in ((0, 6), (1, 5)):
                    if j == last:
                        mo[k][i] = half(mi, k)
                        for n, done in ((0, 6), (1, 5)):
                            if i == done and 2 * n + k < NB3 - 1:
                                val = finish(NB3 * it + 2 * n + k, half(mo[k], n))
                                cp_out_b(NB3 * it + 2 * n + k).start()
                                for e in range(4):
                                    if step + ODUE + e <= 48:
                                        due = step + ODUE + e
                                        pend[due] = pend.get(due, []) + [val[:, e * 128:(e + 1) * 128]]
        ot_s[...] = half(mo[1], 1)
        finish_last(H - 1)
        return carry

    jax.lax.fori_loop(0, NO // NB3, phase3, 0)

    finish(NO - 1, ot_s[...])
    cp_out_b(NO - 1).start()
    for i in range(NO // NB3):
        cp_out_a(i).wait()
    for i in range(NO):
        cp_out_b(i).wait()


@jax.jit
def pallas_concat_heads__ssm_conv_h3__compressed_kv_cla__prompt_kernel(
    A_q: jax.Array,
    A_k: jax.Array,
    A_v: jax.Array,
    A_shift_k: jax.Array,
    A_ssm_k: jax.Array,
    A_ssm_D: jax.Array,
    B_x: jax.Array,
    B_c_kv: jax.Array,
    B_w_q: jax.Array,
    B_w_uk: jax.Array,
    B_w_uv: jax.Array,
    B_w_o: jax.Array,
):
    vm = pltpu.VMEM
    dma = pltpu.SemaphoreType.DMA
    scratch = [
        vm((4, M), BF16),
        vm((M,), BF16),
        vm((5, MP, 128), F32),
        vm((64, 256), U32),
        vm((64, 256), U32),
        vm((8, 128), U32),
        vm((M, S), BF16),
        vm((S // 256 * 7 * 64, MP // 2), U32),
        vm((H // 2, M, D), U32),
        vm((NU, UC // 2, S), U32),
        vm((NU, UC // 2, S), U32),
        vm((NU, UC // 2, S), U32),
        vm((NU, UC // 2, S), U32),
        vm((M, S), BF16),
        vm((S // 2, C), U32),
        vm((NB * 49 * 64, C // 4), U32),
        vm((128, 256), U32),
        vm((H // 2, C, D), U32),
        vm((H // 2, C, D), U32),
        vm((H, M // 2, D), U32),
        vm((4 * 49 * 56, D), U32),
        vm((H * S // 2, D), U32),
        vm((H * S // 2, D), U32),
        vm((M, TO), F32),
        vm((TQ, D), F32),
        vm((TQ, 128), F32),
        vm((S, MA), BF16),
        vm((S, MP), BF16),
        dma((2,)), dma((XCH,)), dma((H // 2,)), dma((NU * 4,)), dma((9,)),
        dma((H // 2,)), dma((H // 2,)), dma((NO // NB3,)), dma((NO,)),
    ]
    out = pl.pallas_call(
        _kernel,
        in_specs=[pl.BlockSpec(memory_space=pl.ANY)] * 12,
        out_specs=pl.BlockSpec(memory_space=pl.ANY),
        out_shape=jax.ShapeDtypeStruct((S, 2 * M), BF16),
        scratch_shapes=scratch,
        compiler_params=pltpu.CompilerParams(
            vmem_limit_bytes=120 * 1024 * 1024,
            disable_semaphore_checks=True,
            disable_bounds_checks=True,
        ),
        name="h3_cla_fused",
    )(
        A_q[0].T, A_k[0].T, A_v[0].T, A_shift_k.T, A_ssm_k, A_ssm_D,
        B_x[0].T, B_c_kv[0], B_w_q, B_w_uk, B_w_uv, jnp.transpose(B_w_o, (0, 2, 1)),
    )
    return out[None]
```

```python
import math

import jax
import jax.numpy as jnp
import jax.experimental.pallas as pl
import jax.experimental.pallas.tpu as pltpu

S = 2048
M = 448
MP = 512
MA = 384
H = 16
D = 256
C = 1024
G = 32
NC = 128 // G
TQ = 128 * NC
NB = S // TQ
NU = 7
UC = M // NU
NBLK = S // 128
XB = (0, 256, 768, 1280, 2048)
XCH = len(XB) - 1
XLAG = 3
TO = 128
NO = S // TO
NB3 = 4
MLAG = 800
SLAG = 1000
NPART = 32
MORDER = (1, 4, 0, 3, 6, 2, 5)
PORDER = (2, 4, 5, 0, 3, 1, 6)
P1PLAN = {0: 'H0 H1 H2 H3', 4: 'X0', 7: 'X1', 11: 'X2', 14: 'X3', 19: 'I00', 24: 'I01', 28: 'I10', 32: 'I11', 36: 'I20', 40: 'I21', 44: 'I30', 48: 'I31'}
CPOS = [16, 17, 18, 20, 21, 22, 23, 25, 26, 29, 30, 33, 34, 37, 38, 41, 42, 45, 46, 47, 49, 50, 51, 52, 53, 54, 55, 1]
P2ORDER = "M101 M401 M001 M301 M601 M201 M501 Q0 M12 M42 P0 Q1 M02 M32 M62 P1 M22 M52 Q2 M13 M43 M03 M33 M63 P2 Q3 M23 M53 P3"

F32 = jnp.float32
BF16 = jnp.bfloat16
U32 = jnp.uint32
HI_MASK = 0xFFFF0000
Q_SCALE = D ** -0.5 * math.log2(math.e)
MASK_VALUE = -1e9


def _dot(a, b):
    return jnp.dot(a, b, preferred_element_type=F32)


def _dot_nt(a, b):
    return jax.lax.dot_general(a, b, (((1,), (1,)), ((), ())), preferred_element_type=F32)


def _pack(x):
    return pltpu.bitcast(x.astype(BF16), U32)


def _ds(start, size, align):
    return pl.ds(start if isinstance(start, int) else pl.multiple_of(start, align), size)


def _sample(x):
    return _or_fold(jnp.concatenate([x[r + 8:r + 16] for r in range(0, x.shape[0], 16)], axis=0))


def _quads(x):
    r, c = x.shape[0] // 2, x.shape[1] // 2
    return x[:r, :c], x[:r, c:], x[r:, :c], x[r:, c:]


def _lhs_op(quad, i):
    return (lambda: quad(0, 0) + quad(1, 1), lambda: quad(1, 0) + quad(1, 1), lambda: quad(0, 0),
            lambda: quad(1, 1), lambda: quad(0, 0) + quad(0, 1), lambda: quad(1, 0) - quad(0, 0),
            lambda: quad(0, 1) - quad(1, 1))[i]()


def _rhs_op(quad, i):
    return (lambda: quad(0, 0) + quad(1, 1), lambda: quad(0, 0), lambda: quad(0, 1) - quad(1, 1),
            lambda: quad(1, 0) - quad(0, 0), lambda: quad(1, 1), lambda: quad(0, 0) + quad(0, 1),
            lambda: quad(1, 0) + quad(1, 1))[i]()


def _lhs_ops(a):
    q = _quads(a)
    return [_lhs_op(lambda r, c: q[2 * r + c], i) for i in range(7)]


def _rhs_ops(b):
    q = _quads(b)
    return [_rhs_op(lambda r, c: q[2 * r + c], i) for i in range(7)]


def _half(m, k):
    if k == 0:
        return jnp.concatenate([(m[0] + m[3]) + (m[6] - m[4]), m[1] + m[3]], axis=0)
    return jnp.concatenate([m[2] + m[4], (m[0] - m[1]) + (m[2] + m[5])], axis=0)


def _combine(m):
    return jnp.concatenate([_half(m, 0), _half(m, 1)], axis=1)


def _or_fold(x):
    bits = pltpu.bitcast(x, U32)
    t = None
    for r in range(bits.shape[0] // 8):
        for c in range(bits.shape[1] // 128):
            e = bits[r * 8:(r + 1) * 8, c * 128:(c + 1) * 128]
            t = e if t is None else t | e
    return t


def _inject(x, tok):
    top = x[:8, :128] | tok
    if x.shape[1] > 128:
        top = jnp.concatenate([top, x[:8, 128:]], axis=1)
    return jnp.concatenate([top, x[8:]], axis=0)


def _recip(x):
    r = pl.reciprocal(x, approx=True)
    return r * (2.0 - x * r)


def _rows(chunks, r0, r1):
    parts = []
    while r0 < r1:
        c = r0 // TQ
        e = min(r1, (c + 1) * TQ)
        parts.append(chunks[c][r0 - c * TQ:e - c * TQ])
        r0 = e
    return parts[0] if len(parts) == 1 else jnp.concatenate(parts, axis=0)


def _steps(i):
    plans = []
    for cls in range(NC):
        last = cls == NC - 1
        base = 0 if last else G * (cls + 1)
        full = NC * i - 1 + last
        plan = []
        m = 0
        while m < full:
            w = 2 if m + 2 <= full else 1
            plan.append((cls, base + 128 * m, base + 128 * (m + w), 0, False))
            m += w
        for t in range(NC):
            if full + t >= 0:
                plan.append((cls, base + 128 * (full + t), base + 128 * (full + t + 1), G * t, True))
        plans.append(plan)
    n = max(len(p) for p in plans)
    return [plans[cls][j - n + len(plans[cls])] for j in range(n) for cls in reversed(range(NC))
            if j - n + len(plans[cls]) >= 0]


def _due(steps, lag):
    ends, out, t = [], [], 0
    for _, k0, k1, row0, _ in steps:
        src = [n for n, e in enumerate(ends) if e + lag <= t]
        out.append(src[-1] if src else None)
        t += (128 - row0) * (k1 - k0) // 256
        ends.append(t)
    return [None if x in out[:n] else x for n, x in enumerate(out)]


def _token(n, nsteps, own, extra):
    t = own
    for k, e in enumerate(extra):
        if k * nsteps // len(extra) == n:
            t = e if t is None else t | e
    return t


def _mix(a, b):
    if not a or not b:
        return a or b
    keyed = [((k + 0.5) / len(a), x) for k, x in enumerate(a)] + [((k + 1.0) / len(b), x) for k, x in enumerate(b)]
    return [x for _, x in sorted(keyed, key=lambda e: e[0])]


def _update(acc, x, row0, op):
    if acc is None:
        return x
    if row0 == 0:
        return op(acc, x)
    return jnp.concatenate([acc[:row0], op(acc[row0:], x)], axis=0)


def _qk(i, qu, ks, zero, extra):
    r = jax.lax.broadcasted_iota(jnp.int32, (G, 128), 0)
    c = jax.lax.broadcasted_iota(jnp.int32, (G, 128), 1)
    msk = c <= r + (128 - G)
    h = G // 2
    qc = [jnp.concatenate([qu[64 * t + h * cls:64 * t + h * (cls + 1)] for t in range(NC)], axis=0)
          for cls in range(NC)]
    steps = _steps(i)
    due = _due(steps, MLAG)
    toks = {}
    run = [None] * NC
    sc, lead = [], []
    for cls in range(NC - 1):
        w = G * (cls + 1)
        s = _dot_nt(_rows(ks, 0, w).astype(BF16), pltpu.bitcast(qc[cls], BF16)).T
        if i == 0:
            top = jnp.where((c <= r + G * cls)[:, :w], s[:G], MASK_VALUE)
            s = jnp.concatenate([top, s[G:]], axis=0)
        lead.append(s)
        run[cls] = jnp.concatenate([s, jnp.full((128, 128 - w), MASK_VALUE, F32)], axis=1)
    for n, (cls, k0, k1, row0, masked) in enumerate(steps):
        x = qc[cls][row0 // 2:]
        t = _token(n, len(steps), toks.get(due[n]), extra)
        x = pltpu.bitcast(x if t is None else _inject(x, t), BF16)
        s = _dot_nt(x, _rows(ks, k0, k1).astype(BF16))
        if masked:
            top = jnp.where(msk, s[:G], MASK_VALUE)
            s = top if row0 + G == 128 else jnp.concatenate([top, s[G:]], axis=0)
        sc.append(s)
        mj = jnp.maximum(s[:, :128], s[:, 128:]) if k1 - k0 == 256 else s
        run[cls] = _update(run[cls], mj, row0, jnp.maximum)
        toks[n] = _or_fold(run[cls]) & zero
    return steps, lead, sc, run


def _softmax_pv(steps, lead, sc, mx, vs, zero, extra):
    m = [jnp.max(mx[cls], axis=1, keepdims=True) for cls in range(NC)]
    groups = []
    for cls in range(NC):
        w, out = [n for n, e in enumerate(steps) if e[0] == cls and e[2] - e[1] == 256], []
        while w:
            k = len(w) if len(w) <= 3 else 2
            out.append(w[:k])
            w = w[k:]
        groups.append(out)
    perm = [n for gi in range(max(len(x) for x in groups)) for cls in reversed(range(NC))
            if gi < len(groups[cls]) for n in groups[cls][gi]]
    ends = [g[-1] for x in groups for g in x]
    perm += sorted((n for n in range(len(steps)) if n not in perm), key=lambda n: (-steps[n][0], n))
    steps = [steps[n] for n in perm]
    due = _due(steps, SLAG)
    toks = {}
    o = [None] * NC
    run = [None] * NC
    macc = [[None] * 7 for _ in range(NC)]
    wait = []
    for cls in range(NC - 1):
        w = G * (cls + 1)
        p = jnp.exp2(lead[cls] - m[cls]).astype(BF16)
        o[cls] = _dot(p, _rows(vs, 0, w).astype(BF16))
        run[cls] = jnp.concatenate([p.astype(F32), jnp.zeros((128, 128 - w), F32)], axis=1)
    for n, (cls, k0, k1, row0, _) in enumerate(steps):
        p = jnp.exp2(sc[perm[n]] - m[cls][row0:])
        t = _token(n, len(steps), toks.get(due[n]), extra)
        if t is not None:
            p = pltpu.bitcast(_inject(pltpu.bitcast(p, U32), t), F32)
        if k1 - k0 == 256:
            lhs = [x.astype(BF16) for x in _lhs_ops(p)]
            wait.append((lhs, [x.astype(BF16) for x in _rhs_ops(_rows(vs, k0, k1))]))
            if perm[n] in ends:
                for j in PORDER:
                    t = None
                    for x, y in wait:
                        t = _update(t, _dot(x[j], y[j]), 0, jnp.add)
                    macc[cls][j] = _update(macc[cls][j], t, 0, jnp.add)
                wait = []
            e = jnp.concatenate([lhs[4].astype(F32), lhs[1].astype(F32)], axis=0)
        else:
            p = p.astype(BF16)
            t = _dot(p, _rows(vs, k0, k1).astype(BF16))
            e = p.astype(F32)
            o[cls] = _update(o[cls], t, row0, jnp.add)
        run[cls] = _update(run[cls], e, row0, jnp.add)
        toks[n] = _or_fold(run[cls]) & zero
    for cls in range(NC):
        if macc[cls][0] is not None:
            o[cls] = o[cls] + _combine(macc[cls])

    def natural(x):
        return jnp.concatenate([x[cls][G * t:G * (t + 1)] for t in range(NC) for cls in range(NC)], axis=0)
    return natural(o), natural(run)


def _normalize(o, lsum):
    return o * _recip(jnp.sum(lsum, axis=1, keepdims=True))


def _kernel(aq_hbm, ak_hbm, av_hbm, sh_hbm, ah_hbm, dd_hbm, xt_hbm, c_hbm,
            wq_hbm, wk_hbm, wv_hbm, wot_hbm,
            out_hbm,
            sh_s, dd_s, coef_s, f_s, fh_s, zero_s, xt_s, x_s, wq_raw, aq_s, ak_s, av_s, ah_s, at_s,
            c_s, cs_s, ws_s, wk_raw, wv_raw, wot_s, wos_s, q_s, ctx_s, ot_s, o7_s, l7_s, stage_a, stage_b,
            sem_small, sem_x, sem_wq, sem_a, sem_c, sem_wk, sem_wv, sem_oa, sem_ob):
    wq32 = wq_hbm.bitcast(U32)
    wk32 = wk_hbm.bitcast(U32)
    wv32 = wv_hbm.bitcast(U32)

    def cp_small(i):
        return pltpu.make_async_copy((sh_hbm, dd_hbm)[i], (sh_s, dd_s)[i], sem_small.at[i])

    def cp_x(i):
        cols = pl.ds(XB[i], XB[i + 1] - XB[i])
        return pltpu.make_async_copy(xt_hbm.at[:, cols], xt_s.at[:, cols], sem_x.at[i])

    def cp_wq(p):
        return pltpu.make_async_copy(wq32.at[:, p, :], wq_raw.at[p], sem_wq.at[p])

    def cp_a(g, i):
        src = (ah_hbm, ak_hbm, av_hbm, aq_hbm)[i].bitcast(U32)
        dst = (ah_s, ak_s, av_s, aq_s)[i]
        n = UC // 2
        start = g * n if isinstance(g, int) else pl.multiple_of(g * n, 8)
        return pltpu.make_async_copy(src.at[pl.ds(start, n), :], dst.at[g], sem_a.at[g * 4 + i])

    def cp_c(i):
        n = 128
        start = i * n if isinstance(i, int) else pl.multiple_of(i * n, n)
        return pltpu.make_async_copy(c_hbm.bitcast(U32).at[pl.ds(start, n), :],
                                     c_s.at[pl.ds(start, n), :], sem_c.at[i])

    def cp_wo():
        return pltpu.make_async_copy(wot_hbm.bitcast(U32), wot_s, sem_c.at[8])

    def c_ops(strip, i):
        blk, part = strip >> 3, strip & 7

        def quad(r, k):
            x = [c_s[_ds(blk * 256 + (2 * r + e) * 64 + part * 8, 8, 8), k * 512:(k + 1) * 512] for e in range(2)]
            return pltpu.bitcast(jnp.concatenate(x, axis=0), BF16).astype(F32)
        tok = None
        for j, y in enumerate(_lhs_ops(_lhs_op(quad, i))):
            cs_s[_ds(((blk * 7 + i) * 7 + j) * 64 + part * 8, 8, 8), :] = _pack(y)
            if j % 2 == 0:
                tok = _sample(y) if tok is None else tok | _sample(y)
        return tok & zero_s[...]

    def cp_wk(p):
        return pltpu.make_async_copy(wk32.at[:, p, :], wk_raw.at[p], sem_wk.at[p])

    def cp_wv(p):
        return pltpu.make_async_copy(wv32.at[:, p, :], wv_raw.at[p], sem_wv.at[p])

    def cp_out_a(i):
        n = NB3 * TO
        start = i * n if isinstance(i, int) else pl.multiple_of(i * n, n)
        return pltpu.make_async_copy(stage_a.at[pl.ds(start, n), :],
                                     out_hbm.at[pl.ds(start, n), pl.ds(0, MA)], sem_oa.at[i])

    def cp_out_b(i):
        start = i * TO if isinstance(i, int) else pl.multiple_of(i * TO, TO)
        return pltpu.make_async_copy(stage_b.at[pl.ds(start, TO), :],
                                     out_hbm.at[pl.ds(start, TO), pl.ds(MA, MP)], sem_ob.at[i])

    cp_x(0).start()
    cp_wq(0).start()
    for i in range(1, XCH):
        cp_x(i).start()
    cp_small(0).start()
    cp_small(1).start()

    tt = jax.lax.broadcasted_iota(jnp.int32, (128, 128), 0)
    rr = jax.lax.broadcasted_iota(jnp.int32, (128, 128), 1)
    ang = ((tt * (2 * rr + 1)) & 511).astype(F32) * (2.0 * math.pi / 512.0)
    fmat = jnp.concatenate([jnp.cos(ang), -jnp.sin(ang)], axis=1).astype(BF16)
    f_s[...] = pltpu.bitcast(fmat, U32)
    fh_s[...] = pltpu.bitcast((fmat.astype(F32) * (1.0 / 128.0)).astype(BF16), U32)
    zero_s[...] = jnp.zeros((8, 128), U32)

    def xpose_x(i):
        for blk in range(XB[i] // 256, XB[i + 1] // 256):
            tiles = []
            for t in (2 * blk, 2 * blk + 1):
                cols = slice(t * 128, (t + 1) * 128)
                parts = [xt_s[g * 128:(g + 1) * 128, cols].astype(F32).T for g in range(3)]
                last = jnp.concatenate([xt_s[MA:M, cols].astype(F32), jnp.zeros((MP - M, 128), F32)], axis=0)
                parts.append(last.T)
                tiles.append(jnp.concatenate(parts, axis=1))
            x = jnp.concatenate(tiles, axis=0)
            for j, op in enumerate(_lhs_ops(x)):
                x_s[(blk * 7 + j) * 64:(blk * 7 + j + 1) * 64, :] = _pack(op)

    def q_weights(p):
        raw = wq_raw[p]
        ops = []
        for w in (raw << 16, raw & jnp.uint32(HI_MASK)):
            w = pltpu.bitcast(w, F32) * Q_SCALE
            ops.append(_rhs_ops(jnp.concatenate([w, jnp.zeros((MP - M, D), F32)], axis=0)))
        return [jnp.concatenate([u, v], axis=1).astype(BF16) for u, v in zip(*ops)]

    def qstep(p, w, ms, n, tok=None):
        blk, j = n // 7, MORDER[n % 7]
        x = x_s[(blk * 7 + j) * 64:(blk * 7 + j + 1) * 64, :]
        if tok is not None:
            x = _inject(x, tok)
        ms[j] = _dot(pltpu.bitcast(x, BF16), w[j])
        if n % 7 == 6:
            for k in range(2):
                q = _combine([ms[e][:, k * 128:(k + 1) * 128] for e in range(7)])
                q_s[_ds((2 * p + k) * (S // 2) + blk * 128, 128, 128), :] = _pack(q)

    cp_x(0).wait()
    xpose_x(0)
    cp_c(0).start()
    cp_c(1).start()
    for g in range(NU):
        cp_wq(g + 1).start()
        for i in range(4):
            cp_a(g, i).start()
        if g < NU - 1:
            cp_c(g + 2).start()
    cp_wk(0).start()
    cp_wv(0).start()
    cp_wo().start()
    for p in range(1, H // 2):
        cp_wk(p).start()
        cp_wv(p).start()
    cp_wq(0).wait()
    w0 = q_weights(0)
    ms0 = {}
    for n in range(XB[1] // 256 * 7 - XLAG):
        qstep(0, w0, ms0, n)
    for i in range(1, XCH):
        cp_x(i).wait()
        if i == XCH - 1:
            cp_small(0).wait()
            cp_small(1).wait()
            cp_c(0).wait()
            cp_c(1).wait()
            prm = [sh_s[j:j + 1, :].astype(F32) for j in range(4)]
            prm.append(dd_s[...].astype(F32).reshape(1, M))
            for j in range(5):
                row = jnp.concatenate([prm[j], jnp.zeros((1, MP - M), F32)], axis=1)
                for t in range(MP // 128):
                    blk = jnp.broadcast_to(row[:, t * 128:(t + 1) * 128], (128, 128))
                    coef_s[j, t * 128:(t + 1) * 128, :] = blk.T
        for n in range(XB[i] // 256 * 7 - XLAG, XB[i] // 256 * 7):
            qstep(0, w0, ms0, n)
        xpose_x(i)
        for n in range(XB[i] // 256 * 7, XB[i + 1] // 256 * 7 - (XLAG if i < XCH - 1 else 0)):
            tok = None
            if i == XCH - 1:
                n0, n1 = XB[i] // 256 * 7, XB[i + 1] // 256 * 7
                for e in range(28):
                    if n0 + e * (n1 - n0) // 28 == n:
                        t = c_ops(e // 7, e % 7)
                        tok = t if tok is None else tok | t
            qstep(0, w0, ms0, n, tok)
    ot_s[...] = jnp.zeros((M, TO), F32)
    o7_s[...] = jnp.zeros((TQ, D), F32)
    l7_s[...] = jnp.ones((TQ, 128), F32)

    def phase1(g, carry):
        cp_wq(g + 1).wait()
        for i in range(4):
            cp_a(g, i).wait()

        @pl.when((g & 1) == 1)
        def _():
            cp_c(g + 1).wait()
            cp_c(g + 2).wait()

        w = q_weights(g + 1)
        fh = pltpu.bitcast(fh_s[...], BF16)
        fx = pltpu.bitcast(f_s[...], BF16)
        lane = jax.lax.broadcasted_iota(jnp.int32, (16, 128), 1)
        sgn = jnp.where((jax.lax.broadcasted_iota(jnp.int32, (8, 128), 1) & 1) == 0, 1.0, -1.0)
        zh, zx, kvs, ys = {}, {}, {}, {}

        def coef(k, j):
            return coef_s[j, pl.ds(pl.multiple_of(g * UC + k * 16, 16), 16), :]

        def hfwd(k):
            lhs = jnp.concatenate([ah_s[g, k * 8:(k + 1) * 8, c * 128:(c + 1) * 128]
                                   for c in range(NBLK)], axis=0)
            zh[k] = _dot(pltpu.bitcast(lhs, BF16), fh)

        def xfwd(k):
            kf = pltpu.bitcast(ak_s[g, k * 8:(k + 1) * 8, :], BF16).astype(F32)
            vf = pltpu.bitcast(av_s[g, k * 8:(k + 1) * 8, :], BF16).astype(F32)
            sh_k = [kf] + [pltpu.roll(kf, j, 1) for j in range(1, 4)]
            cf = [coef(k, j) for j in range(4)]
            kvf = []
            for c in range(NBLK):
                cols = slice(c * 128, (c + 1) * 128)
                t = sh_k[0][:, cols] * cf[0]
                for j in range(1, 4):
                    kj = sh_k[j][:, cols]
                    if c == 0:
                        kj = jnp.where(lane >= j, kj, 0.0)
                    t = t + kj * cf[j]
                kvf.append(t * vf[:, cols])
            kvs[k] = jnp.concatenate(kvf, axis=0).astype(BF16)
            zx[k] = _dot(kvs[k], fx)

        def inv(k, u):
            rows = [slice(c * 16 + u * 8, c * 16 + u * 8 + 8) for c in range(NBLK)]
            xr = [zx[k][r, :128] for r in rows]
            xi = [zx[k][r, 128:] for r in rows]
            h0r = [zh[k][r, :128] for r in rows]
            h0i = [zh[k][r, 128:] for r in rows]
            hr = [h0r[0]] + [h0r[j] - sgn * h0i[j - 1] for j in range(1, NBLK)]
            hi = [h0i[0]] + [h0i[j] + sgn * h0r[j - 1] for j in range(1, NBLK)]
            pr, pi = [], []
            for a0 in range(0, NBLK, 4):
                re = [None] * 4
                im = [None] * 4
                for c0 in range(0, a0 + 4, 4):
                    for da in range(4):
                        for c in range(c0, c0 + 4):
                            j = a0 + da - c
                            if j < 0:
                                continue
                            tr = xr[c] * hr[j] - xi[c] * hi[j]
                            ti = xr[c] * hi[j] + xi[c] * hr[j]
                            re[da] = tr if re[da] is None else re[da] + tr
                            im[da] = ti if im[da] is None else im[da] + ti
                pr += re
                pi += im
            p = jnp.concatenate([jnp.concatenate(pr, axis=0), jnp.concatenate(pi, axis=0)], axis=1)
            ys[k, u] = _dot_nt(p.astype(BF16), fx)
            if u == 1:
                kvr = kvs[k].astype(F32)
                qraw = aq_s[g, k * 8:(k + 1) * 8, :] | jnp.tile(zero_s[...], (1, NBLK))
                qf = pltpu.bitcast(qraw, BF16).astype(F32)
                dd = coef(k, 4)
                row0 = pl.multiple_of(g * UC + k * 16, 16)
                for a in range(NBLK):
                    cols = slice(a * 128, (a + 1) * 128)
                    y = jnp.concatenate([ys[k, 0][a * 8:(a + 1) * 8], ys[k, 1][a * 8:(a + 1) * 8]], axis=0)
                    y = y + kvr[a * 16:(a + 1) * 16] * dd
                    at_s[pl.ds(row0, 16), cols] = (qf[:, cols] * y).astype(BF16)

        ms = {}
        for n in range(S // 256 * 7):
            tok = None
            for step in P1PLAN.get(n, '').split():
                if step[0] == 'H':
                    hfwd(int(step[1]))
                elif step[0] == 'X':
                    xfwd(int(step[1]))
                elif step[0] == 'I':
                    inv(int(step[1]), int(step[2]))
            if n in CPOS:
                e = CPOS.index(n)
                tok = c_ops(4 * (g + 1) + e // 7, e % 7)
            qstep(g + 1, w, ms, n, tok)
        return carry

    jax.lax.fori_loop(0, NU, phase1, 0)

    cp_wo().wait()
    for p in range(H // 2):
        cp_wk(p).wait()
        cp_wv(p).wait()

    def unpack_head(w, h):
        sh = (16 - ((h & 1) << 4)).astype(U32)
        return pltpu.bitcast((w << sh) & jnp.uint32(HI_MASK), F32)

    def first_operands(h):
        w = jnp.concatenate([wk_raw[h >> 1, :256, :128], wk_raw[h >> 1, 256:512, 128:]], axis=1)
        w = unpack_head(w, h)
        ws_s[...] = _pack(w)
        return w

    first_operands(jnp.int32(0))

    def product(ws, blks, i):
        ms = [None] * 7
        for j in MORDER:
            r = [((blk * 7 + i) * 7 + j) * 64 for blk in blks]
            x = jnp.concatenate([cs_s[e:e + 64, :] for e in r], axis=0)
            ms[j] = _dot(pltpu.bitcast(x, BF16), ws[i][j])
        return [_combine([m[k * 128:(k + 1) * 128] for m in ms]) for k in range(len(blks))]

    def finish_last(h):
        ctx = _normalize(o7_s[...], l7_s[...])
        ctx_s[_ds(h * (S // 2) + (NB - 1) * TQ // 2, TQ // 2, TQ // 2), :] = _pack(ctx)
        return ctx

    def phase2(h, carry):
        b = unpack_head(jnp.concatenate([wk_raw[h >> 1], wv_raw[h >> 1]], axis=1), h)
        ws = [[y.astype(BF16) for y in _rhs_ops(x)] for x in _rhs_ops(b)]
        ws[1][1] = pltpu.bitcast(ws_s[:, :128], BF16)
        ws[1][4] = pltpu.bitcast(ws_s[:, 128:], BF16)
        mo = {}
        ks, vs, toks, sc = [], [], {}, {}
        zero = zero_s[...]

        def tokens(x, parts=NPART):
            n = TQ // parts
            return [_or_fold(x[k * n:(k + 1) * n]) & zero for k in range(parts)]

        def wo_ops(k, i):
            unit = jnp.minimum(2 * h + k, 27)
            j = jax.lax.div(unit, 7)
            r0 = (unit - 7 * j) * 8

            def quad(r, c):
                x = [jnp.concatenate([wot_s[j + 4 * (2 * c + f), _ds((2 * r + e) * 56 + r0, 8, 8), :]
                                      for f in range(2)], axis=1) for e in range(2)]
                return pltpu.bitcast(jnp.concatenate(x, axis=0), BF16).astype(F32)
            tok = None
            for n, y in enumerate(_lhs_ops(_lhs_op(quad, i))):
                wos_s[_ds(((j * 7 + i) * 7 + n) * 56 + r0, 8, 8), :] = _pack(y)
                if n % 2 == 0:
                    tok = _sample(y) if tok is None else tok | _sample(y)
            return tok & zero

        nxt = jnp.minimum(h + 1, H - 1)
        toks[-1] = tokens(finish_last(jnp.maximum(h - 1, 0)))
        for step in P2ORDER.split():
            i = int(step[1:])
            if step[0] == 'M':
                blks = [int(e) for e in step[2:]]
                j = int(step[1])
                for blk, m in zip(blks, product(ws, blks, j)):
                    mo[blk, j] = m
                    e = [mo.get((blk, k)) for k in range(7)]
                    if j == 6:
                        ks.append(_half(e, 0))
                    if j == 5:
                        vs.append(_half(e, 1))
            elif step[0] == 'Q':
                q = q_s[_ds(h * (S // 2) + i * TQ // 2, TQ // 2, TQ // 2), :]
                if i >= 1:
                    q = q | jnp.tile(zero, (TQ // 16, D // 128))
                extra = toks.get(i - 2, [])
                for k in {0: (0, 1), 2: (2,)}.get(i, ()):
                    extra = _mix(extra, tokens(vs[k], 8))
                if i >= 2:
                    extra = _mix(extra, [wo_ops(i - 2, e) for e in range(7)])
                if i == NB - 1:
                    w = first_operands(nxt)
                    extra = _mix(extra, [_sample(w[k * 64:(k + 1) * 64]) & zero for k in range(4)])
                sc[i] = _qk(i, q, ks, zero, extra)
            elif i == NB - 1:
                o7_s[...], l7_s[...] = _softmax_pv(*sc[i], vs, zero, toks[i - 1])
            else:
                ctx = _normalize(*_softmax_pv(*sc[i], vs, zero, []))
                ctx_s[_ds(h * (S // 2) + i * TQ // 2, TQ // 2, TQ // 2), :] = _pack(ctx)
                toks[i] = tokens(ctx)
        return carry

    jax.lax.fori_loop(0, H, phase2, 0)

    def finish(i, ot):
        r0 = i * TO if isinstance(i, int) else pl.multiple_of(i * TO, TO)
        top = at_s[MA:M, pl.ds(r0, TO)].astype(F32)
        val = jnp.concatenate([top, ot], axis=0).T
        stage_b[pl.ds(r0, TO), :] = val.astype(BF16)
        return val

    def phase3(it, carry):
        prev = jnp.maximum(NB3 * it - 1, 0)
        val = finish(prev, ot_s[...])
        pend = {3 + k: [val[:, k * 128:(k + 1) * 128]] for k in range(4)}

        @pl.when(it > 0)
        def _():
            cp_out_b(prev).start()

        r0 = pl.multiple_of(it * (NB3 * TO), NB3 * TO)
        apart = []
        for g in range(MA // 128):
            blk = at_s[g * 128:(g + 1) * 128, pl.ds(r0, NB3 * TO)].astype(F32).T
            stage_a[pl.ds(r0, NB3 * TO), g * 128:(g + 1) * 128] = blk.astype(BF16)
            apart.append(blk)
        cp_out_a(it).start()
        for k, y in enumerate(apart):
            for e in range(4):
                pend[16 + 4 * k + e] = [y[e * 128:(e + 1) * 128]]

        def ctx(kq, t):
            rows = pl.multiple_of((NB3 * it + t) * (TO // 2), TO // 2)
            x = [ctx_s[pl.ds(h * (S // 2) + rows, TO // 2), :] for h in range(4 * kq, 4 * kq + 4)]
            return pltpu.bitcast(jnp.concatenate(x, axis=1), BF16)

        mo = [[None] * 7, [None] * 7]
        step = 0
        for i in MORDER:
            sub = {(a, b): _rhs_op(lambda r, c: ctx(2 * r + a, 2 * c + b).astype(F32), i)
                   for a in range(2) for b in range(2)}
            mi = [None] * 7
            for j in MORDER:
                w = _rhs_op(lambda r, c: sub[r, c], j).astype(BF16)
                x = jnp.concatenate([wos_s[((e * 7 + i) * 7 + j) * 56:((e * 7 + i) * 7 + j + 1) * 56, :]
                                     for e in range(4)], axis=1)
                if step in pend:
                    tok = None
                    for y in pend[step]:
                        tok = _sample(y) if tok is None else tok | _sample(y)
                    x = _inject(x, tok & zero_s[...])
                mi[j] = _dot_nt(pltpu.bitcast(x, BF16), w)
                step += 1
                for k, last in ((0, 6), (1, 5)):
                    if j == last:
                        mo[k][i] = _half(mi, k)
                        for n, done in ((0, 6), (1, 5)):
                            if i == done and 2 * n + k < NB3 - 1:
                                val = finish(NB3 * it + 2 * n + k, _half(mo[k], n))
                                cp_out_b(NB3 * it + 2 * n + k).start()
                                for e in range(4):
                                    if step + 4 + e <= 48:
                                        due = step + 4 + e
                                        pend[due] = pend.get(due, []) + [val[:, e * 128:(e + 1) * 128]]
        ot_s[...] = _half(mo[1], 1)
        finish_last(H - 1)
        return carry

    jax.lax.fori_loop(0, NO // NB3, phase3, 0)

    finish(NO - 1, ot_s[...])
    cp_out_b(NO - 1).start()
    for i in range(NO // NB3):
        cp_out_a(i).wait()
    for i in range(NO):
        cp_out_b(i).wait()


@jax.jit
def pallas_concat_heads__ssm_conv_h3__compressed_kv_cla__prompt_kernel(
    A_q: jax.Array,
    A_k: jax.Array,
    A_v: jax.Array,
    A_shift_k: jax.Array,
    A_ssm_k: jax.Array,
    A_ssm_D: jax.Array,
    B_x: jax.Array,
    B_c_kv: jax.Array,
    B_w_q: jax.Array,
    B_w_uk: jax.Array,
    B_w_uv: jax.Array,
    B_w_o: jax.Array,
):
    vm = pltpu.VMEM
    dma = pltpu.SemaphoreType.DMA
    scratch = [
        vm((4, M), BF16),
        vm((M,), BF16),
        vm((5, MP, 128), F32),
        vm((64, 256), U32),
        vm((64, 256), U32),
        vm((8, 128), U32),
        vm((M, S), BF16),
        vm((S // 256 * 7 * 64, MP // 2), U32),
        vm((H // 2, M, D), U32),
        vm((NU, UC // 2, S), U32),
        vm((NU, UC // 2, S), U32),
        vm((NU, UC // 2, S), U32),
        vm((NU, UC // 2, S), U32),
        vm((M, S), BF16),
        vm((S // 2, C), U32),
        vm((NB * 49 * 64, C // 4), U32),
        vm((128, 256), U32),
        vm((H // 2, C, D), U32),
        vm((H // 2, C, D), U32),
        vm((H, M // 2, D), U32),
        vm((4 * 49 * 56, D), U32),
        vm((H * S // 2, D), U32),
        vm((H * S // 2, D), U32),
        vm((M, TO), F32),
        vm((TQ, D), F32),
        vm((TQ, 128), F32),
        vm((S, MA), BF16),
        vm((S, MP), BF16),
        dma((2,)), dma((XCH,)), dma((H // 2,)), dma((NU * 4,)), dma((9,)),
        dma((H // 2,)), dma((H // 2,)), dma((NO // NB3,)), dma((NO,)),
    ]
    out = pl.pallas_call(
        _kernel,
        in_specs=[pl.BlockSpec(memory_space=pl.ANY)] * 12,
        out_specs=pl.BlockSpec(memory_space=pl.ANY),
        out_shape=jax.ShapeDtypeStruct((S, 2 * M), BF16),
        scratch_shapes=scratch,
        compiler_params=pltpu.CompilerParams(
            vmem_limit_bytes=120 * 1024 * 1024,
            disable_semaphore_checks=True,
            disable_bounds_checks=True,
        ),
        name="h3_cla_fused",
    )(
        A_q[0].T, A_k[0].T, A_v[0].T, A_shift_k.T, A_ssm_k, A_ssm_D,
        B_x[0].T, B_c_kv[0], B_w_q, B_w_uk, B_w_uv, jnp.transpose(B_w_o, (0, 2, 1)),
    )
    return out[None]
```

```python
import math

import jax
import jax.numpy as jnp
import jax.experimental.pallas as pl
import jax.experimental.pallas.tpu as pltpu

S = 2048
M = 448
MP = 512
MA = 384
H = 16
D = 256
C = 1024
G = 32
NC = 128 // G
TQ = 128 * NC
NB = S // TQ
NU = 7
UC = M // NU
NBLK = S // 128
XB = (0, 256, 768, 1536, 2048)
XCH = len(XB) - 1
XLAG = 3
TO = 128
NO = S // TO
NB3 = 4
MLAG = 800
SLAG = 1000
NPART = 32
MORDER = (1, 4, 0, 3, 6, 2, 5)
PORDER = (2, 4, 5, 0, 3, 1, 6)
P1PLAN = {0: 'H0 H1 H2 H3', 5: 'X0', 9: 'X1', 13: 'X2', 17: 'X3', 21: 'I00', 25: 'I01', 29: 'I10',
          33: 'I11', 37: 'I20', 41: 'I21', 45: 'I30', 49: 'I31'}
CPOS = [1, 2, 3, 19, 20, 22, 23, 26, 27, 30, 31, 34, 35, 38, 39, 42, 43, 46, 47, 50, 51, 52, 53,
        54, 55, 48, 44, 40]
P2ORDER = ("M101 M401 M001 M301 M601 M201 M501 Q0 M12 M42 P0 Q1 M02 M32 M62 P1 M22 M52 "
           "Q2 M13 M43 M03 M33 M63 P2 Q3 M23 M53 P3")

F32 = jnp.float32
BF16 = jnp.bfloat16
U32 = jnp.uint32
HI_MASK = 0xFFFF0000
Q_SCALE = D ** -0.5 * math.log2(math.e)
MASK_VALUE = -1e9


def _dot(a, b):
    return jnp.dot(a, b, preferred_element_type=F32)


def _dot_nt(a, b):
    return jax.lax.dot_general(a, b, (((1,), (1,)), ((), ())), preferred_element_type=F32)


def _pack(x):
    return pltpu.bitcast(x.astype(BF16), U32)


def _ds(start, size, align):
    return pl.ds(start if isinstance(start, int) else pl.multiple_of(start, align), size)


def _sample(x):
    return _or_fold(jnp.concatenate([x[r + 8:r + 16] for r in range(0, x.shape[0], 16)], axis=0))


def _quads(x):
    r, c = x.shape[0] // 2, x.shape[1] // 2
    return x[:r, :c], x[:r, c:], x[r:, :c], x[r:, c:]


def _lhs_op(quad, i):
    return (lambda: quad(0, 0) + quad(1, 1), lambda: quad(1, 0) + quad(1, 1), lambda: quad(0, 0),
            lambda: quad(1, 1), lambda: quad(0, 0) + quad(0, 1), lambda: quad(1, 0) - quad(0, 0),
            lambda: quad(0, 1) - quad(1, 1))[i]()


def _rhs_op(quad, i):
    return (lambda: quad(0, 0) + quad(1, 1), lambda: quad(0, 0), lambda: quad(0, 1) - quad(1, 1),
            lambda: quad(1, 0) - quad(0, 0), lambda: quad(1, 1), lambda: quad(0, 0) + quad(0, 1),
            lambda: quad(1, 0) + quad(1, 1))[i]()


def _lhs_ops(a):
    q = _quads(a)
    return [_lhs_op(lambda r, c: q[2 * r + c], i) for i in range(7)]


def _rhs_ops(b):
    q = _quads(b)
    return [_rhs_op(lambda r, c: q[2 * r + c], i) for i in range(7)]


def _half(m, k):
    if k == 0:
        return jnp.concatenate([(m[0] + m[3]) + (m[6] - m[4]), m[1] + m[3]], axis=0)
    return jnp.concatenate([m[2] + m[4], (m[0] - m[1]) + (m[2] + m[5])], axis=0)


def _combine(m):
    return jnp.concatenate([_half(m, 0), _half(m, 1)], axis=1)


def _or_fold(x):
    bits = pltpu.bitcast(x, U32)
    t = None
    for r in range(bits.shape[0] // 8):
        for c in range(bits.shape[1] // 128):
            e = bits[r * 8:(r + 1) * 8, c * 128:(c + 1) * 128]
            t = e if t is None else t | e
    return t


def _inject(x, tok):
    top = x[:8, :128] | tok
    if x.shape[1] > 128:
        top = jnp.concatenate([top, x[:8, 128:]], axis=1)
    return jnp.concatenate([top, x[8:]], axis=0)


def _recip(x):
    r = pl.reciprocal(x, approx=True)
    return r * (2.0 - x * r)


def _rows(chunks, r0, r1):
    parts = []
    while r0 < r1:
        c = r0 // TQ
        e = min(r1, (c + 1) * TQ)
        parts.append(chunks[c][r0 - c * TQ:e - c * TQ])
        r0 = e
    return parts[0] if len(parts) == 1 else jnp.concatenate(parts, axis=0)


def _steps(i):
    plans = []
    for cls in range(NC):
        last = cls == NC - 1
        base = 0 if last else G * (cls + 1)
        full = NC * i - 1 + last
        plan = []
        m = 0
        while m < full:
            w = 2 if m + 2 <= full else 1
            plan.append((cls, base + 128 * m, base + 128 * (m + w), 0, False))
            m += w
        for t in range(NC):
            if full + t >= 0:
                plan.append((cls, base + 128 * (full + t), base + 128 * (full + t + 1), G * t, True))
        plans.append(plan)
    n = max(len(p) for p in plans)
    return [plans[cls][j - n + len(plans[cls])] for j in range(n) for cls in reversed(range(NC))
            if j - n + len(plans[cls]) >= 0]


def _due(steps, lag):
    ends, out, t = [], [], 0
    for _, k0, k1, row0, _ in steps:
        src = [n for n, e in enumerate(ends) if e + lag <= t]
        out.append(src[-1] if src else None)
        t += (128 - row0) * (k1 - k0) // 256
        ends.append(t)
    return [None if x in out[:n] else x for n, x in enumerate(out)]


def _token(n, nsteps, own, extra):
    t = own
    for k, e in enumerate(extra):
        if k * nsteps // len(extra) == n:
            t = e if t is None else t | e
    return t


def _mix(a, b):
    if not a or not b:
        return a or b
    keyed = [((k + 0.5) / len(a), x) for k, x in enumerate(a)] + [((k + 1.0) / len(b), x) for k, x in enumerate(b)]
    return [x for _, x in sorted(keyed, key=lambda e: e[0])]


def _update(acc, x, row0, op):
    if acc is None:
        return x
    if row0 == 0:
        return op(acc, x)
    return jnp.concatenate([acc[:row0], op(acc[row0:], x)], axis=0)


def _qk(i, qu, ks, zero, extra):
    r = jax.lax.broadcasted_iota(jnp.int32, (G, 128), 0)
    c = jax.lax.broadcasted_iota(jnp.int32, (G, 128), 1)
    msk = c <= r + (128 - G)
    h = G // 2
    qc = [jnp.concatenate([qu[64 * t + h * cls:64 * t + h * (cls + 1)] for t in range(NC)], axis=0)
          for cls in range(NC)]
    steps = _steps(i)
    due = _due(steps, MLAG)
    toks = {}
    run = [None] * NC
    sc, lead = [], []
    for cls in range(NC - 1):
        w = G * (cls + 1)
        s = _dot_nt(_rows(ks, 0, w).astype(BF16), pltpu.bitcast(qc[cls], BF16)).T
        if i == 0:
            top = jnp.where((c <= r + G * cls)[:, :w], s[:G], MASK_VALUE)
            s = jnp.concatenate([top, s[G:]], axis=0)
        lead.append(s)
        run[cls] = jnp.concatenate([s, jnp.full((128, 128 - w), MASK_VALUE, F32)], axis=1)
    for n, (cls, k0, k1, row0, masked) in enumerate(steps):
        x = qc[cls][row0 // 2:]
        t = _token(n, len(steps), toks.get(due[n]), extra)
        x = pltpu.bitcast(x if t is None else _inject(x, t), BF16)
        s = _dot_nt(x, _rows(ks, k0, k1).astype(BF16))
        if masked:
            top = jnp.where(msk, s[:G], MASK_VALUE)
            s = top if row0 + G == 128 else jnp.concatenate([top, s[G:]], axis=0)
        sc.append(s)
        mj = jnp.maximum(s[:, :128], s[:, 128:]) if k1 - k0 == 256 else s
        run[cls] = _update(run[cls], mj, row0, jnp.maximum)
        toks[n] = _or_fold(run[cls]) & zero
    return steps, lead, sc, run


def _softmax_pv(steps, lead, sc, mx, vs, zero, extra):
    m = [jnp.max(mx[cls], axis=1, keepdims=True) for cls in range(NC)]
    groups = []
    for cls in range(NC):
        w, out = [n for n, e in enumerate(steps) if e[0] == cls and e[2] - e[1] == 256], []
        while w:
            k = len(w) if len(w) <= 3 else 2
            out.append(w[:k])
            w = w[k:]
        groups.append(out)
    perm = [n for gi in range(max(len(x) for x in groups)) for cls in reversed(range(NC))
            if gi < len(groups[cls]) for n in groups[cls][gi]]
    ends = [g[-1] for x in groups for g in x]
    perm += sorted((n for n in range(len(steps)) if n not in perm), key=lambda n: (-steps[n][0], n))
    steps = [steps[n] for n in perm]
    due = _due(steps, SLAG)
    toks = {}
    o = [None] * NC
    run = [None] * NC
    macc = [[None] * 7 for _ in range(NC)]
    wait = []
    for cls in range(NC - 1):
        w = G * (cls + 1)
        p = jnp.exp2(lead[cls] - m[cls]).astype(BF16)
        o[cls] = _dot(p, _rows(vs, 0, w).astype(BF16))
        run[cls] = jnp.concatenate([p.astype(F32), jnp.zeros((128, 128 - w), F32)], axis=1)
    for n, (cls, k0, k1, row0, _) in enumerate(steps):
        p = jnp.exp2(sc[perm[n]] - m[cls][row0:])
        t = _token(n, len(steps), toks.get(due[n]), extra)
        if t is not None:
            p = pltpu.bitcast(_inject(pltpu.bitcast(p, U32), t), F32)
        if k1 - k0 == 256:
            lhs = [x.astype(BF16) for x in _lhs_ops(p)]
            wait.append((lhs, [x.astype(BF16) for x in _rhs_ops(_rows(vs, k0, k1))]))
            if perm[n] in ends:
                for j in PORDER:
                    t = None
                    for x, y in wait:
                        t = _update(t, _dot(x[j], y[j]), 0, jnp.add)
                    macc[cls][j] = _update(macc[cls][j], t, 0, jnp.add)
                wait = []
            e = jnp.concatenate([lhs[4].astype(F32), lhs[1].astype(F32)], axis=0)
        else:
            p = p.astype(BF16)
            t = _dot(p, _rows(vs, k0, k1).astype(BF16))
            e = p.astype(F32)
            o[cls] = _update(o[cls], t, row0, jnp.add)
        run[cls] = _update(run[cls], e, row0, jnp.add)
        toks[n] = _or_fold(run[cls]) & zero
    for cls in range(NC):
        if macc[cls][0] is not None:
            o[cls] = o[cls] + _combine(macc[cls])

    def natural(x):
        return jnp.concatenate([x[cls][G * t:G * (t + 1)] for t in range(NC) for cls in range(NC)], axis=0)
    return natural(o), natural(run)


def _normalize(o, lsum):
    return o * _recip(jnp.sum(lsum, axis=1, keepdims=True))


def _kernel(aq_hbm, ak_hbm, av_hbm, sh_hbm, ah_hbm, dd_hbm, xt_hbm, c_hbm,
            wq_hbm, wk_hbm, wv_hbm, wot_hbm,
            out_hbm,
            sh_s, dd_s, coef_s, f_s, fh_s, zero_s, xt_s, x_s, wq_raw, aq_s, ak_s, av_s, ah_s, at_s,
            c_s, cs_s, ws_s, wk_raw, wv_raw, wot_s, wos_s, q_s, ctx_s, ot_s, o7_s, l7_s, stage_a, stage_b,
            sem_small, sem_x, sem_wq, sem_a, sem_c, sem_wk, sem_wv, sem_oa, sem_ob):
    wq32 = wq_hbm.bitcast(U32)
    wk32 = wk_hbm.bitcast(U32)
    wv32 = wv_hbm.bitcast(U32)

    def cp_small(i):
        return pltpu.make_async_copy((sh_hbm, dd_hbm)[i], (sh_s, dd_s)[i], sem_small.at[i])

    def cp_x(i):
        cols = pl.ds(XB[i], XB[i + 1] - XB[i])
        return pltpu.make_async_copy(xt_hbm.at[:, cols], xt_s.at[:, cols], sem_x.at[i])

    def cp_wq(p):
        return pltpu.make_async_copy(wq32.at[:, p, :], wq_raw.at[p], sem_wq.at[p])

    def cp_a(g, i):
        src = (ah_hbm, ak_hbm, av_hbm, aq_hbm)[i].bitcast(U32)
        dst = (ah_s, ak_s, av_s, aq_s)[i]
        n = UC // 2
        start = g * n if isinstance(g, int) else pl.multiple_of(g * n, 8)
        return pltpu.make_async_copy(src.at[pl.ds(start, n), :], dst.at[g], sem_a.at[g * 4 + i])

    def cp_c(i):
        n = 128
        start = i * n if isinstance(i, int) else pl.multiple_of(i * n, n)
        return pltpu.make_async_copy(c_hbm.bitcast(U32).at[pl.ds(start, n), :],
                                     c_s.at[pl.ds(start, n), :], sem_c.at[i])

    def cp_wo():
        return pltpu.make_async_copy(wot_hbm.bitcast(U32), wot_s, sem_c.at[8])

    def c_ops(strip, i):
        blk, part = strip >> 3, strip & 7

        def quad(r, k):
            x = [c_s[_ds(blk * 256 + (2 * r + e) * 64 + part * 8, 8, 8), k * 512:(k + 1) * 512] for e in range(2)]
            return pltpu.bitcast(jnp.concatenate(x, axis=0), BF16).astype(F32)
        tok = None
        for j, y in enumerate(_lhs_ops(_lhs_op(quad, i))):
            cs_s[_ds(((blk * 7 + i) * 7 + j) * 64 + part * 8, 8, 8), :] = _pack(y)
            if j % 2 == 0:
                tok = _sample(y) if tok is None else tok | _sample(y)
        return tok & zero_s[...]

    def cp_wk(p):
        return pltpu.make_async_copy(wk32.at[:, p, :], wk_raw.at[p], sem_wk.at[p])

    def cp_wv(p):
        return pltpu.make_async_copy(wv32.at[:, p, :], wv_raw.at[p], sem_wv.at[p])

    def cp_out_a(i):
        n = NB3 * TO
        start = i * n if isinstance(i, int) else pl.multiple_of(i * n, n)
        return pltpu.make_async_copy(stage_a.at[pl.ds(start, n), :],
                                     out_hbm.at[pl.ds(start, n), pl.ds(0, MA)], sem_oa.at[i])

    def cp_out_b(i):
        start = i * TO if isinstance(i, int) else pl.multiple_of(i * TO, TO)
        return pltpu.make_async_copy(stage_b.at[pl.ds(start, TO), :],
                                     out_hbm.at[pl.ds(start, TO), pl.ds(MA, MP)], sem_ob.at[i])

    cp_x(0).start()
    cp_wq(0).start()
    for i in range(1, XCH):
        cp_x(i).start()
    cp_small(0).start()
    cp_small(1).start()

    tt = jax.lax.broadcasted_iota(jnp.int32, (128, 128), 0)
    rr = jax.lax.broadcasted_iota(jnp.int32, (128, 128), 1)
    ang = ((tt * (2 * rr + 1)) & 511).astype(F32) * (2.0 * math.pi / 512.0)
    fmat = jnp.concatenate([jnp.cos(ang), -jnp.sin(ang)], axis=1).astype(BF16)
    f_s[...] = pltpu.bitcast(fmat, U32)
    fh_s[...] = pltpu.bitcast((fmat.astype(F32) * (1.0 / 128.0)).astype(BF16), U32)
    zero_s[...] = jnp.zeros((8, 128), U32)

    def xpose_x(i):
        for blk in range(XB[i] // 256, XB[i + 1] // 256):
            tiles = []
            for t in (2 * blk, 2 * blk + 1):
                cols = slice(t * 128, (t + 1) * 128)
                parts = [xt_s[g * 128:(g + 1) * 128, cols].astype(F32).T for g in range(3)]
                last = jnp.concatenate([xt_s[MA:M, cols].astype(F32), jnp.zeros((MP - M, 128), F32)], axis=0)
                parts.append(last.T)
                tiles.append(jnp.concatenate(parts, axis=1))
            x = jnp.concatenate(tiles, axis=0)
            for j, op in enumerate(_lhs_ops(x)):
                x_s[(blk * 7 + j) * 64:(blk * 7 + j + 1) * 64, :] = _pack(op)

    def q_weights(p):
        raw = wq_raw[p]
        ops = []
        for w in (raw << 16, raw & jnp.uint32(HI_MASK)):
            w = pltpu.bitcast(w, F32) * Q_SCALE
            ops.append(_rhs_ops(jnp.concatenate([w, jnp.zeros((MP - M, D), F32)], axis=0)))
        return [jnp.concatenate([u, v], axis=1).astype(BF16) for u, v in zip(*ops)]

    def qstep(p, w, ms, n, tok=None):
        blk, j = n // 7, MORDER[n % 7]
        x = x_s[(blk * 7 + j) * 64:(blk * 7 + j + 1) * 64, :]
        if tok is not None:
            x = _inject(x, tok)
        ms[j] = _dot(pltpu.bitcast(x, BF16), w[j])
        if n % 7 == 6:
            for k in range(2):
                q = _combine([ms[e][:, k * 128:(k + 1) * 128] for e in range(7)])
                q_s[_ds((2 * p + k) * (S // 2) + blk * 128, 128, 128), :] = _pack(q)

    cp_x(0).wait()
    xpose_x(0)
    cp_c(0).start()
    cp_c(1).start()
    for g in range(NU):
        cp_wq(g + 1).start()
        for i in range(4):
            cp_a(g, i).start()
        if g < NU - 1:
            cp_c(g + 2).start()
    cp_wk(0).start()
    cp_wv(0).start()
    cp_wo().start()
    for p in range(1, H // 2):
        cp_wk(p).start()
        cp_wv(p).start()
    cp_wq(0).wait()
    w0 = q_weights(0)
    ms0 = {}
    for n in range(XB[1] // 256 * 7 - XLAG):
        qstep(0, w0, ms0, n)
    for i in range(1, XCH):
        cp_x(i).wait()
        if i == XCH - 1:
            cp_small(0).wait()
            cp_small(1).wait()
            cp_c(0).wait()
            cp_c(1).wait()
            prm = [sh_s[j:j + 1, :].astype(F32) for j in range(4)]
            prm.append(dd_s[...].astype(F32).reshape(1, M))
            for j in range(5):
                row = jnp.concatenate([prm[j], jnp.zeros((1, MP - M), F32)], axis=1)
                for t in range(MP // 128):
                    blk = jnp.broadcast_to(row[:, t * 128:(t + 1) * 128], (128, 128))
                    coef_s[j, t * 128:(t + 1) * 128, :] = blk.T
        for n in range(XB[i] // 256 * 7 - XLAG, XB[i] // 256 * 7):
            qstep(0, w0, ms0, n)
        xpose_x(i)
        for n in range(XB[i] // 256 * 7, XB[i + 1] // 256 * 7 - (XLAG if i < XCH - 1 else 0)):
            tok = None
            if i == XCH - 1:
                n0, n1 = XB[i] // 256 * 7, XB[i + 1] // 256 * 7
                for e in range(28):
                    if n0 + e * (n1 - n0) // 28 == n:
                        t = c_ops(e // 7, e % 7)
                        tok = t if tok is None else tok | t
            qstep(0, w0, ms0, n, tok)
    ot_s[...] = jnp.zeros((M, TO), F32)
    o7_s[...] = jnp.zeros((TQ, D), F32)
    l7_s[...] = jnp.ones((TQ, 128), F32)

    def phase1(g, carry):
        cp_wq(g + 1).wait()
        for i in range(4):
            cp_a(g, i).wait()

        @pl.when((g & 1) == 1)
        def _():
            cp_c(g + 1).wait()
            cp_c(g + 2).wait()

        w = q_weights(g + 1)
        fh = pltpu.bitcast(fh_s[...], BF16)
        fx = pltpu.bitcast(f_s[...], BF16)
        lane = jax.lax.broadcasted_iota(jnp.int32, (16, 128), 1)
        sgn = jnp.where((jax.lax.broadcasted_iota(jnp.int32, (8, 128), 1) & 1) == 0, 1.0, -1.0)
        zh, zx, kvs, ys = {}, {}, {}, {}

        def coef(k, j):
            return coef_s[j, pl.ds(pl.multiple_of(g * UC + k * 16, 16), 16), :]

        def hfwd(k):
            lhs = jnp.concatenate([ah_s[g, k * 8:(k + 1) * 8, c * 128:(c + 1) * 128]
                                   for c in range(NBLK)], axis=0)
            zh[k] = _dot(pltpu.bitcast(lhs, BF16), fh)

        def xfwd(k):
            kf = pltpu.bitcast(ak_s[g, k * 8:(k + 1) * 8, :], BF16).astype(F32)
            vf = pltpu.bitcast(av_s[g, k * 8:(k + 1) * 8, :], BF16).astype(F32)
            sh_k = [kf] + [pltpu.roll(kf, j, 1) for j in range(1, 4)]
            cf = [coef(k, j) for j in range(4)]
            kvf = []
            for c in range(NBLK):
                cols = slice(c * 128, (c + 1) * 128)
                t = sh_k[0][:, cols] * cf[0]
                for j in range(1, 4):
                    kj = sh_k[j][:, cols]
                    if c == 0:
                        kj = jnp.where(lane >= j, kj, 0.0)
                    t = t + kj * cf[j]
                kvf.append(t * vf[:, cols])
            kvs[k] = jnp.concatenate(kvf, axis=0).astype(BF16)
            zx[k] = _dot(kvs[k], fx)

        def inv(k, u):
            rows = [slice(c * 16 + u * 8, c * 16 + u * 8 + 8) for c in range(NBLK)]
            xr = [zx[k][r, :128] for r in rows]
            xi = [zx[k][r, 128:] for r in rows]
            h0r = [zh[k][r, :128] for r in rows]
            h0i = [zh[k][r, 128:] for r in rows]
            hr = [h0r[0]] + [h0r[j] - sgn * h0i[j - 1] for j in range(1, NBLK)]
            hi = [h0i[0]] + [h0i[j] + sgn * h0r[j - 1] for j in range(1, NBLK)]
            pr, pi = [], []
            for a0 in range(0, NBLK, 4):
                re = [None] * 4
                im = [None] * 4
                for c0 in range(0, a0 + 4, 4):
                    for da in range(4):
                        for c in range(c0, c0 + 4):
                            j = a0 + da - c
                            if j < 0:
                                continue
                            tr = xr[c] * hr[j] - xi[c] * hi[j]
                            ti = xr[c] * hi[j] + xi[c] * hr[j]
                            re[da] = tr if re[da] is None else re[da] + tr
                            im[da] = ti if im[da] is None else im[da] + ti
                pr += re
                pi += im
            p = jnp.concatenate([jnp.concatenate(pr, axis=0), jnp.concatenate(pi, axis=0)], axis=1)
            ys[k, u] = _dot_nt(p.astype(BF16), fx)
            if u == 1:
                kvr = kvs[k].astype(F32)
                qraw = aq_s[g, k * 8:(k + 1) * 8, :] | jnp.tile(zero_s[...], (1, NBLK))
                qf = pltpu.bitcast(qraw, BF16).astype(F32)
                dd = coef(k, 4)
                row0 = pl.multiple_of(g * UC + k * 16, 16)
                for a in range(NBLK):
                    cols = slice(a * 128, (a + 1) * 128)
                    y = jnp.concatenate([ys[k, 0][a * 8:(a + 1) * 8], ys[k, 1][a * 8:(a + 1) * 8]], axis=0)
                    y = y + kvr[a * 16:(a + 1) * 16] * dd
                    at_s[pl.ds(row0, 16), cols] = (qf[:, cols] * y).astype(BF16)

        ms = {}
        for n in range(S // 256 * 7):
            tok = None
            for step in P1PLAN.get(n, '').split():
                if step[0] == 'H':
                    hfwd(int(step[1]))
                elif step[0] == 'X':
                    xfwd(int(step[1]))
                elif step[0] == 'I':
                    inv(int(step[1]), int(step[2]))
            for e, pos in enumerate(CPOS):
                if pos == n:
                    t = c_ops(4 * (g + 1) + e // 7, e % 7)
                    tok = t if tok is None else tok | t
            qstep(g + 1, w, ms, n, tok)
        return carry

    jax.lax.fori_loop(0, NU, phase1, 0)

    cp_wo().wait()
    for p in range(H // 2):
        cp_wk(p).wait()
        cp_wv(p).wait()

    def unpack_head(w, h):
        sh = (16 - ((h & 1) << 4)).astype(U32)
        return pltpu.bitcast((w << sh) & jnp.uint32(HI_MASK), F32)

    def first_operands(h):
        w = jnp.concatenate([wk_raw[h >> 1, :256, :128], wk_raw[h >> 1, 256:512, 128:]], axis=1)
        w = unpack_head(w, h)
        ws_s[...] = _pack(w)
        return w

    first_operands(jnp.int32(0))

    def product(ws, blks, i):
        ms = [None] * 7
        for j in MORDER:
            r = [((blk * 7 + i) * 7 + j) * 64 for blk in blks]
            x = jnp.concatenate([cs_s[e:e + 64, :] for e in r], axis=0)
            ms[j] = _dot(pltpu.bitcast(x, BF16), ws[i][j])
        return [_combine([m[k * 128:(k + 1) * 128] for m in ms]) for k in range(len(blks))]

    def finish_last(h):
        ctx = _normalize(o7_s[...], l7_s[...])
        ctx_s[_ds(h * (S // 2) + (NB - 1) * TQ // 2, TQ // 2, TQ // 2), :] = _pack(ctx)
        return ctx

    def phase2(h, carry):
        b = unpack_head(jnp.concatenate([wk_raw[h >> 1], wv_raw[h >> 1]], axis=1), h)
        ws = [[y.astype(BF16) for y in _rhs_ops(x)] for x in _rhs_ops(b)]
        ws[1][1] = pltpu.bitcast(ws_s[:, :128], BF16)
        ws[1][4] = pltpu.bitcast(ws_s[:, 128:], BF16)
        mo = {}
        ks, vs, toks, sc = [], [], {}, {}
        zero = zero_s[...]

        def tokens(x, parts=NPART):
            n = TQ // parts
            return [_or_fold(x[k * n:(k + 1) * n]) & zero for k in range(parts)]

        def wo_ops(k, i):
            unit = jnp.minimum(2 * h + k, 27)
            j = jax.lax.div(unit, 7)
            r0 = (unit - 7 * j) * 8

            def quad(r, c):
                x = [jnp.concatenate([wot_s[j + 4 * (2 * c + f), _ds((2 * r + e) * 56 + r0, 8, 8), :]
                                      for f in range(2)], axis=1) for e in range(2)]
                return pltpu.bitcast(jnp.concatenate(x, axis=0), BF16).astype(F32)
            tok = None
            for n, y in enumerate(_lhs_ops(_lhs_op(quad, i))):
                wos_s[_ds(((j * 7 + i) * 7 + n) * 56 + r0, 8, 8), :] = _pack(y)
                if n % 2 == 0:
                    tok = _sample(y) if tok is None else tok | _sample(y)
            return tok & zero

        nxt = jnp.minimum(h + 1, H - 1)
        toks[-1] = tokens(finish_last(jnp.maximum(h - 1, 0)))
        for step in P2ORDER.split():
            i = int(step[1:])
            if step[0] == 'M':
                blks = [int(e) for e in step[2:]]
                j = int(step[1])
                for blk, m in zip(blks, product(ws, blks, j)):
                    mo[blk, j] = m
                    e = [mo.get((blk, k)) for k in range(7)]
                    if j == 6:
                        ks.append(_half(e, 0))
                    if j == 5:
                        vs.append(_half(e, 1))
            elif step[0] == 'Q':
                q = q_s[_ds(h * (S // 2) + i * TQ // 2, TQ // 2, TQ // 2), :]
                if i >= 1:
                    q = q | jnp.tile(zero, (TQ // 16, D // 128))
                extra = toks.get(i - 2, [])
                for k in {0: (0, 1), 2: (2,)}.get(i, ()):
                    extra = _mix(extra, tokens(vs[k], 8))
                if i >= 2:
                    extra = _mix(extra, [wo_ops(i - 2, e) for e in range(7)])
                if i == NB - 1:
                    w = first_operands(nxt)
                    extra = _mix(extra, [_sample(w[k * 64:(k + 1) * 64]) & zero for k in range(4)])
                sc[i] = _qk(i, q, ks, zero, extra)
            elif i == NB - 1:
                o7_s[...], l7_s[...] = _softmax_pv(*sc[i], vs, zero, toks[i - 1])
            else:
                ctx = _normalize(*_softmax_pv(*sc[i], vs, zero, []))
                ctx_s[_ds(h * (S // 2) + i * TQ // 2, TQ // 2, TQ // 2), :] = _pack(ctx)
                toks[i] = tokens(ctx)
        return carry

    jax.lax.fori_loop(0, H, phase2, 0)

    def finish(i, ot):
        r0 = i * TO if isinstance(i, int) else pl.multiple_of(i * TO, TO)
        top = at_s[MA:M, pl.ds(r0, TO)].astype(F32)
        val = jnp.concatenate([top, ot], axis=0).T
        stage_b[pl.ds(r0, TO), :] = val.astype(BF16)
        return val

    def phase3(it, carry):
        prev = jnp.maximum(NB3 * it - 1, 0)
        val = finish(prev, ot_s[...])
        pend = {3 + k: [val[:, k * 128:(k + 1) * 128]] for k in range(4)}

        @pl.when(it > 0)
        def _():
            cp_out_b(prev).start()

        r0 = pl.multiple_of(it * (NB3 * TO), NB3 * TO)
        apart = []
        for g in range(MA // 128):
            blk = at_s[g * 128:(g + 1) * 128, pl.ds(r0, NB3 * TO)].astype(F32).T
            stage_a[pl.ds(r0, NB3 * TO), g * 128:(g + 1) * 128] = blk.astype(BF16)
            apart.append(blk)
        cp_out_a(it).start()
        for k, y in enumerate(apart):
            for e in range(4):
                pend[16 + 4 * k + e] = [y[e * 128:(e + 1) * 128]]

        def ctx(kq, t):
            rows = pl.multiple_of((NB3 * it + t) * (TO // 2), TO // 2)
            x = [ctx_s[pl.ds(h * (S // 2) + rows, TO // 2), :] for h in range(4 * kq, 4 * kq + 4)]
            return pltpu.bitcast(jnp.concatenate(x, axis=1), BF16)

        mo = [[None] * 7, [None] * 7]
        step = 0
        for i in MORDER:
            sub = {(a, b): _rhs_op(lambda r, c: ctx(2 * r + a, 2 * c + b).astype(F32), i)
                   for a in range(2) for b in range(2)}
            mi = [None] * 7
            for j in MORDER:
                w = _rhs_op(lambda r, c: sub[r, c], j).astype(BF16)
                x = jnp.concatenate([wos_s[((e * 7 + i) * 7 + j) * 56:((e * 7 + i) * 7 + j + 1) * 56, :]
                                     for e in range(4)], axis=1)
                if step in pend:
                    tok = None
                    for y in pend[step]:
                        tok = _sample(y) if tok is None else tok | _sample(y)
                    x = _inject(x, tok & zero_s[...])
                mi[j] = _dot_nt(pltpu.bitcast(x, BF16), w)
                step += 1
                for k, last in ((0, 6), (1, 5)):
                    if j == last:
                        mo[k][i] = _half(mi, k)
                        for n, done in ((0, 6), (1, 5)):
                            if i == done and 2 * n + k < NB3 - 1:
                                val = finish(NB3 * it + 2 * n + k, _half(mo[k], n))
                                cp_out_b(NB3 * it + 2 * n + k).start()
                                for e in range(4):
                                    if step + 4 + e <= 48:
                                        due = step + 4 + e
                                        pend[due] = pend.get(due, []) + [val[:, e * 128:(e + 1) * 128]]
        ot_s[...] = _half(mo[1], 1)
        finish_last(H - 1)
        return carry

    jax.lax.fori_loop(0, NO // NB3, phase3, 0)

    finish(NO - 1, ot_s[...])
    cp_out_b(NO - 1).start()
    for i in range(NO // NB3):
        cp_out_a(i).wait()
    for i in range(NO):
        cp_out_b(i).wait()


@jax.jit
def pallas_concat_heads__ssm_conv_h3__compressed_kv_cla__prompt_kernel(
    A_q: jax.Array,
    A_k: jax.Array,
    A_v: jax.Array,
    A_shift_k: jax.Array,
    A_ssm_k: jax.Array,
    A_ssm_D: jax.Array,
    B_x: jax.Array,
    B_c_kv: jax.Array,
    B_w_q: jax.Array,
    B_w_uk: jax.Array,
    B_w_uv: jax.Array,
    B_w_o: jax.Array,
):
    vm = pltpu.VMEM
    dma = pltpu.SemaphoreType.DMA
    scratch = [
        vm((4, M), BF16),
        vm((M,), BF16),
        vm((5, MP, 128), F32),
        vm((64, 256), U32),
        vm((64, 256), U32),
        vm((8, 128), U32),
        vm((M, S), BF16),
        vm((S // 256 * 7 * 64, MP // 2), U32),
        vm((H // 2, M, D), U32),
        vm((NU, UC // 2, S), U32),
        vm((NU, UC // 2, S), U32),
        vm((NU, UC // 2, S), U32),
        vm((NU, UC // 2, S), U32),
        vm((M, S), BF16),
        vm((S // 2, C), U32),
        vm((NB * 49 * 64, C // 4), U32),
        vm((128, 256), U32),
        vm((H // 2, C, D), U32),
        vm((H // 2, C, D), U32),
        vm((H, M // 2, D), U32),
        vm((4 * 49 * 56, D), U32),
        vm((H * S // 2, D), U32),
        vm((H * S // 2, D), U32),
        vm((M, TO), F32),
        vm((TQ, D), F32),
        vm((TQ, 128), F32),
        vm((S, MA), BF16),
        vm((S, MP), BF16),
        dma((2,)), dma((XCH,)), dma((H // 2,)), dma((NU * 4,)), dma((9,)),
        dma((H // 2,)), dma((H // 2,)), dma((NO // NB3,)), dma((NO,)),
    ]
    out = pl.pallas_call(
        _kernel,
        in_specs=[pl.BlockSpec(memory_space=pl.ANY)] * 12,
        out_specs=pl.BlockSpec(memory_space=pl.ANY),
        out_shape=jax.ShapeDtypeStruct((S, 2 * M), BF16),
        scratch_shapes=scratch,
        compiler_params=pltpu.CompilerParams(
            vmem_limit_bytes=120 * 1024 * 1024,
            disable_semaphore_checks=True,
            disable_bounds_checks=True,
        ),
        name="h3_cla_fused",
    )(
        A_q[0].T, A_k[0].T, A_v[0].T, A_shift_k.T, A_ssm_k, A_ssm_D,
        B_x[0].T, B_c_kv[0], B_w_q, B_w_uk, B_w_uv, jnp.transpose(B_w_o, (0, 2, 1)),
    )
    return out[None]
```

```python
import math

import jax
import jax.numpy as jnp
import jax.experimental.pallas as pl
import jax.experimental.pallas.tpu as pltpu

S = 2048
M = 448
MP = 512
MA = 384
H = 16
D = 256
C = 1024
G = 32
NC = 128 // G
TQ = 128 * NC
NB = S // TQ
NU = 7
UC = M // NU
NBLK = S // 128
XB = (0, 256, 768, 1536, 2048)
XCH = len(XB) - 1
XLAG = 3
TO = 128
NO = S // TO
NB3 = 4
MLAG = 1000
SLAG = 1000
NPART = 16
MORDER = (1, 4, 0, 3, 6, 2, 5)
PORDER = (2, 4, 5, 0, 3, 1, 6)
P1PLAN = {0: 'H0 H1 H2 H3', 5: 'X0', 9: 'X1', 13: 'X2', 17: 'X3', 21: 'I00', 25: 'I01', 29: 'I10',
          33: 'I11', 37: 'I20', 41: 'I21', 45: 'I30', 49: 'I31'}
CPOS = [1, 2, 3, 19, 20, 22, 23, 26, 27, 30, 31, 34, 35, 38, 39, 42, 43, 46, 47, 50, 51, 52, 53,
        54, 55, 48, 44, 40]
P2ORDER = ("M101 M401 M001 M301 M601 M201 M501 Q0 M12 M42 P0 Q1 M02 M32 M62 P1 M22 M52 "
           "Q2 M13 M43 M03 M33 M63 P2 Q3 M23 M53 P3")

F32 = jnp.float32
BF16 = jnp.bfloat16
U32 = jnp.uint32
HI_MASK = 0xFFFF0000
Q_SCALE = D ** -0.5 * math.log2(math.e)
MASK_VALUE = -1e9


def _dot(a, b):
    return jnp.dot(a, b, preferred_element_type=F32)


def _dot_nt(a, b):
    return jax.lax.dot_general(a, b, (((1,), (1,)), ((), ())), preferred_element_type=F32)


def _pack(x):
    return pltpu.bitcast(x.astype(BF16), U32)


def _ds(start, size, align):
    return pl.ds(start if isinstance(start, int) else pl.multiple_of(start, align), size)


def _sample(x):
    return _or_fold(jnp.concatenate([x[r + 8:r + 16] for r in range(0, x.shape[0], 16)], axis=0))


def _quads(x):
    r, c = x.shape[0] // 2, x.shape[1] // 2
    return x[:r, :c], x[:r, c:], x[r:, :c], x[r:, c:]


def _lhs_op(quad, i):
    return (lambda: quad(0, 0) + quad(1, 1), lambda: quad(1, 0) + quad(1, 1), lambda: quad(0, 0),
            lambda: quad(1, 1), lambda: quad(0, 0) + quad(0, 1), lambda: quad(1, 0) - quad(0, 0),
            lambda: quad(0, 1) - quad(1, 1))[i]()


def _rhs_op(quad, i):
    return (lambda: quad(0, 0) + quad(1, 1), lambda: quad(0, 0), lambda: quad(0, 1) - quad(1, 1),
            lambda: quad(1, 0) - quad(0, 0), lambda: quad(1, 1), lambda: quad(0, 0) + quad(0, 1),
            lambda: quad(1, 0) + quad(1, 1))[i]()


def _lhs_ops(a):
    q = _quads(a)
    return [_lhs_op(lambda r, c: q[2 * r + c], i) for i in range(7)]


def _rhs_ops(b):
    q = _quads(b)
    return [_rhs_op(lambda r, c: q[2 * r + c], i) for i in range(7)]


def _half(m, k):
    if k == 0:
        return jnp.concatenate([(m[0] + m[3]) + (m[6] - m[4]), m[1] + m[3]], axis=0)
    return jnp.concatenate([m[2] + m[4], (m[0] - m[1]) + (m[2] + m[5])], axis=0)


def _combine(m):
    return jnp.concatenate([_half(m, 0), _half(m, 1)], axis=1)


def _or_fold(x):
    bits = pltpu.bitcast(x, U32)
    t = None
    for r in range(bits.shape[0] // 8):
        for c in range(bits.shape[1] // 128):
            e = bits[r * 8:(r + 1) * 8, c * 128:(c + 1) * 128]
            t = e if t is None else t | e
    return t


def _inject(x, tok):
    top = x[:8, :128] | tok
    if x.shape[1] > 128:
        top = jnp.concatenate([top, x[:8, 128:]], axis=1)
    return jnp.concatenate([top, x[8:]], axis=0)


def _recip(x):
    r = pl.reciprocal(x, approx=True)
    return r * (2.0 - x * r)


def _rows(chunks, r0, r1):
    parts = []
    while r0 < r1:
        c = r0 // TQ
        e = min(r1, (c + 1) * TQ)
        parts.append(chunks[c][r0 - c * TQ:e - c * TQ])
        r0 = e
    return parts[0] if len(parts) == 1 else jnp.concatenate(parts, axis=0)


def _steps(i):
    plans = []
    for cls in range(NC):
        last = cls == NC - 1
        base = 0 if last else G * (cls + 1)
        full = NC * i - 1 + last
        plan = []
        m = 0
        while m < full:
            w = 2 if m + 2 <= full else 1
            plan.append((cls, base + 128 * m, base + 128 * (m + w), 0, False))
            m += w
        for t in range(NC):
            if full + t >= 0:
                plan.append((cls, base + 128 * (full + t), base + 128 * (full + t + 1), G * t, True))
        plans.append(plan)
    n = max(len(p) for p in plans)
    return [plans[cls][j - n + len(plans[cls])] for j in range(n) for cls in reversed(range(NC))
            if j - n + len(plans[cls]) >= 0]


def _due(steps, lag):
    ends, out, t = [], [], 0
    for _, k0, k1, row0, _ in steps:
        src = [n for n, e in enumerate(ends) if e + lag <= t]
        out.append(src[-1] if src else None)
        t += (128 - row0) * (k1 - k0) // 256
        ends.append(t)
    return [None if x in out[:n] else x for n, x in enumerate(out)]


def _token(n, nsteps, own, extra):
    t = own
    for k, e in enumerate(extra):
        if k * nsteps // len(extra) == n:
            t = e if t is None else t | e
    return t


def _mix(a, b):
    if not a or not b:
        return a or b
    keyed = [((k + 0.5) / len(a), x) for k, x in enumerate(a)] + [((k + 1.0) / len(b), x) for k, x in enumerate(b)]
    return [x for _, x in sorted(keyed, key=lambda e: e[0])]


def _update(acc, x, row0, op):
    if acc is None:
        return x
    if row0 == 0:
        return op(acc, x)
    return jnp.concatenate([acc[:row0], op(acc[row0:], x)], axis=0)


def _qk(i, qu, ks, zero, extra):
    r = jax.lax.broadcasted_iota(jnp.int32, (G, 128), 0)
    c = jax.lax.broadcasted_iota(jnp.int32, (G, 128), 1)
    msk = c <= r + (128 - G)
    h = G // 2
    qc = [jnp.concatenate([qu[64 * t + h * cls:64 * t + h * (cls + 1)] for t in range(NC)], axis=0)
          for cls in range(NC)]
    steps = _steps(i)
    due = _due(steps, MLAG)
    toks = {}
    run = [None] * NC
    sc, lead = [], []
    for cls in range(NC - 1):
        w = G * (cls + 1)
        s = _dot_nt(_rows(ks, 0, w).astype(BF16), pltpu.bitcast(qc[cls], BF16)).T
        if i == 0:
            top = jnp.where((c <= r + G * cls)[:, :w], s[:G], MASK_VALUE)
            s = jnp.concatenate([top, s[G:]], axis=0)
        lead.append(s)
        run[cls] = jnp.concatenate([s, jnp.full((128, 128 - w), MASK_VALUE, F32)], axis=1)
    for n, (cls, k0, k1, row0, masked) in enumerate(steps):
        x = qc[cls][row0 // 2:]
        t = _token(n, len(steps), toks.get(due[n]), extra)
        x = pltpu.bitcast(x if t is None else _inject(x, t), BF16)
        s = _dot_nt(x, _rows(ks, k0, k1).astype(BF16))
        if masked:
            top = jnp.where(msk, s[:G], MASK_VALUE)
            s = top if row0 + G == 128 else jnp.concatenate([top, s[G:]], axis=0)
        sc.append(s)
        mj = jnp.maximum(s[:, :128], s[:, 128:]) if k1 - k0 == 256 else s
        run[cls] = _update(run[cls], mj, row0, jnp.maximum)
        toks[n] = _or_fold(run[cls]) & zero
    return steps, lead, sc, run


def _softmax_pv(steps, lead, sc, mx, vs, zero, extra):
    m = [jnp.max(mx[cls], axis=1, keepdims=True) for cls in range(NC)]
    groups = []
    for cls in range(NC):
        w, out = [n for n, e in enumerate(steps) if e[0] == cls and e[2] - e[1] == 256], []
        while w:
            k = len(w) if len(w) <= 3 else 2
            out.append(w[:k])
            w = w[k:]
        groups.append(out)
    perm = [n for gi in range(max(len(x) for x in groups)) for cls in reversed(range(NC))
            if gi < len(groups[cls]) for n in groups[cls][gi]]
    ends = [g[-1] for x in groups for g in x]
    perm += sorted((n for n in range(len(steps)) if n not in perm), key=lambda n: (-steps[n][0], n))
    steps = [steps[n] for n in perm]
    due = _due(steps, SLAG)
    toks = {}
    o = [None] * NC
    run = [None] * NC
    macc = [[None] * 7 for _ in range(NC)]
    wait = []
    for cls in range(NC - 1):
        w = G * (cls + 1)
        p = jnp.exp2(lead[cls] - m[cls]).astype(BF16)
        o[cls] = _dot(p, _rows(vs, 0, w).astype(BF16))
        run[cls] = jnp.concatenate([p.astype(F32), jnp.zeros((128, 128 - w), F32)], axis=1)
    for n, (cls, k0, k1, row0, _) in enumerate(steps):
        p = jnp.exp2(sc[perm[n]] - m[cls][row0:])
        t = _token(n, len(steps), toks.get(due[n]), extra)
        if t is not None:
            p = pltpu.bitcast(_inject(pltpu.bitcast(p, U32), t), F32)
        if k1 - k0 == 256:
            lhs = [x.astype(BF16) for x in _lhs_ops(p)]
            wait.append((lhs, [x.astype(BF16) for x in _rhs_ops(_rows(vs, k0, k1))]))
            if perm[n] in ends:
                for j in PORDER:
                    t = None
                    for x, y in wait:
                        t = _update(t, _dot(x[j], y[j]), 0, jnp.add)
                    macc[cls][j] = _update(macc[cls][j], t, 0, jnp.add)
                wait = []
            e = jnp.concatenate([lhs[4].astype(F32), lhs[1].astype(F32)], axis=0)
        else:
            p = p.astype(BF16)
            t = _dot(p, _rows(vs, k0, k1).astype(BF16))
            e = p.astype(F32)
            o[cls] = _update(o[cls], t, row0, jnp.add)
        run[cls] = _update(run[cls], e, row0, jnp.add)
        toks[n] = _or_fold(run[cls]) & zero
    for cls in range(NC):
        if macc[cls][0] is not None:
            o[cls] = o[cls] + _combine(macc[cls])

    def natural(x):
        return jnp.concatenate([x[cls][G * t:G * (t + 1)] for t in range(NC) for cls in range(NC)], axis=0)
    return natural(o), natural(run)


def _normalize(o, lsum):
    return o * _recip(jnp.sum(lsum, axis=1, keepdims=True))


def _kernel(aq_hbm, ak_hbm, av_hbm, sh_hbm, ah_hbm, dd_hbm, xt_hbm, c_hbm,
            wq_hbm, wk_hbm, wv_hbm, wot_hbm,
            out_hbm,
            sh_s, dd_s, coef_s, f_s, fh_s, zero_s, xt_s, x_s, wq_raw, aq_s, ak_s, av_s, ah_s, at_s,
            c_s, cs_s, ws_s, wk_raw, wv_raw, wot_s, wos_s, q_s, ctx_s, ot_s, o7_s, l7_s, stage_a, stage_b,
            sem_small, sem_x, sem_wq, sem_a, sem_c, sem_wk, sem_wv, sem_oa, sem_ob):
    wq32 = wq_hbm.bitcast(U32)
    wk32 = wk_hbm.bitcast(U32)
    wv32 = wv_hbm.bitcast(U32)

    def cp_small(i):
        return pltpu.make_async_copy((sh_hbm, dd_hbm)[i], (sh_s, dd_s)[i], sem_small.at[i])

    def cp_x(i):
        cols = pl.ds(XB[i], XB[i + 1] - XB[i])
        return pltpu.make_async_copy(xt_hbm.at[:, cols], xt_s.at[:, cols], sem_x.at[i])

    def cp_wq(p):
        return pltpu.make_async_copy(wq32.at[:, p, :], wq_raw.at[p], sem_wq.at[p])

    def cp_a(g, i):
        src = (ah_hbm, ak_hbm, av_hbm, aq_hbm)[i].bitcast(U32)
        dst = (ah_s, ak_s, av_s, aq_s)[i]
        n = UC // 2
        start = g * n if isinstance(g, int) else pl.multiple_of(g * n, 8)
        return pltpu.make_async_copy(src.at[pl.ds(start, n), :], dst.at[g], sem_a.at[g * 4 + i])

    def cp_c(i):
        n = 128
        start = i * n if isinstance(i, int) else pl.multiple_of(i * n, n)
        return pltpu.make_async_copy(c_hbm.bitcast(U32).at[pl.ds(start, n), :],
                                     c_s.at[pl.ds(start, n), :], sem_c.at[i])

    def cp_wo():
        return pltpu.make_async_copy(wot_hbm.bitcast(U32), wot_s, sem_c.at[8])

    def c_ops(strip, i):
        blk, part = strip >> 3, strip & 7

        def quad(r, k):
            x = [c_s[_ds(blk * 256 + (2 * r + e) * 64 + part * 8, 8, 8), k * 512:(k + 1) * 512] for e in range(2)]
            return pltpu.bitcast(jnp.concatenate(x, axis=0), BF16).astype(F32)
        tok = None
        for j, y in enumerate(_lhs_ops(_lhs_op(quad, i))):
            cs_s[_ds(((blk * 7 + i) * 7 + j) * 64 + part * 8, 8, 8), :] = _pack(y)
            if j % 2 == 0:
                tok = _sample(y) if tok is None else tok | _sample(y)
        return tok & zero_s[...]

    def cp_wk(p):
        return pltpu.make_async_copy(wk32.at[:, p, :], wk_raw.at[p], sem_wk.at[p])

    def cp_wv(p):
        return pltpu.make_async_copy(wv32.at[:, p, :], wv_raw.at[p], sem_wv.at[p])

    def cp_out_a(i):
        n = NB3 * TO
        start = i * n if isinstance(i, int) else pl.multiple_of(i * n, n)
        return pltpu.make_async_copy(stage_a.at[pl.ds(start, n), :],
                                     out_hbm.at[pl.ds(start, n), pl.ds(0, MA)], sem_oa.at[i])

    def cp_out_b(i):
        start = i * TO if isinstance(i, int) else pl.multiple_of(i * TO, TO)
        return pltpu.make_async_copy(stage_b.at[pl.ds(start, TO), :],
                                     out_hbm.at[pl.ds(start, TO), pl.ds(MA, MP)], sem_ob.at[i])

    cp_x(0).start()
    cp_wq(0).start()
    for i in range(1, XCH):
        cp_x(i).start()
    cp_small(0).start()
    cp_small(1).start()

    tt = jax.lax.broadcasted_iota(jnp.int32, (128, 128), 0)
    rr = jax.lax.broadcasted_iota(jnp.int32, (128, 128), 1)
    ang = ((tt * (2 * rr + 1)) & 511).astype(F32) * (2.0 * math.pi / 512.0)
    fmat = jnp.concatenate([jnp.cos(ang), -jnp.sin(ang)], axis=1).astype(BF16)
    f_s[...] = pltpu.bitcast(fmat, U32)
    fh_s[...] = pltpu.bitcast((fmat.astype(F32) * (1.0 / 128.0)).astype(BF16), U32)
    zero_s[...] = jnp.zeros((8, 128), U32)

    def xpose_x(i):
        for blk in range(XB[i] // 256, XB[i + 1] // 256):
            tiles = []
            for t in (2 * blk, 2 * blk + 1):
                cols = slice(t * 128, (t + 1) * 128)
                parts = [xt_s[g * 128:(g + 1) * 128, cols].astype(F32).T for g in range(3)]
                last = jnp.concatenate([xt_s[MA:M, cols].astype(F32), jnp.zeros((MP - M, 128), F32)], axis=0)
                parts.append(last.T)
                tiles.append(jnp.concatenate(parts, axis=1))
            x = jnp.concatenate(tiles, axis=0)
            for j, op in enumerate(_lhs_ops(x)):
                x_s[(blk * 7 + j) * 64:(blk * 7 + j + 1) * 64, :] = _pack(op)

    def q_weights(p):
        raw = wq_raw[p]
        ops = []
        for w in (raw << 16, raw & jnp.uint32(HI_MASK)):
            w = pltpu.bitcast(w, F32) * Q_SCALE
            ops.append(_rhs_ops(jnp.concatenate([w, jnp.zeros((MP - M, D), F32)], axis=0)))
        return [jnp.concatenate([u, v], axis=1).astype(BF16) for u, v in zip(*ops)]

    def qstep(p, w, ms, n, tok=None):
        blk, j = n // 7, MORDER[n % 7]
        x = x_s[(blk * 7 + j) * 64:(blk * 7 + j + 1) * 64, :]
        if tok is not None:
            x = _inject(x, tok)
        ms[j] = _dot(pltpu.bitcast(x, BF16), w[j])
        if n % 7 == 6:
            for k in range(2):
                q = _combine([ms[e][:, k * 128:(k + 1) * 128] for e in range(7)])
                q_s[_ds((2 * p + k) * (S // 2) + blk * 128, 128, 128), :] = _pack(q)

    cp_x(0).wait()
    xpose_x(0)
    cp_c(0).start()
    cp_c(1).start()
    for g in range(NU):
        cp_wq(g + 1).start()
        for i in range(4):
            cp_a(g, i).start()
        if g < NU - 1:
            cp_c(g + 2).start()
    cp_wk(0).start()
    cp_wv(0).start()
    cp_wo().start()
    for p in range(1, H // 2):
        cp_wk(p).start()
        cp_wv(p).start()
    cp_wq(0).wait()
    w0 = q_weights(0)
    ms0 = {}
    for n in range(XB[1] // 256 * 7 - XLAG):
        qstep(0, w0, ms0, n)
    for i in range(1, XCH):
        cp_x(i).wait()
        if i == XCH - 1:
            cp_small(0).wait()
            cp_small(1).wait()
            cp_c(0).wait()
            cp_c(1).wait()
            prm = [sh_s[j:j + 1, :].astype(F32) for j in range(4)]
            prm.append(dd_s[...].astype(F32).reshape(1, M))
            for j in range(5):
                row = jnp.concatenate([prm[j], jnp.zeros((1, MP - M), F32)], axis=1)
                for t in range(MP // 128):
                    blk = jnp.broadcast_to(row[:, t * 128:(t + 1) * 128], (128, 128))
                    coef_s[j, t * 128:(t + 1) * 128, :] = blk.T
        for n in range(XB[i] // 256 * 7 - XLAG, XB[i] // 256 * 7):
            qstep(0, w0, ms0, n)
        xpose_x(i)
        for n in range(XB[i] // 256 * 7, XB[i + 1] // 256 * 7 - (XLAG if i < XCH - 1 else 0)):
            tok = None
            if i == XCH - 1:
                n0, n1 = XB[i] // 256 * 7, XB[i + 1] // 256 * 7
                for e in range(28):
                    if n0 + e * (n1 - n0) // 28 == n:
                        t = c_ops(e // 7, e % 7)
                        tok = t if tok is None else tok | t
            qstep(0, w0, ms0, n, tok)
    ot_s[...] = jnp.zeros((M, TO), F32)
    o7_s[...] = jnp.zeros((TQ, D), F32)
    l7_s[...] = jnp.ones((TQ, 128), F32)

    def phase1(g, carry):
        cp_wq(g + 1).wait()
        for i in range(4):
            cp_a(g, i).wait()

        @pl.when((g & 1) == 1)
        def _():
            cp_c(g + 1).wait()
            cp_c(g + 2).wait()

        w = q_weights(g + 1)
        fh = pltpu.bitcast(fh_s[...], BF16)
        fx = pltpu.bitcast(f_s[...], BF16)
        lane = jax.lax.broadcasted_iota(jnp.int32, (16, 128), 1)
        sgn = jnp.where((jax.lax.broadcasted_iota(jnp.int32, (8, 128), 1) & 1) == 0, 1.0, -1.0)
        zh, zx, kvs, ys = {}, {}, {}, {}

        def coef(k, j):
            return coef_s[j, pl.ds(pl.multiple_of(g * UC + k * 16, 16), 16), :]

        def hfwd(k):
            lhs = jnp.concatenate([ah_s[g, k * 8:(k + 1) * 8, c * 128:(c + 1) * 128]
                                   for c in range(NBLK)], axis=0)
            zh[k] = _dot(pltpu.bitcast(lhs, BF16), fh)

        def xfwd(k):
            kf = pltpu.bitcast(ak_s[g, k * 8:(k + 1) * 8, :], BF16).astype(F32)
            vf = pltpu.bitcast(av_s[g, k * 8:(k + 1) * 8, :], BF16).astype(F32)
            sh_k = [kf] + [pltpu.roll(kf, j, 1) for j in range(1, 4)]
            cf = [coef(k, j) for j in range(4)]
            kvf = []
            for c in range(NBLK):
                cols = slice(c * 128, (c + 1) * 128)
                t = sh_k[0][:, cols] * cf[0]
                for j in range(1, 4):
                    kj = sh_k[j][:, cols]
                    if c == 0:
                        kj = jnp.where(lane >= j, kj, 0.0)
                    t = t + kj * cf[j]
                kvf.append(t * vf[:, cols])
            kvs[k] = jnp.concatenate(kvf, axis=0).astype(BF16)
            zx[k] = _dot(kvs[k], fx)

        def inv(k, u):
            rows = [slice(c * 16 + u * 8, c * 16 + u * 8 + 8) for c in range(NBLK)]
            xr = [zx[k][r, :128] for r in rows]
            xi = [zx[k][r, 128:] for r in rows]
            h0r = [zh[k][r, :128] for r in rows]
            h0i = [zh[k][r, 128:] for r in rows]
            hr = [h0r[0]] + [h0r[j] - sgn * h0i[j - 1] for j in range(1, NBLK)]
            hi = [h0i[0]] + [h0i[j] + sgn * h0r[j - 1] for j in range(1, NBLK)]
            pr, pi = [], []
            for a0 in range(0, NBLK, 4):
                re = [None] * 4
                im = [None] * 4
                for c0 in range(0, a0 + 4, 4):
                    for da in range(4):
                        for c in range(c0, c0 + 4):
                            j = a0 + da - c
                            if j < 0:
                                continue
                            tr = xr[c] * hr[j] - xi[c] * hi[j]
                            ti = xr[c] * hi[j] + xi[c] * hr[j]
                            re[da] = tr if re[da] is None else re[da] + tr
                            im[da] = ti if im[da] is None else im[da] + ti
                pr += re
                pi += im
            p = jnp.concatenate([jnp.concatenate(pr, axis=0), jnp.concatenate(pi, axis=0)], axis=1)
            ys[k, u] = _dot_nt(p.astype(BF16), fx)
            if u == 1:
                kvr = kvs[k].astype(F32)
                qraw = aq_s[g, k * 8:(k + 1) * 8, :] | jnp.tile(zero_s[...], (1, NBLK))
                qf = pltpu.bitcast(qraw, BF16).astype(F32)
                dd = coef(k, 4)
                row0 = pl.multiple_of(g * UC + k * 16, 16)
                for a in range(NBLK):
                    cols = slice(a * 128, (a + 1) * 128)
                    y = jnp.concatenate([ys[k, 0][a * 8:(a + 1) * 8], ys[k, 1][a * 8:(a + 1) * 8]], axis=0)
                    y = y + kvr[a * 16:(a + 1) * 16] * dd
                    at_s[pl.ds(row0, 16), cols] = (qf[:, cols] * y).astype(BF16)

        ms = {}
        for n in range(S // 256 * 7):
            tok = None
            for step in P1PLAN.get(n, '').split():
                if step[0] == 'H':
                    hfwd(int(step[1]))
                elif step[0] == 'X':
                    xfwd(int(step[1]))
                elif step[0] == 'I':
                    inv(int(step[1]), int(step[2]))
            for e, pos in enumerate(CPOS):
                if pos == n:
                    t = c_ops(4 * (g + 1) + e // 7, e % 7)
                    tok = t if tok is None else tok | t
            qstep(g + 1, w, ms, n, tok)
        return carry

    jax.lax.fori_loop(0, NU, phase1, 0)

    cp_wo().wait()
    for p in range(H // 2):
        cp_wk(p).wait()
        cp_wv(p).wait()

    def unpack_head(w, h):
        sh = (16 - ((h & 1) << 4)).astype(U32)
        return pltpu.bitcast((w << sh) & jnp.uint32(HI_MASK), F32)

    def first_operands(h):
        w = jnp.concatenate([wk_raw[h >> 1, :256, :128], wk_raw[h >> 1, 256:512, 128:]], axis=1)
        w = unpack_head(w, h)
        ws_s[...] = _pack(w)
        return w

    first_operands(jnp.int32(0))

    def product(ws, blks, i):
        ms = [None] * 7
        for j in MORDER:
            r = [((blk * 7 + i) * 7 + j) * 64 for blk in blks]
            x = jnp.concatenate([cs_s[e:e + 64, :] for e in r], axis=0)
            ms[j] = _dot(pltpu.bitcast(x, BF16), ws[i][j])
        return [_combine([m[k * 128:(k + 1) * 128] for m in ms]) for k in range(len(blks))]

    def finish_last(h):
        ctx = _normalize(o7_s[...], l7_s[...])
        ctx_s[_ds(h * (S // 2) + (NB - 1) * TQ // 2, TQ // 2, TQ // 2), :] = _pack(ctx)
        return ctx

    def phase2(h, carry):
        b = unpack_head(jnp.concatenate([wk_raw[h >> 1], wv_raw[h >> 1]], axis=1), h)
        ws = [[y.astype(BF16) for y in _rhs_ops(x)] for x in _rhs_ops(b)]
        ws[1][1] = pltpu.bitcast(ws_s[:, :128], BF16)
        ws[1][4] = pltpu.bitcast(ws_s[:, 128:], BF16)
        mo = {}
        ks, vs, toks, sc = [], [], {}, {}
        zero = zero_s[...]

        def tokens(x, parts=NPART):
            n = TQ // parts
            return [_or_fold(x[k * n:(k + 1) * n]) & zero for k in range(parts)]

        def wo_ops(k, i):
            unit = jnp.minimum(2 * h + k, 27)
            j = jax.lax.div(unit, 7)
            r0 = (unit - 7 * j) * 8

            def quad(r, c):
                x = [jnp.concatenate([wot_s[j + 4 * (2 * c + f), _ds((2 * r + e) * 56 + r0, 8, 8), :]
                                      for f in range(2)], axis=1) for e in range(2)]
                return pltpu.bitcast(jnp.concatenate(x, axis=0), BF16).astype(F32)
            tok = None
            for n, y in enumerate(_lhs_ops(_lhs_op(quad, i))):
                wos_s[_ds(((j * 7 + i) * 7 + n) * 56 + r0, 8, 8), :] = _pack(y)
                if n % 2 == 0:
                    tok = _sample(y) if tok is None else tok | _sample(y)
            return tok & zero

        nxt = jnp.minimum(h + 1, H - 1)
        toks[-1] = tokens(finish_last(jnp.maximum(h - 1, 0)))
        for step in P2ORDER.split():
            i = int(step[1:])
            if step[0] == 'M':
                blks = [int(e) for e in step[2:]]
                j = int(step[1])
                for blk, m in zip(blks, product(ws, blks, j)):
                    mo[blk, j] = m
                    e = [mo.get((blk, k)) for k in range(7)]
                    if j == 6:
                        ks.append(_half(e, 0))
                    if j == 5:
                        vs.append(_half(e, 1))
            elif step[0] == 'Q':
                q = q_s[_ds(h * (S // 2) + i * TQ // 2, TQ // 2, TQ // 2), :]
                if i >= 1:
                    q = q | jnp.tile(zero, (TQ // 16, D // 128))
                extra = toks.get(i - 2, [])
                for k in {0: (0, 1), 2: (2,)}.get(i, ()):
                    extra = _mix(extra, tokens(vs[k], 8))
                if i % 2 == 1:
                    extra = _mix(extra, [wo_ops(i // 2, e) for e in range(7)])
                if i == NB - 1:
                    w = first_operands(nxt)
                    extra = _mix(extra, [_sample(w[k * 64:(k + 1) * 64]) & zero for k in range(4)])
                sc[i] = _qk(i, q, ks, zero, extra)
            elif i == NB - 1:
                o7_s[...], l7_s[...] = _softmax_pv(*sc[i], vs, zero, toks[i - 1])
            else:
                ctx = _normalize(*_softmax_pv(*sc[i], vs, zero, []))
                ctx_s[_ds(h * (S // 2) + i * TQ // 2, TQ // 2, TQ // 2), :] = _pack(ctx)
                toks[i] = tokens(ctx)
        return carry

    jax.lax.fori_loop(0, H, phase2, 0)

    def finish(i, ot):
        r0 = i * TO if isinstance(i, int) else pl.multiple_of(i * TO, TO)
        top = at_s[MA:M, pl.ds(r0, TO)].astype(F32)
        val = jnp.concatenate([top, ot], axis=0).T
        stage_b[pl.ds(r0, TO), :] = val.astype(BF16)
        return val

    def phase3(it, carry):
        prev = jnp.maximum(NB3 * it - 1, 0)
        val = finish(prev, ot_s[...])
        pend = {3 + k: [val[:, k * 128:(k + 1) * 128]] for k in range(4)}

        @pl.when(it > 0)
        def _():
            cp_out_b(prev).start()

        r0 = pl.multiple_of(it * (NB3 * TO), NB3 * TO)
        apart = []
        for g in range(MA // 128):
            blk = at_s[g * 128:(g + 1) * 128, pl.ds(r0, NB3 * TO)].astype(F32).T
            stage_a[pl.ds(r0, NB3 * TO), g * 128:(g + 1) * 128] = blk.astype(BF16)
            apart.append(blk)
        cp_out_a(it).start()
        for k, y in enumerate(apart):
            for e in range(4):
                pend[16 + 4 * k + e] = [y[e * 128:(e + 1) * 128]]

        def ctx(kq, t):
            rows = pl.multiple_of((NB3 * it + t) * (TO // 2), TO // 2)
            x = [ctx_s[pl.ds(h * (S // 2) + rows, TO // 2), :] for h in range(4 * kq, 4 * kq + 4)]
            return pltpu.bitcast(jnp.concatenate(x, axis=1), BF16)

        mo = [[None] * 7, [None] * 7]
        step = 0
        for i in MORDER:
            sub = {(a, b): _rhs_op(lambda r, c: ctx(2 * r + a, 2 * c + b).astype(F32), i)
                   for a in range(2) for b in range(2)}
            mi = [None] * 7
            for j in MORDER:
                w = _rhs_op(lambda r, c: sub[r, c], j).astype(BF16)
                x = jnp.concatenate([wos_s[((e * 7 + i) * 7 + j) * 56:((e * 7 + i) * 7 + j + 1) * 56, :]
                                     for e in range(4)], axis=1)
                if step in pend:
                    tok = None
                    for y in pend[step]:
                        tok = _sample(y) if tok is None else tok | _sample(y)
                    x = _inject(x, tok & zero_s[...])
                mi[j] = _dot_nt(pltpu.bitcast(x, BF16), w)
                step += 1
                for k, last in ((0, 6), (1, 5)):
                    if j == last:
                        mo[k][i] = _half(mi, k)
                        for n, done in ((0, 6), (1, 5)):
                            if i == done and 2 * n + k < NB3 - 1:
                                val = finish(NB3 * it + 2 * n + k, _half(mo[k], n))
                                cp_out_b(NB3 * it + 2 * n + k).start()
                                for e in range(4):
                                    if step + 4 + e <= 48:
                                        due = step + 4 + e
                                        pend[due] = pend.get(due, []) + [val[:, e * 128:(e + 1) * 128]]
        ot_s[...] = _half(mo[1], 1)
        finish_last(H - 1)
        return carry

    jax.lax.fori_loop(0, NO // NB3, phase3, 0)

    finish(NO - 1, ot_s[...])
    cp_out_b(NO - 1).start()
    for i in range(NO // NB3):
        cp_out_a(i).wait()
    for i in range(NO):
        cp_out_b(i).wait()


@jax.jit
def pallas_concat_heads__ssm_conv_h3__compressed_kv_cla__prompt_kernel(
    A_q: jax.Array,
    A_k: jax.Array,
    A_v: jax.Array,
    A_shift_k: jax.Array,
    A_ssm_k: jax.Array,
    A_ssm_D: jax.Array,
    B_x: jax.Array,
    B_c_kv: jax.Array,
    B_w_q: jax.Array,
    B_w_uk: jax.Array,
    B_w_uv: jax.Array,
    B_w_o: jax.Array,
):
    vm = pltpu.VMEM
    dma = pltpu.SemaphoreType.DMA
    scratch = [
        vm((4, M), BF16),
        vm((M,), BF16),
        vm((5, MP, 128), F32),
        vm((64, 256), U32),
        vm((64, 256), U32),
        vm((8, 128), U32),
        vm((M, S), BF16),
        vm((S // 256 * 7 * 64, MP // 2), U32),
        vm((H // 2, M, D), U32),
        vm((NU, UC // 2, S), U32),
        vm((NU, UC // 2, S), U32),
        vm((NU, UC // 2, S), U32),
        vm((NU, UC // 2, S), U32),
        vm((M, S), BF16),
        vm((S // 2, C), U32),
        vm((NB * 49 * 64, C // 4), U32),
        vm((128, 256), U32),
        vm((H // 2, C, D), U32),
        vm((H // 2, C, D), U32),
        vm((H, M // 2, D), U32),
        vm((4 * 49 * 56, D), U32),
        vm((H * S // 2, D), U32),
        vm((H * S // 2, D), U32),
        vm((M, TO), F32),
        vm((TQ, D), F32),
        vm((TQ, 128), F32),
        vm((S, MA), BF16),
        vm((S, MP), BF16),
        dma((2,)), dma((XCH,)), dma((H // 2,)), dma((NU * 4,)), dma((9,)),
        dma((H // 2,)), dma((H // 2,)), dma((NO // NB3,)), dma((NO,)),
    ]
    out = pl.pallas_call(
        _kernel,
        in_specs=[pl.BlockSpec(memory_space=pl.ANY)] * 12,
        out_specs=pl.BlockSpec(memory_space=pl.ANY),
        out_shape=jax.ShapeDtypeStruct((S, 2 * M), BF16),
        scratch_shapes=scratch,
        compiler_params=pltpu.CompilerParams(
            vmem_limit_bytes=120 * 1024 * 1024,
            disable_semaphore_checks=True,
            disable_bounds_checks=True,
        ),
        name="h3_cla_fused",
    )(
        A_q[0].T, A_k[0].T, A_v[0].T, A_shift_k.T, A_ssm_k, A_ssm_D,
        B_x[0].T, B_c_kv[0], B_w_q, B_w_uk, B_w_uv, jnp.transpose(B_w_o, (0, 2, 1)),
    )
    return out[None]
```

```python
import math

import jax
import jax.numpy as jnp
import jax.experimental.pallas as pl
import jax.experimental.pallas.tpu as pltpu

S = 2048
M = 448
MP = 512
MA = 384
H = 16
D = 256
C = 1024
G = 32
NC = 128 // G
TQ = 128 * NC
NB = S // TQ
NU = 7
UC = M // NU
NBLK = S // 128
XB = (0, 256, 768, 1536, 2048)
XCH = len(XB) - 1
XLAG = 3
TO = 128
NO = S // TO
NB3 = 4
MLAG = 800
SLAG = 1000
NPART = 16
MORDER = (1, 4, 0, 3, 6, 2, 5)
PORDER = (2, 5, 0, 4, 6, 3, 1)
P1PLAN = {0: 'H0 H1 H2 H3', 5: 'X0', 9: 'X1', 13: 'X2', 17: 'X3', 21: 'I00', 25: 'I01', 29: 'I10',
          33: 'I11', 37: 'I20', 41: 'I21', 45: 'I30', 49: 'I31'}
CPOS = [1, 2, 3, 19, 20, 22, 23, 26, 27, 30, 31, 34, 35, 38, 39, 42, 43, 46, 47, 50, 51, 52, 53,
        54, 55, 48, 44, 40]
P2ORDER = ("M101 M401 M001 M301 M601 M201 M501 Q0 M12 M42 P0 Q1 M02 M32 M62 P1 M22 M52 "
           "Q2 M13 M43 M03 M33 M63 P2 Q3 M23 M53 P3")

F32 = jnp.float32
BF16 = jnp.bfloat16
U32 = jnp.uint32
HI_MASK = 0xFFFF0000
Q_SCALE = D ** -0.5 * math.log2(math.e)
MASK_VALUE = -1e9


def _dot(a, b):
    return jnp.dot(a, b, preferred_element_type=F32)


def _dot_nt(a, b):
    return jax.lax.dot_general(a, b, (((1,), (1,)), ((), ())), preferred_element_type=F32)


def _pack(x):
    return pltpu.bitcast(x.astype(BF16), U32)


def _ds(start, size, align):
    return pl.ds(start if isinstance(start, int) else pl.multiple_of(start, align), size)


def _sample(x):
    return _or_fold(jnp.concatenate([x[r + 8:r + 16] for r in range(0, x.shape[0], 16)], axis=0))


def _quads(x):
    r, c = x.shape[0] // 2, x.shape[1] // 2
    return x[:r, :c], x[:r, c:], x[r:, :c], x[r:, c:]


def _lhs_op(quad, i):
    return (lambda: quad(0, 0) + quad(1, 1), lambda: quad(1, 0) + quad(1, 1), lambda: quad(0, 0),
            lambda: quad(1, 1), lambda: quad(0, 0) + quad(0, 1), lambda: quad(1, 0) - quad(0, 0),
            lambda: quad(0, 1) - quad(1, 1))[i]()


def _rhs_op(quad, i):
    return (lambda: quad(0, 0) + quad(1, 1), lambda: quad(0, 0), lambda: quad(0, 1) - quad(1, 1),
            lambda: quad(1, 0) - quad(0, 0), lambda: quad(1, 1), lambda: quad(0, 0) + quad(0, 1),
            lambda: quad(1, 0) + quad(1, 1))[i]()


def _lhs_ops(a):
    q = _quads(a)
    return [_lhs_op(lambda r, c: q[2 * r + c], i) for i in range(7)]


def _rhs_ops(b):
    q = _quads(b)
    return [_rhs_op(lambda r, c: q[2 * r + c], i) for i in range(7)]


def _half(m, k):
    if k == 0:
        return jnp.concatenate([(m[0] + m[3]) + (m[6] - m[4]), m[1] + m[3]], axis=0)
    return jnp.concatenate([m[2] + m[4], (m[0] - m[1]) + (m[2] + m[5])], axis=0)


def _combine(m):
    return jnp.concatenate([_half(m, 0), _half(m, 1)], axis=1)


def _or_fold(x):
    bits = pltpu.bitcast(x, U32)
    t = None
    for r in range(bits.shape[0] // 8):
        for c in range(bits.shape[1] // 128):
            e = bits[r * 8:(r + 1) * 8, c * 128:(c + 1) * 128]
            t = e if t is None else t | e
    return t


def _inject(x, tok):
    top = x[:8, :128] | tok
    if x.shape[1] > 128:
        top = jnp.concatenate([top, x[:8, 128:]], axis=1)
    return jnp.concatenate([top, x[8:]], axis=0)


def _recip(x):
    r = pl.reciprocal(x, approx=True)
    return r * (2.0 - x * r)


def _rows(chunks, r0, r1):
    parts = []
    while r0 < r1:
        c = r0 // TQ
        e = min(r1, (c + 1) * TQ)
        parts.append(chunks[c][r0 - c * TQ:e - c * TQ])
        r0 = e
    return parts[0] if len(parts) == 1 else jnp.concatenate(parts, axis=0)


def _steps(i):
    plans = []
    for cls in range(NC):
        last = cls == NC - 1
        base = 0 if last else G * (cls + 1)
        full = NC * i - 1 + last
        plan = []
        m = 0
        while m < full:
            w = 2 if m + 2 <= full else 1
            plan.append((cls, base + 128 * m, base + 128 * (m + w), 0, False))
            m += w
        for t in range(NC):
            if full + t >= 0:
                plan.append((cls, base + 128 * (full + t), base + 128 * (full + t + 1), G * t, True))
        plans.append(plan)
    n = max(len(p) for p in plans)
    return [plans[cls][j - n + len(plans[cls])] for j in range(n) for cls in reversed(range(NC))
            if j - n + len(plans[cls]) >= 0]


def _due(steps, lag):
    ends, out, t = [], [], 0
    for _, k0, k1, row0, _ in steps:
        src = [n for n, e in enumerate(ends) if e + lag <= t]
        out.append(src[-1] if src else None)
        t += (128 - row0) * (k1 - k0) // 256
        ends.append(t)
    return [None if x in out[:n] else x for n, x in enumerate(out)]


def _token(n, nsteps, own, extra):
    t = own
    for k, e in enumerate(extra):
        if k * nsteps // len(extra) == n:
            t = e if t is None else t | e
    return t


def _mix(a, b):
    if not a or not b:
        return a or b
    keyed = [((k + 0.5) / len(a), x) for k, x in enumerate(a)] + [((k + 1.0) / len(b), x) for k, x in enumerate(b)]
    return [x for _, x in sorted(keyed, key=lambda e: e[0])]


def _update(acc, x, row0, op):
    if acc is None:
        return x
    if row0 == 0:
        return op(acc, x)
    return jnp.concatenate([acc[:row0], op(acc[row0:], x)], axis=0)


def _qk(i, qu, ks, zero, extra):
    r = jax.lax.broadcasted_iota(jnp.int32, (G, 128), 0)
    c = jax.lax.broadcasted_iota(jnp.int32, (G, 128), 1)
    msk = c <= r + (128 - G)
    h = G // 2
    qc = [jnp.concatenate([qu[64 * t + h * cls:64 * t + h * (cls + 1)] for t in range(NC)], axis=0)
          for cls in range(NC)]
    steps = _steps(i)
    due = _due(steps, MLAG)
    toks = {}
    run = [None] * NC
    sc, lead = [], []
    for cls in range(NC - 1):
        w = G * (cls + 1)
        s = _dot_nt(_rows(ks, 0, w).astype(BF16), pltpu.bitcast(qc[cls], BF16)).T
        if i == 0:
            top = jnp.where((c <= r + G * cls)[:, :w], s[:G], MASK_VALUE)
            s = jnp.concatenate([top, s[G:]], axis=0)
        lead.append(s)
        run[cls] = jnp.concatenate([s, jnp.full((128, 128 - w), MASK_VALUE, F32)], axis=1)
    for n, (cls, k0, k1, row0, masked) in enumerate(steps):
        x = qc[cls][row0 // 2:]
        t = _token(n, len(steps), toks.get(due[n]), extra)
        x = pltpu.bitcast(x if t is None else _inject(x, t), BF16)
        s = _dot_nt(x, _rows(ks, k0, k1).astype(BF16))
        if masked:
            top = jnp.where(msk, s[:G], MASK_VALUE)
            s = top if row0 + G == 128 else jnp.concatenate([top, s[G:]], axis=0)
        sc.append(s)
        mj = jnp.maximum(s[:, :128], s[:, 128:]) if k1 - k0 == 256 else s
        run[cls] = _update(run[cls], mj, row0, jnp.maximum)
        toks[n] = _or_fold(run[cls]) & zero
    return steps, lead, sc, run


def _softmax_pv(steps, lead, sc, mx, vs, zero, extra):
    m = [jnp.max(mx[cls], axis=1, keepdims=True) for cls in range(NC)]
    groups = []
    for cls in range(NC):
        w, out = [n for n, e in enumerate(steps) if e[0] == cls and e[2] - e[1] == 256], []
        while w:
            k = len(w) if len(w) <= 3 else 2
            out.append(w[:k])
            w = w[k:]
        groups.append(out)
    perm = [n for gi in range(max(len(x) for x in groups)) for cls in reversed(range(NC))
            if gi < len(groups[cls]) for n in groups[cls][gi]]
    ends = [g[-1] for x in groups for g in x]
    perm += sorted((n for n in range(len(steps)) if n not in perm), key=lambda n: (-steps[n][0], n))
    steps = [steps[n] for n in perm]
    due = _due(steps, SLAG)
    toks = {}
    o = [None] * NC
    run = [None] * NC
    macc = [[None] * 7 for _ in range(NC)]
    wait = []
    for cls in range(NC - 1):
        w = G * (cls + 1)
        p = jnp.exp2(lead[cls] - m[cls]).astype(BF16)
        o[cls] = _dot(p, _rows(vs, 0, w).astype(BF16))
        run[cls] = jnp.concatenate([p.astype(F32), jnp.zeros((128, 128 - w), F32)], axis=1)
    for n, (cls, k0, k1, row0, _) in enumerate(steps):
        p = jnp.exp2(sc[perm[n]] - m[cls][row0:])
        t = _token(n, len(steps), toks.get(due[n]), extra)
        if t is not None:
            p = pltpu.bitcast(_inject(pltpu.bitcast(p, U32), t), F32)
        if k1 - k0 == 256:
            lhs = [x.astype(BF16) for x in _lhs_ops(p)]
            wait.append((lhs, [x.astype(BF16) for x in _rhs_ops(_rows(vs, k0, k1))]))
            if perm[n] in ends:
                for j in PORDER:
                    t = None
                    for x, y in wait:
                        t = _update(t, _dot(x[j], y[j]), 0, jnp.add)
                    macc[cls][j] = _update(macc[cls][j], t, 0, jnp.add)
                wait = []
            e = jnp.concatenate([lhs[4].astype(F32), lhs[1].astype(F32)], axis=0)
        else:
            p = p.astype(BF16)
            t = _dot(p, _rows(vs, k0, k1).astype(BF16))
            e = p.astype(F32)
            o[cls] = _update(o[cls], t, row0, jnp.add)
        run[cls] = _update(run[cls], e, row0, jnp.add)
        toks[n] = _or_fold(run[cls]) & zero
    for cls in range(NC):
        if macc[cls][0] is not None:
            o[cls] = o[cls] + _combine(macc[cls])

    def natural(x):
        return jnp.concatenate([x[cls][G * t:G * (t + 1)] for t in range(NC) for cls in range(NC)], axis=0)
    return natural(o), natural(run)


def _normalize(o, lsum, unscale):
    r = _recip(jnp.broadcast_to(jnp.sum(lsum, axis=1, keepdims=True), lsum.shape))
    r = r * jnp.tile(unscale, (r.shape[0] // 8, 1))
    return o * jnp.concatenate([r, r], axis=1)


def _kernel(aq_hbm, ak_hbm, av_hbm, sh_hbm, ah_hbm, dd_hbm, xt_hbm, c_hbm,
            wq_hbm, wk_hbm, wv_hbm, wot_hbm,
            out_hbm,
            coef_s, f_s, fh_s, xt_s, x_s, wq_raw, aq_s, ak_s, av_s, ah_s, at_s,
            c_s, cs_s, ws_s, wk_raw, wv_raw, wot_s, wos_s, q_s, ctx_s, ot_s, o7_s, l7_s, stage_a, stage_b,
            vscale_s, zero_s, sh_s, dd_s,
            sem_small, sem_x, sem_wq, sem_a, sem_c, sem_wk, sem_wv, sem_oa, sem_ob):
    wq32 = wq_hbm.bitcast(U32)
    wk32 = wk_hbm.bitcast(U32)
    wv32 = wv_hbm.bitcast(U32)

    def cp_small(i):
        return pltpu.make_async_copy((sh_hbm, dd_hbm)[i], (sh_s, dd_s)[i], sem_small.at[i])

    def cp_x(i):
        cols = pl.ds(XB[i], XB[i + 1] - XB[i])
        return pltpu.make_async_copy(xt_hbm.at[:, cols], xt_s.at[:, cols], sem_x.at[i])

    def cp_wq(p):
        return pltpu.make_async_copy(wq32.at[:, p, :], wq_raw.at[p], sem_wq.at[p])

    def cp_a(g, i):
        src = (ah_hbm, ak_hbm, av_hbm, aq_hbm)[i].bitcast(U32)
        dst = (ah_s, ak_s, av_s, aq_s)[i]
        n = UC // 2
        start = g * n if isinstance(g, int) else pl.multiple_of(g * n, 8)
        return pltpu.make_async_copy(src.at[pl.ds(start, n), :], dst.at[g], sem_a.at[g * 4 + i])

    def cp_c(i):
        n = 128
        start = i * n if isinstance(i, int) else pl.multiple_of(i * n, n)
        return pltpu.make_async_copy(c_hbm.bitcast(U32).at[pl.ds(start, n), :],
                                     c_s.at[pl.ds(start, n), :], sem_c.at[i])

    def cp_wo():
        return pltpu.make_async_copy(wot_hbm.bitcast(U32), wot_s, sem_c.at[8])

    def c_ops(strip, i):
        blk, part = strip >> 3, strip & 7

        def quad(r, k):
            x = [c_s[_ds(blk * 256 + (2 * r + e) * 64 + part * 8, 8, 8), k * 512:(k + 1) * 512] for e in range(2)]
            return pltpu.bitcast(jnp.concatenate(x, axis=0), BF16).astype(F32)
        tok = None
        for j, y in enumerate(_lhs_ops(_lhs_op(quad, i))):
            cs_s[_ds(((blk * 7 + i) * 7 + j) * 64 + part * 8, 8, 8), :] = _pack(y)
            if j % 2 == 0:
                tok = _sample(y) if tok is None else tok | _sample(y)
        return tok & zero_s[...]

    def cp_wk(p):
        return pltpu.make_async_copy(wk32.at[:, p, :], wk_raw.at[p], sem_wk.at[p])

    def cp_wv(p):
        return pltpu.make_async_copy(wv32.at[:, p, :], wv_raw.at[p], sem_wv.at[p])

    def cp_out_a(i):
        n = NB3 * TO
        start = i * n if isinstance(i, int) else pl.multiple_of(i * n, n)
        return pltpu.make_async_copy(stage_a.at[pl.ds(start, n), :],
                                     out_hbm.at[pl.ds(start, n), pl.ds(0, MA)], sem_oa.at[i])

    def cp_out_b(i):
        start = i * TO if isinstance(i, int) else pl.multiple_of(i * TO, TO)
        return pltpu.make_async_copy(stage_b.at[pl.ds(start, TO), :],
                                     out_hbm.at[pl.ds(start, TO), pl.ds(MA, MP)], sem_ob.at[i])

    cp_x(0).start()
    cp_wq(0).start()
    for i in range(1, XCH):
        cp_x(i).start()
    cp_small(0).start()
    cp_small(1).start()

    tt = jax.lax.broadcasted_iota(jnp.int32, (128, 128), 0)
    rr = jax.lax.broadcasted_iota(jnp.int32, (128, 128), 1)
    ang = ((tt * (2 * rr + 1)) & 511).astype(F32) * (2.0 * math.pi / 512.0)
    fmat = jnp.concatenate([jnp.cos(ang), -jnp.sin(ang)], axis=1).astype(BF16)
    f_s[...] = pltpu.bitcast(fmat, U32)
    fh_s[...] = pltpu.bitcast((fmat.astype(F32) * (1.0 / 128.0)).astype(BF16), U32)
    zero_s[...] = jnp.zeros((8, 128), U32)

    def xpose_x(i):
        for blk in range(XB[i] // 256, XB[i + 1] // 256):
            tiles = []
            for t in (2 * blk, 2 * blk + 1):
                cols = slice(t * 128, (t + 1) * 128)
                parts = [xt_s[g * 128:(g + 1) * 128, cols].astype(F32).T for g in range(3)]
                last = jnp.concatenate([xt_s[MA:M, cols].astype(F32), jnp.zeros((MP - M, 128), F32)], axis=0)
                parts.append(last.T)
                tiles.append(jnp.concatenate(parts, axis=1))
            x = jnp.concatenate(tiles, axis=0)
            for j, op in enumerate(_lhs_ops(x)):
                x_s[(blk * 7 + j) * 64:(blk * 7 + j + 1) * 64, :] = _pack(op)

    def q_weights(p):
        raw = wq_raw[p]
        ops = []
        for w in (raw << 16, raw & jnp.uint32(HI_MASK)):
            w = pltpu.bitcast(w, F32) * Q_SCALE
            ops.append(_rhs_ops(jnp.concatenate([w, jnp.zeros((MP - M, D), F32)], axis=0)))
        return [jnp.concatenate([u, v], axis=1).astype(BF16) for u, v in zip(*ops)]

    def qstep(p, w, ms, n, tok=None):
        blk, j = n // 7, MORDER[n % 7]
        x = x_s[(blk * 7 + j) * 64:(blk * 7 + j + 1) * 64, :]
        if tok is not None:
            x = _inject(x, tok)
        ms[j] = _dot(pltpu.bitcast(x, BF16), w[j])
        if n % 7 == 6:
            for k in range(2):
                q = _combine([ms[e][:, k * 128:(k + 1) * 128] for e in range(7)])
                q_s[_ds((2 * p + k) * (S // 2) + blk * 128, 128, 128), :] = _pack(q)

    cp_x(0).wait()
    xpose_x(0)
    cp_c(0).start()
    cp_c(1).start()
    for g in range(NU):
        cp_wq(g + 1).start()
        for i in range(4):
            cp_a(g, i).start()
        if g < NU - 1:
            cp_c(g + 2).start()
    cp_wk(0).start()
    cp_wv(0).start()
    cp_wo().start()
    for p in range(1, H // 2):
        cp_wk(p).start()
        cp_wv(p).start()
    cp_wq(0).wait()
    w0 = q_weights(0)
    ms0 = {}
    for n in range(XB[1] // 256 * 7 - XLAG):
        qstep(0, w0, ms0, n)
    for i in range(1, XCH):
        cp_x(i).wait()
        if i == XCH - 1:
            cp_small(0).wait()
            cp_small(1).wait()
            cp_c(0).wait()
            cp_c(1).wait()
            prm = [sh_s[j:j + 1, :].astype(F32) for j in range(4)]
            prm.append(dd_s[...].astype(F32).reshape(1, M))
            for j in range(5):
                row = jnp.concatenate([prm[j], jnp.zeros((1, MP - M), F32)], axis=1)
                for t in range(MP // 128):
                    blk = jnp.broadcast_to(row[:, t * 128:(t + 1) * 128], (128, 128))
                    coef_s[j, t * 128:(t + 1) * 128, :] = blk.T
        for n in range(XB[i] // 256 * 7 - XLAG, XB[i] // 256 * 7):
            qstep(0, w0, ms0, n)
        xpose_x(i)
        for n in range(XB[i] // 256 * 7, XB[i + 1] // 256 * 7 - (XLAG if i < XCH - 1 else 0)):
            tok = None
            if i == XCH - 1:
                n0, n1 = XB[i] // 256 * 7, XB[i + 1] // 256 * 7
                for e in range(28):
                    if n0 + e * (n1 - n0) // 28 == n:
                        t = c_ops(e // 7, e % 7)
                        tok = t if tok is None else tok | t
            qstep(0, w0, ms0, n, tok)
    ot_s[...] = jnp.zeros((M, TO), F32)
    o7_s[...] = jnp.zeros((TQ, D), F32)
    l7_s[...] = jnp.ones((TQ, 128), F32)

    def phase1(g, carry):
        cp_wq(g + 1).wait()
        for i in range(4):
            cp_a(g, i).wait()

        @pl.when((g & 1) == 1)
        def _():
            cp_c(g + 1).wait()
            cp_c(g + 2).wait()

        w = q_weights(g + 1)
        fh = pltpu.bitcast(fh_s[...], BF16)
        fx = pltpu.bitcast(f_s[...], BF16)
        lane = jax.lax.broadcasted_iota(jnp.int32, (16, 128), 1)
        sgn = jnp.where((jax.lax.broadcasted_iota(jnp.int32, (8, 128), 1) & 1) == 0, 1.0, -1.0)
        zh, zx, kvs, ys = {}, {}, {}, {}

        def coef(k, j):
            return coef_s[j, pl.ds(pl.multiple_of(g * UC + k * 16, 16), 16), :]

        def hfwd(k):
            lhs = jnp.concatenate([ah_s[g, k * 8:(k + 1) * 8, c * 128:(c + 1) * 128]
                                   for c in range(NBLK)], axis=0)
            zh[k] = _dot(pltpu.bitcast(lhs, BF16), fh)

        def xfwd(k):
            kf = pltpu.bitcast(ak_s[g, k * 8:(k + 1) * 8, :], BF16).astype(F32)
            vf = pltpu.bitcast(av_s[g, k * 8:(k + 1) * 8, :], BF16).astype(F32)
            sh_k = [kf] + [pltpu.roll(kf, j, 1) for j in range(1, 4)]
            cf = [coef(k, j) for j in range(4)]
            kvf = []
            for c in range(NBLK):
                cols = slice(c * 128, (c + 1) * 128)
                t = sh_k[0][:, cols] * cf[0]
                for j in range(1, 4):
                    kj = sh_k[j][:, cols]
                    if c == 0:
                        kj = jnp.where(lane >= j, kj, 0.0)
                    t = t + kj * cf[j]
                kvf.append(t * vf[:, cols])
            kvs[k] = jnp.concatenate(kvf, axis=0).astype(BF16)
            zx[k] = _dot(kvs[k], fx)

        def inv(k, u):
            rows = [slice(c * 16 + u * 8, c * 16 + u * 8 + 8) for c in range(NBLK)]
            xr = [zx[k][r, :128] for r in rows]
            xi = [zx[k][r, 128:] for r in rows]
            h0r = [zh[k][r, :128] for r in rows]
            h0i = [zh[k][r, 128:] for r in rows]
            hr = [h0r[0]] + [h0r[j] - sgn * h0i[j - 1] for j in range(1, NBLK)]
            hi = [h0i[0]] + [h0i[j] + sgn * h0r[j - 1] for j in range(1, NBLK)]
            pr, pi = [], []
            for a0 in range(0, NBLK, 4):
                re = [None] * 4
                im = [None] * 4
                for c0 in range(0, a0 + 4, 4):
                    for da in range(4):
                        for c in range(c0, c0 + 4):
                            j = a0 + da - c
                            if j < 0:
                                continue
                            tr = xr[c] * hr[j] - xi[c] * hi[j]
                            ti = xr[c] * hi[j] + xi[c] * hr[j]
                            re[da] = tr if re[da] is None else re[da] + tr
                            im[da] = ti if im[da] is None else im[da] + ti
                pr += re
                pi += im
            p = jnp.concatenate([jnp.concatenate(pr, axis=0), jnp.concatenate(pi, axis=0)], axis=1)
            ys[k, u] = _dot_nt(p.astype(BF16), fx)
            if u == 1:
                kvr = kvs[k].astype(F32)
                qraw = aq_s[g, k * 8:(k + 1) * 8, :] | jnp.tile(zero_s[...], (1, NBLK))
                qf = pltpu.bitcast(qraw, BF16).astype(F32)
                dd = coef(k, 4)
                out = []
                for a in range(NBLK):
                    y = jnp.concatenate([ys[k, 0][a * 8:(a + 1) * 8], ys[k, 1][a * 8:(a + 1) * 8]], axis=0)
                    out.append(y + kvr[a * 16:(a + 1) * 16] * dd)
                at_s[_ds(g * (UC // 2) + k * 8, 8, 8), :] = _pack(qf * jnp.concatenate(out, axis=1))

        ms = {}
        for n in range(S // 256 * 7):
            tok = None
            for step in P1PLAN.get(n, '').split():
                if step[0] == 'H':
                    hfwd(int(step[1]))
                elif step[0] == 'X':
                    xfwd(int(step[1]))
                elif step[0] == 'I':
                    inv(int(step[1]), int(step[2]))
            for e, pos in enumerate(CPOS):
                if pos == n:
                    t = c_ops(4 * (g + 1) + e // 7, e % 7)
                    tok = t if tok is None else tok | t
            qstep(g + 1, w, ms, n, tok)
        return carry

    jax.lax.fori_loop(0, NU, phase1, 0)

    cp_wo().wait()
    for p in range(H // 2):
        cp_wk(p).wait()
        cp_wv(p).wait()

    def unpack_head(w, h):
        sh = (16 - ((h & 1) << 4)).astype(U32)
        return pltpu.bitcast((w << sh) & jnp.uint32(HI_MASK), F32)

    def first_operands(h):
        w = jnp.concatenate([wk_raw[h >> 1, :256, :128], wk_raw[h >> 1, 256:512, 128:]], axis=1)
        w = unpack_head(w, h)
        ws_s[...] = _pack(w)
        return w

    first_operands(jnp.int32(0))

    def exponent(raw):
        x = jnp.max(pltpu.bitcast(raw[0, :64, :] & jnp.uint32(0x7F800000), F32), axis=0, keepdims=True)
        x = jnp.broadcast_to(jnp.max(x, axis=1, keepdims=True), (8, 128))
        return pltpu.bitcast(x, jnp.int32) >> 23
    shift = jnp.clip(exponent(wk_raw) - exponent(wv_raw), -60, 60)
    vscale_s[0] = pltpu.bitcast((127 + shift) << 23, F32)
    vscale_s[1] = pltpu.bitcast((127 - shift) << 23, F32)

    def product(ws, blks, i):
        ms = [None] * 7
        for j in MORDER:
            r = [((blk * 7 + i) * 7 + j) * 64 for blk in blks]
            x = jnp.concatenate([cs_s[e:e + 64, :] for e in r], axis=0)
            ms[j] = _dot(pltpu.bitcast(x, BF16), ws[i][j])
        return [_combine([m[k * 128:(k + 1) * 128] for m in ms]) for k in range(len(blks))]

    def finish_last(h):
        ctx = _normalize(o7_s[...], l7_s[...], vscale_s[1])
        ctx_s[_ds(h * (S // 2) + (NB - 1) * TQ // 2, TQ // 2, TQ // 2), :] = _pack(ctx)
        return ctx

    def phase2(h, carry):
        b = jnp.concatenate([unpack_head(wk_raw[h >> 1], h),
                             unpack_head(wv_raw[h >> 1], h) * jnp.tile(vscale_s[0], (C // 8, D // 128))], axis=1)
        ws = [[y.astype(BF16) for y in _rhs_ops(x)] for x in _rhs_ops(b)]
        ws[1][1] = pltpu.bitcast(ws_s[:, :128], BF16)
        ws[1][4] = pltpu.bitcast(ws_s[:, 128:], BF16)
        mo = {}
        ks, vs, toks, sc = [], [], {}, {}
        zero = zero_s[...]

        def tokens(x, parts=NPART):
            n = TQ // parts
            return [_or_fold(x[k * n:(k + 1) * n]) & zero for k in range(parts)]

        def wo_ops(k, i):
            unit = jnp.minimum(2 * h + k, 27)
            j = jax.lax.div(unit, 7)
            r0 = (unit - 7 * j) * 8

            def quad(r, c):
                x = [jnp.concatenate([wot_s[j + 4 * (2 * c + f), _ds((2 * r + e) * 56 + r0, 8, 8), :]
                                      for f in range(2)], axis=1) for e in range(2)]
                return pltpu.bitcast(jnp.concatenate(x, axis=0), BF16).astype(F32)
            tok = None
            for n, y in enumerate(_lhs_ops(_lhs_op(quad, i))):
                wos_s[_ds(((j * 7 + i) * 7 + n) * 56 + r0, 8, 8), :] = _pack(y)
                if n % 2 == 0:
                    tok = _sample(y) if tok is None else tok | _sample(y)
            return tok & zero

        nxt = jnp.minimum(h + 1, H - 1)
        toks[-1] = tokens(finish_last(jnp.maximum(h - 1, 0)))
        for step in P2ORDER.split():
            i = int(step[1:])
            if step[0] == 'M':
                blks = [int(e) for e in step[2:]]
                j = int(step[1])
                for blk, m in zip(blks, product(ws, blks, j)):
                    mo[blk, j] = m
                    e = [mo.get((blk, k)) for k in range(7)]
                    if j == 6:
                        ks.append(_half(e, 0))
                    if j == 5:
                        vs.append(_half(e, 1))
            elif step[0] == 'Q':
                q = q_s[_ds(h * (S // 2) + i * TQ // 2, TQ // 2, TQ // 2), :]
                extra = toks.get(i - 2, [])
                for k in {0: (0, 1), 2: (2,)}.get(i, ()):
                    extra = _mix(extra, tokens(vs[k], 8))
                if i % 2 == 1:
                    extra = _mix(extra, [wo_ops(i // 2, e) for e in range(7)])
                if i == NB - 1:
                    w = first_operands(nxt)
                    extra = _mix(extra, [_sample(w[k * 64:(k + 1) * 64]) & zero for k in range(4)])
                sc[i] = _qk(i, q, ks, zero, extra)
            elif i == NB - 1:
                o7_s[...], l7_s[...] = _softmax_pv(*sc[i], vs, zero, toks[i - 1])
            else:
                ctx = _normalize(*_softmax_pv(*sc[i], vs, zero, []), vscale_s[1])
                ctx_s[_ds(h * (S // 2) + i * TQ // 2, TQ // 2, TQ // 2), :] = _pack(ctx)
                toks[i] = tokens(ctx)
        return carry

    jax.lax.fori_loop(0, H, phase2, 0)

    def finish(i, ot):
        r0 = i * TO if isinstance(i, int) else pl.multiple_of(i * TO, TO)
        top = pltpu.bitcast(at_s[MA // 2:M // 2, pl.ds(r0, TO)], BF16).astype(F32)
        val = jnp.concatenate([top, ot], axis=0).T
        stage_b[pl.ds(r0, TO), :] = val.astype(BF16)
        return val

    def phase3(it, carry):
        prev = jnp.maximum(NB3 * it - 1, 0)
        val = finish(prev, ot_s[...])
        pend = {3 + k: [val[:, k * 128:(k + 1) * 128]] for k in range(4)}

        @pl.when(it > 0)
        def _():
            cp_out_b(prev).start()

        r0 = pl.multiple_of(it * (NB3 * TO), NB3 * TO)
        apart = []
        for g in range(MA // 128):
            blk = pltpu.bitcast(at_s[g * 64:(g + 1) * 64, pl.ds(r0, NB3 * TO)], BF16).astype(F32).T
            stage_a[pl.ds(r0, NB3 * TO), g * 128:(g + 1) * 128] = blk.astype(BF16)
            apart.append(blk)
        cp_out_a(it).start()
        for k, y in enumerate(apart):
            for e in range(4):
                pend[16 + 4 * k + e] = [y[e * 128:(e + 1) * 128]]

        def ctx(kq, t):
            rows = pl.multiple_of((NB3 * it + t) * (TO // 2), TO // 2)
            x = [ctx_s[pl.ds(h * (S // 2) + rows, TO // 2), :] for h in range(4 * kq, 4 * kq + 4)]
            return pltpu.bitcast(jnp.concatenate(x, axis=1), BF16)

        mo = [[None] * 7, [None] * 7]
        step = 0
        for i in MORDER:
            sub = {(a, b): _rhs_op(lambda r, c: ctx(2 * r + a, 2 * c + b).astype(F32), i)
                   for a in range(2) for b in range(2)}
            mi = [None] * 7
            for j in MORDER:
                w = _rhs_op(lambda r, c: sub[r, c], j).astype(BF16)
                x = jnp.concatenate([wos_s[((e * 7 + i) * 7 + j) * 56:((e * 7 + i) * 7 + j + 1) * 56, :]
                                     for e in range(4)], axis=1)
                if step in pend:
                    tok = None
                    for y in pend[step]:
                        tok = _sample(y) if tok is None else tok | _sample(y)
                    x = _inject(x, tok & zero_s[...])
                mi[j] = _dot_nt(pltpu.bitcast(x, BF16), w)
                step += 1
                for k, last in ((0, 6), (1, 5)):
                    if j == last:
                        mo[k][i] = _half(mi, k)
                        for n, done in ((0, 6), (1, 5)):
                            if i == done and 2 * n + k < NB3 - 1:
                                val = finish(NB3 * it + 2 * n + k, _half(mo[k], n))
                                cp_out_b(NB3 * it + 2 * n + k).start()
                                for e in range(4):
                                    if step + 4 + e <= 48:
                                        due = step + 4 + e
                                        pend[due] = pend.get(due, []) + [val[:, e * 128:(e + 1) * 128]]
        ot_s[...] = _half(mo[1], 1)
        finish_last(H - 1)
        return carry

    jax.lax.fori_loop(0, NO // NB3, phase3, 0)

    finish(NO - 1, ot_s[...])
    cp_out_b(NO - 1).start()
    for i in range(NO // NB3):
        cp_out_a(i).wait()
    for i in range(NO):
        cp_out_b(i).wait()


@jax.jit
def pallas_concat_heads__ssm_conv_h3__compressed_kv_cla__prompt_kernel(
    A_q: jax.Array,
    A_k: jax.Array,
    A_v: jax.Array,
    A_shift_k: jax.Array,
    A_ssm_k: jax.Array,
    A_ssm_D: jax.Array,
    B_x: jax.Array,
    B_c_kv: jax.Array,
    B_w_q: jax.Array,
    B_w_uk: jax.Array,
    B_w_uv: jax.Array,
    B_w_o: jax.Array,
):
    vm = pltpu.VMEM
    dma = pltpu.SemaphoreType.DMA
    scratch = [
        vm((5, MP, 128), F32),
        vm((64, 256), U32),
        vm((64, 256), U32),
        vm((M, S), BF16),
        vm((S // 256 * 7 * 64, MP // 2), U32),
        vm((H // 2, M, D), U32),
        vm((NU, UC // 2, S), U32),
        vm((NU, UC // 2, S), U32),
        vm((NU, UC // 2, S), U32),
        vm((NU, UC // 2, S), U32),
        vm((M // 2, S), U32),
        vm((S // 2, C), U32),
        vm((NB * 49 * 64, C // 4), U32),
        vm((128, 256), U32),
        vm((H // 2, C, D), U32),
        vm((H // 2, C, D), U32),
        vm((H, M // 2, D), U32),
        vm((4 * 49 * 56, D), U32),
        vm((H * S // 2, D), U32),
        vm((H * S // 2, D), U32),
        vm((M, TO), F32),
        vm((TQ, D), F32),
        vm((TQ, 128), F32),
        vm((S, MA), BF16),
        vm((S, MP), BF16),
        vm((2, 8, 128), F32),
        vm((8, 128), U32),
        vm((4, M), BF16),
        vm((M,), BF16),
        dma((2,)), dma((XCH,)), dma((H // 2,)), dma((NU * 4,)), dma((9,)),
        dma((H // 2,)), dma((H // 2,)), dma((NO // NB3,)), dma((NO,)),
    ]
    out = pl.pallas_call(
        _kernel,
        in_specs=[pl.BlockSpec(memory_space=pl.ANY)] * 12,
        out_specs=pl.BlockSpec(memory_space=pl.ANY),
        out_shape=jax.ShapeDtypeStruct((S, 2 * M), BF16),
        scratch_shapes=scratch,
        compiler_params=pltpu.CompilerParams(
            vmem_limit_bytes=124 * 1024 * 1024,
            disable_semaphore_checks=True,
            disable_bounds_checks=True,
        ),
        name="h3_cla_fused",
    )(
        A_q[0].T, A_k[0].T, A_v[0].T, A_shift_k.T, A_ssm_k, A_ssm_D,
        B_x[0].T, B_c_kv[0], B_w_q, B_w_uk, B_w_uv, jnp.transpose(B_w_o, (0, 2, 1)),
    )
    return out[None]
```
